```python
import jax
import jax.numpy as jnp

def _softmax(x, axis=-1):
    return jax.nn.softmax(x, axis=axis)

def _gelu(x):
    return jax.nn.gelu(x, approximate=True)

def _silu(x):
    return jax.nn.silu(x)

def _sigmoid(x):
    return jax.nn.sigmoid(x)

def _layernorm(x, axis=-1, eps=1e-05):
    m = jnp.mean(x, axis=axis, keepdims=True)
    v = jnp.var(x, axis=axis, keepdims=True)
    return (x - m) / jnp.sqrt(v + eps)

def _scatter_add(tgt, idx, src, axis=0):
    return tgt.at[idx].add(src)

def _segment_sum(src, seg, n):
    return jax.ops.segment_sum(src, seg, n)

class _Rng:

    def __init__(self, key):
        self._k = key

    def _next(self):
        self._k, sub = jax.random.split(self._k)
        return sub

    def normal(self, shape):
        return jax.random.normal(self._next(), shape, dtype=jnp.bfloat16)

    def randint(self, lo, hi, shape):
        return jax.random.randint(self._next(), shape, lo, hi, dtype=jnp.int32)

    def uniform(self, shape, lo=0.0, hi=1.0):
        return jax.random.uniform(self._next(), shape, jnp.bfloat16, lo, hi)

    def permutation(self, n):
        return jax.random.permutation(self._next(), n)
kernel_name = 'sequential_preLN__memory_aug_infini_attn__moe_arch_mod__prompt'

def setup_inputs():
    _rng = _Rng(jax.random.key(int.from_bytes(__import__("os").urandom(4), "little")))
    _w = lambda a: (lambda t: t.astype(jnp.bfloat16) if jnp.issubdtype(t.dtype, jnp.floating) else t)(jnp.asarray(a))

    def _A_setup():
        B, S, D, H = (1, 2048, 576, 32)
        N = 4
        L = max(1, S // N)
        sc = D ** (-0.5)
        return {'x': _w((lambda *s: _rng.normal(s) * 0.05)(B, N * L, D)), 'wq': _w((lambda *s: _rng.normal(s) * 0.05)(D, D) * sc), 'wk': _w((lambda *s: _rng.normal(s) * 0.05)(D, D) * sc), 'wv': _w((lambda *s: _rng.normal(s) * 0.05)(D, D) * sc), 'wo': _w((lambda *s: _rng.normal(s) * 0.05)(D, D) * sc), 'beta': _w((lambda *s: _rng.normal(s) * 0.05)(H))}
    _A_in = _A_setup()

    def _B_setup():
        B, S, D, F, C = (1, 2048, 576, 4608, 1)
        return {'x': _w((lambda *s: _rng.normal(s) * 0.05)(B, S, D)), 'w_r': _w((lambda *s: _rng.normal(s) * 0.05)(D)), 'w_gate': _w((lambda *s: _rng.normal(s) * 0.05)(D, F)), 'w_up': _w((lambda *s: _rng.normal(s) * 0.05)(D, F)), 'w_down': _w((lambda *s: _rng.normal(s) * 0.05)(F, D))}
    _B_in = _B_setup()
    return {'A_x': _A_in['x'], 'A_wq': _A_in['wq'], 'A_wk': _A_in['wk'], 'A_wv': _A_in['wv'], 'A_wo': _A_in['wo'], 'A_beta': _A_in['beta'], 'B_x': _B_in['x'], 'B_w_r': _B_in['w_r'], 'B_w_gate': _B_in['w_gate'], 'B_w_up': _B_in['w_up'], 'B_w_down': _B_in['w_down']}

def reference(A_x, A_wq, A_wk, A_wv, A_wo, A_beta, B_x, B_w_r, B_w_gate, B_w_up, B_w_down):

    def _A_ref(x, wq, wk, wv, wo, beta):
        B, S, D = x.shape
        H = 32
        Dh = D // H
        N = 4
        L = S // N
        q = (lambda x, *d: x.transpose(*d))((x @ wq).reshape(B, S, H, Dh), 0, 2, 1, 3).reshape(B, H, N, L, Dh)
        k = (lambda x, *d: x.transpose(*d))((x @ wk).reshape(B, S, H, Dh), 0, 2, 1, 3).reshape(B, H, N, L, Dh)
        v = (lambda x, *d: x.transpose(*d))((x @ wv).reshape(B, S, H, Dh), 0, 2, 1, 3).reshape(B, H, N, L, Dh)
        phi = lambda t: jnp.where(t > 0, t + 1.0, jnp.exp(t))
        scale = Dh ** (-0.5)
        ar = jnp.arange(L)
        mask = (lambda x, dt: x.astype(dt))(ar[:, None] < ar[None, :], x.dtype) * -1000000000.0
        g = _sigmoid(beta).reshape(1, H, 1, 1)
        M = jnp.einsum('bhd,bhe->bhde', q[:, :, 0, 0, :] * 0.0, q[:, :, 0, 0, :] * 0.0)
        z = q[:, :, 0, 0, :] * 0.0
        outs = []
        for s in range(N):
            qs, ks, vs = (q[:, :, s].copy(), k[:, :, s].copy(), v[:, :, s].copy())
            logits = jnp.einsum('bhqd,bhkd->bhqk', qs, ks) * scale + mask
            p = _softmax(logits, axis=-1)
            a_dot = jnp.einsum('bhqk,bhkd->bhqd', p, vs)
            pq = phi(qs)
            num = jnp.einsum('bhld,bhde->bhle', pq, M)
            den = jnp.einsum('bhld,bhd->bhl', pq, z)[..., None] + 1e-06
            a_mem = num / den
            o = g * a_mem + (1.0 - g) * a_dot
            outs.append(o)
            pk = phi(ks)
            M = M + jnp.einsum('bhld,bhle->bhde', pk, vs)
            z = z + jnp.einsum('bhld->bhd', pk)
        o = (lambda x, *d: x.transpose(*d))(jnp.stack(outs, 2).reshape(B, H, S, Dh), 0, 2, 1, 3).reshape(B, S, D)
        return o @ wo

    def _B_ref(x, w_r, w_gate, w_up, w_down):
        B, S, D = x.shape
        C = 1
        r = x @ w_r
        idx = jnp.argsort(-r, axis=-1)[:, :C]
        idx_e = jnp.repeat(idx.reshape(B, C, 1), D, axis=2)
        x_sel = jnp.take_along_axis(x, idx_e, axis=1)
        g = _silu(x_sel @ w_gate)
        u = x_sel @ w_up
        y = g * u @ w_down
        r_sel = _sigmoid(jnp.take_along_axis(r, idx, axis=1))
        y = y * r_sel.reshape(B, C, 1)
        b_off = (jnp.arange(B) * S).reshape(B, 1)
        flat_idx = (idx + b_off).reshape(B * C)
        zero = (x * 0.0).reshape(B * S, D)
        upd = _scatter_add(zero, flat_idx, y.reshape(B * C, D), axis=0)
        return x + upd.reshape(B, S, D)
    x = A_x
    h = x + _A_ref(_layernorm(x, axis=-1), A_wq, A_wk, A_wv, A_wo, A_beta)
    h2 = h + _B_ref(_layernorm(h, axis=-1), B_w_r, B_w_gate, B_w_up, B_w_down)
    return h2
```

```python
import math

import jax
import jax.numpy as jnp
from jax import lax
import jax.experimental.pallas as pl
import jax.experimental.pallas.tpu as pltpu

F32 = jnp.float32
BF16 = jnp.bfloat16
U32 = jnp.uint32

S = 2048
D = 576
H = 32
DH = 18
NSEG = 4
L = 512
FF = 4608
T = 128
NG = 5
GH = (7, 7, 7, 7, 4)
VS = 20
EPS = 1e-5
QSCALE = DH ** (-0.5) * math.log2(math.e)
MASKVAL = -1000000000.0 * math.log2(math.e)
SOFF = (0, 128, 384, 768)
GWIN = tuple(((140 * g) // 16 * 16, -(-(140 * g + 20 * GH[g]) // 16) * 16) for g in range(NG))
QR = 592
FC = 512
import os
import contextlib
PROF = bool(int(os.environ.get('PROF', '0')))


def _scope(name):
    return jax.named_scope(name) if PROF else contextlib.nullcontext()


DIST = int(os.environ.get('DIST', '4'))
ORD = os.environ.get('ORD', 'unit')

NT = (((1,), (1,)), ((), ()))


def _bf(x_u32):
    return pltpu.bitcast(x_u32, BF16)


def _u32(x_bf):
    return pltpu.bitcast(x_bf, U32)


def _rb(x):
    return x.astype(BF16).astype(F32)


def _phi(t):
    return jnp.where(t > 0, t + 1.0, jnp.exp(t))


def _layernorm(x, axis):
    m = jnp.mean(x, axis=axis, keepdims=True)
    c = x - m
    v = jnp.mean(c * c, axis=axis, keepdims=True)
    den = _rb(jnp.sqrt(_rb(_rb(v) + EPS)))
    return c * (1.0 / den)


def _kernel(x_hbm, wq_hbm, wk_hbm, wv_hbm, wo_hbm, beta_hbm, wr_hbm, wg_hbm, wu_hbm, wd_hbm,
            out_hbm,
            x_v, w_v, wqkv, wot, xn, qt, pqt, kk, pkt, vt, memt, bd, s_buf, m_buf, m_blk,
            ot, att, h_s, out_s, r_s, bias, gtab, ones_tab, keep_tab,
            wg_v, wu_v, wd_v, beta_v, wr_v, wr16,
            sem_x, sem_w, sem_f, sem_o, sem_s):
    def x_copy(s):
        return pltpu.make_async_copy(x_hbm.at[0, :, pl.ds(s * L, L)], x_v.at[:, pl.ds(s * L, L)],
                                     sem_x.at[s])

    w_srcs = (wk_hbm, wq_hbm, wv_hbm, wo_hbm)

    def w_copy(i):
        return pltpu.make_async_copy(w_srcs[i], w_v.at[i], sem_w.at[i])

    f_pairs = ((wg_hbm, wg_v), (wu_hbm, wu_v), (wd_hbm, wd_v))

    def f_copy(i):
        return pltpu.make_async_copy(f_pairs[i][0], f_pairs[i][1], sem_f.at[i])

    def o_copy(s):
        return pltpu.make_async_copy(out_s.at[:, pl.ds(s * L, L)], out_hbm.at[0, :, pl.ds(s * L, L)],
                                     sem_o.at[s])

    beta_copy = pltpu.make_async_copy(beta_hbm, beta_v, sem_s.at[0])
    wr_copy = pltpu.make_async_copy(wr_hbm, wr_v, sem_s.at[1])

    beta_copy.start()
    wr_copy.start()
    x_copy(0).start()
    for i in range(3):
        w_copy(i).start()
    with _scope('p0_const'):
        kr = lax.broadcasted_iota(jnp.int32, (T, T), 0)
        qc = lax.broadcasted_iota(jnp.int32, (T, T), 1)
        bias[...] = jnp.where(kr > qc, MASKVAL, 0.0).astype(F32)
        bd[...] = jnp.zeros(bd.shape, F32)
        att[...] = jnp.zeros(att.shape, F32)
        row = lax.broadcasted_iota(jnp.int32, (640, T), 0)
        ones_tab[...] = jnp.where(row % VS == DH, 1.0, 0.0).astype(F32)
        for g in range(NG):
            row = lax.broadcasted_iota(jnp.int32, (160, T), 0) + (GWIN[g][0] - 140 * g)
            lane = lax.broadcasted_iota(jnp.int32, (160, T), 1)
            keep = ((row >= 0) & (row < 20 * GH[g]) & (lane >= (row // VS) * DH)
                    & (lane < (row // VS) * DH + DH))
            keep_tab[g] = jnp.where(keep, 1.0, 0.0).astype(F32)
        pqt[NG - 1] = jnp.zeros(pqt.shape[1:], U32)
        pkt[NG - 1] = jnp.zeros(pkt.shape[1:], U32)
        kk[NG - 1] = jnp.zeros(kk.shape[1:], U32)

    with _scope('p1_w'):
        wqkv[...] = jnp.zeros(wqkv.shape, U32)
        w_copy(3).start()
        x_copy(1).start()
        for i, base in ((0, QR // 2), (1, 0)):
            w_copy(i).wait()
            wt = _u32(w_v[i].T)
            for g in range(NG):
                n = 9 * GH[g]
                wqkv[base + 64 * g:base + 64 * g + n, :] = wt[63 * g:63 * g + n, :]
        w_copy(2).wait()
        wt = _u32(w_v[2].T)
        for h in range(H):
            wqkv[QR + 10 * h:QR + 10 * h + 9, :] = wt[9 * h:9 * h + 9, :]
        w_copy(3).wait()
        wt = _u32(w_v[3])
        wpad = jnp.concatenate(
            [piece for h in range(H) for piece in (wt[9 * h:9 * h + 9, :], jnp.zeros((1, D), U32))], axis=0)
        wot[...] = _u32(_bf(wpad).T)

    with _scope('p0_beta_wait'):
        beta_copy.wait()
        wr_copy.wait()
    with _scope('p0_beta'):
        beta = beta_v[...].astype(F32).reshape(1, H)
        hl = lax.broadcasted_iota(jnp.int32, (H, H), 1)
        hs = lax.broadcasted_iota(jnp.int32, (H, H), 0)
        bcol = jnp.sum(jnp.where(hl == hs, jnp.broadcast_to(beta, (H, H)), 0.0), axis=1, keepdims=True)
        gate = _rb(jax.nn.sigmoid(bcol))
        gtab[0] = jnp.broadcast_to(gate, (H, T))
        gtab[1] = jnp.broadcast_to(_rb(1.0 - gate), (H, T))

        r16 = lax.broadcasted_iota(jnp.int32, (16, D), 0)
        wr_row = wr_v[...].astype(F32).reshape(1, D)
        wr16[...] = jnp.where(r16 == 0, jnp.broadcast_to(wr_row, (16, D)), 0.0).astype(BF16)

    def ln1_unit(s, jt):
        cols = pl.ds(pl.multiple_of(s * L + jt * T, T), T)
        xn[:, jt * T:(jt + 1) * T] = _u32(_layernorm(x_v[:, cols].astype(F32), 0).astype(BF16))

    def q_unit(jt, g):
        cols = slice(jt * T, (jt + 1) * T)
        n = min(64, QR // 2 - 64 * g)
        q = jnp.dot(_bf(wqkv[64 * g:64 * g + n, :]), _bf(xn[:, cols]), preferred_element_type=F32)
        qt[g, 0:n, cols] = _u32((q * QSCALE).astype(BF16))
        pqt[g, 0:n, cols] = _u32(_phi(q).astype(BF16))

    def k_unit(jt, g):
        cols = slice(jt * T, (jt + 1) * T)
        n = min(64, QR // 2 - 64 * g)
        b0 = QR // 2 + 64 * g
        k = jnp.dot(_bf(wqkv[b0:b0 + n, :]), _bf(xn[:, cols]), preferred_element_type=F32)
        pkt[g, 0:n, cols] = _u32(_phi(k).astype(BF16))
        kb = k.astype(BF16)
        if n < 64:
            kb = jnp.concatenate([kb, jnp.zeros((T - 2 * n, T), BF16)], axis=0)
        kk[g, jt * 64:(jt + 1) * 64, :] = _u32(kb.T)

    def v_unit(jt, c):
        cols = slice(jt * T, (jt + 1) * T)
        b0 = QR + 64 * c
        v = jnp.dot(_bf(wqkv[b0:b0 + 64, :]), _bf(xn[:, cols]), preferred_element_type=F32)
        vt[64 * c:64 * (c + 1), cols] = _u32((v + ones_tab[T * c:T * (c + 1), :]).astype(BF16))

    def mem_read_unit(g):
        w0, w1 = GWIN[g]
        b = bd[g, 0:w1 - w0, :].astype(BF16)
        res = jnp.dot(b, _bf(pqt[g]), preferred_element_type=F32)
        lo, hi = 140 * g, 140 * g + 20 * GH[g]
        memt[lo:hi, :] = res[lo - w0:hi - w0]

    def mem_update_unit(g):
        w0, w1 = GWIN[g]
        upd = lax.dot_general(_bf(vt[w0 // 2:w1 // 2, :]), _bf(pkt[g]), NT, preferred_element_type=F32)
        n = w1 - w0
        bd[g, 0:n, :] = bd[g, 0:n, :] + jnp.where(keep_tab[g, 0:n, :] > 0.5, upd, 0.0)

    def s_unit(h, jq):
        g, j = divmod(h, 7)
        nk = T * (jq + 1)
        off = SOFF[jq]
        r = lax.broadcasted_iota(jnp.int32, (64, T), 0)
        qu = qt[g, :, jq * T:(jq + 1) * T]
        qm = _bf(jnp.where((r >= 9 * j) & (r < 9 * j + 9), qu, U32(0)))
        sc = jnp.dot(_bf(kk[g, 0:nk // 2, :]), qm, preferred_element_type=F32)
        sd = sc[nk - T:] + bias[...]
        m = jnp.max(sd, axis=0, keepdims=True)
        if jq > 0:
            so = sc[:nk - T]
            m = jnp.maximum(m, jnp.max(so, axis=0, keepdims=True))
            s_buf[h, off:off + nk - T, :] = so
        s_buf[h, off + nk - T:off + nk, :] = sd
        m_buf[h, jq * 8:(jq + 1) * 8, :] = jnp.broadcast_to(m, (8, T))

    def pv_unit(h, jq):
        w0 = (VS * h) // 16 * 16
        o = VS * h - w0
        nk = T * (jq + 1)
        off = SOFF[jq]
        cols = slice(jq * T, (jq + 1) * T)
        m = m_buf[h, jq * 8:jq * 8 + 1, :]
        p = jnp.exp2(s_buf[h, off:off + nk, :] - m).astype(BF16)
        pv = jnp.dot(_bf(vt[w0 // 2:w0 // 2 + 16, 0:nk]), p, preferred_element_type=F32)
        mem = memt[w0:w0 + 32, cols]
        a = gtab[1, h:h + 1, :] / pv[o + DH:o + DH + 1, :]
        b = gtab[0, h:h + 1, :] / (mem[o + DH:o + DH + 1, :] + 1e-6)
        res = pv * a + mem * b
        ot[VS * h:VS * h + VS, cols] = res[o:o + VS]

    def s_blk(h, jq, kb):
        g, j = divmod(h, 7)
        off = SOFF[jq] + kb * T
        r = lax.broadcasted_iota(jnp.int32, (64, T), 0)
        qu = qt[g, :, jq * T:(jq + 1) * T]
        qm = _bf(jnp.where((r >= 9 * j) & (r < 9 * j + 9), qu, U32(0)))
        sc = jnp.dot(_bf(kk[g, kb * 64:(kb + 1) * 64, :]), qm, preferred_element_type=F32)
        if kb == jq:
            sc = sc + bias[...]
        s_buf[h, off:off + T, :] = sc
        blk = SOFF[jq] // T + kb
        m_blk[h, blk * 8:(blk + 1) * 8, :] = jnp.max(sc.reshape(16, 8, T), axis=0)

    def pv_blk(h, jq, kb, st):
        w0 = (VS * h) // 16 * 16
        o = VS * h - w0
        off = SOFF[jq] + kb * T
        cols = slice(jq * T, (jq + 1) * T)
        if kb == 0:
            b0 = SOFF[jq] // T
            mm = m_blk[h, b0 * 8:(b0 + jq + 1) * 8, :]
            st['m'] = jnp.max(mm, axis=0, keepdims=True)
        p = jnp.exp2(s_buf[h, off:off + T, :] - st['m']).astype(BF16)
        part = jnp.dot(_bf(vt[w0 // 2:w0 // 2 + 16, kb * T:(kb + 1) * T]), p, preferred_element_type=F32)
        st['pv'] = part if kb == 0 else st['pv'] + part
        if kb == jq:
            pv = st['pv']
            mem = memt[w0:w0 + 32, cols]
            a = gtab[1, h:h + 1, :] / pv[o + DH:o + DH + 1, :]
            b = gtab[0, h:h + 1, :] / (mem[o + DH:o + DH + 1, :] + 1e-6)
            res = pv * a + mem * b
            ot[VS * h:VS * h + VS, cols] = res[o:o + VS]

    def e2_unit(s, jt):
        cols = pl.ds(pl.multiple_of(s * L + jt * T, T), T)
        hh = x_v[:, cols].astype(F32) + att[:, jt * T:(jt + 1) * T]
        y = _layernorm(hh, 0)
        yb = y.astype(BF16)
        h_s[:, cols] = _u32(hh.astype(BF16))
        out_s[:, cols] = (hh + y).astype(BF16)
        rr = jnp.dot(wr16[...], yb, preferred_element_type=F32)
        r_s[s, :, jt * T:(jt + 1) * T] = jnp.broadcast_to(_rb(rr[0:1, :]), (8, T))

    with _scope('p2_ln'):
        x_copy(0).wait()
        for jt in range(4):
            ln1_unit(0, jt)

    def seg_body(s, carry):
        with _scope('seg'):
            return seg_body_(s, carry)

    def seg_body_(s, carry):
        @pl.when(s < NSEG - 1)
        def _():
            x_copy(s + 1).wait()

        @pl.when(s < NSEG - 2)
        def _():
            x_copy(s + 2).start()

        sp = jnp.maximum(s - 1, 0)
        sn = jnp.minimum(s + 1, NSEG - 1)
        for jt in range(4):
            for g in range(NG):
                q_unit(jt, g)
            e2_unit(sp, jt)
            for g in range(NG):
                k_unit(jt, g)
            for g in range(NG):
                v_unit(jt, g)
        for g in range(NG):
            mem_read_unit(g)
        for g in range(NG):
            mem_update_unit(g)
        if ORD == 'unit':
            for h in range(DIST):
                for jq in range(4):
                    s_unit(h, jq)
            for h in range(H):
                for jq in range(4):
                    pv_unit(h, jq)
                    if h + DIST < H:
                        s_unit(h + DIST, jq)
                if h % 8 == 3:
                    ln1_unit(sn, h // 8)
        else:
            blks = [(jq, kb) for jq in range(4) for kb in range(jq + 1)]
            for h in range(DIST):
                for jq, kb in blks:
                    s_blk(h, jq, kb)
            for h in range(H):
                st = {}
                for jq, kb in blks:
                    pv_blk(h, jq, kb, st)
                    if h + DIST < H:
                        s_blk(h + DIST, jq, kb)
                if h % 8 == 3:
                    ln1_unit(sn, h // 8)
        att[...] = jnp.dot(_bf(wot[...]), ot[...].astype(BF16), preferred_element_type=F32)

        @pl.when(s > 0)
        def _():
            o_copy(s - 1).start()

        for i in range(3):
            @pl.when(s == i)
            def _():
                f_copy(i).start()
        return carry

    lax.fori_loop(0, int(os.environ.get('NIT', NSEG)), seg_body, 0)
    with _scope('epi'):
        for jt in range(4):
            e2_unit(NSEG - 1, jt)
        o_copy(NSEG - 1).start()

    with _scope('ffn'):
        r_all = r_s[...].reshape(NSEG * 8, L)
        tok = ((lax.broadcasted_iota(jnp.int32, (NSEG * 8, L), 0) // 8) * L
               + lax.broadcasted_iota(jnp.int32, (NSEG * 8, L), 1))
        rmax = jnp.max(jnp.max(r_all, axis=1, keepdims=True), axis=0, keepdims=True)
        idx = jnp.clip(jnp.min(jnp.where(r_all == rmax, tok, S)), 0, S - 1)
        base = pl.multiple_of((idx // T) * T, T)
        lane = idx - base
        tile = pl.ds(base, T)

        htile = _bf(h_s[:, tile]).astype(F32)
        ytile = _layernorm(htile, 0).astype(BF16)
        onehot = (lax.broadcasted_iota(jnp.int32, (16, T), 1) == lane).astype(BF16)
        xs = lax.dot_general(onehot, ytile, NT, preferred_element_type=F32).astype(BF16)
        for i in range(3):
            f_copy(i).wait()
        acc = jnp.zeros((D, T), F32)
        for c in range(FF // FC):
            fc = slice(c * FC, (c + 1) * FC)
            gt = _rb(jnp.dot(xs, wg_v[:, fc], preferred_element_type=F32))
            up = _rb(jnp.dot(xs, wu_v[:, fc], preferred_element_type=F32))
            act = _rb(_rb(gt * jax.nn.sigmoid(gt)) * up)[0:1, :]
            for t in range(FC // T):
                acc = acc + wd_v[:, c * FC + t * T:c * FC + (t + 1) * T].astype(F32) * act[:, t * T:(t + 1) * T]
        ycol = _rb(jnp.sum(acc, axis=1, keepdims=True))
        ycol = _rb(ycol * _rb(jax.nn.sigmoid(rmax)))

        NIT = int(os.environ.get('NIT', NSEG))
        for s in range(NIT, NSEG - 1):
            x_copy(s + 1).wait()
        for s in range(NSEG):
            if s < NIT - 1 or s == NSEG - 1:
                o_copy(s).wait()
        sel = lax.broadcasted_iota(jnp.int32, (D, T), 1) == lane
        new = htile + _rb(ytile.astype(F32) + ycol)
        out_s[:, tile] = jnp.where(sel, new, out_s[:, tile].astype(F32)).astype(BF16)
        fix = pltpu.make_async_copy(out_s.at[:, tile], out_hbm.at[0, :, tile], sem_o.at[0])
        fix.start()
        fix.wait()


@jax.jit
def pallas_sequential_preLN__memory_aug_infini_attn__moe_arch_mod__prompt_kernel(
    A_x: jax.Array,
    A_wq: jax.Array,
    A_wk: jax.Array,
    A_wv: jax.Array,
    A_wo: jax.Array,
    A_beta: jax.Array,
    B_x: jax.Array,
    B_w_r: jax.Array,
    B_w_gate: jax.Array,
    B_w_up: jax.Array,
    B_w_down: jax.Array,
):
    del B_x
    hbm = pl.BlockSpec(memory_space=pltpu.HBM)
    scratch = [
        pltpu.VMEM((D, S), BF16),
        pltpu.VMEM((4, D, D), BF16),
        pltpu.VMEM((QR + 320, D), U32),
        pltpu.VMEM((D // 2, 640), U32),
        pltpu.VMEM((D // 2, L), U32),
        pltpu.VMEM((NG, 64, L), U32),
        pltpu.VMEM((NG, 64, L), U32),
        pltpu.VMEM((NG, L // 2, T), U32),
        pltpu.VMEM((NG, 64, L), U32),
        pltpu.VMEM((320, L), U32),
        pltpu.VMEM((640, L), F32),
        pltpu.VMEM((NG, 160, T), F32),
        pltpu.VMEM((H, 1280, T), F32),
        pltpu.VMEM((H, 32, T), F32),
        pltpu.VMEM((H, 80, T), F32),
        pltpu.VMEM((640, L), F32),
        pltpu.VMEM((D, L), F32),
        pltpu.VMEM((D // 2, S), U32),
        pltpu.VMEM((D, S), BF16),
        pltpu.VMEM((NSEG, 8, L), F32),
        pltpu.VMEM((T, T), F32),
        pltpu.VMEM((2, H, T), F32),
        pltpu.VMEM((640, T), F32),
        pltpu.VMEM((NG, 160, T), F32),
        pltpu.VMEM((D, FF), BF16),
        pltpu.VMEM((D, FF), BF16),
        pltpu.VMEM((D, FF), BF16),
        pltpu.VMEM((H,), BF16),
        pltpu.VMEM((D,), BF16),
        pltpu.VMEM((16, D), BF16),
        pltpu.SemaphoreType.DMA((NSEG,)),
        pltpu.SemaphoreType.DMA((4,)),
        pltpu.SemaphoreType.DMA((3,)),
        pltpu.SemaphoreType.DMA((NSEG,)),
        pltpu.SemaphoreType.DMA((2,)),
    ]
    out_t = pl.pallas_call(
        _kernel,
        out_shape=jax.ShapeDtypeStruct((1, D, S), BF16),
        in_specs=[hbm] * 10,
        out_specs=hbm,
        scratch_shapes=scratch,
        compiler_params=pltpu.CompilerParams(vmem_limit_bytes=110 * 1024 * 1024),
        name="infini_moe",
    )(jnp.transpose(A_x, (0, 2, 1)), A_wq, A_wk, A_wv, A_wo, A_beta, B_w_r,
      B_w_gate, B_w_up, jnp.transpose(B_w_down, (1, 0)))
    return jnp.transpose(out_t, (0, 2, 1))
```

```python
import functools
import math

import jax
import jax.numpy as jnp
from jax import lax
import jax.experimental.pallas as pl
import jax.experimental.pallas.tpu as pltpu

F32 = jnp.float32
BF16 = jnp.bfloat16
U32 = jnp.uint32

S = 2048
D = 576
H = 32
DH = 18
NSEG = 4
L = 512
FF = 4608
T = 128
NG = 5
GH = (7, 7, 7, 7, 4)
VS = 20
EPS = 1e-5
QSCALE = DH ** (-0.5) * math.log2(math.e)
MASKVAL = -1000000000.0 * math.log2(math.e)
SOFF = (0, 128, 384, 768)
GWIN = tuple(((140 * g) // 16 * 16, -(-(140 * g + 20 * GH[g]) // 16) * 16) for g in range(NG))
QR = 592
FC = 512
import os
import contextlib
PROF = bool(int(os.environ.get('PROF', '0')))


def _scope(name):
    return jax.named_scope(name) if PROF else contextlib.nullcontext()


HS = int(os.environ.get('HS', '16'))

NT = (((1,), (1,)), ((), ()))


def _bf(x_u32):
    return pltpu.bitcast(x_u32, BF16)


def _u32(x_bf):
    return pltpu.bitcast(x_bf, U32)


def _rb(x):
    return x.astype(BF16).astype(F32)


def _phi(t):
    return jnp.where(t > 0, t + 1.0, jnp.exp(t))


def _layernorm(x, axis):
    m = jnp.mean(x, axis=axis, keepdims=True)
    c = x - m
    v = jnp.mean(c * c, axis=axis, keepdims=True)
    den = _rb(jnp.sqrt(_rb(_rb(v) + EPS)))
    return c * (1.0 / den)


def _ln_scale(pivot, s1, s2):
    md = s1 * (1.0 / D)
    v = jnp.maximum(s2 * (1.0 / D) - md * md, 0.0)
    den = _rb(jnp.sqrt(_rb(_rb(v) + EPS)))
    return pivot + md, 1.0 / den


def _kernel(x_hbm, wq_hbm, wk_hbm, wv_hbm, wo_hbm, beta_hbm, wr_hbm, wg_hbm, wu_hbm, wd_hbm,
            out_hbm,
            x_v, w_v, wqkv, wot, xn, qt, pqt, kk, pkt, vt, memt, bd, s_buf, m_blk,
            ot, att, ln_st, h_s, out_s, r_s, bias, gtab, ones_tab, keep_tab,
            wg_v, wu_v, wd_v, beta_v, wr_v, wr16,
            sem_x, sem_w, sem_f, sem_o, sem_s):
    def x_copy(s):
        return pltpu.make_async_copy(x_hbm.at[0, :, pl.ds(s * L, L)], x_v.at[:, pl.ds(s * L, L)],
                                     sem_x.at[s])

    w_srcs = (wk_hbm, wq_hbm, wv_hbm, wo_hbm)

    def w_copy(i):
        return pltpu.make_async_copy(w_srcs[i], w_v.at[i], sem_w.at[i])

    f_pairs = ((wg_hbm, wg_v), (wu_hbm, wu_v), (wd_hbm, wd_v))

    def f_copy(i):
        return pltpu.make_async_copy(f_pairs[i][0], f_pairs[i][1], sem_f.at[i])

    def o_copy(s):
        return pltpu.make_async_copy(out_s.at[:, pl.ds(s * L, L)], out_hbm.at[0, :, pl.ds(s * L, L)],
                                     sem_o.at[s])

    beta_copy = pltpu.make_async_copy(beta_hbm, beta_v, sem_s.at[0])
    wr_copy = pltpu.make_async_copy(wr_hbm, wr_v, sem_s.at[1])

    def seg_cols(s, jt):
        if isinstance(s, int):
            return slice(s * L + jt * T, s * L + (jt + 1) * T)
        return pl.ds(pl.multiple_of(s * L + jt * T, T), T)

    def ln1_stats(s, jt):
        cols = seg_cols(s, jt)
        pivot = a1 = a2 = None
        for c in range(D // 32):
            x = x_v[32 * c:32 * (c + 1), cols].astype(F32)
            if c == 0:
                pivot = x[0:1, :]
            d = (x - pivot).reshape(4, 8, T)
            p1 = (d[0] + d[1]) + (d[2] + d[3])
            dd = d * d
            p2 = (dd[0] + dd[1]) + (dd[2] + dd[3])
            a1 = p1 if c == 0 else a1 + p1
            a2 = p2 if c == 0 else a2 + p2
        m, inv = _ln_scale(pivot, jnp.sum(a1, axis=0, keepdims=True), jnp.sum(a2, axis=0, keepdims=True))
        ln_st[jt, 0:1, :] = m
        ln_st[jt, 8:9, :] = inv

    def ln1_norm(s, jt):
        x = x_v[:, seg_cols(s, jt)].astype(F32)
        xn[:, jt * T:(jt + 1) * T] = _u32(((x - ln_st[jt, 0:1, :]) * ln_st[jt, 8:9, :]).astype(BF16))

    def q_unit(jt, g):
        cols = slice(jt * T, (jt + 1) * T)
        n = min(64, QR // 2 - 64 * g)
        q = jnp.dot(_bf(wqkv[64 * g:64 * g + n, :]), _bf(xn[:, cols]), preferred_element_type=F32)
        qt[g, 0:n, cols] = _u32((q * QSCALE).astype(BF16))
        pqt[g, 0:n, cols] = _u32(_phi(q).astype(BF16))

    def k_unit(jt, g):
        cols = slice(jt * T, (jt + 1) * T)
        n = min(64, QR // 2 - 64 * g)
        b0 = QR // 2 + 64 * g
        k = jnp.dot(_bf(wqkv[b0:b0 + n, :]), _bf(xn[:, cols]), preferred_element_type=F32)
        pkt[g, 0:n, cols] = _u32(_phi(k).astype(BF16))
        kb = k.astype(BF16)
        if n < 64:
            kb = jnp.concatenate([kb, jnp.zeros((T - 2 * n, T), BF16)], axis=0)
        kk[g, jt * 64:(jt + 1) * 64, :] = _u32(kb.T)

    def v_unit(jt, c):
        cols = slice(jt * T, (jt + 1) * T)
        b0 = QR + 64 * c
        v = jnp.dot(_bf(wqkv[b0:b0 + 64, :]), _bf(xn[:, cols]), preferred_element_type=F32)
        vt[64 * c:64 * (c + 1), cols] = _u32((v + ones_tab[T * c:T * (c + 1), :]).astype(BF16))

    def mem_read_unit(g):
        w0, w1 = GWIN[g]
        b = bd[g, 0:w1 - w0, :].astype(BF16)
        res = jnp.dot(b, _bf(pqt[g]), preferred_element_type=F32)
        lo, hi = 140 * g, 140 * g + 20 * GH[g]
        memt[lo:hi, :] = res[lo - w0:hi - w0]

    def mem_update_unit(g):
        w0, w1 = GWIN[g]
        upd = lax.dot_general(_bf(vt[w0 // 2:w1 // 2, :]), _bf(pkt[g]), NT, preferred_element_type=F32)
        n = w1 - w0
        bd[g, 0:n, :] = bd[g, 0:n, :] + jnp.where(keep_tab[g, 0:n, :] > 0.5, upd, 0.0)

    def s_blk(h, jq, kb):
        g, j = divmod(h, 7)
        off = SOFF[jq] + kb * T
        r = lax.broadcasted_iota(jnp.int32, (64, T), 0)
        qu = qt[g, :, jq * T:(jq + 1) * T]
        qm = _bf(jnp.where((r >= 9 * j) & (r < 9 * j + 9), qu, U32(0)))
        sc = jnp.dot(_bf(kk[g, kb * 64:(kb + 1) * 64, :]), qm, preferred_element_type=F32)
        if kb == jq:
            sc = sc + bias[...]
        s_buf[h, off:off + T, :] = sc
        blk = SOFF[jq] // T + kb
        m_blk[h, blk * 8:(blk + 1) * 8, :] = jnp.max(sc.reshape(16, 8, T), axis=0)

    def pv_blk(h, jq, kb, st):
        w0 = (VS * h) // 16 * 16
        o = VS * h - w0
        off = SOFF[jq] + kb * T
        cols = slice(jq * T, (jq + 1) * T)
        if kb == 0:
            b0 = SOFF[jq] // T
            mm = m_blk[h, b0 * 8:(b0 + jq + 1) * 8, :]
            st['m'] = jnp.max(mm, axis=0, keepdims=True)
        p = jnp.exp2(s_buf[h, off:off + T, :] - st['m']).astype(BF16)
        part = jnp.dot(_bf(vt[w0 // 2:w0 // 2 + 16, kb * T:(kb + 1) * T]), p, preferred_element_type=F32)
        st['pv'] = part if kb == 0 else st['pv'] + part
        if kb == jq:
            pv = st['pv']
            res = pv * (gtab[1, h:h + 1, :] / pv[o + DH:o + DH + 1, :])
            mem = memt[w0:w0 + 32, cols]
            res = res + mem * (gtab[0, h:h + 1, :] / (mem[o + DH:o + DH + 1, :] + 1e-6))
            ot[VS * h // 2:VS * h // 2 + VS // 2, cols] = _u32(res.astype(BF16))[o // 2:o // 2 + VS // 2]

    def o_unit(s, jt, c, st):
        r0, r1 = T * c, min(T * (c + 1), D)
        tile = slice(jt * T, (jt + 1) * T)
        a = jnp.dot(_bf(wot[r0 // 2:r1 // 2, :]), _bf(ot[:, tile]), preferred_element_type=F32)
        hh = x_v[r0:r1, seg_cols(s, jt)].astype(F32) + a
        att[r0:r1, tile] = hh
        if c == 0:
            st['p'] = hh[0:1, :]
        d = hh - st['p']
        s1 = jnp.sum(d, axis=0, keepdims=True)
        s2 = jnp.sum(d * d, axis=0, keepdims=True)
        st['s1'] = s1 if c == 0 else st['s1'] + s1
        st['s2'] = s2 if c == 0 else st['s2'] + s2

    def e2_unit(s, jt, st):
        cols = seg_cols(s, jt)
        m, inv = _ln_scale(st['p'], st['s1'], st['s2'])
        hh = att[:, jt * T:(jt + 1) * T]
        y = (hh - m) * inv
        h_s[:, cols] = _u32(hh.astype(BF16))
        out_s[:, cols] = (hh + y).astype(BF16)
        rr = jnp.dot(wr16[...], y.astype(BF16), preferred_element_type=F32)
        r_s[s, :, jt * T:(jt + 1) * T] = jnp.broadcast_to(_rb(rr[0:1, :]), (8, T))

    def prep_qk(i, base):
        wt = _u32(w_v[i].T)
        for g in range(NG):
            n = 9 * GH[g]
            wqkv[base + 64 * g:base + 64 * g + n, :] = wt[63 * g:63 * g + n, :]

    def prep_v():
        wt = _u32(w_v[2].T)
        for h in range(H):
            wqkv[QR + 10 * h:QR + 10 * h + 9, :] = wt[9 * h:9 * h + 9, :]

    def prep_o():
        wt = _u32(w_v[3])
        wpad = jnp.concatenate(
            [piece for h in range(H) for piece in (wt[9 * h:9 * h + 9, :], jnp.zeros((1, D), U32))], axis=0)
        wot[...] = _u32(_bf(wpad).T)

    BLKS = [(jq, kb) for jq in range(4) for kb in range(jq + 1)]

    def s_items(heads):
        return [functools.partial(s_blk, h, jq, kb) for h in heads for jq, kb in BLKS]

    def pv_items(heads):
        items = []
        for h in heads:
            st = {}
            items += [functools.partial(pv_blk, h, jq, kb, st) for jq, kb in BLKS]
        return items

    def interleave(*seqs):
        seqs = [q for q in seqs if q]
        order = []
        for i, q in enumerate(seqs):
            order += [((j + 0.5) / len(q), i, j) for j in range(len(q))]
        for _, i, j in sorted(order):
            seqs[i][j]()

    def proj_items(fn):
        return [functools.partial(fn, jt, g) for jt in range(4) for g in range(NG)]

    def out_items(s):
        sts = [{} for _ in range(4)]
        o_items = [functools.partial(o_unit, s, jt, c, sts[jt]) for jt in range(4) for c in range(NG)]
        e_items = [functools.partial(e2_unit, s, jt, sts[jt]) for jt in range(4)]
        return o_items, e_items

    HA = list(range(HS))
    HB = list(range(HS, H))

    x_copy(0).start()
    w_copy(1).start()
    beta_copy.start()
    wr_copy.start()
    with _scope('p0_const'):
        kr = lax.broadcasted_iota(jnp.int32, (T, T), 0)
        qc = lax.broadcasted_iota(jnp.int32, (T, T), 1)
        bias[...] = jnp.where(kr > qc, MASKVAL, 0.0).astype(F32)
        wqkv[...] = jnp.zeros(wqkv.shape, U32)
        w_copy(0).start()
        bd[...] = jnp.zeros(bd.shape, F32)
        memt[...] = jnp.zeros(memt.shape, F32)
        row = lax.broadcasted_iota(jnp.int32, (640, T), 0)
        ones_tab[...] = jnp.where(row % VS == DH, 1.0, 0.0).astype(F32)
        for g in range(NG):
            row = lax.broadcasted_iota(jnp.int32, (160, T), 0) + (GWIN[g][0] - 140 * g)
            lane = lax.broadcasted_iota(jnp.int32, (160, T), 1)
            keep = ((row >= 0) & (row < 20 * GH[g]) & (lane >= (row // VS) * DH)
                    & (lane < (row // VS) * DH + DH))
            keep_tab[g] = jnp.where(keep, 1.0, 0.0).astype(F32)
        pqt[NG - 1] = jnp.zeros(pqt.shape[1:], U32)
        pkt[NG - 1] = jnp.zeros(pkt.shape[1:], U32)

    with _scope('p1_ln'):
        x_copy(0).wait()
        w_copy(2).start()
        for jt in range(4):
            ln1_stats(0, jt)
            ln1_norm(0, jt)
    with _scope('p2_wq'):
        w_copy(1).wait()
        prep_qk(1, 0)
    with _scope('p3_q'):
        w_copy(0).wait()
        w_copy(3).start()
        prep_qk(0, QR // 2)
        for jt in range(4):
            for g in range(NG):
                q_unit(jt, g)
    with _scope('p4_k'):
        w_copy(2).wait()
        for i in range(1, NSEG):
            x_copy(i).start()
        prep_v()
        for jt in range(4):
            for g in range(NG):
                k_unit(jt, g)
    with _scope('p5_v'):
        w_copy(3).wait()
        beta_copy.wait()
        wr_copy.wait()
        prep_o()
        beta = beta_v[...].astype(F32).reshape(1, H)
        hl = lax.broadcasted_iota(jnp.int32, (H, H), 1)
        hs = lax.broadcasted_iota(jnp.int32, (H, H), 0)
        bcol = jnp.sum(jnp.where(hl == hs, jnp.broadcast_to(beta, (H, H)), 0.0), axis=1, keepdims=True)
        gate = _rb(jax.nn.sigmoid(bcol))
        gtab[0] = jnp.broadcast_to(gate, (H, T))
        gtab[1] = jnp.broadcast_to(_rb(1.0 - gate), (H, T))
        r16 = lax.broadcasted_iota(jnp.int32, (16, D), 0)
        wr_row = wr_v[...].astype(F32).reshape(1, D)
        wr16[...] = jnp.where(r16 == 0, jnp.broadcast_to(wr_row, (16, D)), 0.0).astype(BF16)
        for jt in range(4):
            for g in range(NG):
                v_unit(jt, g)
        for it in s_items(HA):
            it()
        for i in range(1, NSEG):
            x_copy(i).wait()
        for jt in range(4):
            ln1_stats(1, jt)

    def seg_body(s, carry):
        with _scope('seg_x'):
            interleave(pv_items(HA), s_items(HB))

        @pl.when(s < NSEG - 1)
        def _():
            with _scope('seg_y'):
                ln = [functools.partial(ln1_norm, s + 1, jt) for jt in range(4)]
                qs = proj_items(q_unit)
                mxu1 = ([ln[0]] + [functools.partial(mem_update_unit, g) for g in range(NG)]
                        + [ln[1]] + qs[0:5] + [ln[2]] + qs[5:10] + [ln[3]] + qs[10:20]
                        + proj_items(k_unit))
                interleave(pv_items(HB), mxu1)
                o_items, e_items = out_items(s)
                for it in o_items:
                    it()
                interleave(proj_items(v_unit) + [functools.partial(mem_read_unit, g) for g in range(NG)],
                           e_items[0:2])
                sn = jnp.minimum(s + 2, NSEG - 1)
                interleave(s_items(HA), e_items[2:4] + [functools.partial(ln1_stats, sn, jt) for jt in range(4)])
                o_copy(s).start()

                @pl.when(s == 0)
                def _():
                    f_copy(0).start()
                    f_copy(1).start()

                @pl.when(s == 1)
                def _():
                    f_copy(2).start()

        @pl.when(s == NSEG - 1)
        def _():
            with _scope('seg_z'):
                for it in pv_items(HB):
                    it()
                o_items, e_items = out_items(s)
                for jt in range(4):
                    for it in o_items[jt * NG:(jt + 1) * NG]:
                        it()
                    if jt > 0:
                        e_items[jt - 1]()
                e_items[3]()
                o_copy(s).start()
        return carry

    lax.fori_loop(0, NSEG, seg_body, 0)
    with _scope('ffn'):
        r_all = r_s[...].reshape(NSEG * 8, L)
        tok = ((lax.broadcasted_iota(jnp.int32, (NSEG * 8, L), 0) // 8) * L
               + lax.broadcasted_iota(jnp.int32, (NSEG * 8, L), 1))
        rmax = jnp.max(jnp.max(r_all, axis=1, keepdims=True), axis=0, keepdims=True)
        idx = jnp.clip(jnp.min(jnp.where(r_all == rmax, tok, S)), 0, S - 1)
        base = pl.multiple_of((idx // T) * T, T)
        lane = idx - base
        tile = pl.ds(base, T)

        htile = _bf(h_s[:, tile]).astype(F32)
        ytile = _layernorm(htile, 0).astype(BF16)
        onehot = (lax.broadcasted_iota(jnp.int32, (16, T), 1) == lane).astype(BF16)
        xs = lax.dot_general(onehot, ytile, NT, preferred_element_type=F32).astype(BF16)
        for i in range(3):
            f_copy(i).wait()
        acc = jnp.zeros((D, T), F32)
        for c in range(FF // FC):
            fc = slice(c * FC, (c + 1) * FC)
            gt = _rb(jnp.dot(xs, wg_v[:, fc], preferred_element_type=F32))
            up = _rb(jnp.dot(xs, wu_v[:, fc], preferred_element_type=F32))
            act = _rb(_rb(gt * jax.nn.sigmoid(gt)) * up)[0:1, :]
            for t in range(FC // T):
                acc = acc + wd_v[:, c * FC + t * T:c * FC + (t + 1) * T].astype(F32) * act[:, t * T:(t + 1) * T]
        ycol = _rb(jnp.sum(acc, axis=1, keepdims=True))
        ycol = _rb(ycol * _rb(jax.nn.sigmoid(rmax)))

        for s in range(NSEG):
            o_copy(s).wait()
        sel = lax.broadcasted_iota(jnp.int32, (D, T), 1) == lane
        new = htile + _rb(ytile.astype(F32) + ycol)
        out_s[:, tile] = jnp.where(sel, new, out_s[:, tile].astype(F32)).astype(BF16)
        fix = pltpu.make_async_copy(out_s.at[:, tile], out_hbm.at[0, :, tile], sem_o.at[0])
        fix.start()
        fix.wait()


@jax.jit
def pallas_sequential_preLN__memory_aug_infini_attn__moe_arch_mod__prompt_kernel(
    A_x: jax.Array,
    A_wq: jax.Array,
    A_wk: jax.Array,
    A_wv: jax.Array,
    A_wo: jax.Array,
    A_beta: jax.Array,
    B_x: jax.Array,
    B_w_r: jax.Array,
    B_w_gate: jax.Array,
    B_w_up: jax.Array,
    B_w_down: jax.Array,
):
    del B_x
    hbm = pl.BlockSpec(memory_space=pltpu.HBM)
    scratch = [
        pltpu.VMEM((D, S), BF16),
        pltpu.VMEM((4, D, D), BF16),
        pltpu.VMEM((QR + 320, D), U32),
        pltpu.VMEM((D // 2, 640), U32),
        pltpu.VMEM((D // 2, L), U32),
        pltpu.VMEM((NG, 64, L), U32),
        pltpu.VMEM((NG, 64, L), U32),
        pltpu.VMEM((NG, L // 2, T), U32),
        pltpu.VMEM((NG, 64, L), U32),
        pltpu.VMEM((320, L), U32),
        pltpu.VMEM((640, L), F32),
        pltpu.VMEM((NG, 160, T), F32),
        pltpu.VMEM((H, 1280, T), F32),
        pltpu.VMEM((H, 80, T), F32),
        pltpu.VMEM((320, L), U32),
        pltpu.VMEM((D, L), F32),
        pltpu.VMEM((4, 16, T), F32),
        pltpu.VMEM((D // 2, S), U32),
        pltpu.VMEM((D, S), BF16),
        pltpu.VMEM((NSEG, 8, L), F32),
        pltpu.VMEM((T, T), F32),
        pltpu.VMEM((2, H, T), F32),
        pltpu.VMEM((640, T), F32),
        pltpu.VMEM((NG, 160, T), F32),
        pltpu.VMEM((D, FF), BF16),
        pltpu.VMEM((D, FF), BF16),
        pltpu.VMEM((D, FF), BF16),
        pltpu.VMEM((H,), BF16),
        pltpu.VMEM((D,), BF16),
        pltpu.VMEM((16, D), BF16),
        pltpu.SemaphoreType.DMA((NSEG,)),
        pltpu.SemaphoreType.DMA((4,)),
        pltpu.SemaphoreType.DMA((3,)),
        pltpu.SemaphoreType.DMA((NSEG,)),
        pltpu.SemaphoreType.DMA((2,)),
    ]
    out_t = pl.pallas_call(
        _kernel,
        out_shape=jax.ShapeDtypeStruct((1, D, S), BF16),
        in_specs=[hbm] * 10,
        out_specs=hbm,
        scratch_shapes=scratch,
        compiler_params=pltpu.CompilerParams(vmem_limit_bytes=110 * 1024 * 1024),
        name="infini_moe",
    )(jnp.transpose(A_x, (0, 2, 1)), A_wq, A_wk, A_wv, A_wo, A_beta, B_w_r,
      B_w_gate, B_w_up, jnp.transpose(B_w_down, (1, 0)))
    return jnp.transpose(out_t, (0, 2, 1))
```

```python
import functools
import math

import jax
import jax.numpy as jnp
from jax import lax
import jax.experimental.pallas as pl
import jax.experimental.pallas.tpu as pltpu

F32 = jnp.float32
BF16 = jnp.bfloat16
U32 = jnp.uint32

S = 2048
D = 576
H = 32
DH = 18
NSEG = 4
L = 512
FF = 4608
T = 128
NG = 5
GH = (7, 7, 7, 7, 4)
VS = 20
EPS = 1e-5
QSCALE = DH ** (-0.5) * math.log2(math.e)
MASKVAL = -1000000000.0 * math.log2(math.e)
SOFF = (0, 128, 384, 768)
MOFF = (0, 2, 5, 9)
GWIN = tuple(((140 * g) // 16 * 16, -(-(140 * g + 20 * GH[g]) // 16) * 16) for g in range(NG))
QR = 592
FC = 512
import os
import contextlib
PROF = bool(int(os.environ.get('PROF', '0')))


def _scope(name):
    return jax.named_scope(name) if PROF else contextlib.nullcontext()


HS = int(os.environ.get('HS', '16'))
PACK = int(os.environ.get('PACK', '0'))
NS0 = int(os.environ.get('NS0', '8'))
KE = (VS * HS) // T * T

NT = (((1,), (1,)), ((), ()))


def _bf(x_u32):
    return pltpu.bitcast(x_u32, BF16)


def _u32(x_bf):
    return pltpu.bitcast(x_bf, U32)


def _pack_rows(y):
    if not PACK:
        return _u32(y.astype(BF16))
    n = y.shape[0]
    parts = []
    full = n // 32 * 32
    if full:
        y4 = y[0:full].reshape(full // 32, 2, 16, T)
        parts.append(pltpu.pack_elementwise([y4[:, 0], y4[:, 1]], packed_dtype=BF16).reshape(full // 2, T))
    if n > full:
        parts.append(pltpu.pack_elementwise([y[full:full + 8], y[full + 8:full + 16]], packed_dtype=BF16))
    return parts[0] if len(parts) == 1 else jnp.concatenate(parts, axis=0)


def _rb(x):
    return x.astype(BF16).astype(F32)


def _phi(t):
    return jnp.where(t > 0, t + 1.0, jnp.exp(t))


def _layernorm(x, axis):
    m = jnp.mean(x, axis=axis, keepdims=True)
    c = x - m
    v = jnp.mean(c * c, axis=axis, keepdims=True)
    den = _rb(jnp.sqrt(_rb(_rb(v) + EPS)))
    return c * (1.0 / den)


def _ln_scale(pivot, s1, s2):
    md = s1 * (1.0 / D)
    v = jnp.maximum(s2 * (1.0 / D) - md * md, 0.0)
    den = _rb(jnp.sqrt(_rb(_rb(v) + EPS)))
    return pivot + md, 1.0 / den


def _kernel(x_hbm, wq_hbm, wk_hbm, wv_hbm, wo_hbm, beta_hbm, wr_hbm, wg_hbm, wu_hbm, wd_hbm,
            out_hbm,
            x_v, w_v, wqkv, wot, xn, qt, pqt, kk, pkt, vt, memt, bd, s_buf, m_blk,
            ot, att, ln_st, h_s, out_s, r_s, bias, bias2, gtab, ones_tab, keep_tab,
            wg_v, wu_v, wd_v, beta_v, wr_v, wr16, dtmp,
            zero_s, sem_x, sem_w, sem_f, sem_o, sem_s):
    def x_copy(s):
        return pltpu.make_async_copy(x_hbm.at[0, :, pl.ds(s * L, L)], x_v.at[:, pl.ds(s * L, L)],
                                     sem_x.at[s])

    w_srcs = (wk_hbm, wq_hbm, wv_hbm, wo_hbm)

    def w_copy(i):
        return pltpu.make_async_copy(w_srcs[i], w_v.at[i], sem_w.at[i])

    f_pairs = ((wg_hbm, wg_v), (wu_hbm, wu_v), (wd_hbm, wd_v))

    def f_copy(i):
        return pltpu.make_async_copy(f_pairs[i][0], f_pairs[i][1], sem_f.at[i])

    def o_copy(s):
        return pltpu.make_async_copy(out_s.at[:, pl.ds(s * L, L)], out_hbm.at[0, :, pl.ds(s * L, L)],
                                     sem_o.at[s])

    beta_copy = pltpu.make_async_copy(beta_hbm, beta_v, sem_s.at[0])
    wr_copy = pltpu.make_async_copy(wr_hbm, wr_v, sem_s.at[1])

    def seg_cols(s, jt):
        if isinstance(s, int):
            return slice(s * L + jt * T, s * L + (jt + 1) * T)
        return pl.ds(pl.multiple_of(s * L + jt * T, T), T)

    def ln1_stats(s, jt, tok=None):
        cols = seg_cols(s, jt)
        pivot = a1 = a2 = None
        for c in range(D // 32):
            x = x_v[32 * c:32 * (c + 1), cols].astype(F32)
            if c == 0:
                pivot = x[0:1, :]
                if tok is not None:
                    pivot = pivot + tok()
            d = (x - pivot).reshape(4, 8, T)
            p1 = (d[0] + d[1]) + (d[2] + d[3])
            dd = d * d
            p2 = (dd[0] + dd[1]) + (dd[2] + dd[3])
            a1 = p1 if c == 0 else a1 + p1
            a2 = p2 if c == 0 else a2 + p2
        m, inv = _ln_scale(pivot, jnp.sum(a1, axis=0, keepdims=True), jnp.sum(a2, axis=0, keepdims=True))
        ln_st[s, jt, 0:1, :] = m
        ln_st[s, jt, 8:9, :] = inv

    def ln1_norm(s, jt):
        x = x_v[:, seg_cols(s, jt)].astype(F32)
        xn[:, jt * T:(jt + 1) * T] = _u32(((x - ln_st[s, jt, 0:1, :]) * ln_st[s, jt, 8:9, :]).astype(BF16))

    def q_unit(jt, g):
        cols = slice(jt * T, (jt + 1) * T)
        n = min(64, QR // 2 - 64 * g)
        q = jnp.dot(_bf(wqkv[64 * g:64 * g + n, :]), _bf(xn[:, cols]), preferred_element_type=F32)
        qt[g, 0:n, cols] = _pack_rows(q * QSCALE)
        pqt[g, 0:n, cols] = _pack_rows(_phi(q))

    def k_unit(jt, g):
        cols = slice(jt * T, (jt + 1) * T)
        n = min(64, QR // 2 - 64 * g)
        b0 = QR // 2 + 64 * g
        k = jnp.dot(_bf(wqkv[b0:b0 + n, :]), _bf(xn[:, cols]), preferred_element_type=F32)
        pkt[g, 0:n, cols] = _pack_rows(_phi(k))
        kb = _pack_rows(k)
        if n < 64:
            kb = jnp.concatenate([kb, jnp.zeros((64 - n, T), U32)], axis=0)
        kk[g, jt * 64:(jt + 1) * 64, :] = _u32(_bf(kb).T)

    def v_unit(jt, c):
        cols = slice(jt * T, (jt + 1) * T)
        b0 = QR + 64 * c
        v = jnp.dot(_bf(wqkv[b0:b0 + 64, :]), _bf(xn[:, cols]), preferred_element_type=F32)
        vt[64 * c:64 * (c + 1), cols] = _pack_rows(v + ones_tab[T * c:T * (c + 1), :])

    def mem_read_unit(g):
        w0, w1 = GWIN[g]
        b = bd[g, 0:w1 - w0, :].astype(BF16)
        res = jnp.dot(b, _bf(pqt[g]), preferred_element_type=F32)
        lo, hi = 140 * g, 140 * g + 20 * GH[g]
        memt[lo:hi, :] = res[lo - w0:hi - w0]

    def mem_update_unit(g):
        w0, w1 = GWIN[g]
        upd = lax.dot_general(_bf(vt[w0 // 2:w1 // 2, :]), _bf(pkt[g]), NT, preferred_element_type=F32)
        n = w1 - w0
        bd[g, 0:n, :] = bd[g, 0:n, :] + jnp.where(keep_tab[g, 0:n, :] > 0.5, upd, 0.0)

    def head_rows(j):
        r = lax.broadcasted_iota(jnp.int32, (64, T), 0)
        return (r >= 9 * j) & (r < 9 * j + 9)

    def s_blk(h, jq, kb, half=False):
        g, j = divmod(h, 7)
        off = SOFF[jq] + kb * T
        n = 64 if half else T
        qm = _bf(jnp.where(head_rows(j), qt[g, :, jq * T:(jq + 1) * T], U32(0)))
        sc = jnp.dot(_bf(kk[g, kb * 64:kb * 64 + n // 2, :]), qm, preferred_element_type=F32)
        if kb == jq:
            sc = sc + bias[0:n, :]
        s_buf[h, off:off + n, :] = sc
        slot = MOFF[jq] + kb
        m_blk[h, slot * 8:(slot + 1) * 8, :] = jnp.max(sc.reshape(n // 8, 8, T), axis=0)

    def s_pair(ha, jq):
        g, j = divmod(ha, 7)
        off = SOFF[jq] + jq * T + 64
        lo = lax.broadcasted_iota(jnp.int32, (64, T), 1) < 64
        qu = qt[g, :, jq * T:(jq + 1) * T]
        qmix = jnp.where(lo, pltpu.roll(qu, 64, 1), qu)
        qm = _bf(jnp.where((lo & head_rows(j)) | (~lo & head_rows(j + 1)), qmix, U32(0)))
        sc = jnp.dot(_bf(kk[g, jq * 64 + 32:jq * 64 + 64, :]), qm, preferred_element_type=F32) + bias2[...]
        s_buf[ha, off:off + 64, :] = sc
        pm = jnp.max(sc.reshape(8, 8, T), axis=0)
        hi = lax.broadcasted_iota(jnp.int32, (8, T), 1) >= 64
        slot = MOFF[jq] + jq + 1
        m_blk[ha, slot * 8:(slot + 1) * 8, :] = jnp.where(hi, pltpu.roll(pm, 64, 1), -jnp.inf)
        m_blk[ha + 1, slot * 8:(slot + 1) * 8, :] = jnp.where(hi, pm, -jnp.inf)

    def row_max(h, jq, nslots):
        return jnp.max(m_blk[h, MOFF[jq] * 8:(MOFF[jq] + nslots) * 8, :], axis=0, keepdims=True)

    def pv_blk(h, jq, kb, st, role):
        w0 = (VS * h) // 16 * 16
        o = VS * h - w0
        off = SOFF[jq] + kb * T
        cols = slice(jq * T, (jq + 1) * T)
        key = role or 'a'
        z = st['z']
        if kb == 0 and role != 'b':
            st['ma'] = row_max(h, jq, jq + 1 if role is None else jq + 2)
            if role == 'a':
                st['mb'] = row_max(h + 1, jq, jq + 2)
        m = st['m' + key]
        if kb < jq or role is None:
            p = jnp.exp2(s_buf[h + z, off:off + T, :] - m).astype(BF16)
        else:
            if role == 'a':
                hi1 = lax.broadcasted_iota(jnp.int32, (1, T), 1) >= 64
                hi = lax.broadcasted_iota(jnp.int32, (64, T), 1) >= 64
                m2 = jnp.where(hi1, st['mb'], pltpu.roll(st['ma'], 64, 1))
                e2 = jnp.exp2(s_buf[h + z, off + 64:off + T, :] - m2)
                p2 = jnp.where(hi, pltpu.roll(e2, 64, 1), 0.0)
                st['p2b'] = jnp.where(hi, e2, 0.0)
            else:
                p2 = st['p2b']
            p1 = jnp.exp2(s_buf[h + z, off:off + 64, :] - m)
            p = jnp.concatenate([p1, p2], axis=0).astype(BF16)
        part = jnp.dot(_bf(vt[w0 // 2:w0 // 2 + 16, kb * T:(kb + 1) * T]), p, preferred_element_type=F32)
        st['pv' + key] = part if kb == 0 else st['pv' + key] + part
        if kb == jq:
            pv = st['pv' + key]
            res = pv * (gtab[1, h:h + 1, :] / pv[o + DH:o + DH + 1, :])
            mem = memt[w0:w0 + 32, cols]
            res = res + mem * (gtab[0, h:h + 1, :] / (mem[o + DH:o + DH + 1, :] + 1e-6))
            ot[VS * h // 2:VS * h // 2 + VS // 2, cols] = _u32(res.astype(BF16))[o // 2:o // 2 + VS // 2]

    def o_early(s, jt, c):
        r0, r1 = T * c, min(T * (c + 1), D)
        tile = slice(jt * T, (jt + 1) * T)
        a = jnp.dot(_bf(wot[r0 // 2:r1 // 2, 0:KE]), _bf(ot[0:KE // 2, tile]), preferred_element_type=F32)
        att[r0:r1, tile] = x_v[r0:r1, seg_cols(s, jt)].astype(F32) + a

    def o_unit(s, jt, c, st):
        r0, r1 = T * c, min(T * (c + 1), D)
        tile = slice(jt * T, (jt + 1) * T)
        a = jnp.dot(_bf(wot[r0 // 2:r1 // 2, KE:640]), _bf(ot[KE // 2:320, tile]), preferred_element_type=F32)
        hh = att[r0:r1, tile] + a
        att[r0:r1, tile] = hh
        if c == 0:
            st['p'] = hh[0:1, :]
        d = hh - st['p']
        s1 = jnp.sum(d, axis=0, keepdims=True)
        s2 = jnp.sum(d * d, axis=0, keepdims=True)
        st['s1'] = s1 if c == 0 else st['s1'] + s1
        st['s2'] = s2 if c == 0 else st['s2'] + s2

    def e2_unit(s, jt, st):
        cols = seg_cols(s, jt)
        m, inv = _ln_scale(st['p'], st['s1'], st['s2'])
        hh = att[:, jt * T:(jt + 1) * T]
        y = (hh - m) * inv
        h_s[:, cols] = pltpu.pack_elementwise([hh[0:D // 2], hh[D // 2:D]], packed_dtype=BF16)
        out_s[:, cols] = (hh + y).astype(BF16)
        rr = jnp.dot(wr16[...], y.astype(BF16), preferred_element_type=F32)
        r_s[s, :, jt * T:(jt + 1) * T] = jnp.broadcast_to(_rb(rr[0:1, :]), (8, T))

    def prep_qk(i, base):
        wt = _u32(w_v[i].T)
        for g in range(NG):
            n = 9 * GH[g]
            wqkv[base + 64 * g:base + 64 * g + n, :] = wt[63 * g:63 * g + n, :]
        deinterleave(base, 4 * 64)
        deinterleave(base + 4 * 64, QR // 2 - 4 * 64)

    def prep_v():
        wt = _u32(w_v[2].T)
        for h in range(H):
            wqkv[QR + 10 * h:QR + 10 * h + 9, :] = wt[9 * h:9 * h + 9, :]
        deinterleave(QR, 320)

    def deinterleave(base, nwords):
        lo16 = U32(0xFFFF)
        hi16 = U32(0xFFFF0000)
        for lt in range(NG if PACK else 0):
            w = min(T, D - T * lt)
            lanes = slice(T * lt, T * lt + w)
            dtmp[0:nwords, 0:w] = wqkv[base:base + nwords, lanes]
            b = 0
            while b < nwords:
                half = 8 if nwords - b >= 16 else 4
                ev = dtmp[pl.ds(b, half, stride=2), :]
                od = dtmp[pl.ds(b + 1, half, stride=2), :]
                wqkv[base + b:base + b + half, lanes] = ((ev & lo16) | (od << 16))[:, 0:w]
                wqkv[base + b + half:base + b + 2 * half, lanes] = ((ev >> 16) | (od & hi16))[:, 0:w]
                b += 2 * half

    def prep_o():
        wt = _u32(w_v[3])
        wpad = jnp.concatenate(
            [piece for h in range(H) for piece in (wt[9 * h:9 * h + 9, :], jnp.zeros((1, D), U32))], axis=0)
        wot[...] = _u32(_bf(wpad).T)

    BLKS = [(jq, kb) for jq in range(4) for kb in range(jq + 1)]

    def head_sets(heads):
        sets, i = [], 0
        while i < len(heads):
            h = heads[i]
            if h % 7 % 2 == 0 and h % 7 < 6 and i + 1 < len(heads):
                sets.append((h, h + 1))
                i += 2
            else:
                assert h % 7 == 6
                sets.append((h,))
                i += 1
        return sets

    def s_items(heads, small_tail=0):
        big, small = [], []
        for hs in head_sets(heads):
            for jq, kb in BLKS:
                halved = len(hs) == 2 and kb == jq
                for h in hs:
                    (small if halved else big).append(functools.partial(s_blk, h, jq, kb, halved))
                if halved:
                    small.append(functools.partial(s_pair, hs[0], jq))
        tail = small[len(small) - small_tail:] if small_tail else []
        small = small[:len(small) - small_tail] if small_tail else small
        order = sorted([((j + 0.5) / len(big), 0, j) for j in range(len(big))]
                       + [((j + 0.5) / len(small), 1, j) for j in range(len(small))])
        return [(big, small)[w][j] for _, w, j in order] + tail

    def phase_x():
        sb = s_items(HB)
        for it in sb[0:NS0]:
            it()
        interleave(pv_items(HA), sb[NS0:])

    def pv_items(heads, z=0):
        items = []
        for hs in head_sets(heads):
            st = {'z': z}
            roles = ('a', 'b') if len(hs) == 2 else (None,)
            for jq, kb in BLKS:
                for h, role in zip(hs, roles):
                    items.append(functools.partial(pv_blk, h, jq, kb, st, role))
        return items

    def interleave(*seqs):
        seqs = [q for q in seqs if q]
        order = []
        for i, q in enumerate(seqs):
            order += [((j + 0.5) / len(q), i, j) for j in range(len(q))]
        for _, i, j in sorted(order):
            seqs[i][j]()

    def proj_items(fn):
        return [functools.partial(fn, jt, g) for jt in range(4) for g in range(NG)]

    def out_items(s):
        sts = [{} for _ in range(4)]
        o_items = [functools.partial(o_unit, s, jt, c, sts[jt]) for jt in range(4) for c in range(NG)]
        e_items = [functools.partial(e2_unit, s, jt, sts[jt]) for jt in range(4)]
        early = [functools.partial(o_early, s, jt, c) for jt in range(4) for c in range(NG)]
        return early, o_items, e_items

    HA = list(range(HS))
    HB = list(range(HS, H))

    x_copy(0).start()
    w_copy(1).start()
    zero_s[0] = 0
    beta_copy.start()
    wr_copy.start()
    with _scope('p0_const'):
        kr = lax.broadcasted_iota(jnp.int32, (T, T), 0)
        qc = lax.broadcasted_iota(jnp.int32, (T, T), 1)
        bias[...] = jnp.where(kr > qc, MASKVAL, 0.0).astype(F32)
        kr2 = lax.broadcasted_iota(jnp.int32, (64, T), 0)
        qc2 = lax.broadcasted_iota(jnp.int32, (64, T), 1)
        bias2[...] = jnp.where(kr2 > (qc2 & 63), MASKVAL, 0.0).astype(F32)
        wqkv[...] = jnp.zeros(wqkv.shape, U32)
        bd[...] = jnp.zeros(bd.shape, F32)
        memt[...] = jnp.zeros(memt.shape, F32)
        row = lax.broadcasted_iota(jnp.int32, (640, T), 0)
        sub = row & 31
        nat = (row - sub) + jnp.where(sub < 16, 2 * sub, 2 * sub - 31)
        if not PACK:
            nat = row
        ones_tab[...] = jnp.where(nat % VS == DH, 1.0, 0.0).astype(F32)
        dtmp[...] = jnp.zeros(dtmp.shape, U32)
        for g in range(NG):
            row = lax.broadcasted_iota(jnp.int32, (160, T), 0) + (GWIN[g][0] - 140 * g)
            lane = lax.broadcasted_iota(jnp.int32, (160, T), 1)
            keep = ((row >= 0) & (row < 20 * GH[g]) & (lane >= (row // VS) * DH)
                    & (lane < (row // VS) * DH + DH))
            keep_tab[g] = jnp.where(keep, 1.0, 0.0).astype(F32)
        pqt[NG - 1] = jnp.zeros(pqt.shape[1:], U32)
        pkt[NG - 1] = jnp.zeros(pkt.shape[1:], U32)

    with _scope('p1_ln'):
        x_copy(0).wait()
        w_copy(0).start()
        for jt in range(4):
            ln1_stats(0, jt)
            ln1_norm(0, jt)
    with _scope('p2_wq'):
        w_copy(1).wait()
        w_copy(2).start()
        prep_qk(1, 0)
        for g in range(NG):
            for jt in range(2):
                q_unit(jt, g)
    with _scope('p3_q'):
        w_copy(0).wait()
        w_copy(3).start()
        prep_qk(0, QR // 2)
        for jt in range(2, 4):
            for g in range(NG):
                q_unit(jt, g)
    with _scope('p4_k'):
        w_copy(2).wait()
        for i in range(1, NSEG):
            x_copy(i).start()
        prep_v()
        for jt in range(4):
            for g in range(NG):
                k_unit(jt, g)
    with _scope('p5_v'):
        w_copy(3).wait()
        beta_copy.wait()
        wr_copy.wait()
        for i in range(1, NSEG):
            x_copy(i).wait()
        prep_o()
        beta = beta_v[...].astype(F32).reshape(1, H)
        hl = lax.broadcasted_iota(jnp.int32, (H, H), 1)
        hs = lax.broadcasted_iota(jnp.int32, (H, H), 0)
        bcol = jnp.sum(jnp.where(hl == hs, jnp.broadcast_to(beta, (H, H)), 0.0), axis=1, keepdims=True)
        gate = _rb(jax.nn.sigmoid(bcol))
        gtab[0] = jnp.broadcast_to(gate, (H, T))
        gtab[1] = jnp.broadcast_to(_rb(1.0 - gate), (H, T))
        r16 = lax.broadcasted_iota(jnp.int32, (16, D), 0)
        wr_row = wr_v[...].astype(F32).reshape(1, D)
        wr16[...] = jnp.where(r16 == 0, jnp.broadcast_to(wr_row, (16, D)), 0.0).astype(BF16)
        interleave(proj_items(v_unit) + s_items(HA, 16),
                   [functools.partial(ln1_stats, i, jt) for i in range(1, NSEG) for jt in range(4)])

    def seg_body(s, carry):
        with _scope('seg_xy'):
            z = zero_s[0]
            phase_x()
            ln = [functools.partial(ln1_norm, s + 1, jt) for jt in range(4)]
            qs = proj_items(q_unit)
            early, o_items, e_items = out_items(s)
            for it in [ln[0]] + early[0:10] + [ln[1]]:
                it()
            mxu1 = ([functools.partial(mem_update_unit, g) for g in range(NG)]
                    + qs[0:5] + [ln[2]] + early[10:20] + qs[5:10] + [ln[3]]
                    + qs[10:20] + proj_items(k_unit))
            interleave(pv_items(HB, z), mxu1)
            for it in o_items:
                it()
            interleave(proj_items(v_unit) + [functools.partial(mem_read_unit, g) for g in range(NG)],
                       e_items[0:2])
            interleave(s_items(HA, 16), e_items[2:4])
            o_copy(s).start()

            @pl.when(s == 0)
            def _():
                f_copy(0).start()
                f_copy(1).start()

            @pl.when(s == 1)
            def _():
                f_copy(2).start()
        return carry

    lax.fori_loop(0, NSEG - 1, seg_body, 0)

    with _scope('seg_xz'):
        z = zero_s[0]
        phase_x()
        early, o_items, e_items = out_items(NSEG - 1)
        for it in early[0:8]:
            it()
        interleave(pv_items(HB, z), early[8:])
        for jt in range(4):
            for it in o_items[jt * NG:(jt + 1) * NG]:
                it()
            if jt > 0:
                e_items[jt - 1]()
        e_items[3]()
        o_copy(NSEG - 1).start()

    with _scope('ffn'):
        r_all = r_s[...].reshape(NSEG * 8, L)
        tok = ((lax.broadcasted_iota(jnp.int32, (NSEG * 8, L), 0) // 8) * L
               + lax.broadcasted_iota(jnp.int32, (NSEG * 8, L), 1))
        rmax = jnp.max(jnp.max(r_all, axis=1, keepdims=True), axis=0, keepdims=True)
        idx = jnp.clip(jnp.min(jnp.where(r_all == rmax, tok, S)), 0, S - 1)
        base = pl.multiple_of((idx // T) * T, T)
        lane = idx - base
        tile = pl.ds(base, T)

        hw = h_s[:, tile]
        htile = jnp.concatenate([pltpu.bitcast(hw << 16, F32), pltpu.bitcast(hw & U32(0xFFFF0000), F32)], axis=0)
        ytile = _layernorm(htile, 0).astype(BF16)
        onehot = (lax.broadcasted_iota(jnp.int32, (16, T), 1) == lane).astype(BF16)
        xs = lax.dot_general(onehot, ytile, NT, preferred_element_type=F32).astype(BF16)
        for i in range(3):
            f_copy(i).wait()
        acc = jnp.zeros((D, T), F32)
        for c in range(FF // FC):
            fc = slice(c * FC, (c + 1) * FC)
            gt = _rb(jnp.dot(xs, wg_v[:, fc], preferred_element_type=F32))
            up = _rb(jnp.dot(xs, wu_v[:, fc], preferred_element_type=F32))
            act = _rb(_rb(gt * jax.nn.sigmoid(gt)) * up)[0:1, :]
            for t in range(FC // T):
                acc = acc + wd_v[:, c * FC + t * T:c * FC + (t + 1) * T].astype(F32) * act[:, t * T:(t + 1) * T]
        ycol = _rb(jnp.sum(acc, axis=1, keepdims=True))
        ycol = _rb(ycol * _rb(jax.nn.sigmoid(rmax)))

        for s in range(NSEG):
            o_copy(s).wait()
        sel = lax.broadcasted_iota(jnp.int32, (D, T), 1) == lane
        new = htile + _rb(ytile.astype(F32) + ycol)
        out_s[:, tile] = jnp.where(sel, new, out_s[:, tile].astype(F32)).astype(BF16)
        fix = pltpu.make_async_copy(out_s.at[:, tile], out_hbm.at[0, :, tile], sem_o.at[0])
        fix.start()
        fix.wait()


@jax.jit
def pallas_sequential_preLN__memory_aug_infini_attn__moe_arch_mod__prompt_kernel(
    A_x: jax.Array,
    A_wq: jax.Array,
    A_wk: jax.Array,
    A_wv: jax.Array,
    A_wo: jax.Array,
    A_beta: jax.Array,
    B_x: jax.Array,
    B_w_r: jax.Array,
    B_w_gate: jax.Array,
    B_w_up: jax.Array,
    B_w_down: jax.Array,
):
    del B_x
    hbm = pl.BlockSpec(memory_space=pltpu.HBM)
    scratch = [
        pltpu.VMEM((D, S), BF16),
        pltpu.VMEM((4, D, D), BF16),
        pltpu.VMEM((QR + 320, D), U32),
        pltpu.VMEM((D // 2, 640), U32),
        pltpu.VMEM((D // 2, L), U32),
        pltpu.VMEM((NG, 64, L), U32),
        pltpu.VMEM((NG, 64, L), U32),
        pltpu.VMEM((NG, L // 2, T), U32),
        pltpu.VMEM((NG, 64, L), U32),
        pltpu.VMEM((320, L), U32),
        pltpu.VMEM((640, L), F32),
        pltpu.VMEM((NG, 160, T), F32),
        pltpu.VMEM((H, 1280, T), F32),
        pltpu.VMEM((H, 112, T), F32),
        pltpu.VMEM((320, L), U32),
        pltpu.VMEM((D, L), F32),
        pltpu.VMEM((NSEG, 4, 16, T), F32),
        pltpu.VMEM((D // 2, S), U32),
        pltpu.VMEM((D, S), BF16),
        pltpu.VMEM((NSEG, 8, L), F32),
        pltpu.VMEM((T, T), F32),
        pltpu.VMEM((64, T), F32),
        pltpu.VMEM((2, H, T), F32),
        pltpu.VMEM((640, T), F32),
        pltpu.VMEM((NG, 160, T), F32),
        pltpu.VMEM((D, FF), BF16),
        pltpu.VMEM((D, FF), BF16),
        pltpu.VMEM((D, FF), BF16),
        pltpu.VMEM((H,), BF16),
        pltpu.VMEM((D,), BF16),
        pltpu.VMEM((16, D), BF16),
        pltpu.VMEM((320, T), U32),
        pltpu.SMEM((1,), jnp.int32),
        pltpu.SemaphoreType.DMA((NSEG,)),
        pltpu.SemaphoreType.DMA((4,)),
        pltpu.SemaphoreType.DMA((3,)),
        pltpu.SemaphoreType.DMA((NSEG,)),
        pltpu.SemaphoreType.DMA((2,)),
    ]
    out_t = pl.pallas_call(
        _kernel,
        out_shape=jax.ShapeDtypeStruct((1, D, S), BF16),
        in_specs=[hbm] * 10,
        out_specs=hbm,
        scratch_shapes=scratch,
        compiler_params=pltpu.CompilerParams(vmem_limit_bytes=110 * 1024 * 1024),
        name="infini_moe",
    )(jnp.transpose(A_x, (0, 2, 1)), A_wq, A_wk, A_wv, A_wo, A_beta, B_w_r,
      B_w_gate, B_w_up, jnp.transpose(B_w_down, (1, 0)))
    return jnp.transpose(out_t, (0, 2, 1))
```

```python
import functools
import math

import jax
import jax.numpy as jnp
from jax import lax
import jax.experimental.pallas as pl
import jax.experimental.pallas.tpu as pltpu

F32 = jnp.float32
BF16 = jnp.bfloat16
U32 = jnp.uint32

S = 2048
D = 576
H = 32
DH = 18
NSEG = 4
L = 512
FF = 4608
T = 128
NG = 5
GH = (7, 7, 7, 7, 4)
VS = 20
EPS = 1e-5
QSCALE = DH ** (-0.5) * math.log2(math.e)
MASKVAL = -1000000000.0 * math.log2(math.e)
SOFF = (0, 128, 384, 768)
MOFF = (0, 2, 5, 9)
GWIN = tuple(((140 * g) // 16 * 16, -(-(140 * g + 20 * GH[g]) // 16) * 16) for g in range(NG))
QR = 592
FC = 512
import os
import contextlib
PROF = bool(int(os.environ.get('PROF', '0')))


def _scope(name):
    return jax.named_scope(name) if PROF else contextlib.nullcontext()


HS = int(os.environ.get('HS', '16'))
PACK = int(os.environ.get('PACK', '0'))
NS0 = int(os.environ.get('NS0', '8'))
HA1 = int(os.environ.get('HA1', '9'))
HM = int(os.environ.get('HM', '23'))
KE = (VS * HS) // T * T
KM = (VS * HM) // T * T

NT = (((1,), (1,)), ((), ()))


def _bf(x_u32):
    return pltpu.bitcast(x_u32, BF16)


def _u32(x_bf):
    return pltpu.bitcast(x_bf, U32)


def _pack_rows(y):
    if not PACK:
        return _u32(y.astype(BF16))
    n = y.shape[0]
    parts = []
    full = n // 32 * 32
    if full:
        y4 = y[0:full].reshape(full // 32, 2, 16, T)
        parts.append(pltpu.pack_elementwise([y4[:, 0], y4[:, 1]], packed_dtype=BF16).reshape(full // 2, T))
    if n > full:
        parts.append(pltpu.pack_elementwise([y[full:full + 8], y[full + 8:full + 16]], packed_dtype=BF16))
    return parts[0] if len(parts) == 1 else jnp.concatenate(parts, axis=0)


def _rb(x):
    return x.astype(BF16).astype(F32)


def _phi(t):
    return jnp.where(t > 0, t + 1.0, jnp.exp(t))


def _layernorm(x, axis):
    m = jnp.mean(x, axis=axis, keepdims=True)
    c = x - m
    v = jnp.mean(c * c, axis=axis, keepdims=True)
    den = _rb(jnp.sqrt(_rb(_rb(v) + EPS)))
    return c * (1.0 / den)


def _ln_scale(pivot, s1, s2):
    md = s1 * (1.0 / D)
    v = jnp.maximum(s2 * (1.0 / D) - md * md, 0.0)
    den = _rb(jnp.sqrt(_rb(_rb(v) + EPS)))
    return pivot + md, 1.0 / den


def _kernel(x_hbm, wq_hbm, wk_hbm, wv_hbm, wo_hbm, beta_hbm, wr_hbm, wg_hbm, wu_hbm, wd_hbm,
            out_hbm,
            x_v, w_v, wqkv, wot, xn, qt, pqt, kk, pkt, vt, memt, bd, s_a, s_b1, s_b2, m_blk,
            ot, att, ln_st, h_s, out_s, r_s, bias, bias2, gtab, ones_tab, keep_tab,
            wg_v, wu_v, wd_v, beta_v, wr_v, wr16, dtmp, xs_v, best_v, fix_v,
            zero_s, sem_x, sem_w, sem_f, sem_o, sem_s):
    def x_copy(s):
        return pltpu.make_async_copy(x_hbm.at[0, :, pl.ds(s * L, L)], x_v.at[:, pl.ds(s * L, L)],
                                     sem_x.at[s])

    w_srcs = (wk_hbm, wq_hbm, wv_hbm, wo_hbm)

    def w_copy(i):
        return pltpu.make_async_copy(w_srcs[i], w_v.at[i], sem_w.at[i])

    f_pairs = ((wg_hbm, wg_v), (wu_hbm, wu_v), (wd_hbm, wd_v))

    def f_copy(i):
        return pltpu.make_async_copy(f_pairs[i][0], f_pairs[i][1], sem_f.at[i])

    def o_copy(s):
        return pltpu.make_async_copy(out_s.at[:, pl.ds(s * L, L)], out_hbm.at[0, :, pl.ds(s * L, L)],
                                     sem_o.at[s])

    beta_copy = pltpu.make_async_copy(beta_hbm, beta_v, sem_s.at[0])
    wr_copy = pltpu.make_async_copy(wr_hbm, wr_v, sem_s.at[1])

    def seg_cols(s, jt):
        if isinstance(s, int):
            return slice(s * L + jt * T, s * L + (jt + 1) * T)
        return pl.ds(pl.multiple_of(s * L + jt * T, T), T)

    def ln1_stats(s, jt, tok=None):
        cols = seg_cols(s, jt)
        pivot = a1 = a2 = None
        for c in range(D // 32):
            x = x_v[32 * c:32 * (c + 1), cols].astype(F32)
            if c == 0:
                pivot = x[0:1, :]
                if tok is not None:
                    pivot = pivot + tok()
            d = (x - pivot).reshape(4, 8, T)
            p1 = (d[0] + d[1]) + (d[2] + d[3])
            dd = d * d
            p2 = (dd[0] + dd[1]) + (dd[2] + dd[3])
            a1 = p1 if c == 0 else a1 + p1
            a2 = p2 if c == 0 else a2 + p2
        m, inv = _ln_scale(pivot, jnp.sum(a1, axis=0, keepdims=True), jnp.sum(a2, axis=0, keepdims=True))
        ln_st[s, jt, 0:1, :] = m
        ln_st[s, jt, 8:9, :] = inv

    def ln1_norm(s, jt, c=None):
        for cc in (range(NG) if c is None else (c,)):
            r0, r1 = T * cc, min(T * (cc + 1), D)
            x = x_v[r0:r1, seg_cols(s, jt)].astype(F32)
            xn[r0 // 2:r1 // 2, jt * T:(jt + 1) * T] = _u32(
                ((x - ln_st[s, jt, 0:1, :]) * ln_st[s, jt, 8:9, :]).astype(BF16))

    def q_unit(jt, g):
        cols = slice(jt * T, (jt + 1) * T)
        n = min(64, QR // 2 - 64 * g)
        q = jnp.dot(_bf(wqkv[64 * g:64 * g + n, :]), _bf(xn[:, cols]), preferred_element_type=F32)
        qt[g, 0:n, cols] = _pack_rows(q * QSCALE)
        pqt[g, 0:n, cols] = _pack_rows(_phi(q))

    def k_unit(jt, g):
        cols = slice(jt * T, (jt + 1) * T)
        n = min(64, QR // 2 - 64 * g)
        b0 = QR // 2 + 64 * g
        k = jnp.dot(_bf(wqkv[b0:b0 + n, :]), _bf(xn[:, cols]), preferred_element_type=F32)
        pkt[g, 0:n, cols] = _pack_rows(_phi(k))
        kb = _pack_rows(k)
        if n < 64:
            kb = jnp.concatenate([kb, jnp.zeros((64 - n, T), U32)], axis=0)
        kk[g, jt * 64:(jt + 1) * 64, :] = _u32(_bf(kb).T)

    def v_unit(jt, c):
        cols = slice(jt * T, (jt + 1) * T)
        b0 = QR + 64 * c
        v = jnp.dot(_bf(wqkv[b0:b0 + 64, :]), _bf(xn[:, cols]), preferred_element_type=F32)
        vt[64 * c:64 * (c + 1), cols] = _pack_rows(v + ones_tab[T * c:T * (c + 1), :])

    def mem_read_unit(g):
        w0, w1 = GWIN[g]
        b = bd[g, 0:w1 - w0, :].astype(BF16)
        res = jnp.dot(b, _bf(pqt[g]), preferred_element_type=F32)
        lo, hi = 140 * g, 140 * g + 20 * GH[g]
        memt[lo:hi, :] = res[lo - w0:hi - w0]

    def mem_update_unit(g):
        w0, w1 = GWIN[g]
        upd = lax.dot_general(_bf(vt[w0 // 2:w1 // 2, :]), _bf(pkt[g]), NT, preferred_element_type=F32)
        n = w1 - w0
        bd[g, 0:n, :] = bd[g, 0:n, :] + jnp.where(keep_tab[g, 0:n, :] > 0.5, upd, 0.0)

    def sbuf(h):
        if h < HS:
            return s_a, h
        return (s_b1, h - HS) if h < HM else (s_b2, h - HM)

    def head_rows(j):
        r = lax.broadcasted_iota(jnp.int32, (64, T), 0)
        return (r >= 9 * j) & (r < 9 * j + 9)

    def s_blk(h, jq, kb, half=False):
        g, j = divmod(h, 7)
        off = SOFF[jq] + kb * T
        n = 64 if half else T
        qm = _bf(jnp.where(head_rows(j), qt[g, :, jq * T:(jq + 1) * T], U32(0)))
        sc = jnp.dot(_bf(kk[g, kb * 64:kb * 64 + n // 2, :]), qm, preferred_element_type=F32)
        if kb == jq:
            sc = sc + bias[0:n, :]
        sb, hi_ = sbuf(h)
        sb[hi_, off:off + n, :] = sc
        slot = MOFF[jq] + kb
        m_blk[h, slot * 8:(slot + 1) * 8, :] = jnp.max(sc.reshape(n // 8, 8, T), axis=0)

    def s_pair(ha, jq):
        g, j = divmod(ha, 7)
        off = SOFF[jq] + jq * T + 64
        lo = lax.broadcasted_iota(jnp.int32, (64, T), 1) < 64
        qu = qt[g, :, jq * T:(jq + 1) * T]
        qmix = jnp.where(lo, pltpu.roll(qu, 64, 1), qu)
        qm = _bf(jnp.where((lo & head_rows(j)) | (~lo & head_rows(j + 1)), qmix, U32(0)))
        sc = jnp.dot(_bf(kk[g, jq * 64 + 32:jq * 64 + 64, :]), qm, preferred_element_type=F32) + bias2[...]
        sb, hi_ = sbuf(ha)
        sb[hi_, off:off + 64, :] = sc
        pm = jnp.max(sc.reshape(8, 8, T), axis=0)
        hi = lax.broadcasted_iota(jnp.int32, (8, T), 1) >= 64
        slot = MOFF[jq] + jq + 1
        m_blk[ha, slot * 8:(slot + 1) * 8, :] = jnp.where(hi, pltpu.roll(pm, 64, 1), -jnp.inf)
        m_blk[ha + 1, slot * 8:(slot + 1) * 8, :] = jnp.where(hi, pm, -jnp.inf)

    def row_max(h, jq, nslots):
        return jnp.max(m_blk[h, MOFF[jq] * 8:(MOFF[jq] + nslots) * 8, :], axis=0, keepdims=True)

    def pv_blk(h, jq, kb, st, role):
        w0 = (VS * h) // 16 * 16
        o = VS * h - w0
        off = SOFF[jq] + kb * T
        cols = slice(jq * T, (jq + 1) * T)
        key = role or 'a'
        sb, hz = sbuf(h)
        hz = hz + st['z']
        if kb == 0 and role != 'b':
            st['ma'] = row_max(h, jq, jq + 1 if role is None else jq + 2)
            if role == 'a':
                st['mb'] = row_max(h + 1, jq, jq + 2)
        m = st['m' + key]
        if kb < jq or role is None:
            p = jnp.exp2(sb[hz, off:off + T, :] - m).astype(BF16)
        else:
            if role == 'a':
                hi1 = lax.broadcasted_iota(jnp.int32, (1, T), 1) >= 64
                hi = lax.broadcasted_iota(jnp.int32, (64, T), 1) >= 64
                m2 = jnp.where(hi1, st['mb'], pltpu.roll(st['ma'], 64, 1))
                e2 = jnp.exp2(sb[hz, off + 64:off + T, :] - m2)
                p2 = jnp.where(hi, pltpu.roll(e2, 64, 1), 0.0)
                st['p2b'] = jnp.where(hi, e2, 0.0)
            else:
                p2 = st['p2b']
            p1 = jnp.exp2(sb[hz, off:off + 64, :] - m)
            p = jnp.concatenate([p1, p2], axis=0).astype(BF16)
        part = jnp.dot(_bf(vt[w0 // 2:w0 // 2 + 16, kb * T:(kb + 1) * T]), p, preferred_element_type=F32)
        st['pv' + key] = part if kb == 0 else st['pv' + key] + part
        if kb == jq:
            pv = st['pv' + key]
            res = pv * (gtab[1, h:h + 1, :] / pv[o + DH:o + DH + 1, :])
            mem = memt[w0:w0 + 32, cols]
            res = res + mem * (gtab[0, h:h + 1, :] / (mem[o + DH:o + DH + 1, :] + 1e-6))
            ot[VS * h // 2:VS * h // 2 + VS // 2, cols] = _u32(res.astype(BF16))[o // 2:o // 2 + VS // 2]

    def o_early(s, jt, c, ke):
        r0, r1 = T * c, min(T * (c + 1), D)
        tile = slice(jt * T, (jt + 1) * T)
        a = jnp.dot(_bf(wot[r0 // 2:r1 // 2, 0:ke]), _bf(ot[0:ke // 2, tile]), preferred_element_type=F32)
        att[r0:r1, tile] = x_v[r0:r1, seg_cols(s, jt)].astype(F32) + a

    def o_unit(s, jt, c, ke, st):
        r0, r1 = T * c, min(T * (c + 1), D)
        tile = slice(jt * T, (jt + 1) * T)
        a = jnp.dot(_bf(wot[r0 // 2:r1 // 2, ke:640]), _bf(ot[ke // 2:320, tile]), preferred_element_type=F32)
        hh = att[r0:r1, tile] + a
        att[r0:r1, tile] = hh
        if c == 0:
            st['p'] = hh[0:1, :]
        d = hh - st['p']
        s1 = jnp.sum(d, axis=0, keepdims=True)
        s2 = jnp.sum(d * d, axis=0, keepdims=True)
        st['s1'] = s1 if c == 0 else st['s1'] + s1
        st['s2'] = s2 if c == 0 else st['s2'] + s2

    def e2_unit(s, jt, c, st):
        r0, r1 = T * c, min(T * (c + 1), D)
        cols = seg_cols(s, jt)
        if c == 0:
            st['m'], st['inv'] = _ln_scale(st['p'], st['s1'], st['s2'])
        hh = att[r0:r1, jt * T:(jt + 1) * T]
        y = (hh - st['m']) * st['inv']
        n = (r1 - r0) // 2
        h_s[r0 // 2:r1 // 2, cols] = pltpu.pack_elementwise([hh[0:n], hh[n:2 * n]], packed_dtype=BF16)
        out_s[r0:r1, cols] = (hh + y).astype(BF16)
        yb = y.astype(BF16)
        rr = jnp.dot(wr16[:, r0:r1], yb, preferred_element_type=F32)
        st['r'] = rr if c == 0 else st['r'] + rr
        cand = st.get('cand')
        if cand is not None:
            cand.setdefault(jt, {'y': []})['y'].append(yb)
        if r1 == D:
            rrow = _rb(st['r'][0:1, :])
            if cand is None:
                r_s[s, :, jt * T:(jt + 1) * T] = jnp.broadcast_to(rrow, (8, T))
            else:
                cand[jt]['r'] = rrow

    def offer_last(best, cand):
        rrow = jnp.concatenate([cand[jt]['r'] for jt in range(4)], axis=1)
        tmax = jnp.max(rrow, axis=1, keepdims=True)
        lane = lax.broadcasted_iota(jnp.int32, (1, L), 1)
        lane_c = jnp.min(jnp.where(rrow == tmax, lane, L), axis=1, keepdims=True)
        xs = None
        for jt in range(4):
            oh = (lax.broadcasted_iota(jnp.int32, (16, T), 1) == lane_c - jt * T).astype(BF16)
            part = jnp.concatenate([lax.dot_general(oh, yc, NT, preferred_element_type=F32)
                                    for yc in cand[jt]['y']], axis=1)
            xs = part if xs is None else xs + part
        take = tmax > best['r']
        best.update(r=jnp.where(take, tmax, best['r']),
                    tok=jnp.where(take, (NSEG - 1) * L + lane_c, best['tok']),
                    xs=jnp.where(take, xs, best['xs']))

    def prep_qk(i, base):
        wt = _u32(w_v[i].T)
        for g in range(NG):
            n = 9 * GH[g]
            wqkv[base + 64 * g:base + 64 * g + n, :] = wt[63 * g:63 * g + n, :]
        deinterleave(base, 4 * 64)
        deinterleave(base + 4 * 64, QR // 2 - 4 * 64)

    def prep_v():
        wt = _u32(w_v[2].T)
        for h in range(H):
            wqkv[QR + 10 * h:QR + 10 * h + 9, :] = wt[9 * h:9 * h + 9, :]
        deinterleave(QR, 320)

    def deinterleave(base, nwords):
        lo16 = U32(0xFFFF)
        hi16 = U32(0xFFFF0000)
        for lt in range(NG if PACK else 0):
            w = min(T, D - T * lt)
            lanes = slice(T * lt, T * lt + w)
            dtmp[0:nwords, 0:w] = wqkv[base:base + nwords, lanes]
            b = 0
            while b < nwords:
                half = 8 if nwords - b >= 16 else 4
                ev = dtmp[pl.ds(b, half, stride=2), :]
                od = dtmp[pl.ds(b + 1, half, stride=2), :]
                wqkv[base + b:base + b + half, lanes] = ((ev & lo16) | (od << 16))[:, 0:w]
                wqkv[base + b + half:base + b + 2 * half, lanes] = ((ev >> 16) | (od & hi16))[:, 0:w]
                b += 2 * half

    def prep_o():
        wt = _u32(w_v[3])
        wpad = jnp.concatenate(
            [piece for h in range(H) for piece in (wt[9 * h:9 * h + 9, :], jnp.zeros((1, D), U32))], axis=0)
        wot[...] = _u32(_bf(wpad).T)

    BLKS = [(jq, kb) for jq in range(4) for kb in range(jq + 1)]

    def head_sets(heads):
        sets, i = [], 0
        while i < len(heads):
            h = heads[i]
            if h % 7 % 2 == 0 and h % 7 < 6 and i + 1 < len(heads):
                sets.append((h, h + 1))
                i += 2
            else:
                assert h % 7 == 6
                sets.append((h,))
                i += 1
        return sets

    def s_items(heads, small_tail=0):
        big, small = [], []
        for hs in head_sets(heads):
            for jq, kb in BLKS:
                halved = len(hs) == 2 and kb == jq
                for h in hs:
                    (small if halved else big).append(functools.partial(s_blk, h, jq, kb, halved))
                if halved:
                    small.append(functools.partial(s_pair, hs[0], jq))
        tail = small[len(small) - small_tail:] if small_tail else []
        small = small[:len(small) - small_tail] if small_tail else small
        order = sorted([((j + 0.5) / len(big), 0, j) for j in range(len(big))]
                       + [((j + 0.5) / len(small), 1, j) for j in range(len(small))])
        return [(big, small)[w][j] for _, w, j in order] + tail

    def phase_x():
        sb = s_items(HB)
        for it in sb[0:NS0]:
            it()
        interleave(pv_items(HA), sb[NS0:])

    def pv_items_by_tile(heads, z):
        out = {}
        for jq in range(4):
            out[jq] = []
            for hs in head_sets(heads):
                st = {'z': z}
                roles = ('a', 'b') if len(hs) == 2 else (None,)
                for kb in range(jq + 1):
                    for h, role in zip(hs, roles):
                        out[jq].append(functools.partial(pv_blk, h, jq, kb, st, role))
        return out

    def pv_items(heads, z=0):
        items = []
        for hs in head_sets(heads):
            st = {'z': z}
            roles = ('a', 'b') if len(hs) == 2 else (None,)
            for jq, kb in BLKS:
                for h, role in zip(hs, roles):
                    items.append(functools.partial(pv_blk, h, jq, kb, st, role))
        return items

    def interleave(*seqs):
        seqs = [q for q in seqs if q]
        order = []
        for i, q in enumerate(seqs):
            order += [((j + 0.5) / len(q), i, j) for j in range(len(q))]
        for _, i, j in sorted(order):
            seqs[i][j]()

    def proj_items(fn):
        return [functools.partial(fn, jt, g) for jt in range(4) for g in range(NG)]

    def out_items(s, ke, cand=None):
        sts = [{'cand': cand} for _ in range(4)]
        o_items = [functools.partial(o_unit, s, jt, c, ke, sts[jt]) for jt in range(4) for c in range(NG)]
        e_items = [functools.partial(e2_unit, s, jt, c, sts[jt]) for jt in range(4) for c in range(NG)]
        early = [functools.partial(o_early, s, jt, c, ke) for jt in range(4) for c in range(NG)]
        return early, o_items, e_items

    HA = list(range(HS))
    HB = list(range(HS, H))

    x_copy(0).start()
    w_copy(1).start()
    zero_s[0] = 0
    beta_copy.start()
    wr_copy.start()
    with _scope('p0_const'):
        kr = lax.broadcasted_iota(jnp.int32, (T, T), 0)
        qc = lax.broadcasted_iota(jnp.int32, (T, T), 1)
        bias[...] = jnp.where(kr > qc, MASKVAL, 0.0).astype(F32)
        kr2 = lax.broadcasted_iota(jnp.int32, (64, T), 0)
        qc2 = lax.broadcasted_iota(jnp.int32, (64, T), 1)
        bias2[...] = jnp.where(kr2 > (qc2 & 63), MASKVAL, 0.0).astype(F32)
        wqkv[...] = jnp.zeros(wqkv.shape, U32)
        bd[...] = jnp.zeros(bd.shape, F32)
        memt[...] = jnp.zeros(memt.shape, F32)
        row = lax.broadcasted_iota(jnp.int32, (640, T), 0)
        sub = row & 31
        nat = (row - sub) + jnp.where(sub < 16, 2 * sub, 2 * sub - 31)
        if not PACK:
            nat = row
        ones_tab[...] = jnp.where(nat % VS == DH, 1.0, 0.0).astype(F32)
        dtmp[...] = jnp.zeros(dtmp.shape, U32)
        for g in range(NG):
            row = lax.broadcasted_iota(jnp.int32, (160, T), 0) + (GWIN[g][0] - 140 * g)
            lane = lax.broadcasted_iota(jnp.int32, (160, T), 1)
            keep = ((row >= 0) & (row < 20 * GH[g]) & (lane >= (row // VS) * DH)
                    & (lane < (row // VS) * DH + DH))
            keep_tab[g] = jnp.where(keep, 1.0, 0.0).astype(F32)
        pqt[NG - 1] = jnp.zeros(pqt.shape[1:], U32)
        pkt[NG - 1] = jnp.zeros(pkt.shape[1:], U32)

    with _scope('p1_ln'):
        x_copy(0).wait()
        w_copy(0).start()
        for jt in range(4):
            ln1_stats(0, jt)
            ln1_norm(0, jt)
    with _scope('p2_wq'):
        w_copy(1).wait()
        w_copy(2).start()
        prep_qk(1, 0)
        for g in range(NG):
            for jt in range(2):
                q_unit(jt, g)
    with _scope('p3_q'):
        w_copy(0).wait()
        w_copy(3).start()
        prep_qk(0, QR // 2)
        for jt in range(2, 4):
            for g in range(NG):
                q_unit(jt, g)
    with _scope('p4_k'):
        w_copy(2).wait()
        for i in range(1, NSEG):
            x_copy(i).start()
        prep_v()
        for jt in range(4):
            for g in range(NG):
                k_unit(jt, g)
    with _scope('p5_v'):
        w_copy(3).wait()
        beta_copy.wait()
        wr_copy.wait()
        for i in range(1, NSEG):
            x_copy(i).wait()
        prep_o()
        beta = beta_v[...].astype(F32).reshape(1, H)
        hl = lax.broadcasted_iota(jnp.int32, (H, H), 1)
        hs = lax.broadcasted_iota(jnp.int32, (H, H), 0)
        bcol = jnp.sum(jnp.where(hl == hs, jnp.broadcast_to(beta, (H, H)), 0.0), axis=1, keepdims=True)
        gate = _rb(jax.nn.sigmoid(bcol))
        gtab[0] = jnp.broadcast_to(gate, (H, T))
        gtab[1] = jnp.broadcast_to(_rb(1.0 - gate), (H, T))
        r16 = lax.broadcasted_iota(jnp.int32, (16, D), 0)
        wr_row = wr_v[...].astype(F32).reshape(1, D)
        wr16[...] = jnp.where(r16 == 0, jnp.broadcast_to(wr_row, (16, D)), 0.0).astype(BF16)
        interleave(proj_items(v_unit) + s_items(HA, 16),
                   [functools.partial(ln1_stats, i, jt) for i in range(1, NSEG) for jt in range(4)])

    def seg_body(s, carry):
        with _scope('seg_xy'):
            z = zero_s[0]
            phase_x()
            ln = [functools.partial(ln1_norm, s + 1, jt) for jt in range(4)]
            qs = proj_items(q_unit)
            early, o_items, e_items = out_items(s, KE)
            for it in [ln[0]] + early[0:10] + [ln[1]]:
                it()
            mxu1 = ([functools.partial(mem_update_unit, g) for g in range(NG)]
                    + qs[0:5] + [ln[2]] + early[10:20] + qs[5:10] + [ln[3]]
                    + qs[10:20] + proj_items(k_unit))
            interleave(pv_items(HB, z), mxu1)
            for it in o_items:
                it()
            interleave(proj_items(v_unit) + [functools.partial(mem_read_unit, g) for g in range(NG)],
                       e_items[0:10])
            interleave(s_items(HA, 16), e_items[10:20])
            o_copy(s).start()

            @pl.when(s == 0)
            def _():
                f_copy(0).start()
                f_copy(1).start()

            @pl.when(s == 1)
            def _():
                f_copy(2).start()
        return carry

    lax.fori_loop(0, NSEG - 1, seg_body, 0)

    def load_h_tile(tile):
        hw = h_s[:, tile]
        hlo = pltpu.bitcast(hw << 16, F32)
        hhi = pltpu.bitcast(hw & U32(0xFFFF0000), F32)
        pieces = []
        for c in range(NG):
            w0, w1 = 64 * c, min(64 * (c + 1), D // 2)
            pieces += [hlo[w0:w1], hhi[w0:w1]]
        return jnp.concatenate(pieces, axis=0)

    with _scope('seg_xz'):
        for i in range(3):
            f_copy(i).wait()
        z = zero_s[0]
        best = {}

        def offer_previous():
            n = (NSEG - 1) * 8
            r_all = r_s[0:NSEG - 1].reshape(n, L)
            tok = ((lax.broadcasted_iota(jnp.int32, (n, L), 0) // 8) * L
                   + lax.broadcasted_iota(jnp.int32, (n, L), 1))
            rmax = jnp.max(jnp.max(r_all, axis=1, keepdims=True), axis=0, keepdims=True)
            idx = jnp.clip(jnp.min(jnp.where(r_all == rmax, tok, S)), 0, S - 1)
            base = pl.multiple_of((idx // T) * T, T)
            yt = _layernorm(load_h_tile(pl.ds(base, T)), 0)
            onehot = (lax.broadcasted_iota(jnp.int32, (16, T), 1) == idx - base).astype(BF16)
            xs = lax.dot_general(onehot, yt.astype(BF16), NT, preferred_element_type=F32)
            best.update(r=rmax, tok=jnp.full((1, 1), idx, jnp.int32), xs=xs)

        ha1, ha2 = HA[:HA1], HA[HA1:]
        hb1, hb2 = list(range(HS, HM)), list(range(HM, H))
        sb1 = s_items(hb1)
        for it in sb1[0:NS0]:
            it()
        interleave(pv_items(ha1), sb1[NS0:])
        offer_previous()
        sb2 = s_items(hb2)
        interleave(pv_items(ha2) + pv_items(hb1, z), sb2)
        cand = {}
        early, o_items, e_items = out_items(NSEG - 1, KM, cand)
        for it in early[0:4]:
            it()
        interleave(pv_items(hb2, z), early[4:])
        for jt in range(4):
            for it in o_items[jt * NG:(jt + 1) * NG]:
                it()
            if jt > 0:
                for it in e_items[(jt - 1) * NG:jt * NG]:
                    it()
        for it in e_items[3 * NG:]:
            it()
        offer_last(best, cand)
        o_copy(NSEG - 1).start()

    xs_v[...] = best['xs'].astype(BF16)
    best_v[...] = jnp.broadcast_to(best['r'], (8, T))
    idx = jnp.clip(jnp.max(best['tok']), 0, S - 1)
    base = pl.multiple_of((idx // T) * T, T)
    tile = pl.ds(base, T)

    @pl.when(zero_s[0] == 0)
    def _ffn():
        with _scope('ffn'):
            xs = xs_v[...]
            acc = jnp.zeros((D, T), F32)
            for c in range(FF // FC):
                fc = slice(c * FC, (c + 1) * FC)
                gt = _rb(jnp.dot(xs, wg_v[:, fc], preferred_element_type=F32))
                up = _rb(jnp.dot(xs, wu_v[:, fc], preferred_element_type=F32))
                act = _rb(_rb(gt * jax.nn.sigmoid(gt)) * up)[0:1, :]
                for t in range(FC // T):
                    acc = acc + (wd_v[:, c * FC + t * T:c * FC + (t + 1) * T].astype(F32)
                                 * act[:, t * T:(t + 1) * T])
            ycol = _rb(jnp.sum(acc, axis=1, keepdims=True))
            ycol = _rb(ycol * _rb(jax.nn.sigmoid(best_v[0:1, 0:1])))
            htile = load_h_tile(tile)
            ytile = _rb(_layernorm(htile, 0))
            sel = lax.broadcasted_iota(jnp.int32, (D, T), 1) == idx - base
            new = htile + _rb(ytile + ycol)
            fix_v[...] = jnp.where(sel, new, out_s[:, tile].astype(F32)).astype(BF16)

    for s in range(NSEG):
        o_copy(s).wait()
    fix = pltpu.make_async_copy(fix_v, out_hbm.at[0, :, tile], sem_o.at[0])
    fix.start()
    fix.wait()


@jax.jit
def pallas_sequential_preLN__memory_aug_infini_attn__moe_arch_mod__prompt_kernel(
    A_x: jax.Array,
    A_wq: jax.Array,
    A_wk: jax.Array,
    A_wv: jax.Array,
    A_wo: jax.Array,
    A_beta: jax.Array,
    B_x: jax.Array,
    B_w_r: jax.Array,
    B_w_gate: jax.Array,
    B_w_up: jax.Array,
    B_w_down: jax.Array,
):
    del B_x
    hbm = pl.BlockSpec(memory_space=pltpu.HBM)
    scratch = [
        pltpu.VMEM((D, S), BF16),
        pltpu.VMEM((4, D, D), BF16),
        pltpu.VMEM((QR + 320, D), U32),
        pltpu.VMEM((D // 2, 640), U32),
        pltpu.VMEM((D // 2, L), U32),
        pltpu.VMEM((NG, 64, L), U32),
        pltpu.VMEM((NG, 64, L), U32),
        pltpu.VMEM((NG, L // 2, T), U32),
        pltpu.VMEM((NG, 64, L), U32),
        pltpu.VMEM((320, L), U32),
        pltpu.VMEM((640, L), F32),
        pltpu.VMEM((NG, 160, T), F32),
        pltpu.VMEM((HS, 1280, T), F32),
        pltpu.VMEM((HM - HS, 1280, T), F32),
        pltpu.VMEM((H - HM, 1280, T), F32),
        pltpu.VMEM((H, 112, T), F32),
        pltpu.VMEM((320, L), U32),
        pltpu.VMEM((D, L), F32),
        pltpu.VMEM((NSEG, 4, 16, T), F32),
        pltpu.VMEM((D // 2, S), U32),
        pltpu.VMEM((D, S), BF16),
        pltpu.VMEM((NSEG, 8, L), F32),
        pltpu.VMEM((T, T), F32),
        pltpu.VMEM((64, T), F32),
        pltpu.VMEM((2, H, T), F32),
        pltpu.VMEM((640, T), F32),
        pltpu.VMEM((NG, 160, T), F32),
        pltpu.VMEM((D, FF), BF16),
        pltpu.VMEM((D, FF), BF16),
        pltpu.VMEM((D, FF), BF16),
        pltpu.VMEM((H,), BF16),
        pltpu.VMEM((D,), BF16),
        pltpu.VMEM((16, D), BF16),
        pltpu.VMEM((320, T), U32),
        pltpu.VMEM((16, D), BF16),
        pltpu.VMEM((8, T), F32),
        pltpu.VMEM((D, T), BF16),
        pltpu.SMEM((1,), jnp.int32),
        pltpu.SemaphoreType.DMA((NSEG,)),
        pltpu.SemaphoreType.DMA((4,)),
        pltpu.SemaphoreType.DMA((3,)),
        pltpu.SemaphoreType.DMA((NSEG,)),
        pltpu.SemaphoreType.DMA((2,)),
    ]
    out_t = pl.pallas_call(
        _kernel,
        out_shape=jax.ShapeDtypeStruct((1, D, S), BF16),
        in_specs=[hbm] * 10,
        out_specs=hbm,
        scratch_shapes=scratch,
        compiler_params=pltpu.CompilerParams(vmem_limit_bytes=110 * 1024 * 1024),
        name="infini_moe",
    )(jnp.transpose(A_x, (0, 2, 1)), A_wq, A_wk, A_wv, A_wo, A_beta, B_w_r,
      B_w_gate, B_w_up, jnp.transpose(B_w_down, (1, 0)))
    return jnp.transpose(out_t, (0, 2, 1))
```

```python
import functools
import math

import jax
import jax.numpy as jnp
from jax import lax
import jax.experimental.pallas as pl
import jax.experimental.pallas.tpu as pltpu

F32 = jnp.float32
BF16 = jnp.bfloat16
U32 = jnp.uint32

S = 2048
D = 576
H = 32
DH = 18
NSEG = 4
L = 512
FF = 4608
T = 128
NG = 5
GH = (7, 7, 7, 7, 4)
VS = 20
EPS = 1e-5
QSCALE = DH ** (-0.5) * math.log2(math.e)
MASKVAL = -1000000000.0 * math.log2(math.e)
SOFF = (0, 128, 384, 768)
MOFF = (0, 2, 5, 9)
GWIN = tuple(((140 * g) // 16 * 16, -(-(140 * g + 20 * GH[g]) // 16) * 16) for g in range(NG))
QR = 592
FCH = {0: (512,) * 9, 1: (128, 384) + (512,) * 8, 2: (256,) * 18, 3: (128, 128, 256) + (512,) * 8,
       4: (128, 256, 384) + (640,) * 6}[int(__import__('os').environ.get('FCV', '2'))]
import os
import contextlib
PROF = bool(int(os.environ.get('PROF', '0')))


def _scope(name):
    return jax.named_scope(name) if PROF else contextlib.nullcontext()


HS = int(os.environ.get('HS', '16'))
PACK = int(os.environ.get('PACK', '0'))
NS0 = int(os.environ.get('NS0', '12'))
HA1 = int(os.environ.get('HA1', '9'))
Y1V = int(os.environ.get('Y1V', '2'))
Y2V = int(os.environ.get('Y2V', '0'))
E2A = int(os.environ.get('E2A', '20'))
TAIL = int(os.environ.get('TAIL', '16'))
STATV = int(os.environ.get('STATV', '0'))
HM = int(os.environ.get('HM', '25'))
KE = (VS * HS) // T * T
KM = (VS * HM) // T * T

NT = (((1,), (1,)), ((), ()))


def _bf(x_u32):
    return pltpu.bitcast(x_u32, BF16)


def _u32(x_bf):
    return pltpu.bitcast(x_bf, U32)


def _pack_rows(y):
    if not PACK:
        return _u32(y.astype(BF16))
    n = y.shape[0]
    parts = []
    full = n // 32 * 32
    if full:
        y4 = y[0:full].reshape(full // 32, 2, 16, T)
        parts.append(pltpu.pack_elementwise([y4[:, 0], y4[:, 1]], packed_dtype=BF16).reshape(full // 2, T))
    if n > full:
        parts.append(pltpu.pack_elementwise([y[full:full + 8], y[full + 8:full + 16]], packed_dtype=BF16))
    return parts[0] if len(parts) == 1 else jnp.concatenate(parts, axis=0)


def _rb(x):
    return x.astype(BF16).astype(F32)


def _phi(t):
    return jnp.where(t > 0, t + 1.0, jnp.exp(t))


def _layernorm(x, axis):
    m = jnp.mean(x, axis=axis, keepdims=True)
    c = x - m
    v = jnp.mean(c * c, axis=axis, keepdims=True)
    den = _rb(jnp.sqrt(_rb(_rb(v) + EPS)))
    return c * (1.0 / den)


def _ln_scale(pivot, s1, s2):
    md = s1 * (1.0 / D)
    v = jnp.maximum(s2 * (1.0 / D) - md * md, 0.0)
    den = _rb(jnp.sqrt(_rb(_rb(v) + EPS)))
    return pivot + md, 1.0 / den


def _kernel(x_hbm, wq_hbm, wk_hbm, wv_hbm, wo_hbm, beta_hbm, wr_hbm, wg_hbm, wu_hbm, wd_hbm,
            out_hbm,
            x_v, w_v, wqkv, wot, xn, qt, pqt, kk, pkt, vt, memt, bd, s_a, s_b1, s_b2, m_blk,
            ot, att, ln_st, h_s, out_s, r_s, bias, bias2, gtab, ones_tab, keep_tab,
            wg_v, wu_v, wd_v, beta_v, wr_v, wr16, dtmp, xs_v, best_v, fix_v, hy_v,
            zero_s, sem_x, sem_w, sem_f, sem_o, sem_s):
    def x_copy(s):
        return pltpu.make_async_copy(x_hbm.at[0, :, pl.ds(s * L, L)], x_v.at[:, pl.ds(s * L, L)],
                                     sem_x.at[s])

    w_srcs = (wk_hbm, wq_hbm, wv_hbm, wo_hbm)

    def w_copy(i):
        return pltpu.make_async_copy(w_srcs[i], w_v.at[i], sem_w.at[i])

    f_pairs = ((wg_hbm, wg_v), (wu_hbm, wu_v), (wd_hbm, wd_v))

    def f_copy(i):
        return pltpu.make_async_copy(f_pairs[i][0], f_pairs[i][1], sem_f.at[i])

    def o_copy(s):
        return pltpu.make_async_copy(out_s.at[:, pl.ds(s * L, L)], out_hbm.at[0, :, pl.ds(s * L, L)],
                                     sem_o.at[s])

    beta_copy = pltpu.make_async_copy(beta_hbm, beta_v, sem_s.at[0])
    wr_copy = pltpu.make_async_copy(wr_hbm, wr_v, sem_s.at[1])

    def seg_cols(s, jt):
        if isinstance(s, int):
            return slice(s * L + jt * T, s * L + (jt + 1) * T)
        return pl.ds(pl.multiple_of(s * L + jt * T, T), T)

    def ln1_stats(s, jt, late=False):
        cols = seg_cols(s, jt)
        pivot = a1 = a2 = None
        for c in range(D // 32):
            x = x_v[32 * c:32 * (c + 1), cols].astype(F32)
            if c == 0:
                pivot = x[0:1, :]
                if late:
                    slot = MOFF[3] + 2
                    bits = pltpu.bitcast(m_blk[HS - 1, slot * 8:slot * 8 + 8, :], U32) & zero_s[0].astype(U32)
                    pivot = pivot + pltpu.bitcast(bits, F32)[0:1, :]
            d = (x - pivot).reshape(4, 8, T)
            p1 = (d[0] + d[1]) + (d[2] + d[3])
            dd = d * d
            p2 = (dd[0] + dd[1]) + (dd[2] + dd[3])
            a1 = p1 if c == 0 else a1 + p1
            a2 = p2 if c == 0 else a2 + p2
        m, inv = _ln_scale(pivot, jnp.sum(a1, axis=0, keepdims=True), jnp.sum(a2, axis=0, keepdims=True))
        ln_st[s, jt, 0:1, :] = m
        ln_st[s, jt, 8:9, :] = inv

    def ln1_norm(s, jt, c=None):
        for cc in (range(NG) if c is None else (c,)):
            r0, r1 = T * cc, min(T * (cc + 1), D)
            x = x_v[r0:r1, seg_cols(s, jt)].astype(F32)
            xn[r0 // 2:r1 // 2, jt * T:(jt + 1) * T] = _u32(
                ((x - ln_st[s, jt, 0:1, :]) * ln_st[s, jt, 8:9, :]).astype(BF16))

    def q_unit(jt, g):
        cols = slice(jt * T, (jt + 1) * T)
        n = min(64, QR // 2 - 64 * g)
        q = jnp.dot(_bf(wqkv[64 * g:64 * g + n, :]), _bf(xn[:, cols]), preferred_element_type=F32)
        qt[g, 0:n, cols] = _pack_rows(q * QSCALE)
        pqt[g, 0:n, cols] = _pack_rows(_phi(q))

    def k_unit(jt, g):
        cols = slice(jt * T, (jt + 1) * T)
        n = min(64, QR // 2 - 64 * g)
        b0 = QR // 2 + 64 * g
        k = jnp.dot(_bf(wqkv[b0:b0 + n, :]), _bf(xn[:, cols]), preferred_element_type=F32)
        pkt[g, 0:n, cols] = _pack_rows(_phi(k))
        kb = _pack_rows(k)
        if n < 64:
            kb = jnp.concatenate([kb, jnp.zeros((64 - n, T), U32)], axis=0)
        kk[g, jt * 64:(jt + 1) * 64, :] = _u32(_bf(kb).T)

    def v_unit(jt, c):
        cols = slice(jt * T, (jt + 1) * T)
        b0 = QR + 64 * c
        v = jnp.dot(_bf(wqkv[b0:b0 + 64, :]), _bf(xn[:, cols]), preferred_element_type=F32)
        vt[64 * c:64 * (c + 1), cols] = _pack_rows(v + ones_tab[T * c:T * (c + 1), :])

    def mem_read_unit(g):
        w0, w1 = GWIN[g]
        b = bd[g, 0:w1 - w0, :].astype(BF16)
        res = jnp.dot(b, _bf(pqt[g]), preferred_element_type=F32)
        lo, hi = 140 * g, 140 * g + 20 * GH[g]
        memt[lo:hi, :] = res[lo - w0:hi - w0]

    def mem_update_unit(g):
        w0, w1 = GWIN[g]
        upd = lax.dot_general(_bf(vt[w0 // 2:w1 // 2, :]), _bf(pkt[g]), NT, preferred_element_type=F32)
        n = w1 - w0
        bd[g, 0:n, :] = bd[g, 0:n, :] + jnp.where(keep_tab[g, 0:n, :] > 0.5, upd, 0.0)

    def sbuf(h):
        if h < HS:
            return s_a, h
        return (s_b1, h - HS) if h < HM else (s_b2, h - HM)

    def head_rows(j):
        r = lax.broadcasted_iota(jnp.int32, (64, T), 0)
        return (r >= 9 * j) & (r < 9 * j + 9)

    def s_blk(h, jq, kb, half=False):
        g, j = divmod(h, 7)
        off = SOFF[jq] + kb * T
        n = 64 if half else T
        qm = _bf(jnp.where(head_rows(j), qt[g, :, jq * T:(jq + 1) * T], U32(0)))
        sc = jnp.dot(_bf(kk[g, kb * 64:kb * 64 + n // 2, :]), qm, preferred_element_type=F32)
        if kb == jq:
            sc = sc + bias[0:n, :]
        sb, hi_ = sbuf(h)
        sb[hi_, off:off + n, :] = sc
        slot = MOFF[jq] + kb
        m_blk[h, slot * 8:(slot + 1) * 8, :] = jnp.max(sc.reshape(n // 8, 8, T), axis=0)

    def s_pair(ha, jq):
        g, j = divmod(ha, 7)
        off = SOFF[jq] + jq * T + 64
        lo = lax.broadcasted_iota(jnp.int32, (64, T), 1) < 64
        qu = qt[g, :, jq * T:(jq + 1) * T]
        qmix = jnp.where(lo, pltpu.roll(qu, 64, 1), qu)
        qm = _bf(jnp.where((lo & head_rows(j)) | (~lo & head_rows(j + 1)), qmix, U32(0)))
        sc = jnp.dot(_bf(kk[g, jq * 64 + 32:jq * 64 + 64, :]), qm, preferred_element_type=F32) + bias2[...]
        sb, hi_ = sbuf(ha)
        sb[hi_, off:off + 64, :] = sc
        pm = jnp.max(sc.reshape(8, 8, T), axis=0)
        hi = lax.broadcasted_iota(jnp.int32, (8, T), 1) >= 64
        slot = MOFF[jq] + jq + 1
        m_blk[ha, slot * 8:(slot + 1) * 8, :] = jnp.where(hi, pltpu.roll(pm, 64, 1), -jnp.inf)
        m_blk[ha + 1, slot * 8:(slot + 1) * 8, :] = jnp.where(hi, pm, -jnp.inf)

    def row_max(h, jq, nslots):
        return jnp.max(m_blk[h, MOFF[jq] * 8:(MOFF[jq] + nslots) * 8, :], axis=0, keepdims=True)

    def pv_blk(h, jq, kb, st, role):
        w0 = (VS * h) // 16 * 16
        o = VS * h - w0
        off = SOFF[jq] + kb * T
        cols = slice(jq * T, (jq + 1) * T)
        key = role or 'a'
        sb, hz = sbuf(h)
        hz = hz + st['z']
        if kb == 0 and role != 'b':
            st['ma'] = row_max(h, jq, jq + 1 if role is None else jq + 2)
            if role == 'a':
                st['mb'] = row_max(h + 1, jq, jq + 2)
        m = st['m' + key]
        if kb < jq or role is None:
            p = jnp.exp2(sb[hz, off:off + T, :] - m).astype(BF16)
        else:
            if role == 'a':
                hi1 = lax.broadcasted_iota(jnp.int32, (1, T), 1) >= 64
                hi = lax.broadcasted_iota(jnp.int32, (64, T), 1) >= 64
                m2 = jnp.where(hi1, st['mb'], pltpu.roll(st['ma'], 64, 1))
                e2 = jnp.exp2(sb[hz, off + 64:off + T, :] - m2)
                p2 = jnp.where(hi, pltpu.roll(e2, 64, 1), 0.0)
                st['p2b'] = jnp.where(hi, e2, 0.0)
            else:
                p2 = st['p2b']
            p1 = jnp.exp2(sb[hz, off:off + 64, :] - m)
            p = jnp.concatenate([p1, p2], axis=0).astype(BF16)
        part = jnp.dot(_bf(vt[w0 // 2:w0 // 2 + 16, kb * T:(kb + 1) * T]), p, preferred_element_type=F32)
        st['pv' + key] = part if kb == 0 else st['pv' + key] + part
        if kb == jq:
            pv = st['pv' + key]
            res = pv * (gtab[1, h:h + 1, :] / pv[o + DH:o + DH + 1, :])
            mem = memt[w0:w0 + 32, cols]
            res = res + mem * (gtab[0, h:h + 1, :] / (mem[o + DH:o + DH + 1, :] + 1e-6))
            ot[VS * h // 2:VS * h // 2 + VS // 2, cols] = _u32(res.astype(BF16))[o // 2:o // 2 + VS // 2]

    def o_early(s, jt, c, ke):
        r0, r1 = T * c, min(T * (c + 1), D)
        tile = slice(jt * T, (jt + 1) * T)
        a = jnp.dot(_bf(wot[r0 // 2:r1 // 2, 0:ke]), _bf(ot[0:ke // 2, tile]), preferred_element_type=F32)
        att[r0:r1, tile] = x_v[r0:r1, seg_cols(s, jt)].astype(F32) + a

    def o_unit(s, jt, c, ke, st):
        r0, r1 = T * c, min(T * (c + 1), D)
        tile = slice(jt * T, (jt + 1) * T)
        a = jnp.dot(_bf(wot[r0 // 2:r1 // 2, ke:640]), _bf(ot[ke // 2:320, tile]), preferred_element_type=F32)
        hh = att[r0:r1, tile] + a
        att[r0:r1, tile] = hh
        if c == 0:
            st['p'] = hh[0:1, :]
        d = hh - st['p']
        s1 = jnp.sum(d, axis=0, keepdims=True)
        s2 = jnp.sum(d * d, axis=0, keepdims=True)
        st['s1'] = s1 if c == 0 else st['s1'] + s1
        st['s2'] = s2 if c == 0 else st['s2'] + s2

    def e2_unit(s, jt, c, st):
        r0, r1 = T * c, min(T * (c + 1), D)
        cols = seg_cols(s, jt)
        if c == 0:
            st['m'], st['inv'] = _ln_scale(st['p'], st['s1'], st['s2'])
        hh = att[r0:r1, jt * T:(jt + 1) * T]
        y = (hh - st['m']) * st['inv']
        n = (r1 - r0) // 2
        h_s[r0 // 2:r1 // 2, cols] = pltpu.pack_elementwise([hh[0:n], hh[n:2 * n]], packed_dtype=BF16)
        out_s[r0:r1, cols] = (hh + y).astype(BF16)
        yb = y.astype(BF16)
        rr = jnp.dot(wr16[:, r0:r1], yb, preferred_element_type=F32)
        st['r'] = rr if c == 0 else st['r'] + rr
        cand = st.get('cand')
        if cand is not None:
            cand.setdefault(jt, {'y': []})['y'].append(yb)
        if r1 == D:
            rrow = _rb(st['r'][0:1, :])
            if cand is None:
                r_s[s, :, jt * T:(jt + 1) * T] = jnp.broadcast_to(rrow, (8, T))
            else:
                cand[jt]['r'] = rrow

    def offer_last(best, cand):
        rrow = jnp.concatenate([cand[jt]['r'] for jt in range(4)], axis=1)
        tmax = jnp.max(rrow, axis=1, keepdims=True)
        lane = lax.broadcasted_iota(jnp.int32, (1, L), 1)
        lane_c = jnp.min(jnp.where(rrow == tmax, lane, L), axis=1, keepdims=True)
        xs = None
        for jt in range(4):
            oh = (lax.broadcasted_iota(jnp.int32, (16, T), 1) == lane_c - jt * T).astype(BF16)
            part = jnp.concatenate([lax.dot_general(oh, yc, NT, preferred_element_type=F32)
                                    for yc in cand[jt]['y']], axis=1)
            xs = part if xs is None else xs + part
        take = tmax > best['r']
        best.update(r=jnp.where(take, tmax, best['r']),
                    tok=jnp.where(take, (NSEG - 1) * L + lane_c, best['tok']),
                    xs=jnp.where(take, xs, best['xs']))

    def prep_qk(i, base):
        wt = _u32(w_v[i].T)
        for g in range(NG):
            n = 9 * GH[g]
            wqkv[base + 64 * g:base + 64 * g + n, :] = wt[63 * g:63 * g + n, :]
        deinterleave(base, 4 * 64)
        deinterleave(base + 4 * 64, QR // 2 - 4 * 64)

    def prep_v():
        wt = _u32(w_v[2].T)
        for h in range(H):
            wqkv[QR + 10 * h:QR + 10 * h + 9, :] = wt[9 * h:9 * h + 9, :]
        deinterleave(QR, 320)

    def deinterleave(base, nwords):
        lo16 = U32(0xFFFF)
        hi16 = U32(0xFFFF0000)
        for lt in range(NG if PACK else 0):
            w = min(T, D - T * lt)
            lanes = slice(T * lt, T * lt + w)
            dtmp[0:nwords, 0:w] = wqkv[base:base + nwords, lanes]
            b = 0
            while b < nwords:
                half = 8 if nwords - b >= 16 else 4
                ev = dtmp[pl.ds(b, half, stride=2), :]
                od = dtmp[pl.ds(b + 1, half, stride=2), :]
                wqkv[base + b:base + b + half, lanes] = ((ev & lo16) | (od << 16))[:, 0:w]
                wqkv[base + b + half:base + b + 2 * half, lanes] = ((ev >> 16) | (od & hi16))[:, 0:w]
                b += 2 * half

    def prep_o():
        wt = _u32(w_v[3])
        wpad = jnp.concatenate(
            [piece for h in range(H) for piece in (wt[9 * h:9 * h + 9, :], jnp.zeros((1, D), U32))], axis=0)
        wot[...] = _u32(_bf(wpad).T)

    BLKS = [(jq, kb) for jq in range(4) for kb in range(jq + 1)]

    def head_sets(heads):
        sets, i = [], 0
        while i < len(heads):
            h = heads[i]
            if h % 7 % 2 == 0 and h % 7 < 6 and i + 1 < len(heads):
                sets.append((h, h + 1))
                i += 2
            else:
                assert h % 7 == 6
                sets.append((h,))
                i += 1
        return sets

    def s_items(heads, small_tail=0):
        big, small = [], []
        for hs in head_sets(heads):
            for jq, kb in BLKS:
                halved = len(hs) == 2 and kb == jq
                for h in hs:
                    (small if halved else big).append(functools.partial(s_blk, h, jq, kb, halved))
                if halved:
                    small.append(functools.partial(s_pair, hs[0], jq))
        tail = small[len(small) - small_tail:] if small_tail else []
        small = small[:len(small) - small_tail] if small_tail else small
        order = sorted([((j + 0.5) / len(big), 0, j) for j in range(len(big))]
                       + [((j + 0.5) / len(small), 1, j) for j in range(len(small))])
        return [(big, small)[w][j] for _, w, j in order] + tail

    def phase_x():
        sb = s_items(HB)
        for it in sb[0:NS0]:
            it()
        interleave(pv_items(HA), sb[NS0:])

    def pv_items_by_tile(heads, z):
        out = {}
        for jq in range(4):
            out[jq] = []
            for hs in head_sets(heads):
                st = {'z': z}
                roles = ('a', 'b') if len(hs) == 2 else (None,)
                for kb in range(jq + 1):
                    for h, role in zip(hs, roles):
                        out[jq].append(functools.partial(pv_blk, h, jq, kb, st, role))
        return out

    def pv_items(heads, z=0):
        items = []
        for hs in head_sets(heads):
            st = {'z': z}
            roles = ('a', 'b') if len(hs) == 2 else (None,)
            for jq, kb in BLKS:
                for h, role in zip(hs, roles):
                    items.append(functools.partial(pv_blk, h, jq, kb, st, role))
        return items

    def interleave(*seqs):
        seqs = [q for q in seqs if q]
        order = []
        for i, q in enumerate(seqs):
            order += [((j + 0.5) / len(q), i, j) for j in range(len(q))]
        for _, i, j in sorted(order):
            seqs[i][j]()

    def proj_items(fn):
        return [functools.partial(fn, jt, g) for jt in range(4) for g in range(NG)]

    def out_items(s, ke, cand=None):
        sts = [{'cand': cand} for _ in range(4)]
        o_items = [functools.partial(o_unit, s, jt, c, ke, sts[jt]) for jt in range(4) for c in range(NG)]
        e_items = [functools.partial(e2_unit, s, jt, c, sts[jt]) for jt in range(4) for c in range(NG)]
        early = [functools.partial(o_early, s, jt, c, ke) for jt in range(4) for c in range(NG)]
        return early, o_items, e_items

    HA = list(range(HS))
    HB = list(range(HS, H))

    x_copy(0).start()
    w_copy(1).start()
    zero_s[0] = 0
    beta_copy.start()
    wr_copy.start()
    with _scope('p0_const'):
        kr = lax.broadcasted_iota(jnp.int32, (T, T), 0)
        qc = lax.broadcasted_iota(jnp.int32, (T, T), 1)
        bias[...] = jnp.where(kr > qc, MASKVAL, 0.0).astype(F32)
        kr2 = lax.broadcasted_iota(jnp.int32, (64, T), 0)
        qc2 = lax.broadcasted_iota(jnp.int32, (64, T), 1)
        bias2[...] = jnp.where(kr2 > (qc2 & 63), MASKVAL, 0.0).astype(F32)
        wqkv[...] = jnp.zeros(wqkv.shape, U32)
        bd[...] = jnp.zeros(bd.shape, F32)
        memt[...] = jnp.zeros(memt.shape, F32)
        row = lax.broadcasted_iota(jnp.int32, (640, T), 0)
        sub = row & 31
        nat = (row - sub) + jnp.where(sub < 16, 2 * sub, 2 * sub - 31)
        if not PACK:
            nat = row
        ones_tab[...] = jnp.where(nat % VS == DH, 1.0, 0.0).astype(F32)
        dtmp[...] = jnp.zeros(dtmp.shape, U32)
        for g in range(NG):
            row = lax.broadcasted_iota(jnp.int32, (160, T), 0) + (GWIN[g][0] - 140 * g)
            lane = lax.broadcasted_iota(jnp.int32, (160, T), 1)
            keep = ((row >= 0) & (row < 20 * GH[g]) & (lane >= (row // VS) * DH)
                    & (lane < (row // VS) * DH + DH))
            keep_tab[g] = jnp.where(keep, 1.0, 0.0).astype(F32)
        pqt[NG - 1] = jnp.zeros(pqt.shape[1:], U32)
        pkt[NG - 1] = jnp.zeros(pkt.shape[1:], U32)

    with _scope('p1_ln'):
        x_copy(0).wait()
        w_copy(0).start()
        for jt in range(4):
            ln1_stats(0, jt)
            ln1_norm(0, jt)
    with _scope('p2_wq'):
        w_copy(1).wait()
        w_copy(2).start()
        prep_qk(1, 0)
        for g in range(NG):
            for jt in range(2):
                q_unit(jt, g)
    with _scope('p3_q'):
        w_copy(0).wait()
        w_copy(3).start()
        prep_qk(0, QR // 2)
        for jt in range(2, 4):
            for g in range(NG):
                q_unit(jt, g)
    with _scope('p4_k'):
        w_copy(2).wait()
        for i in range(1, NSEG):
            x_copy(i).start()
        prep_v()
        for jt in range(4):
            for g in range(NG):
                k_unit(jt, g)
    with _scope('p5_v'):
        w_copy(3).wait()
        beta_copy.wait()
        wr_copy.wait()
        for i in range(1, NSEG):
            x_copy(i).wait()
        prep_o()
        beta = beta_v[...].astype(F32).reshape(1, H)
        hl = lax.broadcasted_iota(jnp.int32, (H, H), 1)
        hs = lax.broadcasted_iota(jnp.int32, (H, H), 0)
        bcol = jnp.sum(jnp.where(hl == hs, jnp.broadcast_to(beta, (H, H)), 0.0), axis=1, keepdims=True)
        gate = _rb(jax.nn.sigmoid(bcol))
        gtab[0] = jnp.broadcast_to(gate, (H, T))
        gtab[1] = jnp.broadcast_to(_rb(1.0 - gate), (H, T))
        r16 = lax.broadcasted_iota(jnp.int32, (16, D), 0)
        wr_row = wr_v[...].astype(F32).reshape(1, D)
        wr16[...] = jnp.where(r16 == 0, jnp.broadcast_to(wr_row, (16, D)), 0.0).astype(BF16)
        if STATV == 0:
            interleave(proj_items(v_unit) + s_items(HA, 16),
                       [functools.partial(ln1_stats, i, jt) for i in range(1, NSEG) for jt in range(4)])
        else:
            for it in proj_items(v_unit) + s_items(HA, 16):
                it()
            for jt in range(4):
                ln1_stats(1, jt, True)

    def seg_body(s, carry):
        with _scope('seg_xy'):
            z = zero_s[0]
            phase_x()
            ln = [functools.partial(ln1_norm, s + 1, jt) for jt in range(4)]
            qs = proj_items(q_unit)
            early, o_items, e_items = out_items(s, KE)
            upd = [functools.partial(mem_update_unit, g) for g in range(NG)]
            ks = proj_items(k_unit)
            if Y1V == 0:
                pre = [ln[0]] + early[0:10] + [ln[1]]
                mxu1 = upd + qs[0:5] + [ln[2]] + early[10:20] + qs[5:10] + [ln[3]] + qs[10:20] + ks
            elif Y1V == 1:
                pre = [ln[0], ln[1]] + early[0:10]
                mxu1 = [ln[2]] + upd + [ln[3]] + early[10:20] + qs + ks
            elif Y1V == 2:
                pre = [ln[0]] + early[0:8] + [ln[1]]
                mxu1 = early[8:14] + [ln[2]] + upd + qs[0:5] + early[14:20] + [ln[3]] + qs[5:20] + ks
            elif Y1V == 3:
                pre = ln + early[0:10]
                mxu1 = upd + early[10:20] + qs + ks
            else:
                pre = [ln[0]] + early[0:10] + [ln[1]]
                mxu1 = (upd + qs[0:5] + ks[0:5] + [ln[2]] + early[10:20] + qs[5:10] + ks[5:10] + [ln[3]]
                        + qs[10:15] + ks[10:15] + qs[15:20] + ks[15:20])
            for it in pre:
                it()
            interleave(pv_items(HB, z), mxu1)
            vr = proj_items(v_unit) + [functools.partial(mem_read_unit, g) for g in range(NG)]
            if Y2V == 0:
                for it in o_items:
                    it()
                interleave(vr, e_items[0:E2A])
            elif Y2V == 1:
                interleave(o_items, vr[0:10])
                interleave(vr[10:], e_items[0:E2A])
            else:
                for it in o_items[0:10]:
                    it()
                interleave(o_items[10:], vr[0:5])
                interleave(vr[5:], e_items[0:E2A])
            interleave(s_items(HA, TAIL), e_items[E2A:])
            if STATV == 1:
                for jt in range(4):
                    ln1_stats(jnp.minimum(s + 2, NSEG - 1), jt, True)
            o_copy(s).start()

            @pl.when(s == 0)
            def _():
                f_copy(0).start()
                f_copy(1).start()

            @pl.when(s == 1)
            def _():
                f_copy(2).start()
        return carry

    lax.fori_loop(0, NSEG - 1, seg_body, 0)

    def load_h_tile(tile):
        hw = h_s[:, tile]
        hlo = pltpu.bitcast(hw << 16, F32)
        hhi = pltpu.bitcast(hw & U32(0xFFFF0000), F32)
        pieces = []
        for c in range(NG):
            w0, w1 = 64 * c, min(64 * (c + 1), D // 2)
            pieces += [hlo[w0:w1], hhi[w0:w1]]
        return jnp.concatenate(pieces, axis=0)

    with _scope('seg_xz'):
        for i in range(3):
            f_copy(i).wait()
        z = zero_s[0]
        best = {}

        def offer_previous():
            n = (NSEG - 1) * 8
            r_all = r_s[0:NSEG - 1].reshape(n, L)
            tok = ((lax.broadcasted_iota(jnp.int32, (n, L), 0) // 8) * L
                   + lax.broadcasted_iota(jnp.int32, (n, L), 1))
            rmax = jnp.max(jnp.max(r_all, axis=1, keepdims=True), axis=0, keepdims=True)
            idx = jnp.clip(jnp.min(jnp.where(r_all == rmax, tok, S)), 0, S - 1)
            base = pl.multiple_of((idx // T) * T, T)
            yt = _layernorm(load_h_tile(pl.ds(base, T)), 0)
            onehot = (lax.broadcasted_iota(jnp.int32, (16, T), 1) == idx - base).astype(BF16)
            xs = lax.dot_general(onehot, yt.astype(BF16), NT, preferred_element_type=F32)
            best.update(r=rmax, tok=jnp.full((1, 1), idx, jnp.int32), xs=xs)

        ha1, ha2 = HA[:HA1], HA[HA1:]
        hb1, hb2 = list(range(HS, HM)), list(range(HM, H))
        sb1 = s_items(hb1)
        for it in sb1[0:NS0]:
            it()
        interleave(pv_items(ha1), sb1[NS0:])
        offer_previous()
        sb2 = s_items(hb2)
        interleave(pv_items(ha2) + pv_items(hb1, z), sb2)
        cand = {}
        early, o_items, e_items = out_items(NSEG - 1, KM, cand)
        for it in early[0:4]:
            it()
        interleave(pv_items(hb2, z), early[4:])
        for jt in range(4):
            for it in o_items[jt * NG:(jt + 1) * NG]:
                it()
            if jt > 0:
                for it in e_items[(jt - 1) * NG:jt * NG]:
                    it()
        for it in e_items[3 * NG:]:
            it()
        offer_last(best, cand)
        o_copy(NSEG - 1).start()

    xs_v[...] = best['xs'].astype(BF16)
    best_v[...] = jnp.broadcast_to(best['r'], (8, T))
    idx = jnp.clip(jnp.max(best['tok']), 0, S - 1)
    base = pl.multiple_of((idx // T) * T, T)
    tile = pl.ds(base, T)
    htile = load_h_tile(tile)
    hy_v[0] = htile
    hy_v[1] = _rb(_layernorm(htile, 0))
    hy_v[2] = out_s[:, tile].astype(F32)

    @pl.when(zero_s[0] == 0)
    def _ffn():
        with _scope('ffn'):
            xs = xs_v[...]
            acc = jnp.zeros((D, T), F32)
            f0 = 0
            for fw in FCH:
                fc = slice(f0, f0 + fw)
                gt = _rb(jnp.dot(xs, wg_v[:, fc], preferred_element_type=F32))
                up = _rb(jnp.dot(xs, wu_v[:, fc], preferred_element_type=F32))
                act = _rb(_rb(gt * jax.nn.sigmoid(gt)) * up)[0:1, :]
                for t in range(fw // T):
                    acc = acc + (wd_v[:, f0 + t * T:f0 + (t + 1) * T].astype(F32) * act[:, t * T:(t + 1) * T])
                f0 += fw
            ycol = _rb(jnp.sum(acc, axis=1, keepdims=True))
            ycol = _rb(ycol * _rb(jax.nn.sigmoid(best_v[0:1, 0:1])))
            sel = lax.broadcasted_iota(jnp.int32, (D, T), 1) == idx - base
            new = hy_v[0] + _rb(hy_v[1] + ycol)
            fix_v[...] = jnp.where(sel, new, hy_v[2]).astype(BF16)

    for s in range(NSEG):
        o_copy(s).wait()
    fix = pltpu.make_async_copy(fix_v, out_hbm.at[0, :, tile], sem_o.at[0])
    fix.start()
    fix.wait()


@jax.jit
def pallas_sequential_preLN__memory_aug_infini_attn__moe_arch_mod__prompt_kernel(
    A_x: jax.Array,
    A_wq: jax.Array,
    A_wk: jax.Array,
    A_wv: jax.Array,
    A_wo: jax.Array,
    A_beta: jax.Array,
    B_x: jax.Array,
    B_w_r: jax.Array,
    B_w_gate: jax.Array,
    B_w_up: jax.Array,
    B_w_down: jax.Array,
):
    del B_x
    hbm = pl.BlockSpec(memory_space=pltpu.HBM)
    scratch = [
        pltpu.VMEM((D, S), BF16),
        pltpu.VMEM((4, D, D), BF16),
        pltpu.VMEM((QR + 320, D), U32),
        pltpu.VMEM((D // 2, 640), U32),
        pltpu.VMEM((D // 2, L), U32),
        pltpu.VMEM((NG, 64, L), U32),
        pltpu.VMEM((NG, 64, L), U32),
        pltpu.VMEM((NG, L // 2, T), U32),
        pltpu.VMEM((NG, 64, L), U32),
        pltpu.VMEM((320, L), U32),
        pltpu.VMEM((640, L), F32),
        pltpu.VMEM((NG, 160, T), F32),
        pltpu.VMEM((HS, 1280, T), F32),
        pltpu.VMEM((HM - HS, 1280, T), F32),
        pltpu.VMEM((H - HM, 1280, T), F32),
        pltpu.VMEM((H, 112, T), F32),
        pltpu.VMEM((320, L), U32),
        pltpu.VMEM((D, L), F32),
        pltpu.VMEM((NSEG, 4, 16, T), F32),
        pltpu.VMEM((D // 2, S), U32),
        pltpu.VMEM((D, S), BF16),
        pltpu.VMEM((NSEG, 8, L), F32),
        pltpu.VMEM((T, T), F32),
        pltpu.VMEM((64, T), F32),
        pltpu.VMEM((2, H, T), F32),
        pltpu.VMEM((640, T), F32),
        pltpu.VMEM((NG, 160, T), F32),
        pltpu.VMEM((D, FF), BF16),
        pltpu.VMEM((D, FF), BF16),
        pltpu.VMEM((D, FF), BF16),
        pltpu.VMEM((H,), BF16),
        pltpu.VMEM((D,), BF16),
        pltpu.VMEM((16, D), BF16),
        pltpu.VMEM((320, T), U32),
        pltpu.VMEM((16, D), BF16),
        pltpu.VMEM((8, T), F32),
        pltpu.VMEM((D, T), BF16),
        pltpu.VMEM((3, D, T), F32),
        pltpu.SMEM((1,), jnp.int32),
        pltpu.SemaphoreType.DMA((NSEG,)),
        pltpu.SemaphoreType.DMA((4,)),
        pltpu.SemaphoreType.DMA((3,)),
        pltpu.SemaphoreType.DMA((NSEG,)),
        pltpu.SemaphoreType.DMA((2,)),
    ]
    out_t = pl.pallas_call(
        _kernel,
        out_shape=jax.ShapeDtypeStruct((1, D, S), BF16),
        in_specs=[hbm] * 10,
        out_specs=hbm,
        scratch_shapes=scratch,
        compiler_params=pltpu.CompilerParams(vmem_limit_bytes=110 * 1024 * 1024),
        name="infini_moe",
    )(jnp.transpose(A_x, (0, 2, 1)), A_wq, A_wk, A_wv, A_wo, A_beta, B_w_r,
      B_w_gate, B_w_up, jnp.transpose(B_w_down, (1, 0)))
    return jnp.transpose(out_t, (0, 2, 1))
```

```python
import functools
import math

import jax
import jax.numpy as jnp
from jax import lax
import jax.experimental.pallas as pl
import jax.experimental.pallas.tpu as pltpu

F32 = jnp.float32
BF16 = jnp.bfloat16
U32 = jnp.uint32

S = 2048
D = 576
H = 32
DH = 18
NSEG = 4
L = 512
FF = 4608
T = 128
NG = 5
GH = (7, 7, 7, 7, 4)
VS = 20
EPS = 1e-5
QSCALE = DH ** (-0.5) * math.log2(math.e)
MASKVAL = -1000000000.0 * math.log2(math.e)
SOFF = (0, 128, 384, 768)
MOFF = (0, 2, 5, 9)
GWIN = tuple(((140 * g) // 16 * 16, -(-(140 * g + 20 * GH[g]) // 16) * 16) for g in range(NG))
QR = 592
FCH = (256,) * 18
import os
import contextlib
PROF = bool(int(os.environ.get('PROF', '0')))


def _scope(name):
    return jax.named_scope(name) if PROF else contextlib.nullcontext()


HS = int(os.environ.get('HS', '16'))
PACK = int(os.environ.get('PACK', '0'))
NS0 = int(os.environ.get('NS0', '12'))
HA1 = int(os.environ.get('HA1', '9'))
Y1V = int(os.environ.get('Y1V', '2'))
Y2V = int(os.environ.get('Y2V', '0'))
E2A = int(os.environ.get('E2A', '20'))
TAIL = int(os.environ.get('TAIL', '16'))
STATV = int(os.environ.get('STATV', '0'))
HM = int(os.environ.get('HM', '25'))
KE = (VS * HS) // T * T
KM = (VS * HM) // T * T

NT = (((1,), (1,)), ((), ()))


def _bf(x_u32):
    return pltpu.bitcast(x_u32, BF16)


def _u32(x_bf):
    return pltpu.bitcast(x_bf, U32)


def _pack_rows(y):
    if not PACK:
        return _u32(y.astype(BF16))
    n = y.shape[0]
    parts = []
    full = n // 32 * 32
    if full:
        y4 = y[0:full].reshape(full // 32, 2, 16, T)
        parts.append(pltpu.pack_elementwise([y4[:, 0], y4[:, 1]], packed_dtype=BF16).reshape(full // 2, T))
    if n > full:
        parts.append(pltpu.pack_elementwise([y[full:full + 8], y[full + 8:full + 16]], packed_dtype=BF16))
    return parts[0] if len(parts) == 1 else jnp.concatenate(parts, axis=0)


def _rb(x):
    return x.astype(BF16).astype(F32)


def _phi(t):
    return jnp.where(t > 0, t + 1.0, jnp.exp(t))


def _layernorm(x, axis):
    m = jnp.mean(x, axis=axis, keepdims=True)
    c = x - m
    v = jnp.mean(c * c, axis=axis, keepdims=True)
    den = _rb(jnp.sqrt(_rb(_rb(v) + EPS)))
    return c * (1.0 / den)


def _ln_scale(pivot, s1, s2):
    md = s1 * (1.0 / D)
    v = jnp.maximum(s2 * (1.0 / D) - md * md, 0.0)
    den = _rb(jnp.sqrt(_rb(_rb(v) + EPS)))
    return pivot + md, 1.0 / den


def _kernel(x_hbm, wq_hbm, wk_hbm, wv_hbm, wo_hbm, beta_hbm, wr_hbm, wg_hbm, wu_hbm, wd_hbm,
            out_hbm,
            x_v, w_v, wqkv, wot, xn, qt, pqt, kk, pkt, vt, memt, bd, s_a, s_b1, s_b2, m_blk,
            ot, att, ln_st, y_s, out_s, r_s, bias, bias2, gtab, ones_tab, keep_tab,
            wg_v, wu_v, wd_v, beta_v, wr_v, wr16, dtmp, xs_v, best_v, fix_v,
            zero_s, sem_x, sem_w, sem_f, sem_o, sem_s):
    def x_copy(s):
        return pltpu.make_async_copy(x_hbm.at[0, :, pl.ds(s * L, L)], x_v.at[:, pl.ds(s * L, L)],
                                     sem_x.at[s])

    w_srcs = (wk_hbm, wq_hbm, wv_hbm, wo_hbm)

    def w_copy(i):
        return pltpu.make_async_copy(w_srcs[i], w_v.at[i], sem_w.at[i])

    f_pairs = ((wg_hbm, wg_v), (wu_hbm, wu_v), (wd_hbm, wd_v))

    def f_copy(i):
        return pltpu.make_async_copy(f_pairs[i][0], f_pairs[i][1], sem_f.at[i])

    def o_copy(s):
        return pltpu.make_async_copy(out_s.at[:, pl.ds(s * L, L)], out_hbm.at[0, :, pl.ds(s * L, L)],
                                     sem_o.at[s])

    beta_copy = pltpu.make_async_copy(beta_hbm, beta_v, sem_s.at[0])
    wr_copy = pltpu.make_async_copy(wr_hbm, wr_v, sem_s.at[1])

    def seg_cols(s, jt):
        if isinstance(s, int):
            return slice(s * L + jt * T, s * L + (jt + 1) * T)
        return pl.ds(pl.multiple_of(s * L + jt * T, T), T)

    def ln1_stats(s, jt, late=False):
        cols = seg_cols(s, jt)
        pivot = a1 = a2 = None
        for c in range(D // 32):
            x = x_v[32 * c:32 * (c + 1), cols].astype(F32)
            if c == 0:
                pivot = x[0:1, :]
                if late:
                    slot = MOFF[3] + 2
                    bits = pltpu.bitcast(m_blk[HS - 1, slot * 8:slot * 8 + 8, :], U32) & zero_s[0].astype(U32)
                    pivot = pivot + pltpu.bitcast(bits, F32)[0:1, :]
            d = (x - pivot).reshape(4, 8, T)
            p1 = (d[0] + d[1]) + (d[2] + d[3])
            dd = d * d
            p2 = (dd[0] + dd[1]) + (dd[2] + dd[3])
            a1 = p1 if c == 0 else a1 + p1
            a2 = p2 if c == 0 else a2 + p2
        m, inv = _ln_scale(pivot, jnp.sum(a1, axis=0, keepdims=True), jnp.sum(a2, axis=0, keepdims=True))
        ln_st[s, jt, 0:1, :] = m
        ln_st[s, jt, 8:9, :] = inv

    def ln1_norm(s, jt, c=None):
        for cc in (range(NG) if c is None else (c,)):
            r0, r1 = T * cc, min(T * (cc + 1), D)
            x = x_v[r0:r1, seg_cols(s, jt)].astype(F32)
            xn[r0 // 2:r1 // 2, jt * T:(jt + 1) * T] = _u32(
                ((x - ln_st[s, jt, 0:1, :]) * ln_st[s, jt, 8:9, :]).astype(BF16))

    def q_unit(jt, g):
        cols = slice(jt * T, (jt + 1) * T)
        n = min(64, QR // 2 - 64 * g)
        q = jnp.dot(_bf(wqkv[64 * g:64 * g + n, :]), _bf(xn[:, cols]), preferred_element_type=F32)
        qt[g, 0:n, cols] = _pack_rows(q * QSCALE)
        pqt[g, 0:n, cols] = _pack_rows(_phi(q))

    def k_unit(jt, g):
        cols = slice(jt * T, (jt + 1) * T)
        n = min(64, QR // 2 - 64 * g)
        b0 = QR // 2 + 64 * g
        k = jnp.dot(_bf(wqkv[b0:b0 + n, :]), _bf(xn[:, cols]), preferred_element_type=F32)
        pkt[g, 0:n, cols] = _pack_rows(_phi(k))
        kb = _pack_rows(k)
        if n < 64:
            kb = jnp.concatenate([kb, jnp.zeros((64 - n, T), U32)], axis=0)
        kk[g, jt * 64:(jt + 1) * 64, :] = _u32(_bf(kb).T)

    def v_unit(jt, c):
        cols = slice(jt * T, (jt + 1) * T)
        b0 = QR + 64 * c
        v = jnp.dot(_bf(wqkv[b0:b0 + 64, :]), _bf(xn[:, cols]), preferred_element_type=F32)
        vt[64 * c:64 * (c + 1), cols] = _pack_rows(v + ones_tab[T * c:T * (c + 1), :])

    def mem_read_unit(g):
        w0, w1 = GWIN[g]
        b = bd[g, 0:w1 - w0, :].astype(BF16)
        res = jnp.dot(b, _bf(pqt[g]), preferred_element_type=F32)
        lo, hi = 140 * g, 140 * g + 20 * GH[g]
        memt[lo:hi, :] = res[lo - w0:hi - w0]

    def mem_update_unit(g):
        w0, w1 = GWIN[g]
        upd = lax.dot_general(_bf(vt[w0 // 2:w1 // 2, :]), _bf(pkt[g]), NT, preferred_element_type=F32)
        n = w1 - w0
        bd[g, 0:n, :] = bd[g, 0:n, :] + jnp.where(keep_tab[g, 0:n, :] > 0.5, upd, 0.0)

    def sbuf(h):
        if h < HS:
            return s_a, h
        return (s_b1, h - HS) if h < HM else (s_b2, h - HM)

    def head_rows(j):
        r = lax.broadcasted_iota(jnp.int32, (64, T), 0)
        return (r >= 9 * j) & (r < 9 * j + 9)

    def s_blk(h, jq, kb, half=False):
        g, j = divmod(h, 7)
        off = SOFF[jq] + kb * T
        n = 64 if half else T
        qm = _bf(jnp.where(head_rows(j), qt[g, :, jq * T:(jq + 1) * T], U32(0)))
        sc = jnp.dot(_bf(kk[g, kb * 64:kb * 64 + n // 2, :]), qm, preferred_element_type=F32)
        if kb == jq:
            sc = sc + bias[0:n, :]
        sb, hi_ = sbuf(h)
        sb[hi_, off:off + n, :] = sc
        slot = MOFF[jq] + kb
        m_blk[h, slot * 8:(slot + 1) * 8, :] = jnp.max(sc.reshape(n // 8, 8, T), axis=0)

    def s_pair(ha, jq):
        g, j = divmod(ha, 7)
        off = SOFF[jq] + jq * T + 64
        lo = lax.broadcasted_iota(jnp.int32, (64, T), 1) < 64
        qu = qt[g, :, jq * T:(jq + 1) * T]
        qmix = jnp.where(lo, pltpu.roll(qu, 64, 1), qu)
        qm = _bf(jnp.where((lo & head_rows(j)) | (~lo & head_rows(j + 1)), qmix, U32(0)))
        sc = jnp.dot(_bf(kk[g, jq * 64 + 32:jq * 64 + 64, :]), qm, preferred_element_type=F32) + bias2[...]
        sb, hi_ = sbuf(ha)
        sb[hi_, off:off + 64, :] = sc
        pm = jnp.max(sc.reshape(8, 8, T), axis=0)
        hi = lax.broadcasted_iota(jnp.int32, (8, T), 1) >= 64
        slot = MOFF[jq] + jq + 1
        m_blk[ha, slot * 8:(slot + 1) * 8, :] = jnp.where(hi, pltpu.roll(pm, 64, 1), -jnp.inf)
        m_blk[ha + 1, slot * 8:(slot + 1) * 8, :] = jnp.where(hi, pm, -jnp.inf)

    def row_max(h, jq, nslots):
        return jnp.max(m_blk[h, MOFF[jq] * 8:(MOFF[jq] + nslots) * 8, :], axis=0, keepdims=True)

    def pv_blk(h, jq, kb, st, role):
        w0 = (VS * h) // 16 * 16
        o = VS * h - w0
        off = SOFF[jq] + kb * T
        cols = slice(jq * T, (jq + 1) * T)
        key = role or 'a'
        sb, hz = sbuf(h)
        hz = hz + st['z']
        if kb == 0 and role != 'b':
            st['ma'] = row_max(h, jq, jq + 1 if role is None else jq + 2)
            if role == 'a':
                st['mb'] = row_max(h + 1, jq, jq + 2)
        m = st['m' + key]
        if kb < jq or role is None:
            p = jnp.exp2(sb[hz, off:off + T, :] - m).astype(BF16)
        else:
            if role == 'a':
                hi1 = lax.broadcasted_iota(jnp.int32, (1, T), 1) >= 64
                hi = lax.broadcasted_iota(jnp.int32, (64, T), 1) >= 64
                m2 = jnp.where(hi1, st['mb'], pltpu.roll(st['ma'], 64, 1))
                e2 = jnp.exp2(sb[hz, off + 64:off + T, :] - m2)
                p2 = jnp.where(hi, pltpu.roll(e2, 64, 1), 0.0)
                st['p2b'] = jnp.where(hi, e2, 0.0)
            else:
                p2 = st['p2b']
            p1 = jnp.exp2(sb[hz, off:off + 64, :] - m)
            p = jnp.concatenate([p1, p2], axis=0).astype(BF16)
        part = jnp.dot(_bf(vt[w0 // 2:w0 // 2 + 16, kb * T:(kb + 1) * T]), p, preferred_element_type=F32)
        st['pv' + key] = part if kb == 0 else st['pv' + key] + part
        if kb == jq:
            pv = st['pv' + key]
            res = pv * (gtab[1, h:h + 1, :] / pv[o + DH:o + DH + 1, :])
            mem = memt[w0:w0 + 32, cols]
            res = res + mem * (gtab[0, h:h + 1, :] / (mem[o + DH:o + DH + 1, :] + 1e-6))
            ot[VS * h // 2:VS * h // 2 + VS // 2, cols] = _u32(res.astype(BF16))[o // 2:o // 2 + VS // 2]

    def o_early(s, jt, c, ke):
        r0, r1 = T * c, min(T * (c + 1), D)
        tile = slice(jt * T, (jt + 1) * T)
        a = jnp.dot(_bf(wot[r0 // 2:r1 // 2, 0:ke]), _bf(ot[0:ke // 2, tile]), preferred_element_type=F32)
        att[r0:r1, tile] = x_v[r0:r1, seg_cols(s, jt)].astype(F32) + a

    def o_unit(s, jt, c, ke, st):
        r0, r1 = T * c, min(T * (c + 1), D)
        tile = slice(jt * T, (jt + 1) * T)
        a = jnp.dot(_bf(wot[r0 // 2:r1 // 2, ke:640]), _bf(ot[ke // 2:320, tile]), preferred_element_type=F32)
        hh = att[r0:r1, tile] + a
        att[r0:r1, tile] = hh
        if c == 0:
            st['p'] = hh[0:1, :]
        d = hh - st['p']
        s1 = jnp.sum(d, axis=0, keepdims=True)
        s2 = jnp.sum(d * d, axis=0, keepdims=True)
        st['s1'] = s1 if c == 0 else st['s1'] + s1
        st['s2'] = s2 if c == 0 else st['s2'] + s2

    def e2_unit(s, jt, c, st):
        r0, r1 = T * c, min(T * (c + 1), D)
        cols = seg_cols(s, jt)
        if c == 0:
            st['m'], st['inv'] = _ln_scale(st['p'], st['s1'], st['s2'])
        hh = att[r0:r1, jt * T:(jt + 1) * T]
        y = (hh - st['m']) * st['inv']
        n = (r1 - r0) // 2
        cand = st.get('cand')
        if cand is None:
            y_s[r0 // 2:r1 // 2, cols] = pltpu.pack_elementwise([y[0:n], y[n:2 * n]], packed_dtype=BF16)
        out_s[r0:r1, cols] = (hh + y).astype(BF16)
        yb = y.astype(BF16)
        rr = jnp.dot(wr16[:, r0:r1], yb, preferred_element_type=F32)
        st['r'] = rr if c == 0 else st['r'] + rr
        if cand is not None:
            cand.setdefault(jt, {'y': []})['y'].append(yb)
        if r1 == D:
            rrow = _rb(st['r'][0:1, :])
            if cand is None:
                r_s[s, :, jt * T:(jt + 1) * T] = jnp.broadcast_to(rrow, (8, T))
            else:
                cand[jt]['r'] = rrow

    def offer_last(best, cand):
        rrow = jnp.concatenate([cand[jt]['r'] for jt in range(4)], axis=1)
        tmax = jnp.max(rrow, axis=1, keepdims=True)
        lane = lax.broadcasted_iota(jnp.int32, (1, L), 1)
        lane_c = jnp.min(jnp.where(rrow == tmax, lane, L), axis=1, keepdims=True)
        xs = None
        for jt in range(4):
            oh = (lax.broadcasted_iota(jnp.int32, (16, T), 1) == lane_c - jt * T).astype(BF16)
            part = jnp.concatenate([lax.dot_general(oh, yc, NT, preferred_element_type=F32)
                                    for yc in cand[jt]['y']], axis=1)
            xs = part if xs is None else xs + part
        take = tmax > best['r']
        best.update(r=jnp.where(take, tmax, best['r']),
                    tok=jnp.where(take, (NSEG - 1) * L + lane_c, best['tok']),
                    xs=jnp.where(take, xs, best['xs']))

    def prep_qk(i, base):
        wt = _u32(w_v[i].T)
        for g in range(NG):
            n = 9 * GH[g]
            wqkv[base + 64 * g:base + 64 * g + n, :] = wt[63 * g:63 * g + n, :]
        deinterleave(base, 4 * 64)
        deinterleave(base + 4 * 64, QR // 2 - 4 * 64)

    def prep_v():
        wt = _u32(w_v[2].T)
        for h in range(H):
            wqkv[QR + 10 * h:QR + 10 * h + 9, :] = wt[9 * h:9 * h + 9, :]
        deinterleave(QR, 320)

    def deinterleave(base, nwords):
        lo16 = U32(0xFFFF)
        hi16 = U32(0xFFFF0000)
        for lt in range(NG if PACK else 0):
            w = min(T, D - T * lt)
            lanes = slice(T * lt, T * lt + w)
            dtmp[0:nwords, 0:w] = wqkv[base:base + nwords, lanes]
            b = 0
            while b < nwords:
                half = 8 if nwords - b >= 16 else 4
                ev = dtmp[pl.ds(b, half, stride=2), :]
                od = dtmp[pl.ds(b + 1, half, stride=2), :]
                wqkv[base + b:base + b + half, lanes] = ((ev & lo16) | (od << 16))[:, 0:w]
                wqkv[base + b + half:base + b + 2 * half, lanes] = ((ev >> 16) | (od & hi16))[:, 0:w]
                b += 2 * half

    def prep_o():
        wt = _u32(w_v[3])
        wpad = jnp.concatenate(
            [piece for h in range(H) for piece in (wt[9 * h:9 * h + 9, :], jnp.zeros((1, D), U32))], axis=0)
        wot[...] = _u32(_bf(wpad).T)

    BLKS = [(jq, kb) for jq in range(4) for kb in range(jq + 1)]

    def head_sets(heads):
        sets, i = [], 0
        while i < len(heads):
            h = heads[i]
            if h % 7 % 2 == 0 and h % 7 < 6 and i + 1 < len(heads):
                sets.append((h, h + 1))
                i += 2
            else:
                assert h % 7 == 6
                sets.append((h,))
                i += 1
        return sets

    def s_items(heads, small_tail=0):
        big, small = [], []
        for hs in head_sets(heads):
            for jq, kb in BLKS:
                halved = len(hs) == 2 and kb == jq
                for h in hs:
                    (small if halved else big).append(functools.partial(s_blk, h, jq, kb, halved))
                if halved:
                    small.append(functools.partial(s_pair, hs[0], jq))
        tail = small[len(small) - small_tail:] if small_tail else []
        small = small[:len(small) - small_tail] if small_tail else small
        order = sorted([((j + 0.5) / len(big), 0, j) for j in range(len(big))]
                       + [((j + 0.5) / len(small), 1, j) for j in range(len(small))])
        return [(big, small)[w][j] for _, w, j in order] + tail

    def phase_x():
        sb = s_items(HB)
        for it in sb[0:NS0]:
            it()
        interleave(pv_items(HA), sb[NS0:])

    def pv_items_by_tile(heads, z):
        out = {}
        for jq in range(4):
            out[jq] = []
            for hs in head_sets(heads):
                st = {'z': z}
                roles = ('a', 'b') if len(hs) == 2 else (None,)
                for kb in range(jq + 1):
                    for h, role in zip(hs, roles):
                        out[jq].append(functools.partial(pv_blk, h, jq, kb, st, role))
        return out

    def pv_items(heads, z=0):
        items = []
        for hs in head_sets(heads):
            st = {'z': z}
            roles = ('a', 'b') if len(hs) == 2 else (None,)
            for jq, kb in BLKS:
                for h, role in zip(hs, roles):
                    items.append(functools.partial(pv_blk, h, jq, kb, st, role))
        return items

    def interleave(*seqs):
        seqs = [q for q in seqs if q]
        order = []
        for i, q in enumerate(seqs):
            order += [((j + 0.5) / len(q), i, j) for j in range(len(q))]
        for _, i, j in sorted(order):
            seqs[i][j]()

    def proj_items(fn):
        return [functools.partial(fn, jt, g) for jt in range(4) for g in range(NG)]

    def out_items(s, ke, cand=None):
        sts = [{'cand': cand} for _ in range(4)]
        o_items = [functools.partial(o_unit, s, jt, c, ke, sts[jt]) for jt in range(4) for c in range(NG)]
        e_items = [functools.partial(e2_unit, s, jt, c, sts[jt]) for jt in range(4) for c in range(NG)]
        early = [functools.partial(o_early, s, jt, c, ke) for jt in range(4) for c in range(NG)]
        return early, o_items, e_items

    HA = list(range(HS))
    HB = list(range(HS, H))

    x_copy(0).start()
    w_copy(1).start()
    zero_s[0] = 0
    beta_copy.start()
    wr_copy.start()
    with _scope('p0_const'):
        kr = lax.broadcasted_iota(jnp.int32, (T, T), 0)
        qc = lax.broadcasted_iota(jnp.int32, (T, T), 1)
        bias[...] = jnp.where(kr > qc, MASKVAL, 0.0).astype(F32)
        kr2 = lax.broadcasted_iota(jnp.int32, (64, T), 0)
        qc2 = lax.broadcasted_iota(jnp.int32, (64, T), 1)
        bias2[...] = jnp.where(kr2 > (qc2 & 63), MASKVAL, 0.0).astype(F32)
        wqkv[...] = jnp.zeros(wqkv.shape, U32)
        bd[...] = jnp.zeros(bd.shape, F32)
        memt[...] = jnp.zeros(memt.shape, F32)
        row = lax.broadcasted_iota(jnp.int32, (640, T), 0)
        sub = row & 31
        nat = (row - sub) + jnp.where(sub < 16, 2 * sub, 2 * sub - 31)
        if not PACK:
            nat = row
        ones_tab[...] = jnp.where(nat % VS == DH, 1.0, 0.0).astype(F32)
        dtmp[...] = jnp.zeros(dtmp.shape, U32)
        for g in range(NG):
            row = lax.broadcasted_iota(jnp.int32, (160, T), 0) + (GWIN[g][0] - 140 * g)
            lane = lax.broadcasted_iota(jnp.int32, (160, T), 1)
            keep = ((row >= 0) & (row < 20 * GH[g]) & (lane >= (row // VS) * DH)
                    & (lane < (row // VS) * DH + DH))
            keep_tab[g] = jnp.where(keep, 1.0, 0.0).astype(F32)
        qt[NG - 1] = jnp.zeros(qt.shape[1:], U32)
        pqt[NG - 1] = jnp.zeros(pqt.shape[1:], U32)
        pkt[NG - 1] = jnp.zeros(pkt.shape[1:], U32)

    with _scope('p1_ln'):
        x_copy(0).wait()
        w_copy(0).start()
        for jt in range(4):
            ln1_stats(0, jt)
            ln1_norm(0, jt)
    with _scope('p2_wq'):
        w_copy(1).wait()
        w_copy(2).start()
        prep_qk(1, 0)
        for g in range(NG):
            for jt in range(2):
                q_unit(jt, g)
    with _scope('p3_q'):
        w_copy(0).wait()
        w_copy(3).start()
        prep_qk(0, QR // 2)
        for jt in range(2, 4):
            for g in range(NG):
                q_unit(jt, g)
    with _scope('p4_k'):
        w_copy(2).wait()
        for i in range(1, NSEG):
            x_copy(i).start()
        prep_v()
        for jt in range(4):
            for g in range(NG):
                k_unit(jt, g)
    with _scope('p5_v'):
        w_copy(3).wait()
        beta_copy.wait()
        wr_copy.wait()
        for i in range(1, NSEG):
            x_copy(i).wait()
        prep_o()
        beta = beta_v[...].astype(F32).reshape(1, H)
        hl = lax.broadcasted_iota(jnp.int32, (H, H), 1)
        hs = lax.broadcasted_iota(jnp.int32, (H, H), 0)
        bcol = jnp.sum(jnp.where(hl == hs, jnp.broadcast_to(beta, (H, H)), 0.0), axis=1, keepdims=True)
        gate = _rb(jax.nn.sigmoid(bcol))
        gtab[0] = jnp.broadcast_to(gate, (H, T))
        gtab[1] = jnp.broadcast_to(_rb(1.0 - gate), (H, T))
        r16 = lax.broadcasted_iota(jnp.int32, (16, D), 0)
        wr_row = wr_v[...].astype(F32).reshape(1, D)
        wr16[...] = jnp.where(r16 == 0, jnp.broadcast_to(wr_row, (16, D)), 0.0).astype(BF16)
        if STATV == 0:
            interleave(proj_items(v_unit) + s_items(HA, 16),
                       [functools.partial(ln1_stats, i, jt) for i in range(1, NSEG) for jt in range(4)])
        else:
            for it in proj_items(v_unit) + s_items(HA, 16):
                it()
            for jt in range(4):
                ln1_stats(1, jt, True)

    def seg_body(s, carry):
        with _scope('seg_xy'):
            z = zero_s[0]
            phase_x()
            ln = [functools.partial(ln1_norm, s + 1, jt) for jt in range(4)]
            qs = proj_items(q_unit)
            early, o_items, e_items = out_items(s, KE)
            upd = [functools.partial(mem_update_unit, g) for g in range(NG)]
            ks = proj_items(k_unit)
            if Y1V == 0:
                pre = [ln[0]] + early[0:10] + [ln[1]]
                mxu1 = upd + qs[0:5] + [ln[2]] + early[10:20] + qs[5:10] + [ln[3]] + qs[10:20] + ks
            elif Y1V == 1:
                pre = [ln[0], ln[1]] + early[0:10]
                mxu1 = [ln[2]] + upd + [ln[3]] + early[10:20] + qs + ks
            elif Y1V == 2:
                pre = [ln[0]] + early[0:8] + [ln[1]]
                mxu1 = early[8:14] + [ln[2]] + upd + qs[0:5] + early[14:20] + [ln[3]] + qs[5:20] + ks
            elif Y1V == 3:
                pre = ln + early[0:10]
                mxu1 = upd + early[10:20] + qs + ks
            else:
                pre = [ln[0]] + early[0:10] + [ln[1]]
                mxu1 = (upd + qs[0:5] + ks[0:5] + [ln[2]] + early[10:20] + qs[5:10] + ks[5:10] + [ln[3]]
                        + qs[10:15] + ks[10:15] + qs[15:20] + ks[15:20])
            for it in pre:
                it()
            interleave(pv_items(HB, z), mxu1)
            vr = proj_items(v_unit) + [functools.partial(mem_read_unit, g) for g in range(NG)]
            if Y2V == 0:
                for it in o_items:
                    it()
                interleave(vr, e_items[0:E2A])
            elif Y2V == 1:
                interleave(o_items, vr[0:10])
                interleave(vr[10:], e_items[0:E2A])
            else:
                for it in o_items[0:10]:
                    it()
                interleave(o_items[10:], vr[0:5])
                interleave(vr[5:], e_items[0:E2A])
            interleave(s_items(HA, TAIL), e_items[E2A:])
            if STATV == 1:
                for jt in range(4):
                    ln1_stats(jnp.minimum(s + 2, NSEG - 1), jt, True)
            o_copy(s).start()

            @pl.when(s == 0)
            def _():
                f_copy(0).start()
                f_copy(1).start()

            @pl.when(s == 1)
            def _():
                f_copy(2).start()
        return carry

    lax.fori_loop(0, NSEG - 1, seg_body, 0)

    with _scope('seg_xz'):
        for i in range(3):
            f_copy(i).wait()
        z = zero_s[0]
        best = {}

        def offer_previous():
            n = (NSEG - 1) * 8
            r_all = r_s[0:NSEG - 1].reshape(n, L)
            tok = ((lax.broadcasted_iota(jnp.int32, (n, L), 0) // 8) * L
                   + lax.broadcasted_iota(jnp.int32, (n, L), 1))
            rmax = jnp.max(jnp.max(r_all, axis=1, keepdims=True), axis=0, keepdims=True)
            idx = jnp.clip(jnp.min(jnp.where(r_all == rmax, tok, S)), 0, S - 1)
            base = pl.multiple_of((idx // T) * T, T)
            onehot = (lax.broadcasted_iota(jnp.int32, (16, T), 1) == idx - base).astype(BF16)
            yw = y_s[:, pl.ds(base, T)]
            pieces = []
            for c in range(NG):
                w0, w1 = 64 * c, min(64 * (c + 1), D // 2)
                n2 = w1 - w0
                xp = lax.dot_general(onehot, _bf(yw[w0:w1]), NT, preferred_element_type=F32)
                rr = lax.broadcasted_iota(jnp.int32, (2 * n2, 2 * n2), 0)
                cc = lax.broadcasted_iota(jnp.int32, (2 * n2, 2 * n2), 1)
                unmix = (rr == jnp.where(cc < n2, 2 * cc, 2 * (cc - n2) + 1)).astype(BF16)
                pieces.append(jnp.dot(xp.astype(BF16), unmix, preferred_element_type=F32))
            best.update(r=rmax, tok=jnp.full((1, 1), idx, jnp.int32), xs=jnp.concatenate(pieces, axis=1))

        ha1, ha2 = HA[:HA1], HA[HA1:]
        hb1, hb2 = list(range(HS, HM)), list(range(HM, H))
        sb1 = s_items(hb1)
        for it in sb1[0:NS0]:
            it()
        interleave(pv_items(ha1), sb1[NS0:])
        offer_previous()
        sb2 = s_items(hb2)
        interleave(pv_items(ha2) + pv_items(hb1, z), sb2)
        cand = {}
        early, o_items, e_items = out_items(NSEG - 1, KM, cand)
        for it in early[0:4]:
            it()
        interleave(pv_items(hb2, z), early[4:])
        for jt in range(4):
            for it in o_items[jt * NG:(jt + 1) * NG]:
                it()
            if jt > 0:
                for it in e_items[(jt - 1) * NG:jt * NG]:
                    it()
        for it in e_items[3 * NG:]:
            it()
        offer_last(best, cand)
        o_copy(NSEG - 1).start()

    xs_v[...] = best['xs'].astype(BF16)
    best_v[...] = jnp.broadcast_to(best['r'], (8, T))
    idx = jnp.clip(jnp.max(best['tok']), 0, S - 1)
    base = pl.multiple_of((idx // T) * T, T)
    tile = pl.ds(base, T)

    @pl.when(zero_s[0] == 0)
    def _ffn():
        with _scope('ffn'):
            xs = xs_v[...]
            acc = None
            f0 = 0
            for fw in FCH:
                fc = slice(f0, f0 + fw)
                gt = _rb(jnp.dot(xs, wg_v[:, fc], preferred_element_type=F32))
                up = _rb(jnp.dot(xs, wu_v[:, fc], preferred_element_type=F32))
                act = _rb(_rb(gt * jax.nn.sigmoid(gt)) * up)[0:1, :]
                for t in range(fw // T):
                    a = act[:, t * T:(t + 1) * T]
                    term = wd_v[:, f0 + t * T:f0 + (t + 1) * T].astype(F32) * a
                    acc = term if acc is None else acc + term
                f0 += fw
            ycol = _rb(jnp.sum(acc, axis=1, keepdims=True))
            ycol = _rb(ycol * _rb(jax.nn.sigmoid(best_v[0:1, 0:1])))
            sel = lax.broadcasted_iota(jnp.int32, (D, T), 1) == idx - base
            old = out_s[:, tile].astype(F32)
            fix_v[...] = jnp.where(sel, old + ycol, old).astype(BF16)

    for s in range(NSEG):
        o_copy(s).wait()
    fix = pltpu.make_async_copy(fix_v, out_hbm.at[0, :, tile], sem_o.at[0])
    fix.start()
    fix.wait()


@jax.jit
def pallas_sequential_preLN__memory_aug_infini_attn__moe_arch_mod__prompt_kernel(
    A_x: jax.Array,
    A_wq: jax.Array,
    A_wk: jax.Array,
    A_wv: jax.Array,
    A_wo: jax.Array,
    A_beta: jax.Array,
    B_x: jax.Array,
    B_w_r: jax.Array,
    B_w_gate: jax.Array,
    B_w_up: jax.Array,
    B_w_down: jax.Array,
):
    del B_x
    hbm = pl.BlockSpec(memory_space=pltpu.HBM)
    scratch = [
        pltpu.VMEM((D, S), BF16),
        pltpu.VMEM((4, D, D), BF16),
        pltpu.VMEM((QR + 320, D), U32),
        pltpu.VMEM((D // 2, 640), U32),
        pltpu.VMEM((D // 2, L), U32),
        pltpu.VMEM((NG, 64, L), U32),
        pltpu.VMEM((NG, 64, L), U32),
        pltpu.VMEM((NG, L // 2, T), U32),
        pltpu.VMEM((NG, 64, L), U32),
        pltpu.VMEM((320, L), U32),
        pltpu.VMEM((640, L), F32),
        pltpu.VMEM((NG, 160, T), F32),
        pltpu.VMEM((HS, 1280, T), F32),
        pltpu.VMEM((HM - HS, 1280, T), F32),
        pltpu.VMEM((H - HM, 1280, T), F32),
        pltpu.VMEM((H, 112, T), F32),
        pltpu.VMEM((320, L), U32),
        pltpu.VMEM((D, L), F32),
        pltpu.VMEM((NSEG, 4, 16, T), F32),
        pltpu.VMEM((D // 2, S), U32),
        pltpu.VMEM((D, S), BF16),
        pltpu.VMEM((NSEG, 8, L), F32),
        pltpu.VMEM((T, T), F32),
        pltpu.VMEM((64, T), F32),
        pltpu.VMEM((2, H, T), F32),
        pltpu.VMEM((640, T), F32),
        pltpu.VMEM((NG, 160, T), F32),
        pltpu.VMEM((D, FF), BF16),
        pltpu.VMEM((D, FF), BF16),
        pltpu.VMEM((D, FF), BF16),
        pltpu.VMEM((H,), BF16),
        pltpu.VMEM((D,), BF16),
        pltpu.VMEM((16, D), BF16),
        pltpu.VMEM((320, T), U32),
        pltpu.VMEM((16, D), BF16),
        pltpu.VMEM((8, T), F32),
        pltpu.VMEM((D, T), BF16),
        pltpu.SMEM((1,), jnp.int32),
        pltpu.SemaphoreType.DMA((NSEG,)),
        pltpu.SemaphoreType.DMA((4,)),
        pltpu.SemaphoreType.DMA((3,)),
        pltpu.SemaphoreType.DMA((NSEG,)),
        pltpu.SemaphoreType.DMA((2,)),
    ]
    out_t = pl.pallas_call(
        _kernel,
        out_shape=jax.ShapeDtypeStruct((1, D, S), BF16),
        in_specs=[hbm] * 10,
        out_specs=hbm,
        scratch_shapes=scratch,
        compiler_params=pltpu.CompilerParams(vmem_limit_bytes=110 * 1024 * 1024),
        name="infini_moe",
    )(jnp.transpose(A_x, (0, 2, 1)), A_wq, A_wk, A_wv, A_wo, A_beta, B_w_r,
      B_w_gate, B_w_up, jnp.transpose(B_w_down, (1, 0)))
    return jnp.transpose(out_t, (0, 2, 1))
```

```python
import functools
import math

import jax
import jax.numpy as jnp
from jax import lax
import jax.experimental.pallas as pl
import jax.experimental.pallas.tpu as pltpu

F32 = jnp.float32
BF16 = jnp.bfloat16
U32 = jnp.uint32

S = 2048
D = 576
H = 32
DH = 18
NSEG = 4
L = 512
FF = 4608
T = 128
NG = 5
GH = (7, 7, 7, 7, 4)
VS = 20
EPS = 1e-5
QSCALE = DH ** (-0.5) * math.log2(math.e)
MASKVAL = -1000000000.0 * math.log2(math.e)
SOFF = (0, 128, 384, 768)
MOFF = (0, 2, 5, 9)
GWIN = tuple(((140 * g) // 16 * 16, -(-(140 * g + 20 * GH[g]) // 16) * 16) for g in range(NG))
QR = 592
FCH = (256,) * 18
import os
import contextlib
PROF = bool(int(os.environ.get('PROF', '0')))


def _scope(name):
    return jax.named_scope(name) if PROF else contextlib.nullcontext()


HS = int(os.environ.get('HS', '16'))
PACK = int(os.environ.get('PACK', '0'))
NS0 = int(os.environ.get('NS0', '16'))
HA1 = int(os.environ.get('HA1', '9'))
Y1V = int(os.environ.get('Y1V', '2'))
Y2V = int(os.environ.get('Y2V', '0'))
E2A = int(os.environ.get('E2A', '20'))
TAIL = int(os.environ.get('TAIL', '16'))
STATV = int(os.environ.get('STATV', '0'))
HM = int(os.environ.get('HM', '25'))
KE = (VS * HS) // T * T
KM = (VS * HM) // T * T

NT = (((1,), (1,)), ((), ()))


def _bf(x_u32):
    return pltpu.bitcast(x_u32, BF16)


def _u32(x_bf):
    return pltpu.bitcast(x_bf, U32)


def _pack_rows(y):
    if not PACK:
        return _u32(y.astype(BF16))
    n = y.shape[0]
    parts = []
    full = n // 32 * 32
    if full:
        y4 = y[0:full].reshape(full // 32, 2, 16, T)
        parts.append(pltpu.pack_elementwise([y4[:, 0], y4[:, 1]], packed_dtype=BF16).reshape(full // 2, T))
    if n > full:
        parts.append(pltpu.pack_elementwise([y[full:full + 8], y[full + 8:full + 16]], packed_dtype=BF16))
    return parts[0] if len(parts) == 1 else jnp.concatenate(parts, axis=0)


def _rb(x):
    return x.astype(BF16).astype(F32)


def _phi(t):
    return jnp.where(t > 0, t + 1.0, jnp.exp(t))


def _layernorm(x, axis):
    m = jnp.mean(x, axis=axis, keepdims=True)
    c = x - m
    v = jnp.mean(c * c, axis=axis, keepdims=True)
    den = _rb(jnp.sqrt(_rb(_rb(v) + EPS)))
    return c * (1.0 / den)


def _ln_scale(pivot, s1, s2):
    md = s1 * (1.0 / D)
    v = jnp.maximum(s2 * (1.0 / D) - md * md, 0.0)
    den = _rb(jnp.sqrt(_rb(_rb(v) + EPS)))
    return pivot + md, 1.0 / den


def _kernel(x_hbm, wq_hbm, wk_hbm, wv_hbm, wo_hbm, beta_hbm, wr_hbm, wg_hbm, wu_hbm, wd_hbm,
            out_hbm,
            x_v, w_v, wqkv, wot, xn, qt, pqt, kk, pkt, vt, memt, bd, s_a, s_b1, s_b2, m_blk,
            ot, att, ln_st, y_s, out_s, r_s, bias, bias2, gtab, ones_tab, keep_tab,
            wg_v, wu_v, wd_v, beta_v, wr_v, wr16, dtmp, xs_v, best_v, fix_v,
            zero_s, sem_x, sem_w, sem_f, sem_o, sem_s):
    def x_copy(s):
        return pltpu.make_async_copy(x_hbm.at[0, :, pl.ds(s * L, L)], x_v.at[:, pl.ds(s * L, L)],
                                     sem_x.at[s])

    x_rest = pltpu.make_async_copy(x_hbm.at[0, :, pl.ds(L, S - L)], x_v.at[:, pl.ds(L, S - L)], sem_x.at[1])

    w_srcs = (wk_hbm, wq_hbm, wv_hbm, wo_hbm)

    def w_copy(i):
        return pltpu.make_async_copy(w_srcs[i], w_v.at[i], sem_w.at[i])

    f_pairs = ((wg_hbm, wg_v), (wu_hbm, wu_v), (wd_hbm, wd_v))

    def f_copy(i):
        return pltpu.make_async_copy(f_pairs[i][0], f_pairs[i][1], sem_f.at[i])

    def o_copy(s):
        return pltpu.make_async_copy(out_s.at[:, pl.ds(s * L, L)], out_hbm.at[0, :, pl.ds(s * L, L)],
                                     sem_o.at[s])

    beta_copy = pltpu.make_async_copy(beta_hbm, beta_v, sem_s.at[0])
    wr_copy = pltpu.make_async_copy(wr_hbm, wr_v, sem_s.at[1])

    def seg_cols(s, jt):
        if isinstance(s, int):
            return slice(s * L + jt * T, s * L + (jt + 1) * T)
        return pl.ds(pl.multiple_of(s * L + jt * T, T), T)

    def ln1_stats(s, jt, late=False):
        cols = seg_cols(s, jt)
        pivot = a1 = a2 = None
        for c in range(D // 32):
            x = x_v[32 * c:32 * (c + 1), cols].astype(F32)
            if c == 0:
                pivot = x[0:1, :]
                if late:
                    slot = MOFF[3] + 2
                    bits = pltpu.bitcast(m_blk[HS - 1, slot * 8:slot * 8 + 8, :], U32) & zero_s[0].astype(U32)
                    pivot = pivot + pltpu.bitcast(bits, F32)[0:1, :]
            d = (x - pivot).reshape(4, 8, T)
            p1 = (d[0] + d[1]) + (d[2] + d[3])
            dd = d * d
            p2 = (dd[0] + dd[1]) + (dd[2] + dd[3])
            a1 = p1 if c == 0 else a1 + p1
            a2 = p2 if c == 0 else a2 + p2
        m, inv = _ln_scale(pivot, jnp.sum(a1, axis=0, keepdims=True), jnp.sum(a2, axis=0, keepdims=True))
        ln_st[s, jt, 0:1, :] = m
        ln_st[s, jt, 8:9, :] = inv

    def ln1_norm(s, jt, c=None):
        for cc in (range(NG) if c is None else (c,)):
            r0, r1 = T * cc, min(T * (cc + 1), D)
            x = x_v[r0:r1, seg_cols(s, jt)].astype(F32)
            xn[r0 // 2:r1 // 2, jt * T:(jt + 1) * T] = _u32(
                ((x - ln_st[s, jt, 0:1, :]) * ln_st[s, jt, 8:9, :]).astype(BF16))

    def q_unit(jt, g):
        cols = slice(jt * T, (jt + 1) * T)
        n = min(64, QR // 2 - 64 * g)
        q = jnp.dot(_bf(wqkv[64 * g:64 * g + n, :]), _bf(xn[:, cols]), preferred_element_type=F32)
        qt[g, 0:n, cols] = _pack_rows(q * QSCALE)
        pqt[g, 0:n, cols] = _pack_rows(_phi(q))

    def k_unit(jt, g):
        cols = slice(jt * T, (jt + 1) * T)
        n = min(64, QR // 2 - 64 * g)
        b0 = QR // 2 + 64 * g
        k = jnp.dot(_bf(wqkv[b0:b0 + n, :]), _bf(xn[:, cols]), preferred_element_type=F32)
        pkt[g, 0:n, cols] = _pack_rows(_phi(k))
        kb = _pack_rows(k)
        if n < 64:
            kb = jnp.concatenate([kb, jnp.zeros((64 - n, T), U32)], axis=0)
        kk[g, jt * 64:(jt + 1) * 64, :] = _u32(_bf(kb).T)

    def v_unit(jt, c):
        cols = slice(jt * T, (jt + 1) * T)
        b0 = QR + 64 * c
        v = jnp.dot(_bf(wqkv[b0:b0 + 64, :]), _bf(xn[:, cols]), preferred_element_type=F32)
        vt[64 * c:64 * (c + 1), cols] = _pack_rows(v + ones_tab[T * c:T * (c + 1), :])

    def mem_read_unit(g):
        w0, w1 = GWIN[g]
        b = bd[g, 0:w1 - w0, :].astype(BF16)
        res = jnp.dot(b, _bf(pqt[g]), preferred_element_type=F32)
        lo, hi = 140 * g, 140 * g + 20 * GH[g]
        memt[lo:hi, :] = res[lo - w0:hi - w0]

    def mem_update_unit(g):
        w0, w1 = GWIN[g]
        upd = lax.dot_general(_bf(vt[w0 // 2:w1 // 2, :]), _bf(pkt[g]), NT, preferred_element_type=F32)
        n = w1 - w0
        bd[g, 0:n, :] = bd[g, 0:n, :] + jnp.where(keep_tab[g, 0:n, :] > 0.5, upd, 0.0)

    def sbuf(h):
        if h < HS:
            return s_a, h
        return (s_b1, h - HS) if h < HM else (s_b2, h - HM)

    def head_rows(j):
        r = lax.broadcasted_iota(jnp.int32, (64, T), 0)
        return (r >= 9 * j) & (r < 9 * j + 9)

    def s_blk(h, jq, kb, half=False):
        g, j = divmod(h, 7)
        off = SOFF[jq] + kb * T
        n = 64 if half else T
        qm = _bf(jnp.where(head_rows(j), qt[g, :, jq * T:(jq + 1) * T], U32(0)))
        sc = jnp.dot(_bf(kk[g, kb * 64:kb * 64 + n // 2, :]), qm, preferred_element_type=F32)
        if kb == jq:
            sc = sc + bias[0:n, :]
        sb, hi_ = sbuf(h)
        sb[hi_, off:off + n, :] = sc
        slot = MOFF[jq] + kb
        m_blk[h, slot * 8:(slot + 1) * 8, :] = jnp.max(sc.reshape(n // 8, 8, T), axis=0)

    def s_pair(ha, jq):
        g, j = divmod(ha, 7)
        off = SOFF[jq] + jq * T + 64
        lo = lax.broadcasted_iota(jnp.int32, (64, T), 1) < 64
        qu = qt[g, :, jq * T:(jq + 1) * T]
        qmix = jnp.where(lo, pltpu.roll(qu, 64, 1), qu)
        qm = _bf(jnp.where((lo & head_rows(j)) | (~lo & head_rows(j + 1)), qmix, U32(0)))
        sc = jnp.dot(_bf(kk[g, jq * 64 + 32:jq * 64 + 64, :]), qm, preferred_element_type=F32) + bias2[...]
        sb, hi_ = sbuf(ha)
        sb[hi_, off:off + 64, :] = sc
        pm = jnp.max(sc.reshape(8, 8, T), axis=0)
        hi = lax.broadcasted_iota(jnp.int32, (8, T), 1) >= 64
        slot = MOFF[jq] + jq + 1
        m_blk[ha, slot * 8:(slot + 1) * 8, :] = jnp.where(hi, pltpu.roll(pm, 64, 1), -jnp.inf)
        m_blk[ha + 1, slot * 8:(slot + 1) * 8, :] = jnp.where(hi, pm, -jnp.inf)

    def row_max(h, jq, nslots):
        return jnp.max(m_blk[h, MOFF[jq] * 8:(MOFF[jq] + nslots) * 8, :], axis=0, keepdims=True)

    def pv_blk(h, jq, kb, st, role):
        w0 = (VS * h) // 16 * 16
        o = VS * h - w0
        off = SOFF[jq] + kb * T
        cols = slice(jq * T, (jq + 1) * T)
        key = role or 'a'
        sb, hz = sbuf(h)
        hz = hz + st['z']
        if kb == 0 and role != 'b':
            st['ma'] = row_max(h, jq, jq + 1 if role is None else jq + 2)
            if role == 'a':
                st['mb'] = row_max(h + 1, jq, jq + 2)
        m = st['m' + key]
        if kb < jq or role is None:
            p = jnp.exp2(sb[hz, off:off + T, :] - m).astype(BF16)
        else:
            if role == 'a':
                hi1 = lax.broadcasted_iota(jnp.int32, (1, T), 1) >= 64
                hi = lax.broadcasted_iota(jnp.int32, (64, T), 1) >= 64
                m2 = jnp.where(hi1, st['mb'], pltpu.roll(st['ma'], 64, 1))
                e2 = jnp.exp2(sb[hz, off + 64:off + T, :] - m2)
                p2 = jnp.where(hi, pltpu.roll(e2, 64, 1), 0.0)
                st['p2b'] = jnp.where(hi, e2, 0.0)
            else:
                p2 = st['p2b']
            p1 = jnp.exp2(sb[hz, off:off + 64, :] - m)
            p = jnp.concatenate([p1, p2], axis=0).astype(BF16)
        part = jnp.dot(_bf(vt[w0 // 2:w0 // 2 + 16, kb * T:(kb + 1) * T]), p, preferred_element_type=F32)
        st['pv' + key] = part if kb == 0 else st['pv' + key] + part
        if kb == jq:
            pv = st['pv' + key]
            res = pv * (gtab[1, h:h + 1, :] / pv[o + DH:o + DH + 1, :])
            mem = memt[w0:w0 + 32, cols]
            res = res + mem * (gtab[0, h:h + 1, :] / (mem[o + DH:o + DH + 1, :] + 1e-6))
            ot[VS * h // 2:VS * h // 2 + VS // 2, cols] = _u32(res.astype(BF16))[o // 2:o // 2 + VS // 2]

    def o_early(s, jt, c, ke):
        r0, r1 = T * c, min(T * (c + 1), D)
        tile = slice(jt * T, (jt + 1) * T)
        a = jnp.dot(_bf(wot[r0 // 2:r1 // 2, 0:ke]), _bf(ot[0:ke // 2, tile]), preferred_element_type=F32)
        att[r0:r1, tile] = x_v[r0:r1, seg_cols(s, jt)].astype(F32) + a

    def o_unit(s, jt, c, ke, st):
        r0, r1 = T * c, min(T * (c + 1), D)
        tile = slice(jt * T, (jt + 1) * T)
        a = jnp.dot(_bf(wot[r0 // 2:r1 // 2, ke:640]), _bf(ot[ke // 2:320, tile]), preferred_element_type=F32)
        hh = att[r0:r1, tile] + a
        att[r0:r1, tile] = hh
        if c == 0:
            st['p'] = hh[0:1, :]
        d = hh - st['p']
        s1 = jnp.sum(d, axis=0, keepdims=True)
        s2 = jnp.sum(d * d, axis=0, keepdims=True)
        st['s1'] = s1 if c == 0 else st['s1'] + s1
        st['s2'] = s2 if c == 0 else st['s2'] + s2

    def e2_unit(s, jt, c, st):
        r0, r1 = T * c, min(T * (c + 1), D)
        cols = seg_cols(s, jt)
        if c == 0:
            st['m'], st['inv'] = _ln_scale(st['p'], st['s1'], st['s2'])
        hh = att[r0:r1, jt * T:(jt + 1) * T]
        y = (hh - st['m']) * st['inv']
        n = (r1 - r0) // 2
        cand = st.get('cand')
        if cand is None:
            y_s[r0 // 2:r1 // 2, cols] = pltpu.pack_elementwise([y[0:n], y[n:2 * n]], packed_dtype=BF16)
        out_s[r0:r1, cols] = (hh + y).astype(BF16)
        yb = y.astype(BF16)
        rr = jnp.dot(wr16[:, r0:r1], yb, preferred_element_type=F32)
        st['r'] = rr if c == 0 else st['r'] + rr
        if cand is not None:
            cand.setdefault(jt, {'y': []})['y'].append(yb)
        if r1 == D:
            rrow = _rb(st['r'][0:1, :])
            if cand is None:
                r_s[s, :, jt * T:(jt + 1) * T] = jnp.broadcast_to(rrow, (8, T))
            else:
                cand[jt]['r'] = rrow

    def offer_last(best, cand):
        rrow = jnp.concatenate([cand[jt]['r'] for jt in range(4)], axis=1)
        tmax = jnp.max(rrow, axis=1, keepdims=True)
        lane = lax.broadcasted_iota(jnp.int32, (1, L), 1)
        lane_c = jnp.min(jnp.where(rrow == tmax, lane, L), axis=1, keepdims=True)
        xs = None
        for jt in range(4):
            oh = (lax.broadcasted_iota(jnp.int32, (16, T), 1) == lane_c - jt * T).astype(BF16)
            part = jnp.concatenate([lax.dot_general(oh, yc, NT, preferred_element_type=F32)
                                    for yc in cand[jt]['y']], axis=1)
            xs = part if xs is None else xs + part
        take = tmax > best['r']
        best.update(r=jnp.where(take, tmax, best['r']),
                    tok=jnp.where(take, (NSEG - 1) * L + lane_c, best['tok']),
                    xs=jnp.where(take, xs, best['xs']))

    def prep_qk(i, base):
        wt = _u32(w_v[i].T)
        for g in range(NG):
            n = 9 * GH[g]
            wqkv[base + 64 * g:base + 64 * g + n, :] = wt[63 * g:63 * g + n, :]
        deinterleave(base, 4 * 64)
        deinterleave(base + 4 * 64, QR // 2 - 4 * 64)

    def prep_v():
        wt = _u32(w_v[2].T)
        for h in range(H):
            wqkv[QR + 10 * h:QR + 10 * h + 9, :] = wt[9 * h:9 * h + 9, :]
        deinterleave(QR, 320)

    def deinterleave(base, nwords):
        lo16 = U32(0xFFFF)
        hi16 = U32(0xFFFF0000)
        for lt in range(NG if PACK else 0):
            w = min(T, D - T * lt)
            lanes = slice(T * lt, T * lt + w)
            dtmp[0:nwords, 0:w] = wqkv[base:base + nwords, lanes]
            b = 0
            while b < nwords:
                half = 8 if nwords - b >= 16 else 4
                ev = dtmp[pl.ds(b, half, stride=2), :]
                od = dtmp[pl.ds(b + 1, half, stride=2), :]
                wqkv[base + b:base + b + half, lanes] = ((ev & lo16) | (od << 16))[:, 0:w]
                wqkv[base + b + half:base + b + 2 * half, lanes] = ((ev >> 16) | (od & hi16))[:, 0:w]
                b += 2 * half

    def prep_o():
        wt = _u32(w_v[3])
        wpad = jnp.concatenate(
            [piece for h in range(H) for piece in (wt[9 * h:9 * h + 9, :], jnp.zeros((1, D), U32))], axis=0)
        wot[...] = _u32(_bf(wpad).T)

    BLKS = [(jq, kb) for jq in range(4) for kb in range(jq + 1)]

    def head_sets(heads):
        sets, i = [], 0
        while i < len(heads):
            h = heads[i]
            if h % 7 % 2 == 0 and h % 7 < 6 and i + 1 < len(heads):
                sets.append((h, h + 1))
                i += 2
            else:
                assert h % 7 == 6
                sets.append((h,))
                i += 1
        return sets

    def s_items(heads, small_tail=0):
        big, small = [], []
        for hs in head_sets(heads):
            for jq, kb in BLKS:
                halved = len(hs) == 2 and kb == jq
                for h in hs:
                    (small if halved else big).append(functools.partial(s_blk, h, jq, kb, halved))
                if halved:
                    small.append(functools.partial(s_pair, hs[0], jq))
        tail = small[len(small) - small_tail:] if small_tail else []
        small = small[:len(small) - small_tail] if small_tail else small
        order = sorted([((j + 0.5) / len(big), 0, j) for j in range(len(big))]
                       + [((j + 0.5) / len(small), 1, j) for j in range(len(small))])
        return [(big, small)[w][j] for _, w, j in order] + tail

    def phase_x():
        sb = s_items(HB)
        for it in sb[0:NS0]:
            it()
        interleave(pv_items(HA), sb[NS0:])

    def pv_items_by_tile(heads, z):
        out = {}
        for jq in range(4):
            out[jq] = []
            for hs in head_sets(heads):
                st = {'z': z}
                roles = ('a', 'b') if len(hs) == 2 else (None,)
                for kb in range(jq + 1):
                    for h, role in zip(hs, roles):
                        out[jq].append(functools.partial(pv_blk, h, jq, kb, st, role))
        return out

    def pv_items(heads, z=0):
        items = []
        for hs in head_sets(heads):
            st = {'z': z}
            roles = ('a', 'b') if len(hs) == 2 else (None,)
            for jq, kb in BLKS:
                for h, role in zip(hs, roles):
                    items.append(functools.partial(pv_blk, h, jq, kb, st, role))
        return items

    def interleave(*seqs):
        seqs = [q for q in seqs if q]
        order = []
        for i, q in enumerate(seqs):
            order += [((j + 0.5) / len(q), i, j) for j in range(len(q))]
        for _, i, j in sorted(order):
            seqs[i][j]()

    def proj_items(fn):
        return [functools.partial(fn, jt, g) for jt in range(4) for g in range(NG)]

    def out_items(s, ke, cand=None):
        sts = [{'cand': cand} for _ in range(4)]
        o_items = [functools.partial(o_unit, s, jt, c, ke, sts[jt]) for jt in range(4) for c in range(NG)]
        e_items = [functools.partial(e2_unit, s, jt, c, sts[jt]) for jt in range(4) for c in range(NG)]
        early = [functools.partial(o_early, s, jt, c, ke) for jt in range(4) for c in range(NG)]
        return early, o_items, e_items

    HA = list(range(HS))
    HB = list(range(HS, H))

    x_copy(0).start()
    w_copy(1).start()
    zero_s[0] = 0
    beta_copy.start()
    wr_copy.start()
    with _scope('p0_const'):
        kr = lax.broadcasted_iota(jnp.int32, (T, T), 0)
        qc = lax.broadcasted_iota(jnp.int32, (T, T), 1)
        bias[...] = jnp.where(kr > qc, MASKVAL, 0.0).astype(F32)
        kr2 = lax.broadcasted_iota(jnp.int32, (64, T), 0)
        qc2 = lax.broadcasted_iota(jnp.int32, (64, T), 1)
        bias2[...] = jnp.where(kr2 > (qc2 & 63), MASKVAL, 0.0).astype(F32)
        wqkv[...] = jnp.zeros(wqkv.shape, U32)
        bd[...] = jnp.zeros(bd.shape, F32)
        memt[...] = jnp.zeros(memt.shape, F32)
        row = lax.broadcasted_iota(jnp.int32, (640, T), 0)
        sub = row & 31
        nat = (row - sub) + jnp.where(sub < 16, 2 * sub, 2 * sub - 31)
        if not PACK:
            nat = row
        ones_tab[...] = jnp.where(nat % VS == DH, 1.0, 0.0).astype(F32)
        dtmp[...] = jnp.zeros(dtmp.shape, U32)
        for g in range(NG):
            row = lax.broadcasted_iota(jnp.int32, (160, T), 0) + (GWIN[g][0] - 140 * g)
            lane = lax.broadcasted_iota(jnp.int32, (160, T), 1)
            keep = ((row >= 0) & (row < 20 * GH[g]) & (lane >= (row // VS) * DH)
                    & (lane < (row // VS) * DH + DH))
            keep_tab[g] = jnp.where(keep, 1.0, 0.0).astype(F32)
        qt[NG - 1] = jnp.zeros(qt.shape[1:], U32)
        pqt[NG - 1] = jnp.zeros(pqt.shape[1:], U32)
        pkt[NG - 1] = jnp.zeros(pkt.shape[1:], U32)

    with _scope('p1_ln'):
        x_copy(0).wait()
        w_copy(0).start()
        for jt in range(4):
            ln1_stats(0, jt)
            ln1_norm(0, jt)
    with _scope('p2_wq'):
        w_copy(1).wait()
        w_copy(2).start()
        prep_qk(1, 0)
        for g in range(NG):
            for jt in range(2):
                q_unit(jt, g)
    with _scope('p3_q'):
        w_copy(0).wait()
        x_rest.start()
        w_copy(3).start()
        prep_qk(0, QR // 2)
        for jt in range(2, 4):
            for g in range(NG):
                q_unit(jt, g)
    with _scope('p4_k'):
        w_copy(2).wait()
        prep_v()
        for jt in range(4):
            for g in range(NG):
                k_unit(jt, g)
    with _scope('p5_v'):
        w_copy(3).wait()
        beta_copy.wait()
        wr_copy.wait()
        x_rest.wait()
        prep_o()
        beta = beta_v[...].astype(F32).reshape(1, H)
        hl = lax.broadcasted_iota(jnp.int32, (H, H), 1)
        hs = lax.broadcasted_iota(jnp.int32, (H, H), 0)
        bcol = jnp.sum(jnp.where(hl == hs, jnp.broadcast_to(beta, (H, H)), 0.0), axis=1, keepdims=True)
        gate = _rb(jax.nn.sigmoid(bcol))
        gtab[0] = jnp.broadcast_to(gate, (H, T))
        gtab[1] = jnp.broadcast_to(_rb(1.0 - gate), (H, T))
        r16 = lax.broadcasted_iota(jnp.int32, (16, D), 0)
        wr_row = wr_v[...].astype(F32).reshape(1, D)
        wr16[...] = jnp.where(r16 == 0, jnp.broadcast_to(wr_row, (16, D)), 0.0).astype(BF16)
        if STATV == 0:
            interleave(proj_items(v_unit) + s_items(HA, 16),
                       [functools.partial(ln1_stats, i, jt) for i in range(1, NSEG) for jt in range(4)])
        else:
            for it in proj_items(v_unit) + s_items(HA, 16):
                it()
            for jt in range(4):
                ln1_stats(1, jt, True)

    def seg_body(s, carry):
        with _scope('seg_xy'):
            z = zero_s[0]
            phase_x()
            ln = [functools.partial(ln1_norm, s + 1, jt) for jt in range(4)]
            qs = proj_items(q_unit)
            early, o_items, e_items = out_items(s, KE)
            upd = [functools.partial(mem_update_unit, g) for g in range(NG)]
            ks = proj_items(k_unit)
            if Y1V == 0:
                pre = [ln[0]] + early[0:10] + [ln[1]]
                mxu1 = upd + qs[0:5] + [ln[2]] + early[10:20] + qs[5:10] + [ln[3]] + qs[10:20] + ks
            elif Y1V == 1:
                pre = [ln[0], ln[1]] + early[0:10]
                mxu1 = [ln[2]] + upd + [ln[3]] + early[10:20] + qs + ks
            elif Y1V == 2:
                pre = [ln[0]] + early[0:8] + [ln[1]]
                mxu1 = early[8:14] + [ln[2]] + upd + qs[0:5] + early[14:20] + [ln[3]] + qs[5:20] + ks
            elif Y1V == 3:
                pre = ln + early[0:10]
                mxu1 = upd + early[10:20] + qs + ks
            else:
                pre = [ln[0]] + early[0:10] + [ln[1]]
                mxu1 = (upd + qs[0:5] + ks[0:5] + [ln[2]] + early[10:20] + qs[5:10] + ks[5:10] + [ln[3]]
                        + qs[10:15] + ks[10:15] + qs[15:20] + ks[15:20])
            for it in pre:
                it()
            interleave(pv_items(HB, z), mxu1)
            vr = proj_items(v_unit) + [functools.partial(mem_read_unit, g) for g in range(NG)]
            if Y2V == 0:
                for it in o_items:
                    it()
                interleave(vr, e_items[0:E2A])
            elif Y2V == 1:
                interleave(o_items, vr[0:10])
                interleave(vr[10:], e_items[0:E2A])
            else:
                for it in o_items[0:10]:
                    it()
                interleave(o_items[10:], vr[0:5])
                interleave(vr[5:], e_items[0:E2A])
            interleave(s_items(HA, TAIL), e_items[E2A:])
            if STATV == 1:
                for jt in range(4):
                    ln1_stats(jnp.minimum(s + 2, NSEG - 1), jt, True)
            o_copy(s).start()

            @pl.when(s == 0)
            def _():
                f_copy(0).start()
                f_copy(1).start()

            @pl.when(s == 1)
            def _():
                f_copy(2).start()
        return carry

    lax.fori_loop(0, NSEG - 1, seg_body, 0)

    with _scope('seg_xz'):
        for i in range(3):
            f_copy(i).wait()
        z = zero_s[0]
        best = {}

        def offer_previous():
            n = (NSEG - 1) * 8
            r_all = r_s[0:NSEG - 1].reshape(n, L)
            tok = ((lax.broadcasted_iota(jnp.int32, (n, L), 0) // 8) * L
                   + lax.broadcasted_iota(jnp.int32, (n, L), 1))
            rmax = jnp.max(jnp.max(r_all, axis=1, keepdims=True), axis=0, keepdims=True)
            idx = jnp.clip(jnp.min(jnp.where(r_all == rmax, tok, S)), 0, S - 1)
            base = pl.multiple_of((idx // T) * T, T)
            onehot = (lax.broadcasted_iota(jnp.int32, (16, T), 1) == idx - base).astype(BF16)
            yw = y_s[:, pl.ds(base, T)]
            pieces = []
            for c in range(NG):
                w0, w1 = 64 * c, min(64 * (c + 1), D // 2)
                n2 = w1 - w0
                xp = lax.dot_general(onehot, _bf(yw[w0:w1]), NT, preferred_element_type=F32)
                rr = lax.broadcasted_iota(jnp.int32, (2 * n2, 2 * n2), 0)
                cc = lax.broadcasted_iota(jnp.int32, (2 * n2, 2 * n2), 1)
                unmix = (rr == jnp.where(cc < n2, 2 * cc, 2 * (cc - n2) + 1)).astype(BF16)
                pieces.append(jnp.dot(xp.astype(BF16), unmix, preferred_element_type=F32))
            best.update(r=rmax, tok=jnp.full((1, 1), idx, jnp.int32), xs=jnp.concatenate(pieces, axis=1))

        ha1, ha2 = HA[:HA1], HA[HA1:]
        hb1, hb2 = list(range(HS, HM)), list(range(HM, H))
        sb1 = s_items(hb1)
        for it in sb1[0:NS0]:
            it()
        interleave(pv_items(ha1), sb1[NS0:])
        offer_previous()
        sb2 = s_items(hb2)
        interleave(pv_items(ha2) + pv_items(hb1, z), sb2)
        cand = {}
        early, o_items, e_items = out_items(NSEG - 1, KM, cand)
        for it in early[0:4]:
            it()
        interleave(pv_items(hb2, z), early[4:])
        for jt in range(4):
            for it in o_items[jt * NG:(jt + 1) * NG]:
                it()
            if jt > 0:
                for it in e_items[(jt - 1) * NG:jt * NG]:
                    it()
        for it in e_items[3 * NG:]:
            it()
        offer_last(best, cand)
        o_copy(NSEG - 1).start()

    xs_v[...] = best['xs'].astype(BF16)
    best_v[...] = jnp.broadcast_to(best['r'], (8, T))
    idx = jnp.clip(jnp.max(best['tok']), 0, S - 1)
    base = pl.multiple_of((idx // T) * T, T)
    tile = pl.ds(base, T)

    @pl.when(zero_s[0] == 0)
    def _ffn():
        with _scope('ffn'):
            xs = xs_v[...]
            acc = None
            f0 = 0
            for fw in FCH:
                fc = slice(f0, f0 + fw)
                gt = _rb(jnp.dot(xs, wg_v[:, fc], preferred_element_type=F32))
                up = _rb(jnp.dot(xs, wu_v[:, fc], preferred_element_type=F32))
                act = _rb(_rb(gt * jax.nn.sigmoid(gt)) * up)[0:1, :]
                for t in range(fw // T):
                    a = act[:, t * T:(t + 1) * T]
                    term = wd_v[:, f0 + t * T:f0 + (t + 1) * T].astype(F32) * a
                    acc = term if acc is None else acc + term
                f0 += fw
            ycol = _rb(jnp.sum(acc, axis=1, keepdims=True))
            ycol = _rb(ycol * _rb(jax.nn.sigmoid(best_v[0:1, 0:1])))
            sel = lax.broadcasted_iota(jnp.int32, (D, T), 1) == idx - base
            old = out_s[:, tile].astype(F32)
            fix_v[...] = jnp.where(sel, old + ycol, old).astype(BF16)

    for s in range(NSEG):
        o_copy(s).wait()
    fix = pltpu.make_async_copy(fix_v, out_hbm.at[0, :, tile], sem_o.at[0])
    fix.start()
    fix.wait()


@jax.jit
def pallas_sequential_preLN__memory_aug_infini_attn__moe_arch_mod__prompt_kernel(
    A_x: jax.Array,
    A_wq: jax.Array,
    A_wk: jax.Array,
    A_wv: jax.Array,
    A_wo: jax.Array,
    A_beta: jax.Array,
    B_x: jax.Array,
    B_w_r: jax.Array,
    B_w_gate: jax.Array,
    B_w_up: jax.Array,
    B_w_down: jax.Array,
):
    del B_x
    hbm = pl.BlockSpec(memory_space=pltpu.HBM)
    scratch = [
        pltpu.VMEM((D, S), BF16),
        pltpu.VMEM((4, D, D), BF16),
        pltpu.VMEM((QR + 320, D), U32),
        pltpu.VMEM((D // 2, 640), U32),
        pltpu.VMEM((D // 2, L), U32),
        pltpu.VMEM((NG, 64, L), U32),
        pltpu.VMEM((NG, 64, L), U32),
        pltpu.VMEM((NG, L // 2, T), U32),
        pltpu.VMEM((NG, 64, L), U32),
        pltpu.VMEM((320, L), U32),
        pltpu.VMEM((640, L), F32),
        pltpu.VMEM((NG, 160, T), F32),
        pltpu.VMEM((HS, 1280, T), F32),
        pltpu.VMEM((HM - HS, 1280, T), F32),
        pltpu.VMEM((H - HM, 1280, T), F32),
        pltpu.VMEM((H, 112, T), F32),
        pltpu.VMEM((320, L), U32),
        pltpu.VMEM((D, L), F32),
        pltpu.VMEM((NSEG, 4, 16, T), F32),
        pltpu.VMEM((D // 2, S), U32),
        pltpu.VMEM((D, S), BF16),
        pltpu.VMEM((NSEG, 8, L), F32),
        pltpu.VMEM((T, T), F32),
        pltpu.VMEM((64, T), F32),
        pltpu.VMEM((2, H, T), F32),
        pltpu.VMEM((640, T), F32),
        pltpu.VMEM((NG, 160, T), F32),
        pltpu.VMEM((D, FF), BF16),
        pltpu.VMEM((D, FF), BF16),
        pltpu.VMEM((D, FF), BF16),
        pltpu.VMEM((H,), BF16),
        pltpu.VMEM((D,), BF16),
        pltpu.VMEM((16, D), BF16),
        pltpu.VMEM((320, T), U32),
        pltpu.VMEM((16, D), BF16),
        pltpu.VMEM((8, T), F32),
        pltpu.VMEM((D, T), BF16),
        pltpu.SMEM((1,), jnp.int32),
        pltpu.SemaphoreType.DMA((2,)),
        pltpu.SemaphoreType.DMA((4,)),
        pltpu.SemaphoreType.DMA((3,)),
        pltpu.SemaphoreType.DMA((NSEG,)),
        pltpu.SemaphoreType.DMA((2,)),
    ]
    out_t = pl.pallas_call(
        _kernel,
        out_shape=jax.ShapeDtypeStruct((1, D, S), BF16),
        in_specs=[hbm] * 10,
        out_specs=hbm,
        scratch_shapes=scratch,
        compiler_params=pltpu.CompilerParams(vmem_limit_bytes=110 * 1024 * 1024),
        name="infini_moe",
    )(jnp.transpose(A_x, (0, 2, 1)), A_wq, A_wk, A_wv, A_wo, A_beta, B_w_r,
      B_w_gate, B_w_up, jnp.transpose(B_w_down, (1, 0)))
    return jnp.transpose(out_t, (0, 2, 1))
```

```python
import functools
import math

import jax
import jax.numpy as jnp
from jax import lax
import jax.experimental.pallas as pl
import jax.experimental.pallas.tpu as pltpu

F32 = jnp.float32
BF16 = jnp.bfloat16
U32 = jnp.uint32

S = 2048
D = 576
H = 32
DH = 18
NSEG = 4
L = 512
FF = 4608
T = 128
NG = 5
GH = (7, 7, 7, 7, 4)
VS = 20
EPS = 1e-5
QSCALE = DH ** (-0.5) * math.log2(math.e)
MASKVAL = -1000000000.0 * math.log2(math.e)
SOFF = (0, 128, 384, 768)
MOFF = (0, 2, 5, 9)
GWIN = tuple(((140 * g) // 16 * 16, -(-(140 * g + 20 * GH[g]) // 16) * 16) for g in range(NG))
QR = 592
FCH = (256,) * 18

HS = 16
HM = 25
HA1 = 9
NS0 = 16
TAIL = 16
KE = (VS * HS) // T * T
KM = (VS * HM) // T * T

NT = (((1,), (1,)), ((), ()))


def _bf(x_u32):
    return pltpu.bitcast(x_u32, BF16)


def _u32(x_bf):
    return pltpu.bitcast(x_bf, U32)


def _pack(y):
    return _u32(y.astype(BF16))


def _rb(x):
    return x.astype(BF16).astype(F32)


def _phi(t):
    return jnp.where(t > 0, t + 1.0, jnp.exp(t))


def _ln_scale(pivot, s1, s2):
    md = s1 * (1.0 / D)
    v = jnp.maximum(s2 * (1.0 / D) - md * md, 0.0)
    den = _rb(jnp.sqrt(_rb(_rb(v) + EPS)))
    return pivot + md, 1.0 / den


def _kernel(x_hbm, wq_hbm, wk_hbm, wv_hbm, wo_hbm, beta_hbm, wr_hbm, wg_hbm, wu_hbm, wd_hbm,
            out_hbm,
            x_v, w_v, wqkv, wot, xn, qt, pqt, kk, pkt, vt, memt, bd, s_a, s_b1, s_b2, m_blk,
            ot, att, ln_st, y_s, out_s, r_s, bias, bias2, gtab, ones_tab, keep_tab,
            wg_v, wu_v, wd_v, beta_v, wr_v, wr16, xs_v, best_v, fix_v,
            zero_s, sem_x, sem_w, sem_f, sem_o, sem_s):
    def x_copy(s):
        return pltpu.make_async_copy(x_hbm.at[0, :, pl.ds(s * L, L)], x_v.at[:, pl.ds(s * L, L)],
                                     sem_x.at[s])

    x_rest = pltpu.make_async_copy(x_hbm.at[0, :, pl.ds(L, S - L)], x_v.at[:, pl.ds(L, S - L)], sem_x.at[1])

    w_srcs = (wk_hbm, wq_hbm, wv_hbm, wo_hbm)

    def w_copy(i):
        return pltpu.make_async_copy(w_srcs[i], w_v.at[i], sem_w.at[i])

    f_pairs = ((wg_hbm, wg_v), (wu_hbm, wu_v), (wd_hbm, wd_v))

    def f_copy(i):
        return pltpu.make_async_copy(f_pairs[i][0], f_pairs[i][1], sem_f.at[i])

    def o_copy(s):
        return pltpu.make_async_copy(out_s.at[:, pl.ds(s * L, L)], out_hbm.at[0, :, pl.ds(s * L, L)],
                                     sem_o.at[s])

    beta_copy = pltpu.make_async_copy(beta_hbm, beta_v, sem_s.at[0])
    wr_copy = pltpu.make_async_copy(wr_hbm, wr_v, sem_s.at[1])

    def seg_cols(s, jt):
        if isinstance(s, int):
            return slice(s * L + jt * T, s * L + (jt + 1) * T)
        return pl.ds(pl.multiple_of(s * L + jt * T, T), T)

    def ln1_stats(s, jt):
        cols = seg_cols(s, jt)
        pivot = a1 = a2 = None
        for c in range(D // 32):
            x = x_v[32 * c:32 * (c + 1), cols].astype(F32)
            if c == 0:
                pivot = x[0:1, :]
            d = (x - pivot).reshape(4, 8, T)
            p1 = (d[0] + d[1]) + (d[2] + d[3])
            dd = d * d
            p2 = (dd[0] + dd[1]) + (dd[2] + dd[3])
            a1 = p1 if c == 0 else a1 + p1
            a2 = p2 if c == 0 else a2 + p2
        m, inv = _ln_scale(pivot, jnp.sum(a1, axis=0, keepdims=True), jnp.sum(a2, axis=0, keepdims=True))
        ln_st[s, jt, 0:1, :] = m
        ln_st[s, jt, 8:9, :] = inv

    def ln1_norm(s, jt):
        for c in range(NG):
            r0, r1 = T * c, min(T * (c + 1), D)
            x = x_v[r0:r1, seg_cols(s, jt)].astype(F32)
            xn[r0 // 2:r1 // 2, jt * T:(jt + 1) * T] = _u32(
                ((x - ln_st[s, jt, 0:1, :]) * ln_st[s, jt, 8:9, :]).astype(BF16))

    def q_unit(jt, g):
        cols = slice(jt * T, (jt + 1) * T)
        n = min(64, QR // 2 - 64 * g)
        q = jnp.dot(_bf(wqkv[64 * g:64 * g + n, :]), _bf(xn[:, cols]), preferred_element_type=F32)
        qt[g, 0:n, cols] = _pack(q * QSCALE)
        pqt[g, 0:n, cols] = _pack(_phi(q))

    def k_unit(jt, g):
        cols = slice(jt * T, (jt + 1) * T)
        n = min(64, QR // 2 - 64 * g)
        b0 = QR // 2 + 64 * g
        k = jnp.dot(_bf(wqkv[b0:b0 + n, :]), _bf(xn[:, cols]), preferred_element_type=F32)
        pkt[g, 0:n, cols] = _pack(_phi(k))
        kb = _pack(k)
        if n < 64:
            kb = jnp.concatenate([kb, jnp.zeros((64 - n, T), U32)], axis=0)
        kk[g, jt * 64:(jt + 1) * 64, :] = _u32(_bf(kb).T)

    def v_unit(jt, c):
        cols = slice(jt * T, (jt + 1) * T)
        b0 = QR + 64 * c
        v = jnp.dot(_bf(wqkv[b0:b0 + 64, :]), _bf(xn[:, cols]), preferred_element_type=F32)
        vt[64 * c:64 * (c + 1), cols] = _pack(v + ones_tab[T * c:T * (c + 1), :])

    def mem_read_unit(g):
        w0, w1 = GWIN[g]
        b = bd[g, 0:w1 - w0, :].astype(BF16)
        res = jnp.dot(b, _bf(pqt[g]), preferred_element_type=F32)
        lo, hi = 140 * g, 140 * g + 20 * GH[g]
        memt[lo:hi, :] = res[lo - w0:hi - w0]

    def mem_update_unit(g):
        w0, w1 = GWIN[g]
        upd = lax.dot_general(_bf(vt[w0 // 2:w1 // 2, :]), _bf(pkt[g]), NT, preferred_element_type=F32)
        n = w1 - w0
        bd[g, 0:n, :] = bd[g, 0:n, :] + jnp.where(keep_tab[g, 0:n, :] > 0.5, upd, 0.0)

    def sbuf(h):
        if h < HS:
            return s_a, h
        return (s_b1, h - HS) if h < HM else (s_b2, h - HM)

    def head_rows(j):
        r = lax.broadcasted_iota(jnp.int32, (64, T), 0)
        return (r >= 9 * j) & (r < 9 * j + 9)

    def s_blk(h, jq, kb, half=False):
        g, j = divmod(h, 7)
        off = SOFF[jq] + kb * T
        n = 64 if half else T
        qm = _bf(jnp.where(head_rows(j), qt[g, :, jq * T:(jq + 1) * T], U32(0)))
        sc = jnp.dot(_bf(kk[g, kb * 64:kb * 64 + n // 2, :]), qm, preferred_element_type=F32)
        if kb == jq:
            sc = sc + bias[0:n, :]
        sb, hi_ = sbuf(h)
        sb[hi_, off:off + n, :] = sc
        slot = MOFF[jq] + kb
        m_blk[h, slot * 8:(slot + 1) * 8, :] = jnp.max(sc.reshape(n // 8, 8, T), axis=0)

    def s_pair(ha, jq):
        g, j = divmod(ha, 7)
        off = SOFF[jq] + jq * T + 64
        lo = lax.broadcasted_iota(jnp.int32, (64, T), 1) < 64
        qu = qt[g, :, jq * T:(jq + 1) * T]
        qmix = jnp.where(lo, pltpu.roll(qu, 64, 1), qu)
        qm = _bf(jnp.where((lo & head_rows(j)) | (~lo & head_rows(j + 1)), qmix, U32(0)))
        sc = jnp.dot(_bf(kk[g, jq * 64 + 32:jq * 64 + 64, :]), qm, preferred_element_type=F32) + bias2[...]
        sb, hi_ = sbuf(ha)
        sb[hi_, off:off + 64, :] = sc
        pm = jnp.max(sc.reshape(8, 8, T), axis=0)
        hi = lax.broadcasted_iota(jnp.int32, (8, T), 1) >= 64
        slot = MOFF[jq] + jq + 1
        m_blk[ha, slot * 8:(slot + 1) * 8, :] = jnp.where(hi, pltpu.roll(pm, 64, 1), -jnp.inf)
        m_blk[ha + 1, slot * 8:(slot + 1) * 8, :] = jnp.where(hi, pm, -jnp.inf)

    def row_max(h, jq, nslots):
        return jnp.max(m_blk[h, MOFF[jq] * 8:(MOFF[jq] + nslots) * 8, :], axis=0, keepdims=True)

    def pv_blk(h, jq, kb, st, role):
        w0 = (VS * h) // 16 * 16
        o = VS * h - w0
        off = SOFF[jq] + kb * T
        cols = slice(jq * T, (jq + 1) * T)
        key = role or 'a'
        sb, hz = sbuf(h)
        hz = hz + st['z']
        if kb == 0 and role != 'b':
            st['ma'] = row_max(h, jq, jq + 1 if role is None else jq + 2)
            if role == 'a':
                st['mb'] = row_max(h + 1, jq, jq + 2)
        m = st['m' + key]
        if kb < jq or role is None:
            p = jnp.exp2(sb[hz, off:off + T, :] - m).astype(BF16)
        else:
            if role == 'a':
                hi1 = lax.broadcasted_iota(jnp.int32, (1, T), 1) >= 64
                hi = lax.broadcasted_iota(jnp.int32, (64, T), 1) >= 64
                m2 = jnp.where(hi1, st['mb'], pltpu.roll(st['ma'], 64, 1))
                e2 = jnp.exp2(sb[hz, off + 64:off + T, :] - m2)
                p2 = jnp.where(hi, pltpu.roll(e2, 64, 1), 0.0)
                st['p2b'] = jnp.where(hi, e2, 0.0)
            else:
                p2 = st['p2b']
            p1 = jnp.exp2(sb[hz, off:off + 64, :] - m)
            p = jnp.concatenate([p1, p2], axis=0).astype(BF16)
        part = jnp.dot(_bf(vt[w0 // 2:w0 // 2 + 16, kb * T:(kb + 1) * T]), p, preferred_element_type=F32)
        st['pv' + key] = part if kb == 0 else st['pv' + key] + part
        if kb == jq:
            pv = st['pv' + key]
            res = pv * (gtab[1, h:h + 1, :] / pv[o + DH:o + DH + 1, :])
            mem = memt[w0:w0 + 32, cols]
            res = res + mem * (gtab[0, h:h + 1, :] / (mem[o + DH:o + DH + 1, :] + 1e-6))
            ot[VS * h // 2:VS * h // 2 + VS // 2, cols] = _u32(res.astype(BF16))[o // 2:o // 2 + VS // 2]

    def o_early(s, jt, c, ke):
        r0, r1 = T * c, min(T * (c + 1), D)
        tile = slice(jt * T, (jt + 1) * T)
        a = jnp.dot(_bf(wot[r0 // 2:r1 // 2, 0:ke]), _bf(ot[0:ke // 2, tile]), preferred_element_type=F32)
        att[r0:r1, tile] = x_v[r0:r1, seg_cols(s, jt)].astype(F32) + a

    def o_unit(s, jt, c, ke, st):
        r0, r1 = T * c, min(T * (c + 1), D)
        tile = slice(jt * T, (jt + 1) * T)
        a = jnp.dot(_bf(wot[r0 // 2:r1 // 2, ke:640]), _bf(ot[ke // 2:320, tile]), preferred_element_type=F32)
        hh = att[r0:r1, tile] + a
        att[r0:r1, tile] = hh
        if c == 0:
            st['p'] = hh[0:1, :]
        d = hh - st['p']
        s1 = jnp.sum(d, axis=0, keepdims=True)
        s2 = jnp.sum(d * d, axis=0, keepdims=True)
        st['s1'] = s1 if c == 0 else st['s1'] + s1
        st['s2'] = s2 if c == 0 else st['s2'] + s2

    def e2_unit(s, jt, c, st):
        r0, r1 = T * c, min(T * (c + 1), D)
        cols = seg_cols(s, jt)
        if c == 0:
            st['m'], st['inv'] = _ln_scale(st['p'], st['s1'], st['s2'])
        hh = att[r0:r1, jt * T:(jt + 1) * T]
        y = (hh - st['m']) * st['inv']
        n = (r1 - r0) // 2
        cand = st.get('cand')
        if cand is None:
            y_s[r0 // 2:r1 // 2, cols] = pltpu.pack_elementwise([y[0:n], y[n:2 * n]], packed_dtype=BF16)
        out_s[r0:r1, cols] = (hh + y).astype(BF16)
        yb = y.astype(BF16)
        rr = jnp.dot(wr16[:, r0:r1], yb, preferred_element_type=F32)
        st['r'] = rr if c == 0 else st['r'] + rr
        if cand is not None:
            cand.setdefault(jt, {'y': []})['y'].append(yb)
        if r1 == D:
            rrow = _rb(st['r'][0:1, :])
            if cand is None:
                r_s[s, :, jt * T:(jt + 1) * T] = jnp.broadcast_to(rrow, (8, T))
            else:
                cand[jt]['r'] = rrow

    def offer_last(best, cand):
        rrow = jnp.concatenate([cand[jt]['r'] for jt in range(4)], axis=1)
        tmax = jnp.max(rrow, axis=1, keepdims=True)
        lane = lax.broadcasted_iota(jnp.int32, (1, L), 1)
        lane_c = jnp.min(jnp.where(rrow == tmax, lane, L), axis=1, keepdims=True)
        xs = None
        for jt in range(4):
            oh = (lax.broadcasted_iota(jnp.int32, (16, T), 1) == lane_c - jt * T).astype(BF16)
            part = jnp.concatenate([lax.dot_general(oh, yc, NT, preferred_element_type=F32)
                                    for yc in cand[jt]['y']], axis=1)
            xs = part if xs is None else xs + part
        take = tmax > best['r']
        best.update(r=jnp.where(take, tmax, best['r']),
                    tok=jnp.where(take, (NSEG - 1) * L + lane_c, best['tok']),
                    xs=jnp.where(take, xs, best['xs']))

    def prep_qk(i, base):
        wt = _u32(w_v[i].T)
        for g in range(NG):
            n = 9 * GH[g]
            wqkv[base + 64 * g:base + 64 * g + n, :] = wt[63 * g:63 * g + n, :]

    def prep_v():
        wt = _u32(w_v[2].T)
        for h in range(H):
            wqkv[QR + 10 * h:QR + 10 * h + 9, :] = wt[9 * h:9 * h + 9, :]

    def prep_o():
        wt = _u32(w_v[3])
        wpad = jnp.concatenate(
            [piece for h in range(H) for piece in (wt[9 * h:9 * h + 9, :], jnp.zeros((1, D), U32))], axis=0)
        wot[...] = _u32(_bf(wpad).T)

    BLKS = [(jq, kb) for jq in range(4) for kb in range(jq + 1)]

    def head_sets(heads):
        sets, i = [], 0
        while i < len(heads):
            h = heads[i]
            if h % 7 % 2 == 0 and h % 7 < 6 and i + 1 < len(heads):
                sets.append((h, h + 1))
                i += 2
            else:
                assert h % 7 == 6
                sets.append((h,))
                i += 1
        return sets

    def s_items(heads, small_tail=0):
        big, small = [], []
        for hs in head_sets(heads):
            for jq, kb in BLKS:
                halved = len(hs) == 2 and kb == jq
                for h in hs:
                    (small if halved else big).append(functools.partial(s_blk, h, jq, kb, halved))
                if halved:
                    small.append(functools.partial(s_pair, hs[0], jq))
        tail = small[len(small) - small_tail:] if small_tail else []
        small = small[:len(small) - small_tail] if small_tail else small
        order = sorted([((j + 0.5) / len(big), 0, j) for j in range(len(big))]
                       + [((j + 0.5) / len(small), 1, j) for j in range(len(small))])
        return [(big, small)[w][j] for _, w, j in order] + tail

    def phase_x():
        sb = s_items(HB)
        for it in sb[0:NS0]:
            it()
        interleave(pv_items(HA), sb[NS0:])

    def pv_items(heads, z=0):
        items = []
        for hs in head_sets(heads):
            st = {'z': z}
            roles = ('a', 'b') if len(hs) == 2 else (None,)
            for jq, kb in BLKS:
                for h, role in zip(hs, roles):
                    items.append(functools.partial(pv_blk, h, jq, kb, st, role))
        return items

    def interleave(*seqs):
        seqs = [q for q in seqs if q]
        order = []
        for i, q in enumerate(seqs):
            order += [((j + 0.5) / len(q), i, j) for j in range(len(q))]
        for _, i, j in sorted(order):
            seqs[i][j]()

    def proj_items(fn):
        return [functools.partial(fn, jt, g) for jt in range(4) for g in range(NG)]

    def out_items(s, ke, cand=None):
        sts = [{'cand': cand} for _ in range(4)]
        o_items = [functools.partial(o_unit, s, jt, c, ke, sts[jt]) for jt in range(4) for c in range(NG)]
        e_items = [functools.partial(e2_unit, s, jt, c, sts[jt]) for jt in range(4) for c in range(NG)]
        early = [functools.partial(o_early, s, jt, c, ke) for jt in range(4) for c in range(NG)]
        return early, o_items, e_items

    HA = list(range(HS))
    HB = list(range(HS, H))

    x_copy(0).start()
    w_copy(1).start()
    zero_s[0] = 0
    beta_copy.start()
    wr_copy.start()
    kr = lax.broadcasted_iota(jnp.int32, (T, T), 0)
    qc = lax.broadcasted_iota(jnp.int32, (T, T), 1)
    bias[...] = jnp.where(kr > qc, MASKVAL, 0.0).astype(F32)
    kr2 = lax.broadcasted_iota(jnp.int32, (64, T), 0)
    qc2 = lax.broadcasted_iota(jnp.int32, (64, T), 1)
    bias2[...] = jnp.where(kr2 > (qc2 & 63), MASKVAL, 0.0).astype(F32)
    wqkv[...] = jnp.zeros(wqkv.shape, U32)
    bd[...] = jnp.zeros(bd.shape, F32)
    memt[...] = jnp.zeros(memt.shape, F32)
    row = lax.broadcasted_iota(jnp.int32, (640, T), 0)
    ones_tab[...] = jnp.where(row % VS == DH, 1.0, 0.0).astype(F32)
    for g in range(NG):
        row = lax.broadcasted_iota(jnp.int32, (160, T), 0) + (GWIN[g][0] - 140 * g)
        lane = lax.broadcasted_iota(jnp.int32, (160, T), 1)
        keep = ((row >= 0) & (row < 20 * GH[g]) & (lane >= (row // VS) * DH)
                & (lane < (row // VS) * DH + DH))
        keep_tab[g] = jnp.where(keep, 1.0, 0.0).astype(F32)
    qt[NG - 1] = jnp.zeros(qt.shape[1:], U32)
    pqt[NG - 1] = jnp.zeros(pqt.shape[1:], U32)
    pkt[NG - 1] = jnp.zeros(pkt.shape[1:], U32)

    x_copy(0).wait()
    w_copy(0).start()
    for jt in range(4):
        ln1_stats(0, jt)
        ln1_norm(0, jt)
    w_copy(1).wait()
    w_copy(2).start()
    prep_qk(1, 0)
    for g in range(NG):
        for jt in range(2):
            q_unit(jt, g)
    w_copy(0).wait()
    x_rest.start()
    w_copy(3).start()
    prep_qk(0, QR // 2)
    for jt in range(2, 4):
        for g in range(NG):
            q_unit(jt, g)
    w_copy(2).wait()
    prep_v()
    for jt in range(4):
        for g in range(NG):
            k_unit(jt, g)
    w_copy(3).wait()
    beta_copy.wait()
    wr_copy.wait()
    x_rest.wait()
    prep_o()
    beta = beta_v[...].astype(F32).reshape(1, H)
    hl = lax.broadcasted_iota(jnp.int32, (H, H), 1)
    hs = lax.broadcasted_iota(jnp.int32, (H, H), 0)
    bcol = jnp.sum(jnp.where(hl == hs, jnp.broadcast_to(beta, (H, H)), 0.0), axis=1, keepdims=True)
    gate = _rb(jax.nn.sigmoid(bcol))
    gtab[0] = jnp.broadcast_to(gate, (H, T))
    gtab[1] = jnp.broadcast_to(_rb(1.0 - gate), (H, T))
    r16 = lax.broadcasted_iota(jnp.int32, (16, D), 0)
    wr_row = wr_v[...].astype(F32).reshape(1, D)
    wr16[...] = jnp.where(r16 == 0, jnp.broadcast_to(wr_row, (16, D)), 0.0).astype(BF16)
    interleave(proj_items(v_unit) + s_items(HA, TAIL),
               [functools.partial(ln1_stats, i, jt) for i in range(1, NSEG) for jt in range(4)])

    def seg_body(s, carry):
        z = zero_s[0]
        phase_x()
        ln = [functools.partial(ln1_norm, s + 1, jt) for jt in range(4)]
        qs = proj_items(q_unit)
        early, o_items, e_items = out_items(s, KE)
        upd = [functools.partial(mem_update_unit, g) for g in range(NG)]
        ks = proj_items(k_unit)
        pre = [ln[0]] + early[0:8] + [ln[1]]
        mxu1 = early[8:14] + [ln[2]] + upd + qs[0:5] + early[14:20] + [ln[3]] + qs[5:20] + ks
        for it in pre:
            it()
        interleave(pv_items(HB, z), mxu1)
        vr = proj_items(v_unit) + [functools.partial(mem_read_unit, g) for g in range(NG)]
        for it in o_items:
            it()
        interleave(vr, e_items)
        for it in s_items(HA, TAIL):
            it()
        o_copy(s).start()

        @pl.when(s == 0)
        def _():
            f_copy(0).start()
            f_copy(1).start()

        @pl.when(s == 1)
        def _():
            f_copy(2).start()
        return carry

    lax.fori_loop(0, NSEG - 1, seg_body, 0)

    for i in range(3):
        f_copy(i).wait()
    z = zero_s[0]
    best = {}

    def offer_previous():
        n = (NSEG - 1) * 8
        r_all = r_s[0:NSEG - 1].reshape(n, L)
        tok = ((lax.broadcasted_iota(jnp.int32, (n, L), 0) // 8) * L
               + lax.broadcasted_iota(jnp.int32, (n, L), 1))
        rmax = jnp.max(jnp.max(r_all, axis=1, keepdims=True), axis=0, keepdims=True)
        idx = jnp.clip(jnp.min(jnp.where(r_all == rmax, tok, S)), 0, S - 1)
        base = pl.multiple_of((idx // T) * T, T)
        onehot = (lax.broadcasted_iota(jnp.int32, (16, T), 1) == idx - base).astype(BF16)
        yw = y_s[:, pl.ds(base, T)]
        pieces = []
        for c in range(NG):
            w0, w1 = 64 * c, min(64 * (c + 1), D // 2)
            n2 = w1 - w0
            xp = lax.dot_general(onehot, _bf(yw[w0:w1]), NT, preferred_element_type=F32)
            rr = lax.broadcasted_iota(jnp.int32, (2 * n2, 2 * n2), 0)
            cc = lax.broadcasted_iota(jnp.int32, (2 * n2, 2 * n2), 1)
            unmix = (rr == jnp.where(cc < n2, 2 * cc, 2 * (cc - n2) + 1)).astype(BF16)
            pieces.append(jnp.dot(xp.astype(BF16), unmix, preferred_element_type=F32))
        best.update(r=rmax, tok=jnp.full((1, 1), idx, jnp.int32), xs=jnp.concatenate(pieces, axis=1))

    ha1, ha2 = HA[:HA1], HA[HA1:]
    hb1, hb2 = list(range(HS, HM)), list(range(HM, H))
    sb1 = s_items(hb1)
    for it in sb1[0:NS0]:
        it()
    interleave(pv_items(ha1), sb1[NS0:])
    offer_previous()
    sb2 = s_items(hb2)
    interleave(pv_items(ha2) + pv_items(hb1, z), sb2)
    cand = {}
    early, o_items, e_items = out_items(NSEG - 1, KM, cand)
    for it in early[0:4]:
        it()
    interleave(pv_items(hb2, z), early[4:])
    for jt in range(4):
        for it in o_items[jt * NG:(jt + 1) * NG]:
            it()
        if jt > 0:
            for it in e_items[(jt - 1) * NG:jt * NG]:
                it()
    for it in e_items[3 * NG:]:
        it()
    offer_last(best, cand)
    o_copy(NSEG - 1).start()

    xs_v[...] = best['xs'].astype(BF16)
    best_v[...] = jnp.broadcast_to(best['r'], (8, T))
    idx = jnp.clip(jnp.max(best['tok']), 0, S - 1)
    base = pl.multiple_of((idx // T) * T, T)
    tile = pl.ds(base, T)

    @pl.when(zero_s[0] == 0)
    def _ffn():
        xs = xs_v[...]
        acc = None
        f0 = 0
        for fw in FCH:
            fc = slice(f0, f0 + fw)
            gt = _rb(jnp.dot(xs, wg_v[:, fc], preferred_element_type=F32))
            up = _rb(jnp.dot(xs, wu_v[:, fc], preferred_element_type=F32))
            act = _rb(_rb(gt * jax.nn.sigmoid(gt)) * up)[0:1, :]
            for t in range(fw // T):
                a = act[:, t * T:(t + 1) * T]
                term = wd_v[:, f0 + t * T:f0 + (t + 1) * T].astype(F32) * a
                acc = term if acc is None else acc + term
            f0 += fw
        ycol = _rb(jnp.sum(acc, axis=1, keepdims=True))
        ycol = _rb(ycol * _rb(jax.nn.sigmoid(best_v[0:1, 0:1])))
        sel = lax.broadcasted_iota(jnp.int32, (D, T), 1) == idx - base
        old = out_s[:, tile].astype(F32)
        fix_v[...] = jnp.where(sel, old + ycol, old).astype(BF16)

    for s in range(NSEG):
        o_copy(s).wait()
    fix = pltpu.make_async_copy(fix_v, out_hbm.at[0, :, tile], sem_o.at[0])
    fix.start()
    fix.wait()


@jax.jit
def pallas_sequential_preLN__memory_aug_infini_attn__moe_arch_mod__prompt_kernel(
    A_x: jax.Array,
    A_wq: jax.Array,
    A_wk: jax.Array,
    A_wv: jax.Array,
    A_wo: jax.Array,
    A_beta: jax.Array,
    B_x: jax.Array,
    B_w_r: jax.Array,
    B_w_gate: jax.Array,
    B_w_up: jax.Array,
    B_w_down: jax.Array,
):
    del B_x
    hbm = pl.BlockSpec(memory_space=pltpu.HBM)
    scratch = [
        pltpu.VMEM((D, S), BF16),
        pltpu.VMEM((4, D, D), BF16),
        pltpu.VMEM((QR + 320, D), U32),
        pltpu.VMEM((D // 2, 640), U32),
        pltpu.VMEM((D // 2, L), U32),
        pltpu.VMEM((NG, 64, L), U32),
        pltpu.VMEM((NG, 64, L), U32),
        pltpu.VMEM((NG, L // 2, T), U32),
        pltpu.VMEM((NG, 64, L), U32),
        pltpu.VMEM((320, L), U32),
        pltpu.VMEM((640, L), F32),
        pltpu.VMEM((NG, 160, T), F32),
        pltpu.VMEM((HS, 1280, T), F32),
        pltpu.VMEM((HM - HS, 1280, T), F32),
        pltpu.VMEM((H - HM, 1280, T), F32),
        pltpu.VMEM((H, 112, T), F32),
        pltpu.VMEM((320, L), U32),
        pltpu.VMEM((D, L), F32),
        pltpu.VMEM((NSEG, 4, 16, T), F32),
        pltpu.VMEM((D // 2, S), U32),
        pltpu.VMEM((D, S), BF16),
        pltpu.VMEM((NSEG, 8, L), F32),
        pltpu.VMEM((T, T), F32),
        pltpu.VMEM((64, T), F32),
        pltpu.VMEM((2, H, T), F32),
        pltpu.VMEM((640, T), F32),
        pltpu.VMEM((NG, 160, T), F32),
        pltpu.VMEM((D, FF), BF16),
        pltpu.VMEM((D, FF), BF16),
        pltpu.VMEM((D, FF), BF16),
        pltpu.VMEM((H,), BF16),
        pltpu.VMEM((D,), BF16),
        pltpu.VMEM((16, D), BF16),
        pltpu.VMEM((16, D), BF16),
        pltpu.VMEM((8, T), F32),
        pltpu.VMEM((D, T), BF16),
        pltpu.SMEM((1,), jnp.int32),
        pltpu.SemaphoreType.DMA((2,)),
        pltpu.SemaphoreType.DMA((4,)),
        pltpu.SemaphoreType.DMA((3,)),
        pltpu.SemaphoreType.DMA((NSEG,)),
        pltpu.SemaphoreType.DMA((2,)),
    ]
    out_t = pl.pallas_call(
        _kernel,
        out_shape=jax.ShapeDtypeStruct((1, D, S), BF16),
        in_specs=[hbm] * 10,
        out_specs=hbm,
        scratch_shapes=scratch,
        compiler_params=pltpu.CompilerParams(vmem_limit_bytes=110 * 1024 * 1024),
        name="infini_moe",
    )(jnp.transpose(A_x, (0, 2, 1)), A_wq, A_wk, A_wv, A_wo, A_beta, B_w_r,
      B_w_gate, B_w_up, jnp.transpose(B_w_down, (1, 0)))
    return jnp.transpose(out_t, (0, 2, 1))
```

```python
import functools
import math

import jax
import jax.numpy as jnp
from jax import lax
import jax.experimental.pallas as pl
import jax.experimental.pallas.tpu as pltpu

F32 = jnp.float32
BF16 = jnp.bfloat16
U32 = jnp.uint32

S = 2048
D = 576
H = 32
DH = 18
NSEG = 4
L = 512
FF = 4608
T = 128
NG = 5
GH = (7, 7, 7, 7, 4)
VS = 20
EPS = 1e-5
QSCALE = DH ** (-0.5) * math.log2(math.e)
MASKVAL = -1000000000.0 * math.log2(math.e)
SOFF = (0, 128, 384, 768)
MOFF = (0, 2, 5, 9)
GWIN = tuple(((140 * g) // 16 * 16, -(-(140 * g + 20 * GH[g]) // 16) * 16) for g in range(NG))
QR = 592
FCH = (256,) * 18

HS = 16
HM = 25
HA1 = 9
NS0 = 16
TAIL = 16
KE = (VS * HS) // T * T
KM = (VS * HM) // T * T

NT = (((1,), (1,)), ((), ()))


def _bf(x_u32):
    return pltpu.bitcast(x_u32, BF16)


def _u32(x_bf):
    return pltpu.bitcast(x_bf, U32)


def _pack(y):
    return _u32(y.astype(BF16))


def _rb(x):
    return x.astype(BF16).astype(F32)


def _phi(t):
    return jnp.where(t > 0, t + 1.0, jnp.exp(t))


def _ln_scale(pivot, s1, s2):
    md = s1 * (1.0 / D)
    v = jnp.maximum(s2 * (1.0 / D) - md * md, 0.0)
    den = _rb(jnp.sqrt(_rb(_rb(v) + EPS)))
    return pivot + md, 1.0 / den


def _kernel(x_hbm, wq_hbm, wk_hbm, wv_hbm, wo_hbm, beta_hbm, wr_hbm, wg_hbm, wu_hbm, wd_hbm,
            out_hbm,
            x_v, w_v, wqkv, wot, xn, qt, pqt, kk, pkt, vt, memt, bd, s_a, s_b1, s_b2, m_blk,
            ot, att, ln_st, y_s, out_s, r_s, bias, bias2, gtab, ones_tab, keep_tab,
            wg_v, wu_v, wd_v, beta_v, wr_v, wr16, xs_v, best_v, fix_v,
            zero_s, sem_x, sem_w, sem_f, sem_o, sem_s):
    def x_copy(s):
        return pltpu.make_async_copy(x_hbm.at[0, :, pl.ds(s * L, L)], x_v.at[:, pl.ds(s * L, L)],
                                     sem_x.at[s])

    x_rest = pltpu.make_async_copy(x_hbm.at[0, :, pl.ds(2 * L, 2 * L)], x_v.at[:, pl.ds(2 * L, 2 * L)], sem_x.at[2])

    w_srcs = (wk_hbm, wq_hbm, wv_hbm, wo_hbm)

    def w_copy(i):
        return pltpu.make_async_copy(w_srcs[i], w_v.at[i], sem_w.at[i])

    f_pairs = ((wg_hbm, wg_v), (wu_hbm, wu_v), (wd_hbm, wd_v))

    def f_copy(i):
        return pltpu.make_async_copy(f_pairs[i][0], f_pairs[i][1], sem_f.at[i])

    def o_copy(s):
        return pltpu.make_async_copy(out_s.at[:, pl.ds(s * L, L)], out_hbm.at[0, :, pl.ds(s * L, L)],
                                     sem_o.at[s])

    beta_copy = pltpu.make_async_copy(beta_hbm, beta_v, sem_s.at[0])
    wr_copy = pltpu.make_async_copy(wr_hbm, wr_v, sem_s.at[1])

    def seg_cols(s, jt):
        if isinstance(s, int):
            return slice(s * L + jt * T, s * L + (jt + 1) * T)
        return pl.ds(pl.multiple_of(s * L + jt * T, T), T)

    def ln1_stats(s, jt):
        cols = seg_cols(s, jt)
        pivot = a1 = a2 = None
        for c in range(D // 32):
            x = x_v[32 * c:32 * (c + 1), cols].astype(F32)
            if c == 0:
                pivot = x[0:1, :]
            d = (x - pivot).reshape(4, 8, T)
            p1 = (d[0] + d[1]) + (d[2] + d[3])
            dd = d * d
            p2 = (dd[0] + dd[1]) + (dd[2] + dd[3])
            a1 = p1 if c == 0 else a1 + p1
            a2 = p2 if c == 0 else a2 + p2
        m, inv = _ln_scale(pivot, jnp.sum(a1, axis=0, keepdims=True), jnp.sum(a2, axis=0, keepdims=True))
        ln_st[s, jt, 0:1, :] = m
        ln_st[s, jt, 8:9, :] = inv

    def ln1_norm(s, jt):
        for c in range(NG):
            r0, r1 = T * c, min(T * (c + 1), D)
            x = x_v[r0:r1, seg_cols(s, jt)].astype(F32)
            xn[r0 // 2:r1 // 2, jt * T:(jt + 1) * T] = _u32(
                ((x - ln_st[s, jt, 0:1, :]) * ln_st[s, jt, 8:9, :]).astype(BF16))

    def q_unit(jt, g):
        cols = slice(jt * T, (jt + 1) * T)
        n = min(64, QR // 2 - 64 * g)
        q = jnp.dot(_bf(wqkv[64 * g:64 * g + n, :]), _bf(xn[:, cols]), preferred_element_type=F32)
        qt[g, 0:n, cols] = _pack(q * QSCALE)
        pqt[g, 0:n, cols] = _pack(_phi(q))

    def k_unit(jt, g):
        cols = slice(jt * T, (jt + 1) * T)
        n = min(64, QR // 2 - 64 * g)
        b0 = QR // 2 + 64 * g
        k = jnp.dot(_bf(wqkv[b0:b0 + n, :]), _bf(xn[:, cols]), preferred_element_type=F32)
        pkt[g, 0:n, cols] = _pack(_phi(k))
        kb = _pack(k)
        if n < 64:
            kb = jnp.concatenate([kb, jnp.zeros((64 - n, T), U32)], axis=0)
        kk[g, jt * 64:(jt + 1) * 64, :] = _u32(_bf(kb).T)

    def v_unit(jt, c):
        cols = slice(jt * T, (jt + 1) * T)
        b0 = QR + 64 * c
        v = jnp.dot(_bf(wqkv[b0:b0 + 64, :]), _bf(xn[:, cols]), preferred_element_type=F32)
        vt[64 * c:64 * (c + 1), cols] = _pack(v + ones_tab[T * c:T * (c + 1), :])

    def mem_read_unit(g):
        w0, w1 = GWIN[g]
        b = bd[g, 0:w1 - w0, :].astype(BF16)
        res = jnp.dot(b, _bf(pqt[g]), preferred_element_type=F32)
        lo, hi = 140 * g, 140 * g + 20 * GH[g]
        memt[lo:hi, :] = res[lo - w0:hi - w0]

    def mem_update_unit(g):
        w0, w1 = GWIN[g]
        upd = lax.dot_general(_bf(vt[w0 // 2:w1 // 2, :]), _bf(pkt[g]), NT, preferred_element_type=F32)
        n = w1 - w0
        bd[g, 0:n, :] = bd[g, 0:n, :] + jnp.where(keep_tab[g, 0:n, :] > 0.5, upd, 0.0)

    def sbuf(h):
        if h < HS:
            return s_a, h
        return (s_b1, h - HS) if h < HM else (s_b2, h - HM)

    def head_rows(j):
        r = lax.broadcasted_iota(jnp.int32, (64, T), 0)
        return (r >= 9 * j) & (r < 9 * j + 9)

    def s_blk(h, jq, kb, half=False):
        g, j = divmod(h, 7)
        off = SOFF[jq] + kb * T
        n = 64 if half else T
        qm = _bf(jnp.where(head_rows(j), qt[g, :, jq * T:(jq + 1) * T], U32(0)))
        sc = jnp.dot(_bf(kk[g, kb * 64:kb * 64 + n // 2, :]), qm, preferred_element_type=F32)
        if kb == jq:
            sc = sc + bias[0:n, :]
        sb, hi_ = sbuf(h)
        sb[hi_, off:off + n, :] = sc
        slot = MOFF[jq] + kb
        m_blk[h, slot * 8:(slot + 1) * 8, :] = jnp.max(sc.reshape(n // 8, 8, T), axis=0)

    def s_pair(ha, jq):
        g, j = divmod(ha, 7)
        off = SOFF[jq] + jq * T + 64
        lo = lax.broadcasted_iota(jnp.int32, (64, T), 1) < 64
        qu = qt[g, :, jq * T:(jq + 1) * T]
        qmix = jnp.where(lo, pltpu.roll(qu, 64, 1), qu)
        qm = _bf(jnp.where((lo & head_rows(j)) | (~lo & head_rows(j + 1)), qmix, U32(0)))
        sc = jnp.dot(_bf(kk[g, jq * 64 + 32:jq * 64 + 64, :]), qm, preferred_element_type=F32) + bias2[...]
        sb, hi_ = sbuf(ha)
        sb[hi_, off:off + 64, :] = sc
        pm = jnp.max(sc.reshape(8, 8, T), axis=0)
        hi = lax.broadcasted_iota(jnp.int32, (8, T), 1) >= 64
        slot = MOFF[jq] + jq + 1
        m_blk[ha, slot * 8:(slot + 1) * 8, :] = jnp.where(hi, pltpu.roll(pm, 64, 1), -jnp.inf)
        m_blk[ha + 1, slot * 8:(slot + 1) * 8, :] = jnp.where(hi, pm, -jnp.inf)

    def row_max(h, jq, nslots):
        return jnp.max(m_blk[h, MOFF[jq] * 8:(MOFF[jq] + nslots) * 8, :], axis=0, keepdims=True)

    def pv_blk(h, jq, kb, st, role):
        w0 = (VS * h) // 16 * 16
        o = VS * h - w0
        off = SOFF[jq] + kb * T
        cols = slice(jq * T, (jq + 1) * T)
        key = role or 'a'
        sb, hz = sbuf(h)
        hz = hz + st['z']
        if kb == 0 and role != 'b':
            st['ma'] = row_max(h, jq, jq + 1 if role is None else jq + 2)
            if role == 'a':
                st['mb'] = row_max(h + 1, jq, jq + 2)
        m = st['m' + key]
        if kb < jq or role is None:
            p = jnp.exp2(sb[hz, off:off + T, :] - m).astype(BF16)
        else:
            if role == 'a':
                hi1 = lax.broadcasted_iota(jnp.int32, (1, T), 1) >= 64
                hi = lax.broadcasted_iota(jnp.int32, (64, T), 1) >= 64
                m2 = jnp.where(hi1, st['mb'], pltpu.roll(st['ma'], 64, 1))
                e2 = jnp.exp2(sb[hz, off + 64:off + T, :] - m2)
                p2 = jnp.where(hi, pltpu.roll(e2, 64, 1), 0.0)
                st['p2b'] = jnp.where(hi, e2, 0.0)
            else:
                p2 = st['p2b']
            p1 = jnp.exp2(sb[hz, off:off + 64, :] - m)
            p = jnp.concatenate([p1, p2], axis=0).astype(BF16)
        part = jnp.dot(_bf(vt[w0 // 2:w0 // 2 + 16, kb * T:(kb + 1) * T]), p, preferred_element_type=F32)
        st['pv' + key] = part if kb == 0 else st['pv' + key] + part
        if kb == jq:
            pv = st['pv' + key]
            res = pv * (gtab[1, h:h + 1, :] / pv[o + DH:o + DH + 1, :])
            mem = memt[w0:w0 + 32, cols]
            res = res + mem * (gtab[0, h:h + 1, :] / (mem[o + DH:o + DH + 1, :] + 1e-6))
            ot[VS * h // 2:VS * h // 2 + VS // 2, cols] = _u32(res.astype(BF16))[o // 2:o // 2 + VS // 2]

    def o_early(s, jt, c, ke):
        r0, r1 = T * c, min(T * (c + 1), D)
        tile = slice(jt * T, (jt + 1) * T)
        a = jnp.dot(_bf(wot[r0 // 2:r1 // 2, 0:ke]), _bf(ot[0:ke // 2, tile]), preferred_element_type=F32)
        att[r0:r1, tile] = x_v[r0:r1, seg_cols(s, jt)].astype(F32) + a

    def o_unit(s, jt, c, ke, st):
        r0, r1 = T * c, min(T * (c + 1), D)
        tile = slice(jt * T, (jt + 1) * T)
        a = jnp.dot(_bf(wot[r0 // 2:r1 // 2, ke:640]), _bf(ot[ke // 2:320, tile]), preferred_element_type=F32)
        hh = att[r0:r1, tile] + a
        att[r0:r1, tile] = hh
        if c == 0:
            st['p'] = hh[0:1, :]
        d = hh - st['p']
        s1 = jnp.sum(d, axis=0, keepdims=True)
        s2 = jnp.sum(d * d, axis=0, keepdims=True)
        st['s1'] = s1 if c == 0 else st['s1'] + s1
        st['s2'] = s2 if c == 0 else st['s2'] + s2

    def e2_unit(s, jt, c, st):
        r0, r1 = T * c, min(T * (c + 1), D)
        cols = seg_cols(s, jt)
        if c == 0:
            st['m'], st['inv'] = _ln_scale(st['p'], st['s1'], st['s2'])
        hh = att[r0:r1, jt * T:(jt + 1) * T]
        y = (hh - st['m']) * st['inv']
        n = (r1 - r0) // 2
        cand = st.get('cand')
        if cand is None:
            y_s[r0 // 2:r1 // 2, cols] = pltpu.pack_elementwise([y[0:n], y[n:2 * n]], packed_dtype=BF16)
        out_s[r0:r1, cols] = (hh + y).astype(BF16)
        yb = y.astype(BF16)
        rr = jnp.dot(wr16[:, r0:r1], yb, preferred_element_type=F32)
        st['r'] = rr if c == 0 else st['r'] + rr
        if cand is not None:
            cand.setdefault(jt, {'y': []})['y'].append(yb)
        if r1 == D:
            rrow = _rb(st['r'][0:1, :])
            if cand is None:
                r_s[s, :, jt * T:(jt + 1) * T] = jnp.broadcast_to(rrow, (8, T))
            else:
                cand[jt]['r'] = rrow

    def offer_last(best, cand):
        rrow = jnp.concatenate([cand[jt]['r'] for jt in range(4)], axis=1)
        tmax = jnp.max(rrow, axis=1, keepdims=True)
        lane = lax.broadcasted_iota(jnp.int32, (1, L), 1)
        lane_c = jnp.min(jnp.where(rrow == tmax, lane, L), axis=1, keepdims=True)
        xs = None
        for jt in range(4):
            oh = (lax.broadcasted_iota(jnp.int32, (16, T), 1) == lane_c - jt * T).astype(BF16)
            part = jnp.concatenate([lax.dot_general(oh, yc, NT, preferred_element_type=F32)
                                    for yc in cand[jt]['y']], axis=1)
            xs = part if xs is None else xs + part
        take = tmax > best['r']
        best.update(r=jnp.where(take, tmax, best['r']),
                    tok=jnp.where(take, (NSEG - 1) * L + lane_c, best['tok']),
                    xs=jnp.where(take, xs, best['xs']))

    def prep_qk(i, base):
        wt = _u32(w_v[i].T)
        for g in range(NG):
            n = 9 * GH[g]
            wqkv[base + 64 * g:base + 64 * g + n, :] = wt[63 * g:63 * g + n, :]

    def prep_v():
        wt = _u32(w_v[2].T)
        for h in range(H):
            wqkv[QR + 10 * h:QR + 10 * h + 9, :] = wt[9 * h:9 * h + 9, :]

    def prep_o():
        wt = _u32(w_v[3])
        wpad = jnp.concatenate(
            [piece for h in range(H) for piece in (wt[9 * h:9 * h + 9, :], jnp.zeros((1, D), U32))], axis=0)
        wot[...] = _u32(_bf(wpad).T)

    BLKS = [(jq, kb) for jq in range(4) for kb in range(jq + 1)]

    def head_sets(heads):
        sets, i = [], 0
        while i < len(heads):
            h = heads[i]
            if h % 7 % 2 == 0 and h % 7 < 6 and i + 1 < len(heads):
                sets.append((h, h + 1))
                i += 2
            else:
                assert h % 7 == 6
                sets.append((h,))
                i += 1
        return sets

    def s_items(heads, small_tail=0):
        big, small = [], []
        for hs in head_sets(heads):
            for jq, kb in BLKS:
                halved = len(hs) == 2 and kb == jq
                for h in hs:
                    (small if halved else big).append(functools.partial(s_blk, h, jq, kb, halved))
                if halved:
                    small.append(functools.partial(s_pair, hs[0], jq))
        tail = small[len(small) - small_tail:] if small_tail else []
        small = small[:len(small) - small_tail] if small_tail else small
        order = sorted([((j + 0.5) / len(big), 0, j) for j in range(len(big))]
                       + [((j + 0.5) / len(small), 1, j) for j in range(len(small))])
        return [(big, small)[w][j] for _, w, j in order] + tail

    def phase_x():
        sb = s_items(HB)
        for it in sb[0:NS0]:
            it()
        interleave(pv_items(HA), sb[NS0:])

    def pv_items(heads, z=0):
        items = []
        for hs in head_sets(heads):
            st = {'z': z}
            roles = ('a', 'b') if len(hs) == 2 else (None,)
            for jq, kb in BLKS:
                for h, role in zip(hs, roles):
                    items.append(functools.partial(pv_blk, h, jq, kb, st, role))
        return items

    def interleave(*seqs):
        seqs = [q for q in seqs if q]
        order = []
        for i, q in enumerate(seqs):
            order += [((j + 0.5) / len(q), i, j) for j in range(len(q))]
        for _, i, j in sorted(order):
            seqs[i][j]()

    def proj_items(fn):
        return [functools.partial(fn, jt, g) for jt in range(4) for g in range(NG)]

    def out_items(s, ke, cand=None):
        sts = [{'cand': cand} for _ in range(4)]
        o_items = [functools.partial(o_unit, s, jt, c, ke, sts[jt]) for jt in range(4) for c in range(NG)]
        e_items = [functools.partial(e2_unit, s, jt, c, sts[jt]) for jt in range(4) for c in range(NG)]
        early = [functools.partial(o_early, s, jt, c, ke) for jt in range(4) for c in range(NG)]
        return early, o_items, e_items

    HA = list(range(HS))
    HB = list(range(HS, H))

    x_copy(0).start()
    w_copy(1).start()
    zero_s[0] = 0
    beta_copy.start()
    wr_copy.start()
    kr = lax.broadcasted_iota(jnp.int32, (T, T), 0)
    qc = lax.broadcasted_iota(jnp.int32, (T, T), 1)
    bias[...] = jnp.where(kr > qc, MASKVAL, 0.0).astype(F32)
    kr2 = lax.broadcasted_iota(jnp.int32, (64, T), 0)
    qc2 = lax.broadcasted_iota(jnp.int32, (64, T), 1)
    bias2[...] = jnp.where(kr2 > (qc2 & 63), MASKVAL, 0.0).astype(F32)
    wqkv[...] = jnp.zeros(wqkv.shape, U32)
    bd[...] = jnp.zeros(bd.shape, F32)
    memt[...] = jnp.zeros(memt.shape, F32)
    row = lax.broadcasted_iota(jnp.int32, (640, T), 0)
    ones_tab[...] = jnp.where(row % VS == DH, 1.0, 0.0).astype(F32)
    for g in range(NG):
        row = lax.broadcasted_iota(jnp.int32, (160, T), 0) + (GWIN[g][0] - 140 * g)
        lane = lax.broadcasted_iota(jnp.int32, (160, T), 1)
        keep = ((row >= 0) & (row < 20 * GH[g]) & (lane >= (row // VS) * DH)
                & (lane < (row // VS) * DH + DH))
        keep_tab[g] = jnp.where(keep, 1.0, 0.0).astype(F32)
    qt[NG - 1] = jnp.zeros(qt.shape[1:], U32)
    pqt[NG - 1] = jnp.zeros(pqt.shape[1:], U32)
    pkt[NG - 1] = jnp.zeros(pkt.shape[1:], U32)

    x_copy(0).wait()
    w_copy(0).start()
    for jt in range(4):
        ln1_stats(0, jt)
        ln1_norm(0, jt)
    w_copy(1).wait()
    w_copy(2).start()
    prep_qk(1, 0)
    for g in range(NG):
        for jt in range(2):
            q_unit(jt, g)
    w_copy(0).wait()
    x_copy(1).start()
    prep_qk(0, QR // 2)
    for jt in range(2, 4):
        for g in range(NG):
            q_unit(jt, g)
    w_copy(2).wait()
    x_rest.start()
    w_copy(3).start()
    prep_v()
    for jt in range(4):
        for g in range(NG):
            k_unit(jt, g)
    beta_copy.wait()
    wr_copy.wait()
    x_copy(1).wait()
    beta = beta_v[...].astype(F32).reshape(1, H)
    hl = lax.broadcasted_iota(jnp.int32, (H, H), 1)
    hs = lax.broadcasted_iota(jnp.int32, (H, H), 0)
    bcol = jnp.sum(jnp.where(hl == hs, jnp.broadcast_to(beta, (H, H)), 0.0), axis=1, keepdims=True)
    gate = _rb(jax.nn.sigmoid(bcol))
    gtab[0] = jnp.broadcast_to(gate, (H, T))
    gtab[1] = jnp.broadcast_to(_rb(1.0 - gate), (H, T))
    r16 = lax.broadcasted_iota(jnp.int32, (16, D), 0)
    wr_row = wr_v[...].astype(F32).reshape(1, D)
    wr16[...] = jnp.where(r16 == 0, jnp.broadcast_to(wr_row, (16, D)), 0.0).astype(BF16)
    interleave(proj_items(v_unit) + s_items(HA, TAIL),
               [functools.partial(ln1_stats, 1, jt) for jt in range(4)])
    x_rest.wait()
    w_copy(3).wait()
    for i in range(2, NSEG):
        for jt in range(4):
            ln1_stats(i, jt)

    def seg_body(s, carry):
        z = zero_s[0]
        prep_o()
        phase_x()
        ln = [functools.partial(ln1_norm, s + 1, jt) for jt in range(4)]
        qs = proj_items(q_unit)
        early, o_items, e_items = out_items(s, KE)
        upd = [functools.partial(mem_update_unit, g) for g in range(NG)]
        ks = proj_items(k_unit)
        pre = [ln[0]] + early[0:8] + [ln[1]]
        mxu1 = early[8:14] + [ln[2]] + upd + qs[0:5] + early[14:20] + [ln[3]] + qs[5:20] + ks
        for it in pre:
            it()
        interleave(pv_items(HB, z), mxu1)
        vr = proj_items(v_unit) + [functools.partial(mem_read_unit, g) for g in range(NG)]
        for it in o_items:
            it()
        interleave(vr, e_items)
        for it in s_items(HA, TAIL):
            it()
        o_copy(s).start()

        @pl.when(s == 0)
        def _():
            f_copy(0).start()
            f_copy(1).start()

        @pl.when(s == 1)
        def _():
            f_copy(2).start()
        return carry

    lax.fori_loop(0, NSEG - 1, seg_body, 0)

    for i in range(3):
        f_copy(i).wait()
    z = zero_s[0]
    best = {}

    def offer_previous():
        n = (NSEG - 1) * 8
        r_all = r_s[0:NSEG - 1].reshape(n, L)
        tok = ((lax.broadcasted_iota(jnp.int32, (n, L), 0) // 8) * L
               + lax.broadcasted_iota(jnp.int32, (n, L), 1))
        rmax = jnp.max(jnp.max(r_all, axis=1, keepdims=True), axis=0, keepdims=True)
        idx = jnp.clip(jnp.min(jnp.where(r_all == rmax, tok, S)), 0, S - 1)
        base = pl.multiple_of((idx // T) * T, T)
        onehot = (lax.broadcasted_iota(jnp.int32, (16, T), 1) == idx - base).astype(BF16)
        yw = y_s[:, pl.ds(base, T)]
        pieces = []
        for c in range(NG):
            w0, w1 = 64 * c, min(64 * (c + 1), D // 2)
            n2 = w1 - w0
            xp = lax.dot_general(onehot, _bf(yw[w0:w1]), NT, preferred_element_type=F32)
            rr = lax.broadcasted_iota(jnp.int32, (2 * n2, 2 * n2), 0)
            cc = lax.broadcasted_iota(jnp.int32, (2 * n2, 2 * n2), 1)
            unmix = (rr == jnp.where(cc < n2, 2 * cc, 2 * (cc - n2) + 1)).astype(BF16)
            pieces.append(jnp.dot(xp.astype(BF16), unmix, preferred_element_type=F32))
        best.update(r=rmax, tok=jnp.full((1, 1), idx, jnp.int32), xs=jnp.concatenate(pieces, axis=1))

    ha1, ha2 = HA[:HA1], HA[HA1:]
    hb1, hb2 = list(range(HS, HM)), list(range(HM, H))
    sb1 = s_items(hb1)
    for it in sb1[0:NS0]:
        it()
    interleave(pv_items(ha1), sb1[NS0:])
    offer_previous()
    sb2 = s_items(hb2)
    interleave(pv_items(ha2) + pv_items(hb1, z), sb2)
    cand = {}
    early, o_items, e_items = out_items(NSEG - 1, KM, cand)
    for it in early[0:4]:
        it()
    interleave(pv_items(hb2, z), early[4:])
    for jt in range(4):
        for it in o_items[jt * NG:(jt + 1) * NG]:
            it()
        if jt > 0:
            for it in e_items[(jt - 1) * NG:jt * NG]:
                it()
    for it in e_items[3 * NG:]:
        it()
    offer_last(best, cand)
    o_copy(NSEG - 1).start()

    xs_v[...] = best['xs'].astype(BF16)
    best_v[...] = jnp.broadcast_to(best['r'], (8, T))
    idx = jnp.clip(jnp.max(best['tok']), 0, S - 1)
    base = pl.multiple_of((idx // T) * T, T)
    tile = pl.ds(base, T)

    @pl.when(zero_s[0] == 0)
    def _ffn():
        xs = xs_v[...]
        acc = None
        f0 = 0
        for fw in FCH:
            fc = slice(f0, f0 + fw)
            gt = _rb(jnp.dot(xs, wg_v[:, fc], preferred_element_type=F32))
            up = _rb(jnp.dot(xs, wu_v[:, fc], preferred_element_type=F32))
            act = _rb(_rb(gt * jax.nn.sigmoid(gt)) * up)[0:1, :]
            for t in range(fw // T):
                a = act[:, t * T:(t + 1) * T]
                term = wd_v[:, f0 + t * T:f0 + (t + 1) * T].astype(F32) * a
                acc = term if acc is None else acc + term
            f0 += fw
        ycol = _rb(jnp.sum(acc, axis=1, keepdims=True))
        ycol = _rb(ycol * _rb(jax.nn.sigmoid(best_v[0:1, 0:1])))
        sel = lax.broadcasted_iota(jnp.int32, (D, T), 1) == idx - base
        old = out_s[:, tile].astype(F32)
        fix_v[...] = jnp.where(sel, old + ycol, old).astype(BF16)

    for s in range(NSEG):
        o_copy(s).wait()
    fix = pltpu.make_async_copy(fix_v, out_hbm.at[0, :, tile], sem_o.at[0])
    fix.start()
    fix.wait()


@jax.jit
def pallas_sequential_preLN__memory_aug_infini_attn__moe_arch_mod__prompt_kernel(
    A_x: jax.Array,
    A_wq: jax.Array,
    A_wk: jax.Array,
    A_wv: jax.Array,
    A_wo: jax.Array,
    A_beta: jax.Array,
    B_x: jax.Array,
    B_w_r: jax.Array,
    B_w_gate: jax.Array,
    B_w_up: jax.Array,
    B_w_down: jax.Array,
):
    del B_x
    hbm = pl.BlockSpec(memory_space=pltpu.HBM)
    scratch = [
        pltpu.VMEM((D, S), BF16),
        pltpu.VMEM((4, D, D), BF16),
        pltpu.VMEM((QR + 320, D), U32),
        pltpu.VMEM((D // 2, 640), U32),
        pltpu.VMEM((D // 2, L), U32),
        pltpu.VMEM((NG, 64, L), U32),
        pltpu.VMEM((NG, 64, L), U32),
        pltpu.VMEM((NG, L // 2, T), U32),
        pltpu.VMEM((NG, 64, L), U32),
        pltpu.VMEM((320, L), U32),
        pltpu.VMEM((640, L), F32),
        pltpu.VMEM((NG, 160, T), F32),
        pltpu.VMEM((HS, 1280, T), F32),
        pltpu.VMEM((HM - HS, 1280, T), F32),
        pltpu.VMEM((H - HM, 1280, T), F32),
        pltpu.VMEM((H, 112, T), F32),
        pltpu.VMEM((320, L), U32),
        pltpu.VMEM((D, L), F32),
        pltpu.VMEM((NSEG, 4, 16, T), F32),
        pltpu.VMEM((D // 2, S), U32),
        pltpu.VMEM((D, S), BF16),
        pltpu.VMEM((NSEG, 8, L), F32),
        pltpu.VMEM((T, T), F32),
        pltpu.VMEM((64, T), F32),
        pltpu.VMEM((2, H, T), F32),
        pltpu.VMEM((640, T), F32),
        pltpu.VMEM((NG, 160, T), F32),
        pltpu.VMEM((D, FF), BF16),
        pltpu.VMEM((D, FF), BF16),
        pltpu.VMEM((D, FF), BF16),
        pltpu.VMEM((H,), BF16),
        pltpu.VMEM((D,), BF16),
        pltpu.VMEM((16, D), BF16),
        pltpu.VMEM((16, D), BF16),
        pltpu.VMEM((8, T), F32),
        pltpu.VMEM((D, T), BF16),
        pltpu.SMEM((1,), jnp.int32),
        pltpu.SemaphoreType.DMA((3,)),
        pltpu.SemaphoreType.DMA((4,)),
        pltpu.SemaphoreType.DMA((3,)),
        pltpu.SemaphoreType.DMA((NSEG,)),
        pltpu.SemaphoreType.DMA((2,)),
    ]
    out_t = pl.pallas_call(
        _kernel,
        out_shape=jax.ShapeDtypeStruct((1, D, S), BF16),
        in_specs=[hbm] * 10,
        out_specs=hbm,
        scratch_shapes=scratch,
        compiler_params=pltpu.CompilerParams(vmem_limit_bytes=110 * 1024 * 1024),
        name="infini_moe",
    )(jnp.transpose(A_x, (0, 2, 1)), A_wq, A_wk, A_wv, A_wo, A_beta, B_w_r,
      B_w_gate, B_w_up, jnp.transpose(B_w_down, (1, 0)))
    return jnp.transpose(out_t, (0, 2, 1))
```

```python
import functools
import math

import jax
import jax.numpy as jnp
from jax import lax
import jax.experimental.pallas as pl
import jax.experimental.pallas.tpu as pltpu

F32 = jnp.float32
BF16 = jnp.bfloat16
U32 = jnp.uint32

S = 2048
D = 576
H = 32
DH = 18
NSEG = 4
L = 512
FF = 4608
T = 128
NG = 5
GH = (7, 7, 7, 7, 4)
VS = 20
EPS = 1e-5
QSCALE = DH ** (-0.5) * math.log2(math.e)
MASKVAL = -1000000000.0 * math.log2(math.e)
SOFF = (0, 128, 384, 768)
MOFF = (0, 2, 5, 9)
GWIN = tuple(((140 * g) // 16 * 16, -(-(140 * g + 20 * GH[g]) // 16) * 16) for g in range(NG))
QR = 592
FCH = (256,) * 18

HS = 16
HM = 25
HA1 = 9
NS0 = 16
TAIL = 16
KE = (VS * HS) // T * T
KM = (VS * HM) // T * T

NT = (((1,), (1,)), ((), ()))


def _bf(x_u32):
    return pltpu.bitcast(x_u32, BF16)


def _u32(x_bf):
    return pltpu.bitcast(x_bf, U32)


def _pack(y):
    return _u32(y.astype(BF16))


def _rb(x):
    return x.astype(BF16).astype(F32)


def _phi(t):
    return jnp.where(t > 0, t + 1.0, jnp.exp(t))


def _ln_scale(pivot, s1, s2):
    md = s1 * (1.0 / D)
    v = jnp.maximum(s2 * (1.0 / D) - md * md, 0.0)
    den = _rb(jnp.sqrt(_rb(_rb(v) + EPS)))
    return pivot + md, 1.0 / den


def _kernel(x_hbm, wq_hbm, wk_hbm, wv_hbm, wo_hbm, beta_hbm, wr_hbm, wg_hbm, wu_hbm, wd_hbm,
            out_hbm,
            x_v, w_v, wqkv, wot, xn, qt, pqt, kk, pkt, vt, memt, bd, s_a, s_b1, s_b2, m_blk,
            ot, att, ln_st, y_s, out_s, r_s, bias, bias2, gtab, ones_tab, keep_tab,
            wg_v, wu_v, wd_v, beta_v, wr_v, wr16, xs_v, best_v, fix_v,
            zero_s, sem_x, sem_w, sem_f, sem_o, sem_s):
    def x_copy(s):
        return pltpu.make_async_copy(x_hbm.at[0, :, pl.ds(s * L, L)], x_v.at[:, pl.ds(s * L, L)],
                                     sem_x.at[s])

    x_rest = pltpu.make_async_copy(x_hbm.at[0, :, pl.ds(2 * L, 2 * L)], x_v.at[:, pl.ds(2 * L, 2 * L)], sem_x.at[2])

    x0a = pltpu.make_async_copy(x_hbm.at[0, :, pl.ds(0, L // 2)], x_v.at[:, pl.ds(0, L // 2)], sem_x.at[0])
    x0b = pltpu.make_async_copy(x_hbm.at[0, :, pl.ds(L // 2, L // 2)], x_v.at[:, pl.ds(L // 2, L // 2)], sem_x.at[3])

    w_srcs = (wk_hbm, wq_hbm, wv_hbm, wo_hbm)

    def w_copy(i):
        return pltpu.make_async_copy(w_srcs[i], w_v.at[i], sem_w.at[i])

    f_pairs = ((wg_hbm, wg_v), (wu_hbm, wu_v), (wd_hbm, wd_v))

    def f_copy(i):
        return pltpu.make_async_copy(f_pairs[i][0], f_pairs[i][1], sem_f.at[i])

    def o_copy(s):
        return pltpu.make_async_copy(out_s.at[:, pl.ds(s * L, L)], out_hbm.at[0, :, pl.ds(s * L, L)],
                                     sem_o.at[s])

    beta_copy = pltpu.make_async_copy(beta_hbm, beta_v, sem_s.at[0])
    wr_copy = pltpu.make_async_copy(wr_hbm, wr_v, sem_s.at[1])

    def seg_cols(s, jt):
        if isinstance(s, int):
            return slice(s * L + jt * T, s * L + (jt + 1) * T)
        return pl.ds(pl.multiple_of(s * L + jt * T, T), T)

    def ln1_stats(s, jt):
        cols = seg_cols(s, jt)
        pivot = a1 = a2 = None
        for c in range(D // 32):
            x = x_v[32 * c:32 * (c + 1), cols].astype(F32)
            if c == 0:
                pivot = x[0:1, :]
            d = (x - pivot).reshape(4, 8, T)
            p1 = (d[0] + d[1]) + (d[2] + d[3])
            dd = d * d
            p2 = (dd[0] + dd[1]) + (dd[2] + dd[3])
            a1 = p1 if c == 0 else a1 + p1
            a2 = p2 if c == 0 else a2 + p2
        m, inv = _ln_scale(pivot, jnp.sum(a1, axis=0, keepdims=True), jnp.sum(a2, axis=0, keepdims=True))
        ln_st[s, jt, 0:1, :] = m
        ln_st[s, jt, 8:9, :] = inv

    def ln1_norm(s, jt):
        for c in range(NG):
            r0, r1 = T * c, min(T * (c + 1), D)
            x = x_v[r0:r1, seg_cols(s, jt)].astype(F32)
            xn[r0 // 2:r1 // 2, jt * T:(jt + 1) * T] = _u32(
                ((x - ln_st[s, jt, 0:1, :]) * ln_st[s, jt, 8:9, :]).astype(BF16))

    def q_unit(jt, g):
        cols = slice(jt * T, (jt + 1) * T)
        n = min(64, QR // 2 - 64 * g)
        q = jnp.dot(_bf(wqkv[64 * g:64 * g + n, :]), _bf(xn[:, cols]), preferred_element_type=F32)
        qt[g, 0:n, cols] = _pack(q * QSCALE)
        pqt[g, 0:n, cols] = _pack(_phi(q))

    def k_unit(jt, g):
        cols = slice(jt * T, (jt + 1) * T)
        n = min(64, QR // 2 - 64 * g)
        b0 = QR // 2 + 64 * g
        k = jnp.dot(_bf(wqkv[b0:b0 + n, :]), _bf(xn[:, cols]), preferred_element_type=F32)
        pkt[g, 0:n, cols] = _pack(_phi(k))
        kb = _pack(k)
        if n < 64:
            kb = jnp.concatenate([kb, jnp.zeros((64 - n, T), U32)], axis=0)
        kk[g, jt * 64:(jt + 1) * 64, :] = _u32(_bf(kb).T)

    def v_unit(jt, c):
        cols = slice(jt * T, (jt + 1) * T)
        b0 = QR + 64 * c
        v = jnp.dot(_bf(wqkv[b0:b0 + 64, :]), _bf(xn[:, cols]), preferred_element_type=F32)
        vt[64 * c:64 * (c + 1), cols] = _pack(v + ones_tab[T * c:T * (c + 1), :])

    def mem_read_unit(g):
        w0, w1 = GWIN[g]
        b = bd[g, 0:w1 - w0, :].astype(BF16)
        res = jnp.dot(b, _bf(pqt[g]), preferred_element_type=F32)
        lo, hi = 140 * g, 140 * g + 20 * GH[g]
        memt[lo:hi, :] = res[lo - w0:hi - w0]

    def mem_update_unit(g):
        w0, w1 = GWIN[g]
        upd = lax.dot_general(_bf(vt[w0 // 2:w1 // 2, :]), _bf(pkt[g]), NT, preferred_element_type=F32)
        n = w1 - w0
        bd[g, 0:n, :] = bd[g, 0:n, :] + jnp.where(keep_tab[g, 0:n, :] > 0.5, upd, 0.0)

    def sbuf(h):
        if h < HS:
            return s_a, h
        return (s_b1, h - HS) if h < HM else (s_b2, h - HM)

    def head_rows(j):
        r = lax.broadcasted_iota(jnp.int32, (64, T), 0)
        return (r >= 9 * j) & (r < 9 * j + 9)

    def s_blk(h, jq, kb, half=False):
        g, j = divmod(h, 7)
        off = SOFF[jq] + kb * T
        n = 64 if half else T
        qm = _bf(jnp.where(head_rows(j), qt[g, :, jq * T:(jq + 1) * T], U32(0)))
        sc = jnp.dot(_bf(kk[g, kb * 64:kb * 64 + n // 2, :]), qm, preferred_element_type=F32)
        if kb == jq:
            sc = sc + bias[0:n, :]
        sb, hi_ = sbuf(h)
        sb[hi_, off:off + n, :] = sc
        slot = MOFF[jq] + kb
        m_blk[h, slot * 8:(slot + 1) * 8, :] = jnp.max(sc.reshape(n // 8, 8, T), axis=0)

    def s_pair(ha, jq):
        g, j = divmod(ha, 7)
        off = SOFF[jq] + jq * T + 64
        lo = lax.broadcasted_iota(jnp.int32, (64, T), 1) < 64
        qu = qt[g, :, jq * T:(jq + 1) * T]
        qmix = jnp.where(lo, pltpu.roll(qu, 64, 1), qu)
        qm = _bf(jnp.where((lo & head_rows(j)) | (~lo & head_rows(j + 1)), qmix, U32(0)))
        sc = jnp.dot(_bf(kk[g, jq * 64 + 32:jq * 64 + 64, :]), qm, preferred_element_type=F32) + bias2[...]
        sb, hi_ = sbuf(ha)
        sb[hi_, off:off + 64, :] = sc
        pm = jnp.max(sc.reshape(8, 8, T), axis=0)
        hi = lax.broadcasted_iota(jnp.int32, (8, T), 1) >= 64
        slot = MOFF[jq] + jq + 1
        m_blk[ha, slot * 8:(slot + 1) * 8, :] = jnp.where(hi, pltpu.roll(pm, 64, 1), -jnp.inf)
        m_blk[ha + 1, slot * 8:(slot + 1) * 8, :] = jnp.where(hi, pm, -jnp.inf)

    def row_max(h, jq, nslots):
        return jnp.max(m_blk[h, MOFF[jq] * 8:(MOFF[jq] + nslots) * 8, :], axis=0, keepdims=True)

    def pv_blk(h, jq, kb, st, role):
        w0 = (VS * h) // 16 * 16
        o = VS * h - w0
        off = SOFF[jq] + kb * T
        cols = slice(jq * T, (jq + 1) * T)
        key = role or 'a'
        sb, hz = sbuf(h)
        hz = hz + st['z']
        if kb == 0 and role != 'b':
            st['ma'] = row_max(h, jq, jq + 1 if role is None else jq + 2)
            if role == 'a':
                st['mb'] = row_max(h + 1, jq, jq + 2)
        m = st['m' + key]
        if kb < jq or role is None:
            p = jnp.exp2(sb[hz, off:off + T, :] - m).astype(BF16)
        else:
            if role == 'a':
                hi1 = lax.broadcasted_iota(jnp.int32, (1, T), 1) >= 64
                hi = lax.broadcasted_iota(jnp.int32, (64, T), 1) >= 64
                m2 = jnp.where(hi1, st['mb'], pltpu.roll(st['ma'], 64, 1))
                e2 = jnp.exp2(sb[hz, off + 64:off + T, :] - m2)
                p2 = jnp.where(hi, pltpu.roll(e2, 64, 1), 0.0)
                st['p2b'] = jnp.where(hi, e2, 0.0)
            else:
                p2 = st['p2b']
            p1 = jnp.exp2(sb[hz, off:off + 64, :] - m)
            p = jnp.concatenate([p1, p2], axis=0).astype(BF16)
        part = jnp.dot(_bf(vt[w0 // 2:w0 // 2 + 16, kb * T:(kb + 1) * T]), p, preferred_element_type=F32)
        st['pv' + key] = part if kb == 0 else st['pv' + key] + part
        if kb == jq:
            pv = st['pv' + key]
            res = pv * (gtab[1, h:h + 1, :] / pv[o + DH:o + DH + 1, :])
            mem = memt[w0:w0 + 32, cols]
            res = res + mem * (gtab[0, h:h + 1, :] / (mem[o + DH:o + DH + 1, :] + 1e-6))
            ot[VS * h // 2:VS * h // 2 + VS // 2, cols] = _u32(res.astype(BF16))[o // 2:o // 2 + VS // 2]

    def o_early(s, jt, c, ke):
        r0, r1 = T * c, min(T * (c + 1), D)
        tile = slice(jt * T, (jt + 1) * T)
        a = jnp.dot(_bf(wot[r0 // 2:r1 // 2, 0:ke]), _bf(ot[0:ke // 2, tile]), preferred_element_type=F32)
        att[r0:r1, tile] = x_v[r0:r1, seg_cols(s, jt)].astype(F32) + a

    def o_unit(s, jt, c, ke, st):
        r0, r1 = T * c, min(T * (c + 1), D)
        tile = slice(jt * T, (jt + 1) * T)
        a = jnp.dot(_bf(wot[r0 // 2:r1 // 2, ke:640]), _bf(ot[ke // 2:320, tile]), preferred_element_type=F32)
        hh = att[r0:r1, tile] + a
        att[r0:r1, tile] = hh
        if c == 0:
            st['p'] = hh[0:1, :]
        d = hh - st['p']
        s1 = jnp.sum(d, axis=0, keepdims=True)
        s2 = jnp.sum(d * d, axis=0, keepdims=True)
        st['s1'] = s1 if c == 0 else st['s1'] + s1
        st['s2'] = s2 if c == 0 else st['s2'] + s2

    def e2_unit(s, jt, c, st):
        r0, r1 = T * c, min(T * (c + 1), D)
        cols = seg_cols(s, jt)
        if c == 0:
            st['m'], st['inv'] = _ln_scale(st['p'], st['s1'], st['s2'])
        hh = att[r0:r1, jt * T:(jt + 1) * T]
        y = (hh - st['m']) * st['inv']
        n = (r1 - r0) // 2
        cand = st.get('cand')
        if cand is None:
            y_s[r0 // 2:r1 // 2, cols] = pltpu.pack_elementwise([y[0:n], y[n:2 * n]], packed_dtype=BF16)
        out_s[r0:r1, cols] = (hh + y).astype(BF16)
        yb = y.astype(BF16)
        rr = jnp.dot(wr16[:, r0:r1], yb, preferred_element_type=F32)
        st['r'] = rr if c == 0 else st['r'] + rr
        if cand is not None:
            cand.setdefault(jt, {'y': []})['y'].append(yb)
        if r1 == D:
            rrow = _rb(st['r'][0:1, :])
            if cand is None:
                r_s[s, :, jt * T:(jt + 1) * T] = jnp.broadcast_to(rrow, (8, T))
            else:
                cand[jt]['r'] = rrow

    def offer_last(best, cand):
        rrow = jnp.concatenate([cand[jt]['r'] for jt in range(4)], axis=1)
        tmax = jnp.max(rrow, axis=1, keepdims=True)
        lane = lax.broadcasted_iota(jnp.int32, (1, L), 1)
        lane_c = jnp.min(jnp.where(rrow == tmax, lane, L), axis=1, keepdims=True)
        xs = None
        for jt in range(4):
            oh = (lax.broadcasted_iota(jnp.int32, (16, T), 1) == lane_c - jt * T).astype(BF16)
            part = jnp.concatenate([lax.dot_general(oh, yc, NT, preferred_element_type=F32)
                                    for yc in cand[jt]['y']], axis=1)
            xs = part if xs is None else xs + part
        take = tmax > best['r']
        best.update(r=jnp.where(take, tmax, best['r']),
                    tok=jnp.where(take, (NSEG - 1) * L + lane_c, best['tok']),
                    xs=jnp.where(take, xs, best['xs']))

    def prep_qk(i, base):
        wt = _u32(w_v[i].T)
        for g in range(NG):
            n = 9 * GH[g]
            wqkv[base + 64 * g:base + 64 * g + n, :] = wt[63 * g:63 * g + n, :]

    def prep_v():
        wt = _u32(w_v[2].T)
        for h in range(H):
            wqkv[QR + 10 * h:QR + 10 * h + 9, :] = wt[9 * h:9 * h + 9, :]

    def prep_o():
        wt = _u32(w_v[3])
        wpad = jnp.concatenate(
            [piece for h in range(H) for piece in (wt[9 * h:9 * h + 9, :], jnp.zeros((1, D), U32))], axis=0)
        wot[...] = _u32(_bf(wpad).T)

    BLKS = [(jq, kb) for jq in range(4) for kb in range(jq + 1)]

    def head_sets(heads):
        sets, i = [], 0
        while i < len(heads):
            h = heads[i]
            if h % 7 % 2 == 0 and h % 7 < 6 and i + 1 < len(heads):
                sets.append((h, h + 1))
                i += 2
            else:
                assert h % 7 == 6
                sets.append((h,))
                i += 1
        return sets

    def s_items(heads, small_tail=0):
        big, small = [], []
        for hs in head_sets(heads):
            for jq, kb in BLKS:
                halved = len(hs) == 2 and kb == jq
                for h in hs:
                    (small if halved else big).append(functools.partial(s_blk, h, jq, kb, halved))
                if halved:
                    small.append(functools.partial(s_pair, hs[0], jq))
        tail = small[len(small) - small_tail:] if small_tail else []
        small = small[:len(small) - small_tail] if small_tail else small
        order = sorted([((j + 0.5) / len(big), 0, j) for j in range(len(big))]
                       + [((j + 0.5) / len(small), 1, j) for j in range(len(small))])
        return [(big, small)[w][j] for _, w, j in order] + tail

    def phase_x():
        sb = s_items(HB)
        for it in sb[0:NS0]:
            it()
        interleave(pv_items(HA), sb[NS0:])

    def pv_items(heads, z=0):
        items = []
        for hs in head_sets(heads):
            st = {'z': z}
            roles = ('a', 'b') if len(hs) == 2 else (None,)
            for jq, kb in BLKS:
                for h, role in zip(hs, roles):
                    items.append(functools.partial(pv_blk, h, jq, kb, st, role))
        return items

    def interleave(*seqs):
        seqs = [q for q in seqs if q]
        order = []
        for i, q in enumerate(seqs):
            order += [((j + 0.5) / len(q), i, j) for j in range(len(q))]
        for _, i, j in sorted(order):
            seqs[i][j]()

    def proj_items(fn):
        return [functools.partial(fn, jt, g) for jt in range(4) for g in range(NG)]

    def out_items(s, ke, cand=None):
        sts = [{'cand': cand} for _ in range(4)]
        o_items = [functools.partial(o_unit, s, jt, c, ke, sts[jt]) for jt in range(4) for c in range(NG)]
        e_items = [functools.partial(e2_unit, s, jt, c, sts[jt]) for jt in range(4) for c in range(NG)]
        early = [functools.partial(o_early, s, jt, c, ke) for jt in range(4) for c in range(NG)]
        return early, o_items, e_items

    HA = list(range(HS))
    HB = list(range(HS, H))

    x0a.start()
    w_copy(1).start()
    x0b.start()
    zero_s[0] = 0
    beta_copy.start()
    wr_copy.start()
    kr = lax.broadcasted_iota(jnp.int32, (T, T), 0)
    qc = lax.broadcasted_iota(jnp.int32, (T, T), 1)
    bias[...] = jnp.where(kr > qc, MASKVAL, 0.0).astype(F32)
    kr2 = lax.broadcasted_iota(jnp.int32, (64, T), 0)
    qc2 = lax.broadcasted_iota(jnp.int32, (64, T), 1)
    bias2[...] = jnp.where(kr2 > (qc2 & 63), MASKVAL, 0.0).astype(F32)
    wqkv[...] = jnp.zeros(wqkv.shape, U32)
    bd[...] = jnp.zeros(bd.shape, F32)
    memt[...] = jnp.zeros(memt.shape, F32)
    row = lax.broadcasted_iota(jnp.int32, (640, T), 0)
    ones_tab[...] = jnp.where(row % VS == DH, 1.0, 0.0).astype(F32)
    for g in range(NG):
        row = lax.broadcasted_iota(jnp.int32, (160, T), 0) + (GWIN[g][0] - 140 * g)
        lane = lax.broadcasted_iota(jnp.int32, (160, T), 1)
        keep = ((row >= 0) & (row < 20 * GH[g]) & (lane >= (row // VS) * DH)
                & (lane < (row // VS) * DH + DH))
        keep_tab[g] = jnp.where(keep, 1.0, 0.0).astype(F32)
    qt[NG - 1] = jnp.zeros(qt.shape[1:], U32)
    pqt[NG - 1] = jnp.zeros(pqt.shape[1:], U32)
    pkt[NG - 1] = jnp.zeros(pkt.shape[1:], U32)

    x0a.wait()
    w_copy(0).start()
    for jt in range(2):
        ln1_stats(0, jt)
        ln1_norm(0, jt)
    w_copy(1).wait()
    w_copy(2).start()
    prep_qk(1, 0)
    for g in range(NG):
        for jt in range(2):
            q_unit(jt, g)
    w_copy(0).wait()
    x0b.wait()
    x_copy(1).start()
    for jt in range(2, 4):
        ln1_stats(0, jt)
        ln1_norm(0, jt)
    prep_qk(0, QR // 2)
    for jt in range(2, 4):
        for g in range(NG):
            q_unit(jt, g)
    w_copy(2).wait()
    x_rest.start()
    w_copy(3).start()
    prep_v()
    for jt in range(4):
        for g in range(NG):
            k_unit(jt, g)
    beta_copy.wait()
    wr_copy.wait()
    x_copy(1).wait()
    beta = beta_v[...].astype(F32).reshape(1, H)
    hl = lax.broadcasted_iota(jnp.int32, (H, H), 1)
    hs = lax.broadcasted_iota(jnp.int32, (H, H), 0)
    bcol = jnp.sum(jnp.where(hl == hs, jnp.broadcast_to(beta, (H, H)), 0.0), axis=1, keepdims=True)
    gate = _rb(jax.nn.sigmoid(bcol))
    gtab[0] = jnp.broadcast_to(gate, (H, T))
    gtab[1] = jnp.broadcast_to(_rb(1.0 - gate), (H, T))
    r16 = lax.broadcasted_iota(jnp.int32, (16, D), 0)
    wr_row = wr_v[...].astype(F32).reshape(1, D)
    wr16[...] = jnp.where(r16 == 0, jnp.broadcast_to(wr_row, (16, D)), 0.0).astype(BF16)
    interleave(proj_items(v_unit) + s_items(HA, TAIL),
               [functools.partial(ln1_stats, 1, jt) for jt in range(4)])
    x_rest.wait()
    w_copy(3).wait()
    for i in range(2, NSEG):
        for jt in range(4):
            ln1_stats(i, jt)

    def seg_body(s, carry):
        z = zero_s[0]
        prep_o()
        phase_x()
        ln = [functools.partial(ln1_norm, s + 1, jt) for jt in range(4)]
        qs = proj_items(q_unit)
        early, o_items, e_items = out_items(s, KE)
        upd = [functools.partial(mem_update_unit, g) for g in range(NG)]
        ks = proj_items(k_unit)
        pre = [ln[0]] + early[0:8] + [ln[1]]
        mxu1 = early[8:14] + [ln[2]] + upd + qs[0:5] + early[14:20] + [ln[3]] + qs[5:20] + ks
        for it in pre:
            it()
        interleave(pv_items(HB, z), mxu1)
        vr = proj_items(v_unit) + [functools.partial(mem_read_unit, g) for g in range(NG)]
        for it in o_items:
            it()
        interleave(vr, e_items)
        for it in s_items(HA, TAIL):
            it()
        o_copy(s).start()

        @pl.when(s == 0)
        def _():
            f_copy(0).start()
            f_copy(1).start()

        @pl.when(s == 1)
        def _():
            f_copy(2).start()
        return carry

    lax.fori_loop(0, NSEG - 1, seg_body, 0)

    for i in range(3):
        f_copy(i).wait()
    z = zero_s[0]
    best = {}

    def offer_previous():
        n = (NSEG - 1) * 8
        r_all = r_s[0:NSEG - 1].reshape(n, L)
        tok = ((lax.broadcasted_iota(jnp.int32, (n, L), 0) // 8) * L
               + lax.broadcasted_iota(jnp.int32, (n, L), 1))
        rmax = jnp.max(jnp.max(r_all, axis=1, keepdims=True), axis=0, keepdims=True)
        idx = jnp.clip(jnp.min(jnp.where(r_all == rmax, tok, S)), 0, S - 1)
        base = pl.multiple_of((idx // T) * T, T)
        onehot = (lax.broadcasted_iota(jnp.int32, (16, T), 1) == idx - base).astype(BF16)
        yw = y_s[:, pl.ds(base, T)]
        pieces = []
        for c in range(NG):
            w0, w1 = 64 * c, min(64 * (c + 1), D // 2)
            n2 = w1 - w0
            xp = lax.dot_general(onehot, _bf(yw[w0:w1]), NT, preferred_element_type=F32)
            rr = lax.broadcasted_iota(jnp.int32, (2 * n2, 2 * n2), 0)
            cc = lax.broadcasted_iota(jnp.int32, (2 * n2, 2 * n2), 1)
            unmix = (rr == jnp.where(cc < n2, 2 * cc, 2 * (cc - n2) + 1)).astype(BF16)
            pieces.append(jnp.dot(xp.astype(BF16), unmix, preferred_element_type=F32))
        best.update(r=rmax, tok=jnp.full((1, 1), idx, jnp.int32), xs=jnp.concatenate(pieces, axis=1))

    ha1, ha2 = HA[:HA1], HA[HA1:]
    hb1, hb2 = list(range(HS, HM)), list(range(HM, H))
    sb1 = s_items(hb1)
    for it in sb1[0:NS0]:
        it()
    interleave(pv_items(ha1), sb1[NS0:])
    offer_previous()
    sb2 = s_items(hb2)
    interleave(pv_items(ha2) + pv_items(hb1, z), sb2)
    cand = {}
    early, o_items, e_items = out_items(NSEG - 1, KM, cand)
    for it in early[0:4]:
        it()
    interleave(pv_items(hb2, z), early[4:])
    for jt in range(4):
        for it in o_items[jt * NG:(jt + 1) * NG]:
            it()
        if jt > 0:
            for it in e_items[(jt - 1) * NG:jt * NG]:
                it()
    for it in e_items[3 * NG:]:
        it()
    offer_last(best, cand)
    o_copy(NSEG - 1).start()

    xs_v[...] = best['xs'].astype(BF16)
    best_v[...] = jnp.broadcast_to(best['r'], (8, T))
    idx = jnp.clip(jnp.max(best['tok']), 0, S - 1)
    base = pl.multiple_of((idx // T) * T, T)
    tile = pl.ds(base, T)

    @pl.when(zero_s[0] == 0)
    def _ffn():
        xs = xs_v[...]
        acc = None
        f0 = 0
        for fw in FCH:
            fc = slice(f0, f0 + fw)
            gt = _rb(jnp.dot(xs, wg_v[:, fc], preferred_element_type=F32))
            up = _rb(jnp.dot(xs, wu_v[:, fc], preferred_element_type=F32))
            act = _rb(_rb(gt * jax.nn.sigmoid(gt)) * up)[0:1, :]
            for t in range(fw // T):
                a = act[:, t * T:(t + 1) * T]
                term = wd_v[:, f0 + t * T:f0 + (t + 1) * T].astype(F32) * a
                acc = term if acc is None else acc + term
            f0 += fw
        ycol = _rb(jnp.sum(acc, axis=1, keepdims=True))
        ycol = _rb(ycol * _rb(jax.nn.sigmoid(best_v[0:1, 0:1])))
        sel = lax.broadcasted_iota(jnp.int32, (D, T), 1) == idx - base
        old = out_s[:, tile].astype(F32)
        fix_v[...] = jnp.where(sel, old + ycol, old).astype(BF16)

    for s in range(NSEG):
        o_copy(s).wait()
    fix = pltpu.make_async_copy(fix_v, out_hbm.at[0, :, tile], sem_o.at[0])
    fix.start()
    fix.wait()


@jax.jit
def pallas_sequential_preLN__memory_aug_infini_attn__moe_arch_mod__prompt_kernel(
    A_x: jax.Array,
    A_wq: jax.Array,
    A_wk: jax.Array,
    A_wv: jax.Array,
    A_wo: jax.Array,
    A_beta: jax.Array,
    B_x: jax.Array,
    B_w_r: jax.Array,
    B_w_gate: jax.Array,
    B_w_up: jax.Array,
    B_w_down: jax.Array,
):
    del B_x
    hbm = pl.BlockSpec(memory_space=pltpu.HBM)
    scratch = [
        pltpu.VMEM((D, S), BF16),
        pltpu.VMEM((4, D, D), BF16),
        pltpu.VMEM((QR + 320, D), U32),
        pltpu.VMEM((D // 2, 640), U32),
        pltpu.VMEM((D // 2, L), U32),
        pltpu.VMEM((NG, 64, L), U32),
        pltpu.VMEM((NG, 64, L), U32),
        pltpu.VMEM((NG, L // 2, T), U32),
        pltpu.VMEM((NG, 64, L), U32),
        pltpu.VMEM((320, L), U32),
        pltpu.VMEM((640, L), F32),
        pltpu.VMEM((NG, 160, T), F32),
        pltpu.VMEM((HS, 1280, T), F32),
        pltpu.VMEM((HM - HS, 1280, T), F32),
        pltpu.VMEM((H - HM, 1280, T), F32),
        pltpu.VMEM((H, 112, T), F32),
        pltpu.VMEM((320, L), U32),
        pltpu.VMEM((D, L), F32),
        pltpu.VMEM((NSEG, 4, 16, T), F32),
        pltpu.VMEM((D // 2, S), U32),
        pltpu.VMEM((D, S), BF16),
        pltpu.VMEM((NSEG, 8, L), F32),
        pltpu.VMEM((T, T), F32),
        pltpu.VMEM((64, T), F32),
        pltpu.VMEM((2, H, T), F32),
        pltpu.VMEM((640, T), F32),
        pltpu.VMEM((NG, 160, T), F32),
        pltpu.VMEM((D, FF), BF16),
        pltpu.VMEM((D, FF), BF16),
        pltpu.VMEM((D, FF), BF16),
        pltpu.VMEM((H,), BF16),
        pltpu.VMEM((D,), BF16),
        pltpu.VMEM((16, D), BF16),
        pltpu.VMEM((16, D), BF16),
        pltpu.VMEM((8, T), F32),
        pltpu.VMEM((D, T), BF16),
        pltpu.SMEM((1,), jnp.int32),
        pltpu.SemaphoreType.DMA((4,)),
        pltpu.SemaphoreType.DMA((4,)),
        pltpu.SemaphoreType.DMA((3,)),
        pltpu.SemaphoreType.DMA((NSEG,)),
        pltpu.SemaphoreType.DMA((2,)),
    ]
    out_t = pl.pallas_call(
        _kernel,
        out_shape=jax.ShapeDtypeStruct((1, D, S), BF16),
        in_specs=[hbm] * 10,
        out_specs=hbm,
        scratch_shapes=scratch,
        compiler_params=pltpu.CompilerParams(vmem_limit_bytes=110 * 1024 * 1024),
        name="infini_moe",
    )(jnp.transpose(A_x, (0, 2, 1)), A_wq, A_wk, A_wv, A_wo, A_beta, B_w_r,
      B_w_gate, B_w_up, jnp.transpose(B_w_down, (1, 0)))
    return jnp.transpose(out_t, (0, 2, 1))
```

```python
import functools
import math

import jax
import jax.numpy as jnp
from jax import lax
import jax.experimental.pallas as pl
import jax.experimental.pallas.tpu as pltpu

F32 = jnp.float32
BF16 = jnp.bfloat16
U32 = jnp.uint32

S = 2048
D = 576
H = 32
DH = 18
NSEG = 4
L = 512
FF = 4608
T = 128
NG = 5
GH = (7, 7, 7, 7, 4)
VS = 20
EPS = 1e-5
QSCALE = DH ** (-0.5) * math.log2(math.e)
MASKVAL = -1000000000.0 * math.log2(math.e)
SOFF = (0, 128, 384, 768)
MOFF = (0, 2, 5, 9)
GWIN = tuple(((140 * g) // 16 * 16, -(-(140 * g + 20 * GH[g]) // 16) * 16) for g in range(NG))
QR = 592
FCH = (256,) * 18

HS = 16
HM = 25
HA1 = 9
NS0 = 16
TAIL = 16
KE = (VS * HS) // T * T
KM = (VS * HM) // T * T

NT = (((1,), (1,)), ((), ()))


def _bf(x_u32):
    return pltpu.bitcast(x_u32, BF16)


def _u32(x_bf):
    return pltpu.bitcast(x_bf, U32)


def _pack(y):
    return _u32(y.astype(BF16))


def _rb(x):
    return x.astype(BF16).astype(F32)


def _phi(t):
    return jnp.where(t > 0, t + 1.0, jnp.exp(t))


def _ln_scale(pivot, s1, s2):
    md = s1 * (1.0 / D)
    v = jnp.maximum(s2 * (1.0 / D) - md * md, 0.0)
    den = _rb(jnp.sqrt(_rb(_rb(v) + EPS)))
    return pivot + md, 1.0 / den


def _kernel(x_hbm, wq_hbm, wk_hbm, wv_hbm, wo_hbm, beta_hbm, wr_hbm, wg_hbm, wu_hbm, wd_hbm,
            out_hbm,
            x_v, w_v, wqkv, wot, xn, qt, pqt, kk, pkt, vt, memt, bd, s_a, s_b1, s_b2, m_blk,
            ot, att, ln_st, y_s, out_s, r_s, bias, bias2, gtab, ones_tab, keep_tab,
            wg_v, wu_v, wd_v, beta_v, wr_v, wr16, xs_v, best_v, fix_v,
            zero_s, sem_x, sem_w, sem_f, sem_o, sem_s):
    def x_copy(s):
        return pltpu.make_async_copy(x_hbm.at[0, :, pl.ds(s * L, L)], x_v.at[:, pl.ds(s * L, L)],
                                     sem_x.at[s])

    x_rest = pltpu.make_async_copy(x_hbm.at[0, :, pl.ds(2 * L, 2 * L)], x_v.at[:, pl.ds(2 * L, 2 * L)], sem_x.at[2])

    x0a = pltpu.make_async_copy(x_hbm.at[0, :, pl.ds(0, L // 2)], x_v.at[:, pl.ds(0, L // 2)], sem_x.at[0])
    x0b = pltpu.make_async_copy(x_hbm.at[0, :, pl.ds(L // 2, L // 2)], x_v.at[:, pl.ds(L // 2, L // 2)], sem_x.at[3])

    w_srcs = (wk_hbm, wq_hbm, wv_hbm, wo_hbm)

    def w_copy(i):
        return pltpu.make_async_copy(w_srcs[i], w_v.at[i], sem_w.at[i])

    f_pairs = ((wg_hbm, wg_v), (wu_hbm, wu_v), (wd_hbm, wd_v))

    def f_copy(i):
        return pltpu.make_async_copy(f_pairs[i][0], f_pairs[i][1], sem_f.at[i])

    def o_copy(s):
        return pltpu.make_async_copy(out_s.at[:, pl.ds(s * L, L)], out_hbm.at[0, :, pl.ds(s * L, L)],
                                     sem_o.at[s])

    beta_copy = pltpu.make_async_copy(beta_hbm, beta_v, sem_s.at[0])
    wr_copy = pltpu.make_async_copy(wr_hbm, wr_v, sem_s.at[1])

    def seg_cols(s, jt):
        if isinstance(s, int):
            return slice(s * L + jt * T, s * L + (jt + 1) * T)
        return pl.ds(pl.multiple_of(s * L + jt * T, T), T)

    def ln1_stats(s, jt):
        cols = seg_cols(s, jt)
        pivot = a1 = a2 = None
        for c in range(D // 32):
            x = x_v[32 * c:32 * (c + 1), cols].astype(F32)
            if c == 0:
                pivot = x[0:1, :]
            d = (x - pivot).reshape(4, 8, T)
            p1 = (d[0] + d[1]) + (d[2] + d[3])
            dd = d * d
            p2 = (dd[0] + dd[1]) + (dd[2] + dd[3])
            a1 = p1 if c == 0 else a1 + p1
            a2 = p2 if c == 0 else a2 + p2
        m, inv = _ln_scale(pivot, jnp.sum(a1, axis=0, keepdims=True), jnp.sum(a2, axis=0, keepdims=True))
        ln_st[s, jt, 0:1, :] = m
        ln_st[s, jt, 8:9, :] = inv

    def ln1_norm(s, jt):
        for c in range(NG):
            r0, r1 = T * c, min(T * (c + 1), D)
            x = x_v[r0:r1, seg_cols(s, jt)].astype(F32)
            xn[r0 // 2:r1 // 2, jt * T:(jt + 1) * T] = _u32(
                ((x - ln_st[s, jt, 0:1, :]) * ln_st[s, jt, 8:9, :]).astype(BF16))

    def q_unit(jt, g):
        cols = slice(jt * T, (jt + 1) * T)
        n = min(64, QR // 2 - 64 * g)
        q = jnp.dot(_bf(wqkv[64 * g:64 * g + n, :]), _bf(xn[:, cols]), preferred_element_type=F32)
        qt[g, 0:n, cols] = _pack(q * QSCALE)
        pqt[g, 0:n, cols] = _pack(_phi(q))

    def k_unit(jt, g):
        cols = slice(jt * T, (jt + 1) * T)
        n = min(64, QR // 2 - 64 * g)
        b0 = QR // 2 + 64 * g
        k = jnp.dot(_bf(wqkv[b0:b0 + n, :]), _bf(xn[:, cols]), preferred_element_type=F32)
        pkt[g, 0:n, cols] = _pack(_phi(k))
        kb = _pack(k)
        if n < 64:
            kb = jnp.concatenate([kb, jnp.zeros((64 - n, T), U32)], axis=0)
        kk[g, jt * 64:(jt + 1) * 64, :] = _u32(_bf(kb).T)

    def v_unit(jt, c):
        cols = slice(jt * T, (jt + 1) * T)
        b0 = QR + 64 * c
        v = jnp.dot(_bf(wqkv[b0:b0 + 64, :]), _bf(xn[:, cols]), preferred_element_type=F32)
        vt[64 * c:64 * (c + 1), cols] = _pack(v + ones_tab[T * c:T * (c + 1), :])

    def mem_read_unit(g):
        w0, w1 = GWIN[g]
        b = bd[g, 0:w1 - w0, :].astype(BF16)
        res = jnp.dot(b, _bf(pqt[g]), preferred_element_type=F32)
        lo, hi = 140 * g, 140 * g + 20 * GH[g]
        memt[lo:hi, :] = res[lo - w0:hi - w0]

    def mem_update_unit(g):
        w0, w1 = GWIN[g]
        upd = lax.dot_general(_bf(vt[w0 // 2:w1 // 2, :]), _bf(pkt[g]), NT, preferred_element_type=F32)
        n = w1 - w0
        bd[g, 0:n, :] = bd[g, 0:n, :] + jnp.where(keep_tab[g, 0:n, :] > 0.5, upd, 0.0)

    def sbuf(h):
        if h < HS:
            return s_a, h
        return (s_b1, h - HS) if h < HM else (s_b2, h - HM)

    def put_scores(h, off, sc):
        sb, hi_ = sbuf(h)
        n = sc.shape[0]
        if h < HS:
            sb[hi_, off:off + n, :] = sc
        else:
            keep = lax.broadcasted_iota(jnp.int32, (n, T), 1) >= zero_s[0]
            pltpu.store(sb.at[hi_, off:off + n, :], sc, mask=keep)

    def head_rows(j):
        r = lax.broadcasted_iota(jnp.int32, (64, T), 0)
        return (r >= 9 * j) & (r < 9 * j + 9)

    def s_blk(h, jq, kb, half=False):
        g, j = divmod(h, 7)
        off = SOFF[jq] + kb * T
        n = 64 if half else T
        qm = _bf(jnp.where(head_rows(j), qt[g, :, jq * T:(jq + 1) * T], U32(0)))
        sc = jnp.dot(_bf(kk[g, kb * 64:kb * 64 + n // 2, :]), qm, preferred_element_type=F32)
        if kb == jq:
            sc = sc + bias[0:n, :]
        put_scores(h, off, sc)
        slot = MOFF[jq] + kb
        m_blk[h, slot * 8:(slot + 1) * 8, :] = jnp.max(sc.reshape(n // 8, 8, T), axis=0)

    def s_pair(ha, jq):
        g, j = divmod(ha, 7)
        off = SOFF[jq] + jq * T + 64
        lo = lax.broadcasted_iota(jnp.int32, (64, T), 1) < 64
        qu = qt[g, :, jq * T:(jq + 1) * T]
        qmix = jnp.where(lo, pltpu.roll(qu, 64, 1), qu)
        qm = _bf(jnp.where((lo & head_rows(j)) | (~lo & head_rows(j + 1)), qmix, U32(0)))
        sc = jnp.dot(_bf(kk[g, jq * 64 + 32:jq * 64 + 64, :]), qm, preferred_element_type=F32) + bias2[...]
        put_scores(ha, off, sc)
        pm = jnp.max(sc.reshape(8, 8, T), axis=0)
        hi = lax.broadcasted_iota(jnp.int32, (8, T), 1) >= 64
        slot = MOFF[jq] + jq + 1
        m_blk[ha, slot * 8:(slot + 1) * 8, :] = jnp.where(hi, pltpu.roll(pm, 64, 1), -jnp.inf)
        m_blk[ha + 1, slot * 8:(slot + 1) * 8, :] = jnp.where(hi, pm, -jnp.inf)

    def row_max(h, jq, nslots):
        return jnp.max(m_blk[h, MOFF[jq] * 8:(MOFF[jq] + nslots) * 8, :], axis=0, keepdims=True)

    def pv_blk(h, jq, kb, st, role):
        w0 = (VS * h) // 16 * 16
        o = VS * h - w0
        off = SOFF[jq] + kb * T
        cols = slice(jq * T, (jq + 1) * T)
        key = role or 'a'
        sb, hz = sbuf(h)
        if kb == 0 and role != 'b':
            st['ma'] = row_max(h, jq, jq + 1 if role is None else jq + 2)
            if role == 'a':
                st['mb'] = row_max(h + 1, jq, jq + 2)
        m = st['m' + key]
        if kb < jq or role is None:
            p = jnp.exp2(sb[hz, off:off + T, :] - m).astype(BF16)
        else:
            if role == 'a':
                hi1 = lax.broadcasted_iota(jnp.int32, (1, T), 1) >= 64
                hi = lax.broadcasted_iota(jnp.int32, (64, T), 1) >= 64
                m2 = jnp.where(hi1, st['mb'], pltpu.roll(st['ma'], 64, 1))
                e2 = jnp.exp2(sb[hz, off + 64:off + T, :] - m2)
                p2 = jnp.where(hi, pltpu.roll(e2, 64, 1), 0.0)
                st['p2b'] = jnp.where(hi, e2, 0.0)
            else:
                p2 = st['p2b']
            p1 = jnp.exp2(sb[hz, off:off + 64, :] - m)
            p = jnp.concatenate([p1, p2], axis=0).astype(BF16)
        part = jnp.dot(_bf(vt[w0 // 2:w0 // 2 + 16, kb * T:(kb + 1) * T]), p, preferred_element_type=F32)
        st['pv' + key] = part if kb == 0 else st['pv' + key] + part
        if kb == jq:
            pv = st['pv' + key]
            res = pv * (gtab[1, h:h + 1, :] / pv[o + DH:o + DH + 1, :])
            mem = memt[w0:w0 + 32, cols]
            res = res + mem * (gtab[0, h:h + 1, :] / (mem[o + DH:o + DH + 1, :] + 1e-6))
            ot[VS * h // 2:VS * h // 2 + VS // 2, cols] = _u32(res.astype(BF16))[o // 2:o // 2 + VS // 2]

    def o_early(s, jt, c, ke):
        r0, r1 = T * c, min(T * (c + 1), D)
        tile = slice(jt * T, (jt + 1) * T)
        a = jnp.dot(_bf(wot[r0 // 2:r1 // 2, 0:ke]), _bf(ot[0:ke // 2, tile]), preferred_element_type=F32)
        att[r0:r1, tile] = x_v[r0:r1, seg_cols(s, jt)].astype(F32) + a

    def o_unit(s, jt, c, ke, st):
        r0, r1 = T * c, min(T * (c + 1), D)
        tile = slice(jt * T, (jt + 1) * T)
        a = jnp.dot(_bf(wot[r0 // 2:r1 // 2, ke:640]), _bf(ot[ke // 2:320, tile]), preferred_element_type=F32)
        hh = att[r0:r1, tile] + a
        att[r0:r1, tile] = hh
        if c == 0:
            st['p'] = hh[0:1, :]
        d = hh - st['p']
        s1 = jnp.sum(d, axis=0, keepdims=True)
        s2 = jnp.sum(d * d, axis=0, keepdims=True)
        st['s1'] = s1 if c == 0 else st['s1'] + s1
        st['s2'] = s2 if c == 0 else st['s2'] + s2

    def e2_unit(s, jt, c, st):
        r0, r1 = T * c, min(T * (c + 1), D)
        cols = seg_cols(s, jt)
        if c == 0:
            st['m'], st['inv'] = _ln_scale(st['p'], st['s1'], st['s2'])
        hh = att[r0:r1, jt * T:(jt + 1) * T]
        y = (hh - st['m']) * st['inv']
        n = (r1 - r0) // 2
        cand = st.get('cand')
        if cand is None:
            y_s[r0 // 2:r1 // 2, cols] = pltpu.pack_elementwise([y[0:n], y[n:2 * n]], packed_dtype=BF16)
        out_s[r0:r1, cols] = (hh + y).astype(BF16)
        yb = y.astype(BF16)
        rr = jnp.dot(wr16[:, r0:r1], yb, preferred_element_type=F32)
        st['r'] = rr if c == 0 else st['r'] + rr
        if cand is not None:
            cand.setdefault(jt, {'y': []})['y'].append(yb)
        if r1 == D:
            rrow = _rb(st['r'][0:1, :])
            if cand is None:
                r_s[s, :, jt * T:(jt + 1) * T] = jnp.broadcast_to(rrow, (8, T))
            else:
                cand[jt]['r'] = rrow

    def offer_last(best, cand):
        rrow = jnp.concatenate([cand[jt]['r'] for jt in range(4)], axis=1)
        tmax = jnp.max(rrow, axis=1, keepdims=True)
        lane = lax.broadcasted_iota(jnp.int32, (1, L), 1)
        lane_c = jnp.min(jnp.where(rrow == tmax, lane, L), axis=1, keepdims=True)
        xs = None
        for jt in range(4):
            oh = (lax.broadcasted_iota(jnp.int32, (16, T), 1) == lane_c - jt * T).astype(BF16)
            part = jnp.concatenate([lax.dot_general(oh, yc, NT, preferred_element_type=F32)
                                    for yc in cand[jt]['y']], axis=1)
            xs = part if xs is None else xs + part
        take = tmax > best['r']
        best.update(r=jnp.where(take, tmax, best['r']),
                    tok=jnp.where(take, (NSEG - 1) * L + lane_c, best['tok']),
                    xs=jnp.where(take, xs, best['xs']))

    def prep_qk(i, base):
        wt = _u32(w_v[i].T)
        for g in range(NG):
            n = 9 * GH[g]
            wqkv[base + 64 * g:base + 64 * g + n, :] = wt[63 * g:63 * g + n, :]

    def prep_v():
        wt = _u32(w_v[2].T)
        for h in range(H):
            wqkv[QR + 10 * h:QR + 10 * h + 9, :] = wt[9 * h:9 * h + 9, :]

    def prep_o():
        wt = _u32(w_v[3])
        wpad = jnp.concatenate(
            [piece for h in range(H) for piece in (wt[9 * h:9 * h + 9, :], jnp.zeros((1, D), U32))], axis=0)
        wot[...] = _u32(_bf(wpad).T)

    BLKS = [(jq, kb) for jq in range(4) for kb in range(jq + 1)]

    def head_sets(heads):
        sets, i = [], 0
        while i < len(heads):
            h = heads[i]
            if h % 7 % 2 == 0 and h % 7 < 6 and i + 1 < len(heads):
                sets.append((h, h + 1))
                i += 2
            else:
                assert h % 7 == 6
                sets.append((h,))
                i += 1
        return sets

    def s_items(heads, small_tail=0):
        big, small = [], []
        for hs in head_sets(heads):
            for jq, kb in BLKS:
                halved = len(hs) == 2 and kb == jq
                for h in hs:
                    (small if halved else big).append(functools.partial(s_blk, h, jq, kb, halved))
                if halved:
                    small.append(functools.partial(s_pair, hs[0], jq))
        tail = small[len(small) - small_tail:] if small_tail else []
        small = small[:len(small) - small_tail] if small_tail else small
        order = sorted([((j + 0.5) / len(big), 0, j) for j in range(len(big))]
                       + [((j + 0.5) / len(small), 1, j) for j in range(len(small))])
        return [(big, small)[w][j] for _, w, j in order] + tail

    def phase_x():
        sb = s_items(HB)
        for it in sb[0:NS0]:
            it()
        interleave(pv_items(HA), sb[NS0:])

    def pv_items(heads, z=0):
        items = []
        for hs in head_sets(heads):
            st = {'z': z}
            roles = ('a', 'b') if len(hs) == 2 else (None,)
            for jq, kb in BLKS:
                for h, role in zip(hs, roles):
                    items.append(functools.partial(pv_blk, h, jq, kb, st, role))
        return items

    def interleave(*seqs):
        seqs = [q for q in seqs if q]
        order = []
        for i, q in enumerate(seqs):
            order += [((j + 0.5) / len(q), i, j) for j in range(len(q))]
        for _, i, j in sorted(order):
            seqs[i][j]()

    def proj_items(fn):
        return [functools.partial(fn, jt, g) for jt in range(4) for g in range(NG)]

    def out_items(s, ke, cand=None):
        sts = [{'cand': cand} for _ in range(4)]
        o_items = [functools.partial(o_unit, s, jt, c, ke, sts[jt]) for jt in range(4) for c in range(NG)]
        e_items = [functools.partial(e2_unit, s, jt, c, sts[jt]) for jt in range(4) for c in range(NG)]
        early = [functools.partial(o_early, s, jt, c, ke) for jt in range(4) for c in range(NG)]
        return early, o_items, e_items

    HA = list(range(HS))
    HB = list(range(HS, H))

    x0a.start()
    w_copy(1).start()
    x0b.start()
    zero_s[0] = 0
    beta_copy.start()
    wr_copy.start()
    kr = lax.broadcasted_iota(jnp.int32, (T, T), 0)
    qc = lax.broadcasted_iota(jnp.int32, (T, T), 1)
    bias[...] = jnp.where(kr > qc, MASKVAL, 0.0).astype(F32)
    kr2 = lax.broadcasted_iota(jnp.int32, (64, T), 0)
    qc2 = lax.broadcasted_iota(jnp.int32, (64, T), 1)
    bias2[...] = jnp.where(kr2 > (qc2 & 63), MASKVAL, 0.0).astype(F32)
    wqkv[...] = jnp.zeros(wqkv.shape, U32)
    bd[...] = jnp.zeros(bd.shape, F32)
    memt[...] = jnp.zeros(memt.shape, F32)
    row = lax.broadcasted_iota(jnp.int32, (640, T), 0)
    ones_tab[...] = jnp.where(row % VS == DH, 1.0, 0.0).astype(F32)
    for g in range(NG):
        row = lax.broadcasted_iota(jnp.int32, (160, T), 0) + (GWIN[g][0] - 140 * g)
        lane = lax.broadcasted_iota(jnp.int32, (160, T), 1)
        keep = ((row >= 0) & (row < 20 * GH[g]) & (lane >= (row // VS) * DH)
                & (lane < (row // VS) * DH + DH))
        keep_tab[g] = jnp.where(keep, 1.0, 0.0).astype(F32)
    qt[NG - 1] = jnp.zeros(qt.shape[1:], U32)
    pqt[NG - 1] = jnp.zeros(pqt.shape[1:], U32)
    pkt[NG - 1] = jnp.zeros(pkt.shape[1:], U32)

    x0a.wait()
    w_copy(0).start()
    for jt in range(2):
        ln1_stats(0, jt)
        ln1_norm(0, jt)
    w_copy(1).wait()
    w_copy(2).start()
    prep_qk(1, 0)
    for g in range(NG):
        for jt in range(2):
            q_unit(jt, g)
    w_copy(0).wait()
    x0b.wait()
    x_copy(1).start()
    for jt in range(2, 4):
        ln1_stats(0, jt)
        ln1_norm(0, jt)
    prep_qk(0, QR // 2)
    for jt in range(2, 4):
        for g in range(NG):
            q_unit(jt, g)
    w_copy(2).wait()
    x_rest.start()
    w_copy(3).start()
    prep_v()
    for jt in range(4):
        for g in range(NG):
            k_unit(jt, g)
    beta_copy.wait()
    wr_copy.wait()
    x_copy(1).wait()
    beta = beta_v[...].astype(F32).reshape(1, H)
    hl = lax.broadcasted_iota(jnp.int32, (H, H), 1)
    hs = lax.broadcasted_iota(jnp.int32, (H, H), 0)
    bcol = jnp.sum(jnp.where(hl == hs, jnp.broadcast_to(beta, (H, H)), 0.0), axis=1, keepdims=True)
    gate = _rb(jax.nn.sigmoid(bcol))
    gtab[0] = jnp.broadcast_to(gate, (H, T))
    gtab[1] = jnp.broadcast_to(_rb(1.0 - gate), (H, T))
    r16 = lax.broadcasted_iota(jnp.int32, (16, D), 0)
    wr_row = wr_v[...].astype(F32).reshape(1, D)
    wr16[...] = jnp.where(r16 == 0, jnp.broadcast_to(wr_row, (16, D)), 0.0).astype(BF16)
    interleave(proj_items(v_unit) + s_items(HA, TAIL),
               [functools.partial(ln1_stats, 1, jt) for jt in range(4)])
    x_rest.wait()
    w_copy(3).wait()
    for i in range(2, NSEG):
        for jt in range(4):
            ln1_stats(i, jt)

    def seg_body(s, carry):
        z = zero_s[0]
        prep_o()
        phase_x()
        ln = [functools.partial(ln1_norm, s + 1, jt) for jt in range(4)]
        qs = proj_items(q_unit)
        early, o_items, e_items = out_items(s, KE)
        upd = [functools.partial(mem_update_unit, g) for g in range(NG)]
        ks = proj_items(k_unit)
        pre = [ln[0]] + early[0:8] + [ln[1]]
        mxu1 = early[8:14] + [ln[2]] + upd + qs[0:5] + early[14:20] + [ln[3]] + qs[5:20] + ks
        for it in pre:
            it()
        interleave(pv_items(HB, z), mxu1)
        vr = proj_items(v_unit) + [functools.partial(mem_read_unit, g) for g in range(NG)]
        for it in o_items:
            it()
        interleave(vr, e_items)
        for it in s_items(HA, TAIL):
            it()
        o_copy(s).start()

        @pl.when(s == 0)
        def _():
            f_copy(0).start()
            f_copy(1).start()

        @pl.when(s == 1)
        def _():
            f_copy(2).start()
        return carry

    lax.fori_loop(0, NSEG - 1, seg_body, 0)

    for i in range(3):
        f_copy(i).wait()
    z = zero_s[0]
    best = {}

    def offer_previous():
        n = (NSEG - 1) * 8
        r_all = r_s[0:NSEG - 1].reshape(n, L)
        tok = ((lax.broadcasted_iota(jnp.int32, (n, L), 0) // 8) * L
               + lax.broadcasted_iota(jnp.int32, (n, L), 1))
        rmax = jnp.max(jnp.max(r_all, axis=1, keepdims=True), axis=0, keepdims=True)
        idx = jnp.clip(jnp.min(jnp.where(r_all == rmax, tok, S)), 0, S - 1)
        base = pl.multiple_of((idx // T) * T, T)
        onehot = (lax.broadcasted_iota(jnp.int32, (16, T), 1) == idx - base).astype(BF16)
        yw = y_s[:, pl.ds(base, T)]
        pieces = []
        for c in range(NG):
            w0, w1 = 64 * c, min(64 * (c + 1), D // 2)
            n2 = w1 - w0
            xp = lax.dot_general(onehot, _bf(yw[w0:w1]), NT, preferred_element_type=F32)
            rr = lax.broadcasted_iota(jnp.int32, (2 * n2, 2 * n2), 0)
            cc = lax.broadcasted_iota(jnp.int32, (2 * n2, 2 * n2), 1)
            unmix = (rr == jnp.where(cc < n2, 2 * cc, 2 * (cc - n2) + 1)).astype(BF16)
            pieces.append(jnp.dot(xp.astype(BF16), unmix, preferred_element_type=F32))
        best.update(r=rmax, tok=jnp.full((1, 1), idx, jnp.int32), xs=jnp.concatenate(pieces, axis=1))

    ha1, ha2 = HA[:HA1], HA[HA1:]
    hb1, hb2 = list(range(HS, HM)), list(range(HM, H))
    sb1 = s_items(hb1)
    for it in sb1[0:NS0]:
        it()
    interleave(pv_items(ha1), sb1[NS0:])
    offer_previous()
    sb2 = s_items(hb2)
    interleave(pv_items(ha2) + pv_items(hb1, z), sb2)
    cand = {}
    early, o_items, e_items = out_items(NSEG - 1, KM, cand)
    for it in early[0:4]:
        it()
    interleave(pv_items(hb2, z), early[4:])
    for jt in range(4):
        for it in o_items[jt * NG:(jt + 1) * NG]:
            it()
        if jt > 0:
            for it in e_items[(jt - 1) * NG:jt * NG]:
                it()
    for it in e_items[3 * NG:]:
        it()
    offer_last(best, cand)
    o_copy(NSEG - 1).start()

    xs_v[...] = best['xs'].astype(BF16)
    best_v[...] = jnp.broadcast_to(best['r'], (8, T))
    idx = jnp.clip(jnp.max(best['tok']), 0, S - 1)
    base = pl.multiple_of((idx // T) * T, T)
    tile = pl.ds(base, T)

    @pl.when(zero_s[0] == 0)
    def _ffn():
        xs = xs_v[...]
        acc = None
        f0 = 0
        for fw in FCH:
            fc = slice(f0, f0 + fw)
            gt = _rb(jnp.dot(xs, wg_v[:, fc], preferred_element_type=F32))
            up = _rb(jnp.dot(xs, wu_v[:, fc], preferred_element_type=F32))
            act = _rb(_rb(gt * jax.nn.sigmoid(gt)) * up)[0:1, :]
            for t in range(fw // T):
                a = act[:, t * T:(t + 1) * T]
                term = wd_v[:, f0 + t * T:f0 + (t + 1) * T].astype(F32) * a
                acc = term if acc is None else acc + term
            f0 += fw
        ycol = _rb(jnp.sum(acc, axis=1, keepdims=True))
        ycol = _rb(ycol * _rb(jax.nn.sigmoid(best_v[0:1, 0:1])))
        sel = lax.broadcasted_iota(jnp.int32, (D, T), 1) == idx - base
        old = out_s[:, tile].astype(F32)
        fix_v[...] = jnp.where(sel, old + ycol, old).astype(BF16)

    for s in range(NSEG):
        o_copy(s).wait()
    fix = pltpu.make_async_copy(fix_v, out_hbm.at[0, :, tile], sem_o.at[0])
    fix.start()
    fix.wait()


@jax.jit
def pallas_sequential_preLN__memory_aug_infini_attn__moe_arch_mod__prompt_kernel(
    A_x: jax.Array,
    A_wq: jax.Array,
    A_wk: jax.Array,
    A_wv: jax.Array,
    A_wo: jax.Array,
    A_beta: jax.Array,
    B_x: jax.Array,
    B_w_r: jax.Array,
    B_w_gate: jax.Array,
    B_w_up: jax.Array,
    B_w_down: jax.Array,
):
    del B_x
    hbm = pl.BlockSpec(memory_space=pltpu.HBM)
    scratch = [
        pltpu.VMEM((D, S), BF16),
        pltpu.VMEM((4, D, D), BF16),
        pltpu.VMEM((QR + 320, D), U32),
        pltpu.VMEM((D // 2, 640), U32),
        pltpu.VMEM((D // 2, L), U32),
        pltpu.VMEM((NG, 64, L), U32),
        pltpu.VMEM((NG, 64, L), U32),
        pltpu.VMEM((NG, L // 2, T), U32),
        pltpu.VMEM((NG, 64, L), U32),
        pltpu.VMEM((320, L), U32),
        pltpu.VMEM((640, L), F32),
        pltpu.VMEM((NG, 160, T), F32),
        pltpu.VMEM((HS, 1280, T), F32),
        pltpu.VMEM((HM - HS, 1280, T), F32),
        pltpu.VMEM((H - HM, 1280, T), F32),
        pltpu.VMEM((H, 112, T), F32),
        pltpu.VMEM((320, L), U32),
        pltpu.VMEM((D, L), F32),
        pltpu.VMEM((NSEG, 4, 16, T), F32),
        pltpu.VMEM((D // 2, S), U32),
        pltpu.VMEM((D, S), BF16),
        pltpu.VMEM((NSEG, 8, L), F32),
        pltpu.VMEM((T, T), F32),
        pltpu.VMEM((64, T), F32),
        pltpu.VMEM((2, H, T), F32),
        pltpu.VMEM((640, T), F32),
        pltpu.VMEM((NG, 160, T), F32),
        pltpu.VMEM((D, FF), BF16),
        pltpu.VMEM((D, FF), BF16),
        pltpu.VMEM((D, FF), BF16),
        pltpu.VMEM((H,), BF16),
        pltpu.VMEM((D,), BF16),
        pltpu.VMEM((16, D), BF16),
        pltpu.VMEM((16, D), BF16),
        pltpu.VMEM((8, T), F32),
        pltpu.VMEM((D, T), BF16),
        pltpu.SMEM((1,), jnp.int32),
        pltpu.SemaphoreType.DMA((4,)),
        pltpu.SemaphoreType.DMA((4,)),
        pltpu.SemaphoreType.DMA((3,)),
        pltpu.SemaphoreType.DMA((NSEG,)),
        pltpu.SemaphoreType.DMA((2,)),
    ]
    out_t = pl.pallas_call(
        _kernel,
        out_shape=jax.ShapeDtypeStruct((1, D, S), BF16),
        in_specs=[hbm] * 10,
        out_specs=hbm,
        scratch_shapes=scratch,
        compiler_params=pltpu.CompilerParams(vmem_limit_bytes=110 * 1024 * 1024),
        name="infini_moe",
    )(jnp.transpose(A_x, (0, 2, 1)), A_wq, A_wk, A_wv, A_wo, A_beta, B_w_r,
      B_w_gate, B_w_up, jnp.transpose(B_w_down, (1, 0)))
    return jnp.transpose(out_t, (0, 2, 1))
```

```python
import functools
import math

import jax
import jax.numpy as jnp
from jax import lax
import jax.experimental.pallas as pl
import jax.experimental.pallas.tpu as pltpu

F32 = jnp.float32
BF16 = jnp.bfloat16
U32 = jnp.uint32

S = 2048
D = 576
H = 32
DH = 18
NSEG = 4
L = 512
FF = 4608
T = 128
NG = 5
GH = (7, 7, 7, 7, 4)
VS = 20
EPS = 1e-5
QSCALE = DH ** (-0.5) * math.log2(math.e)
MASKVAL = -1000000000.0 * math.log2(math.e)
SOFF = (0, 128, 384, 768)
MOFF = (0, 2, 5, 9)
GWIN = tuple(((140 * g) // 16 * 16, -(-(140 * g + 20 * GH[g]) // 16) * 16) for g in range(NG))
QR = 592
FCH = (256,) * 18

HS = 16
HM = 25
HA1 = 9
NS0 = 16
TAIL = 16
KE = (VS * HS) // T * T
KM = (VS * HM) // T * T

NT = (((1,), (1,)), ((), ()))


def _bf(x_u32):
    return pltpu.bitcast(x_u32, BF16)


def _u32(x_bf):
    return pltpu.bitcast(x_bf, U32)


def _pack(y):
    return _u32(y.astype(BF16))


def _rb(x):
    return x.astype(BF16).astype(F32)


def _phi(t):
    return jnp.where(t > 0, t + 1.0, jnp.exp(t))


def _ln_scale(pivot, s1, s2):
    md = s1 * (1.0 / D)
    v = jnp.maximum(s2 * (1.0 / D) - md * md, 0.0)
    den = _rb(jnp.sqrt(_rb(_rb(v) + EPS)))
    return pivot + md, 1.0 / den


def _kernel(x_hbm, wq_hbm, wk_hbm, wv_hbm, wo_hbm, beta_hbm, wr_hbm, wg_hbm, wu_hbm, wd_hbm,
            out_hbm,
            x_v, w_v, wqkv, wot, xn, qt, pqt, kk, pkt, vt, memt, bd, s_a, s_b1, s_b2, m_blk,
            ot, att, ln_st, y_s, out_s, r_s, bias, bias2, gtab, ones_tab, keep_tab,
            wg_v, wu_v, wd_v, beta_v, wr_v, wr16, xs_v, best_v, fix_v,
            zero_s, sem_x, sem_w, sem_f, sem_o, sem_s):
    def x_copy(s):
        return pltpu.make_async_copy(x_hbm.at[0, :, pl.ds(s * L, L)], x_v.at[:, pl.ds(s * L, L)],
                                     sem_x.at[s])

    x_rest = pltpu.make_async_copy(x_hbm.at[0, :, pl.ds(2 * L, 2 * L)], x_v.at[:, pl.ds(2 * L, 2 * L)], sem_x.at[2])

    x0a = pltpu.make_async_copy(x_hbm.at[0, :, pl.ds(0, L // 2)], x_v.at[:, pl.ds(0, L // 2)], sem_x.at[0])
    x0b = pltpu.make_async_copy(x_hbm.at[0, :, pl.ds(L // 2, L // 2)], x_v.at[:, pl.ds(L // 2, L // 2)], sem_x.at[3])

    w_srcs = (wk_hbm, wq_hbm, wv_hbm, wo_hbm)

    def w_copy(i):
        return pltpu.make_async_copy(w_srcs[i], w_v.at[i], sem_w.at[i])

    f_pairs = ((wg_hbm, wg_v), (wu_hbm, wu_v), (wd_hbm, wd_v))

    def f_copy(i):
        return pltpu.make_async_copy(f_pairs[i][0], f_pairs[i][1], sem_f.at[i])

    def o_copy(s):
        return pltpu.make_async_copy(out_s.at[:, pl.ds(s * L, L)], out_hbm.at[0, :, pl.ds(s * L, L)],
                                     sem_o.at[s])

    beta_copy = pltpu.make_async_copy(beta_hbm, beta_v, sem_s.at[0])
    wr_copy = pltpu.make_async_copy(wr_hbm, wr_v, sem_s.at[1])

    def seg_cols(s, jt):
        if isinstance(s, int):
            return slice(s * L + jt * T, s * L + (jt + 1) * T)
        return pl.ds(pl.multiple_of(s * L + jt * T, T), T)

    def ln1_stats(s, jt):
        cols = seg_cols(s, jt)
        pivot = a1 = a2 = None
        for c in range(D // 32):
            x = x_v[32 * c:32 * (c + 1), cols].astype(F32)
            if c == 0:
                pivot = x[0:1, :]
            d = (x - pivot).reshape(4, 8, T)
            p1 = (d[0] + d[1]) + (d[2] + d[3])
            dd = d * d
            p2 = (dd[0] + dd[1]) + (dd[2] + dd[3])
            a1 = p1 if c == 0 else a1 + p1
            a2 = p2 if c == 0 else a2 + p2
        m, inv = _ln_scale(pivot, jnp.sum(a1, axis=0, keepdims=True), jnp.sum(a2, axis=0, keepdims=True))
        ln_st[s, jt, 0:1, :] = m
        ln_st[s, jt, 8:9, :] = inv

    def ln1_norm(s, jt):
        for c in range(NG):
            r0, r1 = T * c, min(T * (c + 1), D)
            x = x_v[r0:r1, seg_cols(s, jt)].astype(F32)
            xn[r0 // 2:r1 // 2, jt * T:(jt + 1) * T] = _u32(
                ((x - ln_st[s, jt, 0:1, :]) * ln_st[s, jt, 8:9, :]).astype(BF16))

    def q_unit(jt, g):
        cols = slice(jt * T, (jt + 1) * T)
        n = min(64, QR // 2 - 64 * g)
        q = jnp.dot(_bf(wqkv[64 * g:64 * g + n, :]), _bf(xn[:, cols]), preferred_element_type=F32)
        qt[g, 0:n, cols] = _pack(q * QSCALE)
        pqt[g, 0:n, cols] = _pack(_phi(q))

    def k_unit(jt, g):
        cols = slice(jt * T, (jt + 1) * T)
        n = min(64, QR // 2 - 64 * g)
        b0 = QR // 2 + 64 * g
        k = jnp.dot(_bf(wqkv[b0:b0 + n, :]), _bf(xn[:, cols]), preferred_element_type=F32)
        pkt[g, 0:n, cols] = _pack(_phi(k))
        kb = _pack(k)
        if n < 64:
            kb = jnp.concatenate([kb, jnp.zeros((64 - n, T), U32)], axis=0)
        kk[g, jt * 64:(jt + 1) * 64, :] = _u32(_bf(kb).T)

    def v_unit(jt, c):
        cols = slice(jt * T, (jt + 1) * T)
        b0 = QR + 64 * c
        v = jnp.dot(_bf(wqkv[b0:b0 + 64, :]), _bf(xn[:, cols]), preferred_element_type=F32)
        vt[64 * c:64 * (c + 1), cols] = _pack(v + ones_tab[T * c:T * (c + 1), :])

    def mem_read_unit(g):
        w0, w1 = GWIN[g]
        b = bd[g, 0:w1 - w0, :].astype(BF16)
        res = jnp.dot(b, _bf(pqt[g]), preferred_element_type=F32)
        lo, hi = 140 * g, 140 * g + 20 * GH[g]
        memt[lo:hi, :] = res[lo - w0:hi - w0]

    def mem_update_unit(g):
        w0, w1 = GWIN[g]
        upd = lax.dot_general(_bf(vt[w0 // 2:w1 // 2, :]), _bf(pkt[g]), NT, preferred_element_type=F32)
        n = w1 - w0
        bd[g, 0:n, :] = bd[g, 0:n, :] + jnp.where(keep_tab[g, 0:n, :] > 0.5, upd, 0.0)

    def sbuf(h):
        if h < HS:
            return s_a, h
        return (s_b1, h - HS) if h < HM else (s_b2, h - HM)

    def put_scores(h, off, sc):
        sb, hi_ = sbuf(h)
        n = sc.shape[0]
        if h < HS:
            sb[hi_, off:off + n, :] = sc
        else:
            keep = lax.broadcasted_iota(jnp.int32, (n, T), 1) >= zero_s[0]
            pltpu.store(sb.at[hi_, off:off + n, :], sc, mask=keep)

    def head_rows(j):
        r = lax.broadcasted_iota(jnp.int32, (64, T), 0)
        return (r >= 9 * j) & (r < 9 * j + 9)

    def s_blk(h, jq, kb, half=False):
        g, j = divmod(h, 7)
        off = SOFF[jq] + kb * T
        n = 64 if half else T
        qm = _bf(jnp.where(head_rows(j), qt[g, :, jq * T:(jq + 1) * T], U32(0)))
        sc = jnp.dot(_bf(kk[g, kb * 64:kb * 64 + n // 2, :]), qm, preferred_element_type=F32)
        if kb == jq:
            sc = sc + bias[0:n, :]
        put_scores(h, off, sc)
        slot = MOFF[jq] + kb
        m_blk[h, slot * 8:(slot + 1) * 8, :] = jnp.max(sc.reshape(n // 8, 8, T), axis=0)

    def s_pair(ha, jq):
        g, j = divmod(ha, 7)
        off = SOFF[jq] + jq * T + 64
        lo = lax.broadcasted_iota(jnp.int32, (64, T), 1) < 64
        qu = qt[g, :, jq * T:(jq + 1) * T]
        qmix = jnp.where(lo, pltpu.roll(qu, 64, 1), qu)
        qm = _bf(jnp.where((lo & head_rows(j)) | (~lo & head_rows(j + 1)), qmix, U32(0)))
        sc = jnp.dot(_bf(kk[g, jq * 64 + 32:jq * 64 + 64, :]), qm, preferred_element_type=F32) + bias2[...]
        put_scores(ha, off, sc)
        pm = jnp.max(sc.reshape(8, 8, T), axis=0)
        hi = lax.broadcasted_iota(jnp.int32, (8, T), 1) >= 64
        slot = MOFF[jq] + jq + 1
        m_blk[ha, slot * 8:(slot + 1) * 8, :] = jnp.where(hi, pltpu.roll(pm, 64, 1), -jnp.inf)
        m_blk[ha + 1, slot * 8:(slot + 1) * 8, :] = jnp.where(hi, pm, -jnp.inf)

    def row_max(h, jq, nslots):
        return jnp.max(m_blk[h, MOFF[jq] * 8:(MOFF[jq] + nslots) * 8, :], axis=0, keepdims=True)

    def pv_blk(h, jq, kb, st, role):
        w0 = (VS * h) // 16 * 16
        o = VS * h - w0
        off = SOFF[jq] + kb * T
        cols = slice(jq * T, (jq + 1) * T)
        key = role or 'a'
        sb, hz = sbuf(h)
        if kb == 0 and role != 'b':
            st['ma'] = row_max(h, jq, jq + 1 if role is None else jq + 2)
            if role == 'a':
                st['mb'] = row_max(h + 1, jq, jq + 2)
        m = st['m' + key]
        if kb < jq or role is None:
            p = jnp.exp2(sb[hz, off:off + T, :] - m).astype(BF16)
        else:
            if role == 'a':
                hi1 = lax.broadcasted_iota(jnp.int32, (1, T), 1) >= 64
                hi = lax.broadcasted_iota(jnp.int32, (64, T), 1) >= 64
                m2 = jnp.where(hi1, st['mb'], pltpu.roll(st['ma'], 64, 1))
                e2 = jnp.exp2(sb[hz, off + 64:off + T, :] - m2)
                p2 = jnp.where(hi, pltpu.roll(e2, 64, 1), 0.0)
                st['p2b'] = jnp.where(hi, e2, 0.0)
            else:
                p2 = st['p2b']
            p1 = jnp.exp2(sb[hz, off:off + 64, :] - m)
            p = jnp.concatenate([p1, p2], axis=0).astype(BF16)
        part = jnp.dot(_bf(vt[w0 // 2:w0 // 2 + 16, kb * T:(kb + 1) * T]), p, preferred_element_type=F32)
        st['pv' + key] = part if kb == 0 else st['pv' + key] + part
        if kb == jq:
            pv = st['pv' + key]
            res = pv * (gtab[1, h:h + 1, :] / pv[o + DH:o + DH + 1, :])
            mem = memt[w0:w0 + 32, cols]
            res = res + mem * (gtab[0, h:h + 1, :] / (mem[o + DH:o + DH + 1, :] + 1e-6))
            ot[VS * h // 2:VS * h // 2 + VS // 2, cols] = _u32(res.astype(BF16))[o // 2:o // 2 + VS // 2]

    def o_early(s, jt, c, ke):
        r0, r1 = T * c, min(T * (c + 1), D)
        tile = slice(jt * T, (jt + 1) * T)
        a = jnp.dot(_bf(wot[r0 // 2:r1 // 2, 0:ke]), _bf(ot[0:ke // 2, tile]), preferred_element_type=F32)
        att[r0:r1, tile] = x_v[r0:r1, seg_cols(s, jt)].astype(F32) + a

    def o_unit(s, jt, c, ke, st):
        r0, r1 = T * c, min(T * (c + 1), D)
        tile = slice(jt * T, (jt + 1) * T)
        a = jnp.dot(_bf(wot[r0 // 2:r1 // 2, ke:640]), _bf(ot[ke // 2:320, tile]), preferred_element_type=F32)
        hh = att[r0:r1, tile] + a
        att[r0:r1, tile] = hh
        if c == 0:
            st['p'] = hh[0:1, :]
        d = hh - st['p']
        s1 = jnp.sum(d, axis=0, keepdims=True)
        s2 = jnp.sum(d * d, axis=0, keepdims=True)
        st['s1'] = s1 if c == 0 else st['s1'] + s1
        st['s2'] = s2 if c == 0 else st['s2'] + s2

    def e2_unit(s, jt, c, st):
        r0, r1 = T * c, min(T * (c + 1), D)
        cols = seg_cols(s, jt)
        if c == 0:
            st['m'], st['inv'] = _ln_scale(st['p'], st['s1'], st['s2'])
        hh = att[r0:r1, jt * T:(jt + 1) * T]
        y = (hh - st['m']) * st['inv']
        n = (r1 - r0) // 2
        cand = st.get('cand')
        if cand is None:
            y_s[r0 // 2:r1 // 2, cols] = pltpu.pack_elementwise([y[0:n], y[n:2 * n]], packed_dtype=BF16)
        out_s[r0:r1, cols] = (hh + y).astype(BF16)
        yb = y.astype(BF16)
        rr = jnp.dot(wr16[:, r0:r1], yb, preferred_element_type=F32)
        st['r'] = rr if c == 0 else st['r'] + rr
        if cand is not None:
            cand.setdefault(jt, {'y': []})['y'].append(yb)
        if r1 == D:
            rrow = _rb(st['r'][0:1, :])
            if cand is None:
                r_s[s, :, jt * T:(jt + 1) * T] = jnp.broadcast_to(rrow, (8, T))
            else:
                cand[jt]['r'] = rrow

    def offer_last(best, cand):
        rrow = jnp.concatenate([cand[jt]['r'] for jt in range(4)], axis=1)
        tmax = jnp.max(rrow, axis=1, keepdims=True)
        lane = lax.broadcasted_iota(jnp.int32, (1, L), 1)
        lane_c = jnp.min(jnp.where(rrow == tmax, lane, L), axis=1, keepdims=True)
        xs = None
        for jt in range(4):
            oh = (lax.broadcasted_iota(jnp.int32, (16, T), 1) == lane_c - jt * T).astype(BF16)
            part = jnp.concatenate([lax.dot_general(oh, yc, NT, preferred_element_type=F32)
                                    for yc in cand[jt]['y']], axis=1)
            xs = part if xs is None else xs + part
        take = tmax > best['r']
        best.update(r=jnp.where(take, tmax, best['r']),
                    tok=jnp.where(take, (NSEG - 1) * L + lane_c, best['tok']),
                    xs=jnp.where(take, xs, best['xs']))

    def prep_qk(i, base):
        wt = _u32(w_v[i].T)
        for g in range(NG):
            n = 9 * GH[g]
            wqkv[base + 64 * g:base + 64 * g + n, :] = wt[63 * g:63 * g + n, :]

    def prep_v():
        wt = _u32(w_v[2].T)
        for h in range(H):
            wqkv[QR + 10 * h:QR + 10 * h + 9, :] = wt[9 * h:9 * h + 9, :]

    def prep_o():
        wt = _u32(w_v[3])
        wpad = jnp.concatenate(
            [piece for h in range(H) for piece in (wt[9 * h:9 * h + 9, :], jnp.zeros((1, D), U32))], axis=0)
        wot[...] = _u32(_bf(wpad).T)

    BLKS = [(jq, kb) for jq in range(4) for kb in range(jq + 1)]

    def head_sets(heads):
        sets, i = [], 0
        while i < len(heads):
            h = heads[i]
            if h % 7 % 2 == 0 and h % 7 < 6 and i + 1 < len(heads):
                sets.append((h, h + 1))
                i += 2
            else:
                assert h % 7 == 6
                sets.append((h,))
                i += 1
        return sets

    def s_items(heads, small_tail=0):
        big, small = [], []
        for hs in head_sets(heads):
            for jq, kb in BLKS:
                halved = len(hs) == 2 and kb == jq
                for h in hs:
                    (small if halved else big).append(functools.partial(s_blk, h, jq, kb, halved))
                if halved:
                    small.append(functools.partial(s_pair, hs[0], jq))
        tail = small[len(small) - small_tail:] if small_tail else []
        small = small[:len(small) - small_tail] if small_tail else small
        order = sorted([((j + 0.5) / len(big), 0, j) for j in range(len(big))]
                       + [((j + 0.5) / len(small), 1, j) for j in range(len(small))])
        return [(big, small)[w][j] for _, w, j in order] + tail

    def phase_x():
        sb = s_items(HB)
        for it in sb[0:NS0]:
            it()
        interleave(pv_items(HA), sb[NS0:])

    def pv_items(heads):
        items = []
        for hs in head_sets(heads):
            st = {}
            roles = ('a', 'b') if len(hs) == 2 else (None,)
            for jq, kb in BLKS:
                for h, role in zip(hs, roles):
                    items.append(functools.partial(pv_blk, h, jq, kb, st, role))
        return items

    def interleave(*seqs):
        seqs = [q for q in seqs if q]
        order = []
        for i, q in enumerate(seqs):
            order += [((j + 0.5) / len(q), i, j) for j in range(len(q))]
        for _, i, j in sorted(order):
            seqs[i][j]()

    def proj_items(fn):
        return [functools.partial(fn, jt, g) for jt in range(4) for g in range(NG)]

    def out_items(s, ke, cand=None):
        sts = [{'cand': cand} for _ in range(4)]
        o_items = [functools.partial(o_unit, s, jt, c, ke, sts[jt]) for jt in range(4) for c in range(NG)]
        e_items = [functools.partial(e2_unit, s, jt, c, sts[jt]) for jt in range(4) for c in range(NG)]
        early = [functools.partial(o_early, s, jt, c, ke) for jt in range(4) for c in range(NG)]
        return early, o_items, e_items

    HA = list(range(HS))
    HB = list(range(HS, H))

    x0a.start()
    w_copy(1).start()
    x0b.start()
    zero_s[0] = 0
    beta_copy.start()
    wr_copy.start()
    kr = lax.broadcasted_iota(jnp.int32, (T, T), 0)
    qc = lax.broadcasted_iota(jnp.int32, (T, T), 1)
    bias[...] = jnp.where(kr > qc, MASKVAL, 0.0).astype(F32)
    kr2 = lax.broadcasted_iota(jnp.int32, (64, T), 0)
    qc2 = lax.broadcasted_iota(jnp.int32, (64, T), 1)
    bias2[...] = jnp.where(kr2 > (qc2 & 63), MASKVAL, 0.0).astype(F32)
    wqkv[...] = jnp.zeros(wqkv.shape, U32)
    bd[...] = jnp.zeros(bd.shape, F32)
    memt[...] = jnp.zeros(memt.shape, F32)
    row = lax.broadcasted_iota(jnp.int32, (640, T), 0)
    ones_tab[...] = jnp.where(row % VS == DH, 1.0, 0.0).astype(F32)
    for g in range(NG):
        row = lax.broadcasted_iota(jnp.int32, (160, T), 0) + (GWIN[g][0] - 140 * g)
        lane = lax.broadcasted_iota(jnp.int32, (160, T), 1)
        keep = ((row >= 0) & (row < 20 * GH[g]) & (lane >= (row // VS) * DH)
                & (lane < (row // VS) * DH + DH))
        keep_tab[g] = jnp.where(keep, 1.0, 0.0).astype(F32)
    qt[NG - 1] = jnp.zeros(qt.shape[1:], U32)
    pqt[NG - 1] = jnp.zeros(pqt.shape[1:], U32)
    pkt[NG - 1] = jnp.zeros(pkt.shape[1:], U32)

    x0a.wait()
    w_copy(0).start()
    for jt in range(2):
        ln1_stats(0, jt)
        ln1_norm(0, jt)
    w_copy(1).wait()
    w_copy(2).start()
    prep_qk(1, 0)
    for g in range(NG):
        for jt in range(2):
            q_unit(jt, g)
    w_copy(0).wait()
    x0b.wait()
    x_copy(1).start()
    for jt in range(2, 4):
        ln1_stats(0, jt)
        ln1_norm(0, jt)
    prep_qk(0, QR // 2)
    for jt in range(2, 4):
        for g in range(NG):
            q_unit(jt, g)
    w_copy(2).wait()
    x_rest.start()
    w_copy(3).start()
    prep_v()
    for jt in range(4):
        for g in range(NG):
            k_unit(jt, g)
    beta_copy.wait()
    wr_copy.wait()
    x_copy(1).wait()
    beta = beta_v[...].astype(F32).reshape(1, H)
    hl = lax.broadcasted_iota(jnp.int32, (H, H), 1)
    hs = lax.broadcasted_iota(jnp.int32, (H, H), 0)
    bcol = jnp.sum(jnp.where(hl == hs, jnp.broadcast_to(beta, (H, H)), 0.0), axis=1, keepdims=True)
    gate = _rb(jax.nn.sigmoid(bcol))
    gtab[0] = jnp.broadcast_to(gate, (H, T))
    gtab[1] = jnp.broadcast_to(_rb(1.0 - gate), (H, T))
    r16 = lax.broadcasted_iota(jnp.int32, (16, D), 0)
    wr_row = wr_v[...].astype(F32).reshape(1, D)
    wr16[...] = jnp.where(r16 == 0, jnp.broadcast_to(wr_row, (16, D)), 0.0).astype(BF16)
    interleave(proj_items(v_unit) + s_items(HA, TAIL),
               [functools.partial(ln1_stats, 1, jt) for jt in range(4)])
    x_rest.wait()
    w_copy(3).wait()
    for i in range(2, NSEG):
        for jt in range(4):
            ln1_stats(i, jt)

    def seg_body(s, carry):
        prep_o()
        phase_x()
        ln = [functools.partial(ln1_norm, s + 1, jt) for jt in range(4)]
        qs = proj_items(q_unit)
        early, o_items, e_items = out_items(s, KE)
        upd = [functools.partial(mem_update_unit, g) for g in range(NG)]
        ks = proj_items(k_unit)
        pre = [ln[0]] + early[0:8] + [ln[1]]
        mxu1 = early[8:14] + [ln[2]] + upd + qs[0:5] + early[14:20] + [ln[3]] + qs[5:20] + ks
        for it in pre:
            it()
        interleave(pv_items(HB), mxu1)
        vr = proj_items(v_unit) + [functools.partial(mem_read_unit, g) for g in range(NG)]
        for it in o_items:
            it()
        interleave(vr, e_items)
        for it in s_items(HA, TAIL):
            it()
        o_copy(s).start()

        @pl.when(s == 0)
        def _():
            f_copy(0).start()
            f_copy(1).start()

        @pl.when(s == 1)
        def _():
            f_copy(2).start()
        return carry

    lax.fori_loop(0, NSEG - 1, seg_body, 0)

    for i in range(3):
        f_copy(i).wait()
    best = {}

    def offer_previous():
        n = (NSEG - 1) * 8
        r_all = r_s[0:NSEG - 1].reshape(n, L)
        tok = ((lax.broadcasted_iota(jnp.int32, (n, L), 0) // 8) * L
               + lax.broadcasted_iota(jnp.int32, (n, L), 1))
        rmax = jnp.max(jnp.max(r_all, axis=1, keepdims=True), axis=0, keepdims=True)
        idx = jnp.clip(jnp.min(jnp.where(r_all == rmax, tok, S)), 0, S - 1)
        base = pl.multiple_of((idx // T) * T, T)
        onehot = (lax.broadcasted_iota(jnp.int32, (16, T), 1) == idx - base).astype(BF16)
        yw = y_s[:, pl.ds(base, T)]
        pieces = []
        for c in range(NG):
            w0, w1 = 64 * c, min(64 * (c + 1), D // 2)
            n2 = w1 - w0
            xp = lax.dot_general(onehot, _bf(yw[w0:w1]), NT, preferred_element_type=F32)
            rr = lax.broadcasted_iota(jnp.int32, (2 * n2, 2 * n2), 0)
            cc = lax.broadcasted_iota(jnp.int32, (2 * n2, 2 * n2), 1)
            unmix = (rr == jnp.where(cc < n2, 2 * cc, 2 * (cc - n2) + 1)).astype(BF16)
            pieces.append(jnp.dot(xp.astype(BF16), unmix, preferred_element_type=F32))
        best.update(r=rmax, tok=jnp.full((1, 1), idx, jnp.int32), xs=jnp.concatenate(pieces, axis=1))

    ha1, ha2 = HA[:HA1], HA[HA1:]
    hb1, hb2 = list(range(HS, HM)), list(range(HM, H))
    sb1 = s_items(hb1)
    for it in sb1[0:NS0]:
        it()
    interleave(pv_items(ha1), sb1[NS0:])
    offer_previous()
    sb2 = s_items(hb2)
    interleave(pv_items(ha2) + pv_items(hb1), sb2)
    cand = {}
    early, o_items, e_items = out_items(NSEG - 1, KM, cand)
    for it in early[0:4]:
        it()
    interleave(pv_items(hb2), early[4:])
    for jt in range(4):
        for it in o_items[jt * NG:(jt + 1) * NG]:
            it()
        if jt > 0:
            for it in e_items[(jt - 1) * NG:jt * NG]:
                it()
    for it in e_items[3 * NG:]:
        it()
    offer_last(best, cand)
    o_copy(NSEG - 1).start()

    xs_v[...] = best['xs'].astype(BF16)
    best_v[...] = jnp.broadcast_to(best['r'], (8, T))
    idx = jnp.clip(jnp.max(best['tok']), 0, S - 1)
    base = pl.multiple_of((idx // T) * T, T)
    tile = pl.ds(base, T)

    @pl.when(zero_s[0] == 0)
    def _ffn():
        xs = xs_v[...]
        acc = None
        f0 = 0
        for fw in FCH:
            fc = slice(f0, f0 + fw)
            gt = _rb(jnp.dot(xs, wg_v[:, fc], preferred_element_type=F32))
            up = _rb(jnp.dot(xs, wu_v[:, fc], preferred_element_type=F32))
            act = _rb(_rb(gt * jax.nn.sigmoid(gt)) * up)[0:1, :]
            for t in range(fw // T):
                a = act[:, t * T:(t + 1) * T]
                term = wd_v[:, f0 + t * T:f0 + (t + 1) * T].astype(F32) * a
                acc = term if acc is None else acc + term
            f0 += fw
        ycol = _rb(jnp.sum(acc, axis=1, keepdims=True))
        ycol = _rb(ycol * _rb(jax.nn.sigmoid(best_v[0:1, 0:1])))
        sel = lax.broadcasted_iota(jnp.int32, (D, T), 1) == idx - base
        old = out_s[:, tile].astype(F32)
        fix_v[...] = jnp.where(sel, old + ycol, old).astype(BF16)

    for s in range(NSEG):
        o_copy(s).wait()
    fix = pltpu.make_async_copy(fix_v, out_hbm.at[0, :, tile], sem_o.at[0])
    fix.start()
    fix.wait()


@jax.jit
def pallas_sequential_preLN__memory_aug_infini_attn__moe_arch_mod__prompt_kernel(
    A_x: jax.Array,
    A_wq: jax.Array,
    A_wk: jax.Array,
    A_wv: jax.Array,
    A_wo: jax.Array,
    A_beta: jax.Array,
    B_x: jax.Array,
    B_w_r: jax.Array,
    B_w_gate: jax.Array,
    B_w_up: jax.Array,
    B_w_down: jax.Array,
):
    del B_x
    hbm = pl.BlockSpec(memory_space=pltpu.HBM)
    scratch = [
        pltpu.VMEM((D, S), BF16),
        pltpu.VMEM((4, D, D), BF16),
        pltpu.VMEM((QR + 320, D), U32),
        pltpu.VMEM((D // 2, 640), U32),
        pltpu.VMEM((D // 2, L), U32),
        pltpu.VMEM((NG, 64, L), U32),
        pltpu.VMEM((NG, 64, L), U32),
        pltpu.VMEM((NG, L // 2, T), U32),
        pltpu.VMEM((NG, 64, L), U32),
        pltpu.VMEM((320, L), U32),
        pltpu.VMEM((640, L), F32),
        pltpu.VMEM((NG, 160, T), F32),
        pltpu.VMEM((HS, 1280, T), F32),
        pltpu.VMEM((HM - HS, 1280, T), F32),
        pltpu.VMEM((H - HM, 1280, T), F32),
        pltpu.VMEM((H, 112, T), F32),
        pltpu.VMEM((320, L), U32),
        pltpu.VMEM((D, L), F32),
        pltpu.VMEM((NSEG, 4, 16, T), F32),
        pltpu.VMEM((D // 2, S), U32),
        pltpu.VMEM((D, S), BF16),
        pltpu.VMEM((NSEG, 8, L), F32),
        pltpu.VMEM((T, T), F32),
        pltpu.VMEM((64, T), F32),
        pltpu.VMEM((2, H, T), F32),
        pltpu.VMEM((640, T), F32),
        pltpu.VMEM((NG, 160, T), F32),
        pltpu.VMEM((D, FF), BF16),
        pltpu.VMEM((D, FF), BF16),
        pltpu.VMEM((D, FF), BF16),
        pltpu.VMEM((H,), BF16),
        pltpu.VMEM((D,), BF16),
        pltpu.VMEM((16, D), BF16),
        pltpu.VMEM((16, D), BF16),
        pltpu.VMEM((8, T), F32),
        pltpu.VMEM((D, T), BF16),
        pltpu.SMEM((1,), jnp.int32),
        pltpu.SemaphoreType.DMA((4,)),
        pltpu.SemaphoreType.DMA((4,)),
        pltpu.SemaphoreType.DMA((3,)),
        pltpu.SemaphoreType.DMA((NSEG,)),
        pltpu.SemaphoreType.DMA((2,)),
    ]
    out_t = pl.pallas_call(
        _kernel,
        out_shape=jax.ShapeDtypeStruct((1, D, S), BF16),
        in_specs=[hbm] * 10,
        out_specs=hbm,
        scratch_shapes=scratch,
        compiler_params=pltpu.CompilerParams(vmem_limit_bytes=110 * 1024 * 1024),
        name="infini_moe",
    )(jnp.transpose(A_x, (0, 2, 1)), A_wq, A_wk, A_wv, A_wo, A_beta, B_w_r,
      B_w_gate, B_w_up, jnp.transpose(B_w_down, (1, 0)))
    return jnp.transpose(out_t, (0, 2, 1))
```

```python
import functools
import math

import jax
import jax.numpy as jnp
from jax import lax
import jax.experimental.pallas as pl
import jax.experimental.pallas.tpu as pltpu

F32 = jnp.float32
BF16 = jnp.bfloat16
U32 = jnp.uint32

S = 2048
D = 576
H = 32
DH = 18
NSEG = 4
L = 512
FF = 4608
T = 128
NG = 5
GH = (7, 7, 7, 7, 4)
VS = 20
EPS = 1e-5
QSCALE = DH ** (-0.5) * math.log2(math.e)
MASKVAL = -1000000000.0 * math.log2(math.e)
SOFF = (0, 128, 384, 768)
MOFF = (0, 2, 5, 9)
GWIN = tuple(((140 * g) // 16 * 16, -(-(140 * g + 20 * GH[g]) // 16) * 16) for g in range(NG))
QR = 592
FCH = (256,) * 18

HS = 16
HM = 25
HA1 = 9
NS0 = 16
TAIL = 16
KE = (VS * HS) // T * T
KM = (VS * HM) // T * T

NT = (((1,), (1,)), ((), ()))


def _bf(x_u32):
    return pltpu.bitcast(x_u32, BF16)


def _u32(x_bf):
    return pltpu.bitcast(x_bf, U32)


def _pack(y):
    return _u32(y.astype(BF16))


def _rb(x):
    return x.astype(BF16).astype(F32)


def _phi(t):
    return jnp.where(t > 0, t + 1.0, jnp.exp(t))


def _ln_scale(pivot, s1, s2):
    md = s1 * (1.0 / D)
    v = jnp.maximum(s2 * (1.0 / D) - md * md, 0.0)
    den = _rb(jnp.sqrt(_rb(_rb(v) + EPS)))
    return pivot + md, 1.0 / den


def _kernel(x_hbm, wq_hbm, wk_hbm, wv_hbm, wo_hbm, beta_hbm, wr_hbm, wg_hbm, wu_hbm, wd_hbm,
            out_hbm,
            x_v, w_v, wqkv, wot, xn, qt, pqt, kk, pkt, vt, memt, bd, s_a, s_b1, s_b2, m_blk,
            ot, att, ln_st, y_s, out_s, r_s, bias, bias2, gtab, ones_tab, keep_tab,
            wg_v, wu_v, wd_v, beta_v, wr_v, wr16, xs_v, best_v, fix_v,
            zero_s, sem_x, sem_w, sem_f, sem_o, sem_s):
    def x_copy(s):
        return pltpu.make_async_copy(x_hbm.at[0, :, pl.ds(s * L, L)], x_v.at[:, pl.ds(s * L, L)],
                                     sem_x.at[s])

    x_rest = pltpu.make_async_copy(x_hbm.at[0, :, pl.ds(2 * L, 2 * L)], x_v.at[:, pl.ds(2 * L, 2 * L)], sem_x.at[2])

    x0a = pltpu.make_async_copy(x_hbm.at[0, :, pl.ds(0, L // 2)], x_v.at[:, pl.ds(0, L // 2)], sem_x.at[0])
    x0b = pltpu.make_async_copy(x_hbm.at[0, :, pl.ds(L // 2, L // 2)], x_v.at[:, pl.ds(L // 2, L // 2)], sem_x.at[3])

    w_srcs = (wk_hbm, wq_hbm, wv_hbm, wo_hbm)

    def w_copy(i):
        return pltpu.make_async_copy(w_srcs[i], w_v.at[i], sem_w.at[i])

    f_pairs = ((wg_hbm, wg_v), (wu_hbm, wu_v), (wd_hbm, wd_v))

    def f_copy(i):
        return pltpu.make_async_copy(f_pairs[i][0], f_pairs[i][1], sem_f.at[i])

    def o_copy(s):
        return pltpu.make_async_copy(out_s.at[:, pl.ds(s * L, L)], out_hbm.at[0, :, pl.ds(s * L, L)],
                                     sem_o.at[s])

    beta_copy = pltpu.make_async_copy(beta_hbm, beta_v, sem_s.at[0])
    wr_copy = pltpu.make_async_copy(wr_hbm, wr_v, sem_s.at[1])

    def seg_cols(s, jt):
        if isinstance(s, int):
            return slice(s * L + jt * T, s * L + (jt + 1) * T)
        return pl.ds(pl.multiple_of(s * L + jt * T, T), T)

    def ln1_stats(s, jt):
        cols = seg_cols(s, jt)
        pivot = a1 = a2 = None
        for c in range(D // 32):
            x = x_v[32 * c:32 * (c + 1), cols].astype(F32)
            if c == 0:
                pivot = x[0:1, :]
            d = (x - pivot).reshape(4, 8, T)
            p1 = (d[0] + d[1]) + (d[2] + d[3])
            dd = d * d
            p2 = (dd[0] + dd[1]) + (dd[2] + dd[3])
            a1 = p1 if c == 0 else a1 + p1
            a2 = p2 if c == 0 else a2 + p2
        m, inv = _ln_scale(pivot, jnp.sum(a1, axis=0, keepdims=True), jnp.sum(a2, axis=0, keepdims=True))
        ln_st[s, jt, 0:1, :] = m
        ln_st[s, jt, 8:9, :] = inv

    def ln1_norm(s, jt):
        for c in range(NG):
            r0, r1 = T * c, min(T * (c + 1), D)
            x = x_v[r0:r1, seg_cols(s, jt)].astype(F32)
            xn[r0 // 2:r1 // 2, jt * T:(jt + 1) * T] = _u32(
                ((x - ln_st[s, jt, 0:1, :]) * ln_st[s, jt, 8:9, :]).astype(BF16))

    def q_unit(jt, g):
        cols = slice(jt * T, (jt + 1) * T)
        n = min(64, QR // 2 - 64 * g)
        q = jnp.dot(_bf(wqkv[64 * g:64 * g + n, :]), _bf(xn[:, cols]), preferred_element_type=F32)
        qt[g, 0:n, cols] = _pack(q * QSCALE)
        pqt[g, 0:n, cols] = _pack(_phi(q))

    def k_unit(jt, g):
        cols = slice(jt * T, (jt + 1) * T)
        n = min(64, QR // 2 - 64 * g)
        b0 = QR // 2 + 64 * g
        k = jnp.dot(_bf(wqkv[b0:b0 + n, :]), _bf(xn[:, cols]), preferred_element_type=F32)
        pkt[g, 0:n, cols] = _pack(_phi(k))
        kb = _pack(k)
        if n < 64:
            kb = jnp.concatenate([kb, jnp.zeros((64 - n, T), U32)], axis=0)
        kk[g, jt * 64:(jt + 1) * 64, :] = _u32(_bf(kb).T)

    def v_unit(jt, c):
        cols = slice(jt * T, (jt + 1) * T)
        b0 = QR + 64 * c
        v = jnp.dot(_bf(wqkv[b0:b0 + 64, :]), _bf(xn[:, cols]), preferred_element_type=F32)
        vt[64 * c:64 * (c + 1), cols] = _pack(v + ones_tab[T * c:T * (c + 1), :])

    def mem_read_unit(g):
        w0, w1 = GWIN[g]
        b = bd[g, 0:w1 - w0, :].astype(BF16)
        res = jnp.dot(b, _bf(pqt[g]), preferred_element_type=F32)
        lo, hi = 140 * g, 140 * g + 20 * GH[g]
        memt[lo:hi, :] = res[lo - w0:hi - w0]

    def mem_update_unit(g):
        w0, w1 = GWIN[g]
        upd = lax.dot_general(_bf(vt[w0 // 2:w1 // 2, :]), _bf(pkt[g]), NT, preferred_element_type=F32)
        n = w1 - w0
        bd[g, 0:n, :] = bd[g, 0:n, :] + jnp.where(keep_tab[g, 0:n, :] > 0.5, upd, 0.0)

    def sbuf(h):
        if h < HS:
            return s_a, h
        return (s_b1, h - HS) if h < HM else (s_b2, h - HM)

    def put_scores(h, off, sc):
        sb, hi_ = sbuf(h)
        n = sc.shape[0]
        if h < HS:
            sb[hi_, off:off + n, :] = sc
        else:
            keep = lax.broadcasted_iota(jnp.int32, (n, T), 1) >= zero_s[0]
            pltpu.store(sb.at[hi_, off:off + n, :], sc, mask=keep)

    def head_rows(j):
        r = lax.broadcasted_iota(jnp.int32, (64, T), 0)
        return (r >= 9 * j) & (r < 9 * j + 9)

    def s_blk(h, jq, kb, half=False):
        g, j = divmod(h, 7)
        off = SOFF[jq] + kb * T
        n = 64 if half else T
        qm = _bf(jnp.where(head_rows(j), qt[g, :, jq * T:(jq + 1) * T], U32(0)))
        sc = jnp.dot(_bf(kk[g, kb * 64:kb * 64 + n // 2, :]), qm, preferred_element_type=F32)
        if kb == jq:
            sc = sc + bias[0:n, :]
        put_scores(h, off, sc)
        slot = MOFF[jq] + kb
        m_blk[h, slot * 8:(slot + 1) * 8, :] = jnp.max(sc.reshape(n // 8, 8, T), axis=0)

    def s_pair(ha, jq):
        g, j = divmod(ha, 7)
        off = SOFF[jq] + jq * T + 64
        lo = lax.broadcasted_iota(jnp.int32, (64, T), 1) < 64
        qu = qt[g, :, jq * T:(jq + 1) * T]
        qmix = jnp.where(lo, pltpu.roll(qu, 64, 1), qu)
        qm = _bf(jnp.where((lo & head_rows(j)) | (~lo & head_rows(j + 1)), qmix, U32(0)))
        sc = jnp.dot(_bf(kk[g, jq * 64 + 32:jq * 64 + 64, :]), qm, preferred_element_type=F32) + bias2[...]
        put_scores(ha, off, sc)
        pm = jnp.max(sc.reshape(8, 8, T), axis=0)
        hi = lax.broadcasted_iota(jnp.int32, (8, T), 1) >= 64
        slot = MOFF[jq] + jq + 1
        m_blk[ha, slot * 8:(slot + 1) * 8, :] = jnp.where(hi, pltpu.roll(pm, 64, 1), -jnp.inf)
        m_blk[ha + 1, slot * 8:(slot + 1) * 8, :] = jnp.where(hi, pm, -jnp.inf)

    def row_max(h, jq, nslots):
        return jnp.max(m_blk[h, MOFF[jq] * 8:(MOFF[jq] + nslots) * 8, :], axis=0, keepdims=True)

    def pv_blk(h, jq, kb, st, role):
        w0 = (VS * h) // 16 * 16
        o = VS * h - w0
        off = SOFF[jq] + kb * T
        cols = slice(jq * T, (jq + 1) * T)
        key = role or 'a'
        sb, hz = sbuf(h)
        if kb == 0 and role != 'b':
            st['ma'] = row_max(h, jq, jq + 1 if role is None else jq + 2)
            if role == 'a':
                st['mb'] = row_max(h + 1, jq, jq + 2)
        m = st['m' + key]
        if kb < jq or role is None:
            p = jnp.exp2(sb[hz, off:off + T, :] - m).astype(BF16)
        else:
            if role == 'a':
                hi1 = lax.broadcasted_iota(jnp.int32, (1, T), 1) >= 64
                hi = lax.broadcasted_iota(jnp.int32, (64, T), 1) >= 64
                m2 = jnp.where(hi1, st['mb'], pltpu.roll(st['ma'], 64, 1))
                e2 = jnp.exp2(sb[hz, off + 64:off + T, :] - m2)
                p2 = jnp.where(hi, pltpu.roll(e2, 64, 1), 0.0)
                st['p2b'] = jnp.where(hi, e2, 0.0)
            else:
                p2 = st['p2b']
            p1 = jnp.exp2(sb[hz, off:off + 64, :] - m)
            p = jnp.concatenate([p1, p2], axis=0).astype(BF16)
        part = jnp.dot(_bf(vt[w0 // 2:w0 // 2 + 16, kb * T:(kb + 1) * T]), p, preferred_element_type=F32)
        st['pv' + key] = part if kb == 0 else st['pv' + key] + part
        if kb == jq:
            pv = st['pv' + key]
            res = pv * (gtab[1, h:h + 1, :] / pv[o + DH:o + DH + 1, :])
            mem = memt[w0:w0 + 32, cols]
            res = res + mem * (gtab[0, h:h + 1, :] / (mem[o + DH:o + DH + 1, :] + 1e-6))
            ot[VS * h // 2:VS * h // 2 + VS // 2, cols] = _u32(res.astype(BF16))[o // 2:o // 2 + VS // 2]

    def o_early(s, jt, c, ke):
        r0, r1 = T * c, min(T * (c + 1), D)
        tile = slice(jt * T, (jt + 1) * T)
        a = jnp.dot(_bf(wot[r0 // 2:r1 // 2, 0:ke]), _bf(ot[0:ke // 2, tile]), preferred_element_type=F32)
        att[r0:r1, tile] = x_v[r0:r1, seg_cols(s, jt)].astype(F32) + a

    def o_unit(s, jt, c, ke, st):
        r0, r1 = T * c, min(T * (c + 1), D)
        tile = slice(jt * T, (jt + 1) * T)
        a = jnp.dot(_bf(wot[r0 // 2:r1 // 2, ke:640]), _bf(ot[ke // 2:320, tile]), preferred_element_type=F32)
        hh = att[r0:r1, tile] + a
        att[r0:r1, tile] = hh
        if c == 0:
            st['p'] = hh[0:1, :]
        d = hh - st['p']
        s1 = jnp.sum(d, axis=0, keepdims=True)
        s2 = jnp.sum(d * d, axis=0, keepdims=True)
        st['s1'] = s1 if c == 0 else st['s1'] + s1
        st['s2'] = s2 if c == 0 else st['s2'] + s2

    def e2_unit(s, jt, c, st):
        r0, r1 = T * c, min(T * (c + 1), D)
        cols = seg_cols(s, jt)
        if c == 0:
            st['m'], st['inv'] = _ln_scale(st['p'], st['s1'], st['s2'])
        hh = att[r0:r1, jt * T:(jt + 1) * T]
        y = (hh - st['m']) * st['inv']
        cand = st.get('cand')
        out_s[r0:r1, cols] = (hh + y).astype(BF16)
        yb = y.astype(BF16)
        if cand is None:
            y_s[r0 // 2:r1 // 2, cols] = _u32(yb)
        rr = jnp.dot(wr16[:, r0:r1], yb, preferred_element_type=F32)
        st['r'] = rr if c == 0 else st['r'] + rr
        if cand is not None:
            cand.setdefault(jt, {'y': []})['y'].append(yb)
        if r1 == D:
            rrow = _rb(st['r'][0:1, :])
            if cand is None:
                r_s[s, :, jt * T:(jt + 1) * T] = jnp.broadcast_to(rrow, (8, T))
            else:
                cand[jt]['r'] = rrow

    def offer_last(best, cand):
        rrow = jnp.concatenate([cand[jt]['r'] for jt in range(4)], axis=1)
        tmax = jnp.max(rrow, axis=1, keepdims=True)
        lane = lax.broadcasted_iota(jnp.int32, (1, L), 1)
        lane_c = jnp.min(jnp.where(rrow == tmax, lane, L), axis=1, keepdims=True)
        xs = None
        for jt in range(4):
            oh = (lax.broadcasted_iota(jnp.int32, (16, T), 1) == lane_c - jt * T).astype(BF16)
            part = jnp.concatenate([lax.dot_general(oh, yc, NT, preferred_element_type=F32)
                                    for yc in cand[jt]['y']], axis=1)
            xs = part if xs is None else xs + part
        take = tmax > best['r']
        best.update(r=jnp.where(take, tmax, best['r']),
                    tok=jnp.where(take, (NSEG - 1) * L + lane_c, best['tok']),
                    xs=jnp.where(take, xs, best['xs']))

    def prep_qk(i, base):
        wt = _u32(w_v[i].T)
        for g in range(NG):
            n = 9 * GH[g]
            wqkv[base + 64 * g:base + 64 * g + n, :] = wt[63 * g:63 * g + n, :]

    def prep_v():
        wt = _u32(w_v[2].T)
        for h in range(H):
            wqkv[QR + 10 * h:QR + 10 * h + 9, :] = wt[9 * h:9 * h + 9, :]

    def prep_o():
        wt = _u32(w_v[3])
        wpad = jnp.concatenate(
            [piece for h in range(H) for piece in (wt[9 * h:9 * h + 9, :], jnp.zeros((1, D), U32))], axis=0)
        wot[...] = _u32(_bf(wpad).T)

    BLKS = [(jq, kb) for jq in range(4) for kb in range(jq + 1)]

    def head_sets(heads):
        sets, i = [], 0
        while i < len(heads):
            h = heads[i]
            if h % 7 % 2 == 0 and h % 7 < 6 and i + 1 < len(heads):
                sets.append((h, h + 1))
                i += 2
            else:
                assert h % 7 == 6
                sets.append((h,))
                i += 1
        return sets

    def s_items(heads, small_tail=0):
        big, small = [], []
        for hs in head_sets(heads):
            for jq, kb in BLKS:
                halved = len(hs) == 2 and kb == jq
                for h in hs:
                    (small if halved else big).append(functools.partial(s_blk, h, jq, kb, halved))
                if halved:
                    small.append(functools.partial(s_pair, hs[0], jq))
        tail = small[len(small) - small_tail:] if small_tail else []
        small = small[:len(small) - small_tail] if small_tail else small
        order = sorted([((j + 0.5) / len(big), 0, j) for j in range(len(big))]
                       + [((j + 0.5) / len(small), 1, j) for j in range(len(small))])
        return [(big, small)[w][j] for _, w, j in order] + tail

    def phase_x():
        sb = s_items(HB)
        for it in sb[0:NS0]:
            it()
        interleave(pv_items(HA), sb[NS0:])

    def pv_items(heads):
        items = []
        for hs in head_sets(heads):
            st = {}
            roles = ('a', 'b') if len(hs) == 2 else (None,)
            for jq, kb in BLKS:
                for h, role in zip(hs, roles):
                    items.append(functools.partial(pv_blk, h, jq, kb, st, role))
        return items

    def interleave(*seqs):
        seqs = [q for q in seqs if q]
        order = []
        for i, q in enumerate(seqs):
            order += [((j + 0.5) / len(q), i, j) for j in range(len(q))]
        for _, i, j in sorted(order):
            seqs[i][j]()

    def proj_items(fn):
        return [functools.partial(fn, jt, g) for jt in range(4) for g in range(NG)]

    def out_items(s, ke, cand=None):
        sts = [{'cand': cand} for _ in range(4)]
        o_items = [functools.partial(o_unit, s, jt, c, ke, sts[jt]) for jt in range(4) for c in range(NG)]
        e_items = [functools.partial(e2_unit, s, jt, c, sts[jt]) for jt in range(4) for c in range(NG)]
        early = [functools.partial(o_early, s, jt, c, ke) for jt in range(4) for c in range(NG)]
        return early, o_items, e_items

    HA = list(range(HS))
    HB = list(range(HS, H))

    x0a.start()
    w_copy(1).start()
    x0b.start()
    zero_s[0] = 0
    beta_copy.start()
    wr_copy.start()
    kr = lax.broadcasted_iota(jnp.int32, (T, T), 0)
    qc = lax.broadcasted_iota(jnp.int32, (T, T), 1)
    bias[...] = jnp.where(kr > qc, MASKVAL, 0.0).astype(F32)
    kr2 = lax.broadcasted_iota(jnp.int32, (64, T), 0)
    qc2 = lax.broadcasted_iota(jnp.int32, (64, T), 1)
    bias2[...] = jnp.where(kr2 > (qc2 & 63), MASKVAL, 0.0).astype(F32)
    wqkv[...] = jnp.zeros(wqkv.shape, U32)
    bd[...] = jnp.zeros(bd.shape, F32)
    memt[...] = jnp.zeros(memt.shape, F32)
    row = lax.broadcasted_iota(jnp.int32, (640, T), 0)
    ones_tab[...] = jnp.where(row % VS == DH, 1.0, 0.0).astype(F32)
    for g in range(NG):
        row = lax.broadcasted_iota(jnp.int32, (160, T), 0) + (GWIN[g][0] - 140 * g)
        lane = lax.broadcasted_iota(jnp.int32, (160, T), 1)
        keep = ((row >= 0) & (row < 20 * GH[g]) & (lane >= (row // VS) * DH)
                & (lane < (row // VS) * DH + DH))
        keep_tab[g] = jnp.where(keep, 1.0, 0.0).astype(F32)
    qt[NG - 1] = jnp.zeros(qt.shape[1:], U32)
    pqt[NG - 1] = jnp.zeros(pqt.shape[1:], U32)
    pkt[NG - 1] = jnp.zeros(pkt.shape[1:], U32)

    x0a.wait()
    w_copy(0).start()
    for jt in range(2):
        ln1_stats(0, jt)
        ln1_norm(0, jt)
    w_copy(1).wait()
    w_copy(2).start()
    prep_qk(1, 0)
    for g in range(NG):
        for jt in range(2):
            q_unit(jt, g)
    w_copy(0).wait()
    x0b.wait()
    x_copy(1).start()
    for jt in range(2, 4):
        ln1_stats(0, jt)
        ln1_norm(0, jt)
    prep_qk(0, QR // 2)
    for jt in range(2, 4):
        for g in range(NG):
            q_unit(jt, g)
    w_copy(2).wait()
    x_rest.start()
    w_copy(3).start()
    prep_v()
    for jt in range(4):
        for g in range(NG):
            k_unit(jt, g)
    beta_copy.wait()
    wr_copy.wait()
    x_copy(1).wait()
    beta = beta_v[...].astype(F32).reshape(1, H)
    hl = lax.broadcasted_iota(jnp.int32, (H, H), 1)
    hs = lax.broadcasted_iota(jnp.int32, (H, H), 0)
    bcol = jnp.sum(jnp.where(hl == hs, jnp.broadcast_to(beta, (H, H)), 0.0), axis=1, keepdims=True)
    gate = _rb(jax.nn.sigmoid(bcol))
    gtab[0] = jnp.broadcast_to(gate, (H, T))
    gtab[1] = jnp.broadcast_to(_rb(1.0 - gate), (H, T))
    r16 = lax.broadcasted_iota(jnp.int32, (16, D), 0)
    wr_row = wr_v[...].astype(F32).reshape(1, D)
    wr16[...] = jnp.where(r16 == 0, jnp.broadcast_to(wr_row, (16, D)), 0.0).astype(BF16)
    interleave(proj_items(v_unit) + s_items(HA, TAIL),
               [functools.partial(ln1_stats, 1, jt) for jt in range(4)])
    x_rest.wait()
    w_copy(3).wait()
    for i in range(2, NSEG):
        for jt in range(4):
            ln1_stats(i, jt)

    def seg_body(s, carry):
        prep_o()
        phase_x()
        ln = [functools.partial(ln1_norm, s + 1, jt) for jt in range(4)]
        qs = proj_items(q_unit)
        early, o_items, e_items = out_items(s, KE)
        upd = [functools.partial(mem_update_unit, g) for g in range(NG)]
        ks = proj_items(k_unit)
        pre = [ln[0]] + early[0:8] + [ln[1]]
        mxu1 = early[8:14] + [ln[2]] + upd + qs[0:5] + early[14:20] + [ln[3]] + qs[5:20] + ks
        for it in pre:
            it()
        interleave(pv_items(HB), mxu1)
        vr = proj_items(v_unit) + [functools.partial(mem_read_unit, g) for g in range(NG)]
        for it in o_items:
            it()
        interleave(vr, e_items)
        for it in s_items(HA, TAIL):
            it()
        o_copy(s).start()

        @pl.when(s == 0)
        def _():
            f_copy(0).start()
            f_copy(1).start()

        @pl.when(s == 1)
        def _():
            f_copy(2).start()
        return carry

    lax.fori_loop(0, NSEG - 1, seg_body, 0)

    for i in range(3):
        f_copy(i).wait()
    best = {}

    def offer_previous():
        n = (NSEG - 1) * 8
        r_all = r_s[0:NSEG - 1].reshape(n, L)
        tok = ((lax.broadcasted_iota(jnp.int32, (n, L), 0) // 8) * L
               + lax.broadcasted_iota(jnp.int32, (n, L), 1))
        rmax = jnp.max(jnp.max(r_all, axis=1, keepdims=True), axis=0, keepdims=True)
        idx = jnp.clip(jnp.min(jnp.where(r_all == rmax, tok, S)), 0, S - 1)
        base = pl.multiple_of((idx // T) * T, T)
        onehot = (lax.broadcasted_iota(jnp.int32, (16, T), 1) == idx - base).astype(BF16)
        xs = lax.dot_general(onehot, _bf(y_s[:, pl.ds(base, T)]), NT, preferred_element_type=F32)
        best.update(r=rmax, tok=jnp.full((1, 1), idx, jnp.int32), xs=xs)

    ha1, ha2 = HA[:HA1], HA[HA1:]
    hb1, hb2 = list(range(HS, HM)), list(range(HM, H))
    sb1 = s_items(hb1)
    for it in sb1[0:NS0]:
        it()
    interleave(pv_items(ha1), sb1[NS0:])
    offer_previous()
    sb2 = s_items(hb2)
    interleave(pv_items(ha2) + pv_items(hb1), sb2)
    cand = {}
    early, o_items, e_items = out_items(NSEG - 1, KM, cand)
    for it in early[0:4]:
        it()
    interleave(pv_items(hb2), early[4:])
    for jt in range(4):
        for it in o_items[jt * NG:(jt + 1) * NG]:
            it()
        if jt > 0:
            for it in e_items[(jt - 1) * NG:jt * NG]:
                it()
    for it in e_items[3 * NG:]:
        it()
    offer_last(best, cand)
    o_copy(NSEG - 1).start()

    xs_v[...] = best['xs'].astype(BF16)
    best_v[...] = jnp.broadcast_to(best['r'], (8, T))
    idx = jnp.clip(jnp.max(best['tok']), 0, S - 1)
    base = pl.multiple_of((idx // T) * T, T)
    tile = pl.ds(base, T)

    @pl.when(zero_s[0] == 0)
    def _ffn():
        xs = xs_v[...]
        acc = None
        f0 = 0
        for fw in FCH:
            fc = slice(f0, f0 + fw)
            gt = _rb(jnp.dot(xs, wg_v[:, fc], preferred_element_type=F32))
            up = _rb(jnp.dot(xs, wu_v[:, fc], preferred_element_type=F32))
            act = _rb(_rb(gt * jax.nn.sigmoid(gt)) * up)[0:1, :]
            for t in range(fw // T):
                a = act[:, t * T:(t + 1) * T]
                term = wd_v[:, f0 + t * T:f0 + (t + 1) * T].astype(F32) * a
                acc = term if acc is None else acc + term
            f0 += fw
        ycol = _rb(jnp.sum(acc, axis=1, keepdims=True))
        ycol = _rb(ycol * _rb(jax.nn.sigmoid(best_v[0:1, 0:1])))
        sel = lax.broadcasted_iota(jnp.int32, (D, T), 1) == idx - base
        old = out_s[:, tile].astype(F32)
        fix_v[...] = jnp.where(sel, old + ycol, old).astype(BF16)

    for s in range(NSEG):
        o_copy(s).wait()
    fix = pltpu.make_async_copy(fix_v, out_hbm.at[0, :, tile], sem_o.at[0])
    fix.start()
    fix.wait()


@jax.jit
def pallas_sequential_preLN__memory_aug_infini_attn__moe_arch_mod__prompt_kernel(
    A_x: jax.Array,
    A_wq: jax.Array,
    A_wk: jax.Array,
    A_wv: jax.Array,
    A_wo: jax.Array,
    A_beta: jax.Array,
    B_x: jax.Array,
    B_w_r: jax.Array,
    B_w_gate: jax.Array,
    B_w_up: jax.Array,
    B_w_down: jax.Array,
):
    del B_x
    hbm = pl.BlockSpec(memory_space=pltpu.HBM)
    scratch = [
        pltpu.VMEM((D, S), BF16),
        pltpu.VMEM((4, D, D), BF16),
        pltpu.VMEM((QR + 320, D), U32),
        pltpu.VMEM((D // 2, 640), U32),
        pltpu.VMEM((D // 2, L), U32),
        pltpu.VMEM((NG, 64, L), U32),
        pltpu.VMEM((NG, 64, L), U32),
        pltpu.VMEM((NG, L // 2, T), U32),
        pltpu.VMEM((NG, 64, L), U32),
        pltpu.VMEM((320, L), U32),
        pltpu.VMEM((640, L), F32),
        pltpu.VMEM((NG, 160, T), F32),
        pltpu.VMEM((HS, 1280, T), F32),
        pltpu.VMEM((HM - HS, 1280, T), F32),
        pltpu.VMEM((H - HM, 1280, T), F32),
        pltpu.VMEM((H, 112, T), F32),
        pltpu.VMEM((320, L), U32),
        pltpu.VMEM((D, L), F32),
        pltpu.VMEM((NSEG, 4, 16, T), F32),
        pltpu.VMEM((D // 2, S), U32),
        pltpu.VMEM((D, S), BF16),
        pltpu.VMEM((NSEG, 8, L), F32),
        pltpu.VMEM((T, T), F32),
        pltpu.VMEM((64, T), F32),
        pltpu.VMEM((2, H, T), F32),
        pltpu.VMEM((640, T), F32),
        pltpu.VMEM((NG, 160, T), F32),
        pltpu.VMEM((D, FF), BF16),
        pltpu.VMEM((D, FF), BF16),
        pltpu.VMEM((D, FF), BF16),
        pltpu.VMEM((H,), BF16),
        pltpu.VMEM((D,), BF16),
        pltpu.VMEM((16, D), BF16),
        pltpu.VMEM((16, D), BF16),
        pltpu.VMEM((8, T), F32),
        pltpu.VMEM((D, T), BF16),
        pltpu.SMEM((1,), jnp.int32),
        pltpu.SemaphoreType.DMA((4,)),
        pltpu.SemaphoreType.DMA((4,)),
        pltpu.SemaphoreType.DMA((3,)),
        pltpu.SemaphoreType.DMA((NSEG,)),
        pltpu.SemaphoreType.DMA((2,)),
    ]
    out_t = pl.pallas_call(
        _kernel,
        out_shape=jax.ShapeDtypeStruct((1, D, S), BF16),
        in_specs=[hbm] * 10,
        out_specs=hbm,
        scratch_shapes=scratch,
        compiler_params=pltpu.CompilerParams(vmem_limit_bytes=110 * 1024 * 1024),
        name="infini_moe",
    )(jnp.transpose(A_x, (0, 2, 1)), A_wq, A_wk, A_wv, A_wo, A_beta, B_w_r,
      B_w_gate, B_w_up, jnp.transpose(B_w_down, (1, 0)))
    return jnp.transpose(out_t, (0, 2, 1))
```

```python
import functools
import math

import jax
import jax.numpy as jnp
from jax import lax
import jax.experimental.pallas as pl
import jax.experimental.pallas.tpu as pltpu

F32 = jnp.float32
BF16 = jnp.bfloat16
U32 = jnp.uint32

S = 2048
D = 576
H = 32
DH = 18
NSEG = 4
L = 512
FF = 4608
T = 128
NG = 5
GH = (7, 7, 7, 7, 4)
VS = 20
EPS = 1e-5
QSCALE = DH ** (-0.5) * math.log2(math.e)
MASKVAL = -1000000000.0 * math.log2(math.e)
SOFF = (0, 128, 384, 768)
MOFF = (0, 2, 5, 9)
GWIN = tuple(((140 * g) // 16 * 16, -(-(140 * g + 20 * GH[g]) // 16) * 16) for g in range(NG))
QR = 592
FCH = (256,) * 18

HS = 16
HM = 25
HA1 = 9
NS0 = 16
TAIL = 16
KE = (VS * HS) // T * T
KM = (VS * HM) // T * T

NT = (((1,), (1,)), ((), ()))


def _bf(x_u32):
    return pltpu.bitcast(x_u32, BF16)


def _u32(x_bf):
    return pltpu.bitcast(x_bf, U32)


def _pack(y):
    return _u32(y.astype(BF16))


def _rb(x):
    return x.astype(BF16).astype(F32)


def _phi(t):
    return jnp.where(t > 0, t + 1.0, jnp.exp(t))


def _rank_key(r, tok):
    b = pltpu.bitcast(jnp.broadcast_to(r, (8, r.shape[1])), jnp.int32)[0:1]
    b = (b ^ ((b >> 31) & 0x7FFFFFFF)) & -65536
    return b | (0xFFFF - tok)


def _key_score(key):
    u = key & -65536
    u = jnp.where(u < 0, u ^ 0x7FFF0000, u)
    return pltpu.bitcast(jnp.broadcast_to(u, (8, key.shape[1])), F32)[0:1]


def _ln_scale(pivot, s1, s2):
    md = s1 * (1.0 / D)
    v = jnp.maximum(s2 * (1.0 / D) - md * md, 0.0)
    den = _rb(jnp.sqrt(_rb(_rb(v) + EPS)))
    return pivot + md, 1.0 / den


def _kernel(x_hbm, wq_hbm, wk_hbm, wv_hbm, wo_hbm, beta_hbm, wr_hbm, wg_hbm, wu_hbm, wd_hbm,
            out_hbm,
            x_v, w_v, wqkv, wot, xn, qt, pqt, kk, pkt, vt, memt, bd, s_a, s_b1, s_b2, m_blk,
            ot, att, ln_st, y_s, out_s, r_s, bias, bias2, gtab, ones_tab, keep_tab,
            wg_v, wu_v, wd_v, beta_v, wr_v, wr16, xs_v, best_v, fix_v,
            zero_s, sem_x, sem_w, sem_f, sem_o, sem_s):
    def x_copy(s):
        return pltpu.make_async_copy(x_hbm.at[0, :, pl.ds(s * L, L)], x_v.at[:, pl.ds(s * L, L)],
                                     sem_x.at[s])

    x_rest = pltpu.make_async_copy(x_hbm.at[0, :, pl.ds(2 * L, 2 * L)], x_v.at[:, pl.ds(2 * L, 2 * L)], sem_x.at[2])

    x0a = pltpu.make_async_copy(x_hbm.at[0, :, pl.ds(0, L // 2)], x_v.at[:, pl.ds(0, L // 2)], sem_x.at[0])
    x0b = pltpu.make_async_copy(x_hbm.at[0, :, pl.ds(L // 2, L // 2)], x_v.at[:, pl.ds(L // 2, L // 2)], sem_x.at[3])

    w_srcs = (wk_hbm, wq_hbm, wv_hbm, wo_hbm)

    def w_copy(i):
        return pltpu.make_async_copy(w_srcs[i], w_v.at[i], sem_w.at[i])

    f_pairs = ((wg_hbm, wg_v), (wu_hbm, wu_v), (wd_hbm, wd_v))

    def f_copy(i):
        return pltpu.make_async_copy(f_pairs[i][0], f_pairs[i][1], sem_f.at[i])

    def o_copy(s):
        return pltpu.make_async_copy(out_s.at[:, pl.ds(s * L, L)], out_hbm.at[0, :, pl.ds(s * L, L)],
                                     sem_o.at[s])

    beta_copy = pltpu.make_async_copy(beta_hbm, beta_v, sem_s.at[0])
    wr_copy = pltpu.make_async_copy(wr_hbm, wr_v, sem_s.at[1])

    def seg_cols(s, jt):
        if isinstance(s, int):
            return slice(s * L + jt * T, s * L + (jt + 1) * T)
        return pl.ds(pl.multiple_of(s * L + jt * T, T), T)

    def ln1_stats(s, jt):
        cols = seg_cols(s, jt)
        pivot = a1 = a2 = None
        for c in range(D // 32):
            x = x_v[32 * c:32 * (c + 1), cols].astype(F32)
            if c == 0:
                pivot = x[0:1, :]
            d = (x - pivot).reshape(4, 8, T)
            p1 = (d[0] + d[1]) + (d[2] + d[3])
            dd = d * d
            p2 = (dd[0] + dd[1]) + (dd[2] + dd[3])
            a1 = p1 if c == 0 else a1 + p1
            a2 = p2 if c == 0 else a2 + p2
        m, inv = _ln_scale(pivot, jnp.sum(a1, axis=0, keepdims=True), jnp.sum(a2, axis=0, keepdims=True))
        ln_st[s, jt, 0:1, :] = m
        ln_st[s, jt, 8:9, :] = inv

    def ln1_norm(s, jt):
        for c in range(NG):
            r0, r1 = T * c, min(T * (c + 1), D)
            x = x_v[r0:r1, seg_cols(s, jt)].astype(F32)
            xn[r0 // 2:r1 // 2, jt * T:(jt + 1) * T] = _u32(
                ((x - ln_st[s, jt, 0:1, :]) * ln_st[s, jt, 8:9, :]).astype(BF16))

    def q_unit(jt, g):
        cols = slice(jt * T, (jt + 1) * T)
        n = min(64, QR // 2 - 64 * g)
        q = jnp.dot(_bf(wqkv[64 * g:64 * g + n, :]), _bf(xn[:, cols]), preferred_element_type=F32)
        qt[g, 0:n, cols] = _pack(q * QSCALE)
        pqt[g, 0:n, cols] = _pack(_phi(q))

    def k_unit(jt, g):
        cols = slice(jt * T, (jt + 1) * T)
        n = min(64, QR // 2 - 64 * g)
        b0 = QR // 2 + 64 * g
        k = jnp.dot(_bf(wqkv[b0:b0 + n, :]), _bf(xn[:, cols]), preferred_element_type=F32)
        pkt[g, 0:n, cols] = _pack(_phi(k))
        kb = _pack(k)
        if n < 64:
            kb = jnp.concatenate([kb, jnp.zeros((64 - n, T), U32)], axis=0)
        kk[g, jt * 64:(jt + 1) * 64, :] = _u32(_bf(kb).T)

    def v_unit(jt, c):
        cols = slice(jt * T, (jt + 1) * T)
        b0 = QR + 64 * c
        v = jnp.dot(_bf(wqkv[b0:b0 + 64, :]), _bf(xn[:, cols]), preferred_element_type=F32)
        vt[64 * c:64 * (c + 1), cols] = _pack(v + ones_tab[T * c:T * (c + 1), :])

    def mem_read_unit(g):
        w0, w1 = GWIN[g]
        b = bd[g, 0:w1 - w0, :].astype(BF16)
        res = jnp.dot(b, _bf(pqt[g]), preferred_element_type=F32)
        lo, hi = 140 * g, 140 * g + 20 * GH[g]
        memt[lo:hi, :] = res[lo - w0:hi - w0]

    def mem_update_unit(g):
        w0, w1 = GWIN[g]
        upd = lax.dot_general(_bf(vt[w0 // 2:w1 // 2, :]), _bf(pkt[g]), NT, preferred_element_type=F32)
        n = w1 - w0
        bd[g, 0:n, :] = bd[g, 0:n, :] + jnp.where(keep_tab[g, 0:n, :] > 0.5, upd, 0.0)

    def sbuf(h):
        if h < HS:
            return s_a, h
        return (s_b1, h - HS) if h < HM else (s_b2, h - HM)

    def put_scores(h, off, sc):
        sb, hi_ = sbuf(h)
        n = sc.shape[0]
        if h < HS:
            sb[hi_, off:off + n, :] = sc
        else:
            keep = lax.broadcasted_iota(jnp.int32, (n, T), 1) >= zero_s[0]
            pltpu.store(sb.at[hi_, off:off + n, :], sc, mask=keep)

    def head_rows(j):
        r = lax.broadcasted_iota(jnp.int32, (64, T), 0)
        return (r >= 9 * j) & (r < 9 * j + 9)

    def s_blk(h, jq, kb, half=False):
        g, j = divmod(h, 7)
        off = SOFF[jq] + kb * T
        n = 64 if half else T
        qm = _bf(jnp.where(head_rows(j), qt[g, :, jq * T:(jq + 1) * T], U32(0)))
        sc = jnp.dot(_bf(kk[g, kb * 64:kb * 64 + n // 2, :]), qm, preferred_element_type=F32)
        if kb == jq:
            sc = sc + bias[0:n, :]
        put_scores(h, off, sc)
        slot = MOFF[jq] + kb
        m_blk[h, slot * 8:(slot + 1) * 8, :] = jnp.max(sc.reshape(n // 8, 8, T), axis=0)

    def s_pair(ha, jq):
        g, j = divmod(ha, 7)
        off = SOFF[jq] + jq * T + 64
        lo = lax.broadcasted_iota(jnp.int32, (64, T), 1) < 64
        qu = qt[g, :, jq * T:(jq + 1) * T]
        qmix = jnp.where(lo, pltpu.roll(qu, 64, 1), qu)
        qm = _bf(jnp.where((lo & head_rows(j)) | (~lo & head_rows(j + 1)), qmix, U32(0)))
        sc = jnp.dot(_bf(kk[g, jq * 64 + 32:jq * 64 + 64, :]), qm, preferred_element_type=F32) + bias2[...]
        put_scores(ha, off, sc)
        pm = jnp.max(sc.reshape(8, 8, T), axis=0)
        hi = lax.broadcasted_iota(jnp.int32, (8, T), 1) >= 64
        slot = MOFF[jq] + jq + 1
        m_blk[ha, slot * 8:(slot + 1) * 8, :] = jnp.where(hi, pltpu.roll(pm, 64, 1), -jnp.inf)
        m_blk[ha + 1, slot * 8:(slot + 1) * 8, :] = jnp.where(hi, pm, -jnp.inf)

    def row_max(h, jq, nslots):
        return jnp.max(m_blk[h, MOFF[jq] * 8:(MOFF[jq] + nslots) * 8, :], axis=0, keepdims=True)

    def pv_blk(h, jq, kb, st, role):
        w0 = (VS * h) // 16 * 16
        o = VS * h - w0
        off = SOFF[jq] + kb * T
        cols = slice(jq * T, (jq + 1) * T)
        key = role or 'a'
        sb, hz = sbuf(h)
        if kb == 0 and role != 'b':
            st['ma'] = row_max(h, jq, jq + 1 if role is None else jq + 2)
            if role == 'a':
                st['mb'] = row_max(h + 1, jq, jq + 2)
        m = st['m' + key]
        if kb < jq or role is None:
            p = jnp.exp2(sb[hz, off:off + T, :] - m).astype(BF16)
        else:
            if role == 'a':
                hi1 = lax.broadcasted_iota(jnp.int32, (1, T), 1) >= 64
                hi = lax.broadcasted_iota(jnp.int32, (64, T), 1) >= 64
                m2 = jnp.where(hi1, st['mb'], pltpu.roll(st['ma'], 64, 1))
                e2 = jnp.exp2(sb[hz, off + 64:off + T, :] - m2)
                p2 = jnp.where(hi, pltpu.roll(e2, 64, 1), 0.0)
                st['p2b'] = jnp.where(hi, e2, 0.0)
            else:
                p2 = st['p2b']
            p1 = jnp.exp2(sb[hz, off:off + 64, :] - m)
            p = jnp.concatenate([p1, p2], axis=0).astype(BF16)
        part = jnp.dot(_bf(vt[w0 // 2:w0 // 2 + 16, kb * T:(kb + 1) * T]), p, preferred_element_type=F32)
        st['pv' + key] = part if kb == 0 else st['pv' + key] + part
        if kb == jq:
            pv = st['pv' + key]
            res = pv * (gtab[1, h:h + 1, :] / pv[o + DH:o + DH + 1, :])
            mem = memt[w0:w0 + 32, cols]
            res = res + mem * (gtab[0, h:h + 1, :] / (mem[o + DH:o + DH + 1, :] + 1e-6))
            ot[VS * h // 2:VS * h // 2 + VS // 2, cols] = _u32(res.astype(BF16))[o // 2:o // 2 + VS // 2]

    def o_early(s, jt, c, ke):
        r0, r1 = T * c, min(T * (c + 1), D)
        tile = slice(jt * T, (jt + 1) * T)
        a = jnp.dot(_bf(wot[r0 // 2:r1 // 2, 0:ke]), _bf(ot[0:ke // 2, tile]), preferred_element_type=F32)
        att[r0:r1, tile] = x_v[r0:r1, seg_cols(s, jt)].astype(F32) + a

    def o_unit(s, jt, c, ke, st):
        r0, r1 = T * c, min(T * (c + 1), D)
        tile = slice(jt * T, (jt + 1) * T)
        a = jnp.dot(_bf(wot[r0 // 2:r1 // 2, ke:640]), _bf(ot[ke // 2:320, tile]), preferred_element_type=F32)
        hh = att[r0:r1, tile] + a
        att[r0:r1, tile] = hh
        if c == 0:
            st['p'] = hh[0:1, :]
        d = hh - st['p']
        s1 = jnp.sum(d, axis=0, keepdims=True)
        s2 = jnp.sum(d * d, axis=0, keepdims=True)
        st['s1'] = s1 if c == 0 else st['s1'] + s1
        st['s2'] = s2 if c == 0 else st['s2'] + s2

    def e2_unit(s, jt, c, st):
        r0, r1 = T * c, min(T * (c + 1), D)
        cols = seg_cols(s, jt)
        if c == 0:
            st['m'], st['inv'] = _ln_scale(st['p'], st['s1'], st['s2'])
        hh = att[r0:r1, jt * T:(jt + 1) * T]
        y = (hh - st['m']) * st['inv']
        cand = st.get('cand')
        out_s[r0:r1, cols] = (hh + y).astype(BF16)
        yb = y.astype(BF16)
        if cand is None:
            y_s[r0 // 2:r1 // 2, cols] = _u32(yb)
        rr = jnp.dot(wr16[:, r0:r1], yb, preferred_element_type=F32)
        st['r'] = rr if c == 0 else st['r'] + rr
        if cand is not None:
            cand.setdefault(jt, {'y': []})['y'].append(yb)
        if r1 == D:
            rrow = _rb(st['r'][0:1, :])
            if cand is None:
                r_s[s, :, jt * T:(jt + 1) * T] = jnp.broadcast_to(rrow, (8, T))
            else:
                cand[jt]['r'] = rrow

    def offer_last(best, cand):
        lane = lax.broadcasted_iota(jnp.int32, (1, T), 1)
        keys = [_rank_key(cand[jt]['r'], lane + jt * T) for jt in range(4)]
        key = jnp.max(jnp.maximum(jnp.maximum(keys[0], keys[1]), jnp.maximum(keys[2], keys[3])),
                      axis=1, keepdims=True)
        tmax = _key_score(jnp.broadcast_to(key, (1, T)))[:, 0:1]
        lane_c = 0xFFFF - (key & 0xFFFF)
        xs = None
        for jt in range(4):
            oh = (lax.broadcasted_iota(jnp.int32, (16, T), 1) == lane_c - jt * T).astype(BF16)
            part = jnp.concatenate([lax.dot_general(oh, yc, NT, preferred_element_type=F32)
                                    for yc in cand[jt]['y']], axis=1)
            xs = part if xs is None else xs + part
        take = tmax > best['r']
        best.update(r=jnp.where(take, tmax, best['r']),
                    tok=jnp.where(take, (NSEG - 1) * L + lane_c, best['tok']),
                    xs=jnp.where(take, xs, best['xs']))

    def prep_qk(i, base):
        wt = _u32(w_v[i].T)
        for g in range(NG):
            n = 9 * GH[g]
            wqkv[base + 64 * g:base + 64 * g + n, :] = wt[63 * g:63 * g + n, :]

    def prep_v():
        wt = _u32(w_v[2].T)
        for h in range(H):
            wqkv[QR + 10 * h:QR + 10 * h + 9, :] = wt[9 * h:9 * h + 9, :]

    def prep_o():
        wt = _u32(w_v[3])
        wpad = jnp.concatenate(
            [piece for h in range(H) for piece in (wt[9 * h:9 * h + 9, :], jnp.zeros((1, D), U32))], axis=0)
        wot[...] = _u32(_bf(wpad).T)

    BLKS = [(jq, kb) for jq in range(4) for kb in range(jq + 1)]

    def head_sets(heads):
        sets, i = [], 0
        while i < len(heads):
            h = heads[i]
            if h % 7 % 2 == 0 and h % 7 < 6 and i + 1 < len(heads):
                sets.append((h, h + 1))
                i += 2
            else:
                assert h % 7 == 6
                sets.append((h,))
                i += 1
        return sets

    def s_items(heads, small_tail=0):
        big, small = [], []
        for hs in head_sets(heads):
            for jq, kb in BLKS:
                halved = len(hs) == 2 and kb == jq
                for h in hs:
                    (small if halved else big).append(functools.partial(s_blk, h, jq, kb, halved))
                if halved:
                    small.append(functools.partial(s_pair, hs[0], jq))
        tail = small[len(small) - small_tail:] if small_tail else []
        small = small[:len(small) - small_tail] if small_tail else small
        order = sorted([((j + 0.5) / len(big), 0, j) for j in range(len(big))]
                       + [((j + 0.5) / len(small), 1, j) for j in range(len(small))])
        return [(big, small)[w][j] for _, w, j in order] + tail

    def phase_x():
        sb = s_items(HB)
        for it in sb[0:NS0]:
            it()
        interleave(pv_items(HA), sb[NS0:])

    def pv_items(heads):
        items = []
        for hs in head_sets(heads):
            st = {}
            roles = ('a', 'b') if len(hs) == 2 else (None,)
            for jq, kb in BLKS:
                for h, role in zip(hs, roles):
                    items.append(functools.partial(pv_blk, h, jq, kb, st, role))
        return items

    def interleave(*seqs):
        seqs = [q for q in seqs if q]
        order = []
        for i, q in enumerate(seqs):
            order += [((j + 0.5) / len(q), i, j) for j in range(len(q))]
        for _, i, j in sorted(order):
            seqs[i][j]()

    def proj_items(fn):
        return [functools.partial(fn, jt, g) for jt in range(4) for g in range(NG)]

    def out_items(s, ke, cand=None):
        sts = [{'cand': cand} for _ in range(4)]
        o_items = [functools.partial(o_unit, s, jt, c, ke, sts[jt]) for jt in range(4) for c in range(NG)]
        e_items = [functools.partial(e2_unit, s, jt, c, sts[jt]) for jt in range(4) for c in range(NG)]
        early = [functools.partial(o_early, s, jt, c, ke) for jt in range(4) for c in range(NG)]
        return early, o_items, e_items

    HA = list(range(HS))
    HB = list(range(HS, H))

    x0a.start()
    w_copy(1).start()
    x0b.start()
    zero_s[0] = 0
    beta_copy.start()
    wr_copy.start()
    kr = lax.broadcasted_iota(jnp.int32, (T, T), 0)
    qc = lax.broadcasted_iota(jnp.int32, (T, T), 1)
    bias[...] = jnp.where(kr > qc, MASKVAL, 0.0).astype(F32)
    kr2 = lax.broadcasted_iota(jnp.int32, (64, T), 0)
    qc2 = lax.broadcasted_iota(jnp.int32, (64, T), 1)
    bias2[...] = jnp.where(kr2 > (qc2 & 63), MASKVAL, 0.0).astype(F32)
    wqkv[...] = jnp.zeros(wqkv.shape, U32)
    bd[...] = jnp.zeros(bd.shape, F32)
    memt[...] = jnp.zeros(memt.shape, F32)
    row = lax.broadcasted_iota(jnp.int32, (640, T), 0)
    ones_tab[...] = jnp.where(row % VS == DH, 1.0, 0.0).astype(F32)
    for g in range(NG):
        row = lax.broadcasted_iota(jnp.int32, (160, T), 0) + (GWIN[g][0] - 140 * g)
        lane = lax.broadcasted_iota(jnp.int32, (160, T), 1)
        keep = ((row >= 0) & (row < 20 * GH[g]) & (lane >= (row // VS) * DH)
                & (lane < (row // VS) * DH + DH))
        keep_tab[g] = jnp.where(keep, 1.0, 0.0).astype(F32)
    qt[NG - 1] = jnp.zeros(qt.shape[1:], U32)
    pqt[NG - 1] = jnp.zeros(pqt.shape[1:], U32)
    pkt[NG - 1] = jnp.zeros(pkt.shape[1:], U32)

    x0a.wait()
    w_copy(0).start()
    for jt in range(2):
        ln1_stats(0, jt)
        ln1_norm(0, jt)
    w_copy(1).wait()
    w_copy(2).start()
    prep_qk(1, 0)
    for g in range(NG):
        for jt in range(2):
            q_unit(jt, g)
    w_copy(0).wait()
    x0b.wait()
    x_copy(1).start()
    for jt in range(2, 4):
        ln1_stats(0, jt)
        ln1_norm(0, jt)
    prep_qk(0, QR // 2)
    for jt in range(2, 4):
        for g in range(NG):
            q_unit(jt, g)
    w_copy(2).wait()
    x_rest.start()
    w_copy(3).start()
    prep_v()
    for jt in range(4):
        for g in range(NG):
            k_unit(jt, g)
    beta_copy.wait()
    wr_copy.wait()
    x_copy(1).wait()
    beta = beta_v[...].astype(F32).reshape(1, H)
    hl = lax.broadcasted_iota(jnp.int32, (H, H), 1)
    hs = lax.broadcasted_iota(jnp.int32, (H, H), 0)
    bcol = jnp.sum(jnp.where(hl == hs, jnp.broadcast_to(beta, (H, H)), 0.0), axis=1, keepdims=True)
    gate = _rb(jax.nn.sigmoid(bcol))
    gtab[0] = jnp.broadcast_to(gate, (H, T))
    gtab[1] = jnp.broadcast_to(_rb(1.0 - gate), (H, T))
    r16 = lax.broadcasted_iota(jnp.int32, (16, D), 0)
    wr_row = wr_v[...].astype(F32).reshape(1, D)
    wr16[...] = jnp.where(r16 == 0, jnp.broadcast_to(wr_row, (16, D)), 0.0).astype(BF16)
    interleave(proj_items(v_unit) + s_items(HA, TAIL),
               [functools.partial(ln1_stats, 1, jt) for jt in range(4)])
    x_rest.wait()
    w_copy(3).wait()
    for i in range(2, NSEG):
        for jt in range(4):
            ln1_stats(i, jt)

    def seg_body(s, carry):
        prep_o()
        phase_x()
        ln = [functools.partial(ln1_norm, s + 1, jt) for jt in range(4)]
        qs = proj_items(q_unit)
        early, o_items, e_items = out_items(s, KE)
        upd = [functools.partial(mem_update_unit, g) for g in range(NG)]
        ks = proj_items(k_unit)
        pre = [ln[0]] + early[0:8] + [ln[1]]
        mxu1 = early[8:14] + [ln[2]] + upd + qs[0:5] + early[14:20] + [ln[3]] + qs[5:20] + ks
        for it in pre:
            it()
        interleave(pv_items(HB), mxu1)
        vr = proj_items(v_unit) + [functools.partial(mem_read_unit, g) for g in range(NG)]
        for it in o_items:
            it()
        interleave(vr, e_items)
        for it in s_items(HA, TAIL):
            it()
        o_copy(s).start()

        @pl.when(s == 0)
        def _():
            f_copy(0).start()
            f_copy(1).start()

        @pl.when(s == 1)
        def _():
            f_copy(2).start()
        return carry

    lax.fori_loop(0, NSEG - 1, seg_body, 0)

    for i in range(3):
        f_copy(i).wait()
    best = {}

    def offer_previous():
        n = (NSEG - 1) * 8
        r_all = r_s[0:NSEG - 1].reshape(n, L)
        tok = ((lax.broadcasted_iota(jnp.int32, (n, L), 0) // 8) * L
               + lax.broadcasted_iota(jnp.int32, (n, L), 1))
        rmax = jnp.max(jnp.max(r_all, axis=1, keepdims=True), axis=0, keepdims=True)
        idx = jnp.clip(jnp.min(jnp.where(r_all == rmax, tok, S)), 0, S - 1)
        base = pl.multiple_of((idx // T) * T, T)
        onehot = (lax.broadcasted_iota(jnp.int32, (16, T), 1) == idx - base).astype(BF16)
        xs = lax.dot_general(onehot, _bf(y_s[:, pl.ds(base, T)]), NT, preferred_element_type=F32)
        best.update(r=rmax, tok=jnp.full((1, 1), idx, jnp.int32), xs=xs)

    ha1, ha2 = HA[:HA1], HA[HA1:]
    hb1, hb2 = list(range(HS, HM)), list(range(HM, H))
    sb1 = s_items(hb1)
    for it in sb1[0:NS0]:
        it()
    interleave(pv_items(ha1), sb1[NS0:])
    offer_previous()
    sb2 = s_items(hb2)
    interleave(pv_items(ha2) + pv_items(hb1), sb2)
    cand = {}
    early, o_items, e_items = out_items(NSEG - 1, KM, cand)
    for it in early[0:4]:
        it()
    interleave(pv_items(hb2), early[4:])
    for jt in range(4):
        for it in o_items[jt * NG:(jt + 1) * NG]:
            it()
        if jt > 0:
            for it in e_items[(jt - 1) * NG:jt * NG]:
                it()
    for it in e_items[3 * NG:]:
        it()
    offer_last(best, cand)
    o_copy(NSEG - 1).start()

    xs_v[...] = best['xs'].astype(BF16)
    best_v[...] = jnp.broadcast_to(best['r'], (8, T))
    idx = jnp.clip(jnp.max(best['tok']), 0, S - 1)
    base = pl.multiple_of((idx // T) * T, T)
    tile = pl.ds(base, T)

    @pl.when(zero_s[0] == 0)
    def _ffn():
        xs = xs_v[...]
        acc = None
        f0 = 0
        for fw in FCH:
            fc = slice(f0, f0 + fw)
            gt = _rb(jnp.dot(xs, wg_v[:, fc], preferred_element_type=F32))
            up = _rb(jnp.dot(xs, wu_v[:, fc], preferred_element_type=F32))
            act = _rb(_rb(gt * jax.nn.sigmoid(gt)) * up)[0:1, :]
            for t in range(fw // T):
                a = act[:, t * T:(t + 1) * T]
                term = wd_v[:, f0 + t * T:f0 + (t + 1) * T].astype(F32) * a
                acc = term if acc is None else acc + term
            f0 += fw
        ycol = _rb(jnp.sum(acc, axis=1, keepdims=True))
        ycol = _rb(ycol * _rb(jax.nn.sigmoid(best_v[0:1, 0:1])))
        sel = lax.broadcasted_iota(jnp.int32, (D, T), 1) == idx - base
        old = out_s[:, tile].astype(F32)
        fix_v[...] = jnp.where(sel, old + ycol, old).astype(BF16)

    for s in range(NSEG):
        o_copy(s).wait()
    fix = pltpu.make_async_copy(fix_v, out_hbm.at[0, :, tile], sem_o.at[0])
    fix.start()
    fix.wait()


@jax.jit
def pallas_sequential_preLN__memory_aug_infini_attn__moe_arch_mod__prompt_kernel(
    A_x: jax.Array,
    A_wq: jax.Array,
    A_wk: jax.Array,
    A_wv: jax.Array,
    A_wo: jax.Array,
    A_beta: jax.Array,
    B_x: jax.Array,
    B_w_r: jax.Array,
    B_w_gate: jax.Array,
    B_w_up: jax.Array,
    B_w_down: jax.Array,
):
    del B_x
    hbm = pl.BlockSpec(memory_space=pltpu.HBM)
    scratch = [
        pltpu.VMEM((D, S), BF16),
        pltpu.VMEM((4, D, D), BF16),
        pltpu.VMEM((QR + 320, D), U32),
        pltpu.VMEM((D // 2, 640), U32),
        pltpu.VMEM((D // 2, L), U32),
        pltpu.VMEM((NG, 64, L), U32),
        pltpu.VMEM((NG, 64, L), U32),
        pltpu.VMEM((NG, L // 2, T), U32),
        pltpu.VMEM((NG, 64, L), U32),
        pltpu.VMEM((320, L), U32),
        pltpu.VMEM((640, L), F32),
        pltpu.VMEM((NG, 160, T), F32),
        pltpu.VMEM((HS, 1280, T), F32),
        pltpu.VMEM((HM - HS, 1280, T), F32),
        pltpu.VMEM((H - HM, 1280, T), F32),
        pltpu.VMEM((H, 112, T), F32),
        pltpu.VMEM((320, L), U32),
        pltpu.VMEM((D, L), F32),
        pltpu.VMEM((NSEG, 4, 16, T), F32),
        pltpu.VMEM((D // 2, S), U32),
        pltpu.VMEM((D, S), BF16),
        pltpu.VMEM((NSEG, 8, L), F32),
        pltpu.VMEM((T, T), F32),
        pltpu.VMEM((64, T), F32),
        pltpu.VMEM((2, H, T), F32),
        pltpu.VMEM((640, T), F32),
        pltpu.VMEM((NG, 160, T), F32),
        pltpu.VMEM((D, FF), BF16),
        pltpu.VMEM((D, FF), BF16),
        pltpu.VMEM((D, FF), BF16),
        pltpu.VMEM((H,), BF16),
        pltpu.VMEM((D,), BF16),
        pltpu.VMEM((16, D), BF16),
        pltpu.VMEM((16, D), BF16),
        pltpu.VMEM((8, T), F32),
        pltpu.VMEM((D, T), BF16),
        pltpu.SMEM((1,), jnp.int32),
        pltpu.SemaphoreType.DMA((4,)),
        pltpu.SemaphoreType.DMA((4,)),
        pltpu.SemaphoreType.DMA((3,)),
        pltpu.SemaphoreType.DMA((NSEG,)),
        pltpu.SemaphoreType.DMA((2,)),
    ]
    out_t = pl.pallas_call(
        _kernel,
        out_shape=jax.ShapeDtypeStruct((1, D, S), BF16),
        in_specs=[hbm] * 10,
        out_specs=hbm,
        scratch_shapes=scratch,
        compiler_params=pltpu.CompilerParams(vmem_limit_bytes=110 * 1024 * 1024),
        name="infini_moe",
    )(jnp.transpose(A_x, (0, 2, 1)), A_wq, A_wk, A_wv, A_wo, A_beta, B_w_r,
      B_w_gate, B_w_up, jnp.transpose(B_w_down, (1, 0)))
    return jnp.transpose(out_t, (0, 2, 1))
```

```python
import functools
import math

import jax
import jax.numpy as jnp
from jax import lax
import jax.experimental.pallas as pl
import jax.experimental.pallas.tpu as pltpu

F32 = jnp.float32
BF16 = jnp.bfloat16
U32 = jnp.uint32

S = 2048
D = 576
H = 32
DH = 18
NSEG = 4
L = 512
FF = 4608
T = 128
NG = 5
GH = (7, 7, 7, 7, 4)
VS = 20
EPS = 1e-5
QSCALE = DH ** (-0.5) * math.log2(math.e)
MASKVAL = -1000000000.0 * math.log2(math.e)
SOFF = (0, 128, 384, 768)
MOFF = (0, 2, 5, 9)
GWIN = tuple(((140 * g) // 16 * 16, -(-(140 * g + 20 * GH[g]) // 16) * 16) for g in range(NG))
QR = 592
FCH = (256,) * 18

HS = 16
HM = 25
HA1 = 9
NS0 = 16
TAIL = 16
KE = (VS * HS) // T * T
KM = (VS * HM) // T * T

NT = (((1,), (1,)), ((), ()))


def _bf(x_u32):
    return pltpu.bitcast(x_u32, BF16)


def _u32(x_bf):
    return pltpu.bitcast(x_bf, U32)


def _pack(y):
    return _u32(y.astype(BF16))


def _rb(x):
    return x.astype(BF16).astype(F32)


def _phi(t):
    return jnp.where(t > 0, t + 1.0, jnp.exp(t))


def _rank_key(r, tok):
    b = pltpu.bitcast(jnp.broadcast_to(r, (8, r.shape[1])), jnp.int32)[0:1]
    b = (b ^ ((b >> 31) & 0x7FFFFFFF)) & -65536
    return b | (0xFFFF - tok)


def _key_score(key):
    u = key & -65536
    u = jnp.where(u < 0, u ^ 0x7FFF0000, u)
    return pltpu.bitcast(jnp.broadcast_to(u, (8, key.shape[1])), F32)[0:1]


def _ln_scale(pivot, s1, s2):
    md = s1 * (1.0 / D)
    v = jnp.maximum(s2 * (1.0 / D) - md * md, 0.0)
    den = _rb(jnp.sqrt(_rb(_rb(v) + EPS)))
    return pivot + md, 1.0 / den


def _kernel(x_hbm, wq_hbm, wk_hbm, wv_hbm, wo_hbm, beta_hbm, wr_hbm, wg_hbm, wu_hbm, wd_hbm,
            out_hbm,
            x_v, w_v, wqkv, wot, xn, qt, pqt, kk, pkt, vt, memt, bd, s_a, s_b1, s_b2, m_blk,
            ot, att, ln_st, y_s, out_s, r_s, bias, bias2, gtab, ones_tab, keep_tab,
            wg_v, wu_v, wd_v, beta_v, wr_v, wr16, xs_v, best_v, fix_v,
            zero_s, sem_x, sem_w, sem_f, sem_o, sem_s):
    def x_copy(s):
        return pltpu.make_async_copy(x_hbm.at[0, :, pl.ds(s * L, L)], x_v.at[:, pl.ds(s * L, L)],
                                     sem_x.at[s])

    x_rest = pltpu.make_async_copy(x_hbm.at[0, :, pl.ds(L, S - L)], x_v.at[:, pl.ds(L, S - L)], sem_x.at[2])

    x0a = pltpu.make_async_copy(x_hbm.at[0, :, pl.ds(0, L // 2)], x_v.at[:, pl.ds(0, L // 2)], sem_x.at[0])
    x0b = pltpu.make_async_copy(x_hbm.at[0, :, pl.ds(L // 2, L // 2)], x_v.at[:, pl.ds(L // 2, L // 2)], sem_x.at[3])

    w_srcs = (wk_hbm, wq_hbm, wv_hbm, wo_hbm)

    def w_copy(i):
        return pltpu.make_async_copy(w_srcs[i], w_v.at[i], sem_w.at[i])

    f_pairs = ((wg_hbm, wg_v), (wu_hbm, wu_v), (wd_hbm, wd_v))

    def f_copy(i):
        return pltpu.make_async_copy(f_pairs[i][0], f_pairs[i][1], sem_f.at[i])

    def o_copy(s):
        return pltpu.make_async_copy(out_s.at[:, pl.ds(s * L, L)], out_hbm.at[0, :, pl.ds(s * L, L)],
                                     sem_o.at[s])

    beta_copy = pltpu.make_async_copy(beta_hbm, beta_v, sem_s.at[0])
    wr_copy = pltpu.make_async_copy(wr_hbm, wr_v, sem_s.at[1])

    def seg_cols(s, jt):
        if isinstance(s, int):
            return slice(s * L + jt * T, s * L + (jt + 1) * T)
        return pl.ds(pl.multiple_of(s * L + jt * T, T), T)

    def ln1_stats(s, jt):
        cols = seg_cols(s, jt)
        pivot = a1 = a2 = None
        for c in range(D // 32):
            x = x_v[32 * c:32 * (c + 1), cols].astype(F32)
            if c == 0:
                pivot = x[0:1, :]
            d = (x - pivot).reshape(4, 8, T)
            p1 = (d[0] + d[1]) + (d[2] + d[3])
            dd = d * d
            p2 = (dd[0] + dd[1]) + (dd[2] + dd[3])
            a1 = p1 if c == 0 else a1 + p1
            a2 = p2 if c == 0 else a2 + p2
        m, inv = _ln_scale(pivot, jnp.sum(a1, axis=0, keepdims=True), jnp.sum(a2, axis=0, keepdims=True))
        ln_st[s, jt, 0:1, :] = m
        ln_st[s, jt, 8:9, :] = inv

    def ln1_norm(s, jt):
        for c in range(NG):
            r0, r1 = T * c, min(T * (c + 1), D)
            x = x_v[r0:r1, seg_cols(s, jt)].astype(F32)
            xn[r0 // 2:r1 // 2, jt * T:(jt + 1) * T] = _u32(
                ((x - ln_st[s, jt, 0:1, :]) * ln_st[s, jt, 8:9, :]).astype(BF16))

    def q_unit(jt, g):
        cols = slice(jt * T, (jt + 1) * T)
        n = min(64, QR // 2 - 64 * g)
        q = jnp.dot(_bf(wqkv[64 * g:64 * g + n, :]), _bf(xn[:, cols]), preferred_element_type=F32)
        qt[g, 0:n, cols] = _pack(q * QSCALE)
        pqt[g, 0:n, cols] = _pack(_phi(q))

    def k_unit(jt, g):
        cols = slice(jt * T, (jt + 1) * T)
        n = min(64, QR // 2 - 64 * g)
        b0 = QR // 2 + 64 * g
        k = jnp.dot(_bf(wqkv[b0:b0 + n, :]), _bf(xn[:, cols]), preferred_element_type=F32)
        pkt[g, 0:n, cols] = _pack(_phi(k))
        kb = _pack(k)
        if n < 64:
            kb = jnp.concatenate([kb, jnp.zeros((64 - n, T), U32)], axis=0)
        kk[g, jt * 64:(jt + 1) * 64, :] = _u32(_bf(kb).T)

    def v_unit(jt, c):
        cols = slice(jt * T, (jt + 1) * T)
        b0 = QR + 64 * c
        v = jnp.dot(_bf(wqkv[b0:b0 + 64, :]), _bf(xn[:, cols]), preferred_element_type=F32)
        vt[64 * c:64 * (c + 1), cols] = _pack(v + ones_tab[T * c:T * (c + 1), :])

    def mem_read_unit(g):
        w0, w1 = GWIN[g]
        b = bd[g, 0:w1 - w0, :].astype(BF16)
        res = jnp.dot(b, _bf(pqt[g]), preferred_element_type=F32)
        lo, hi = 140 * g, 140 * g + 20 * GH[g]
        memt[lo:hi, :] = res[lo - w0:hi - w0]

    def mem_update_unit(g):
        w0, w1 = GWIN[g]
        upd = lax.dot_general(_bf(vt[w0 // 2:w1 // 2, :]), _bf(pkt[g]), NT, preferred_element_type=F32)
        n = w1 - w0
        bd[g, 0:n, :] = bd[g, 0:n, :] + jnp.where(keep_tab[g, 0:n, :] > 0.5, upd, 0.0)

    def sbuf(h):
        if h < HS:
            return s_a, h
        return (s_b1, h - HS) if h < HM else (s_b2, h - HM)

    def put_scores(h, off, sc):
        sb, hi_ = sbuf(h)
        n = sc.shape[0]
        if h < HS:
            sb[hi_, off:off + n, :] = sc
        else:
            keep = lax.broadcasted_iota(jnp.int32, (n, T), 1) >= zero_s[0]
            pltpu.store(sb.at[hi_, off:off + n, :], sc, mask=keep)

    def head_rows(j):
        r = lax.broadcasted_iota(jnp.int32, (64, T), 0)
        return (r >= 9 * j) & (r < 9 * j + 9)

    def s_blk(h, jq, kb, half=False):
        g, j = divmod(h, 7)
        off = SOFF[jq] + kb * T
        n = 64 if half else T
        qm = _bf(jnp.where(head_rows(j), qt[g, :, jq * T:(jq + 1) * T], U32(0)))
        sc = jnp.dot(_bf(kk[g, kb * 64:kb * 64 + n // 2, :]), qm, preferred_element_type=F32)
        if kb == jq:
            sc = sc + bias[0:n, :]
        put_scores(h, off, sc)
        slot = MOFF[jq] + kb
        m_blk[h, slot * 8:(slot + 1) * 8, :] = jnp.max(sc.reshape(n // 8, 8, T), axis=0)

    def s_pair(ha, jq):
        g, j = divmod(ha, 7)
        off = SOFF[jq] + jq * T + 64
        lo = lax.broadcasted_iota(jnp.int32, (64, T), 1) < 64
        qu = qt[g, :, jq * T:(jq + 1) * T]
        qmix = jnp.where(lo, pltpu.roll(qu, 64, 1), qu)
        qm = _bf(jnp.where((lo & head_rows(j)) | (~lo & head_rows(j + 1)), qmix, U32(0)))
        sc = jnp.dot(_bf(kk[g, jq * 64 + 32:jq * 64 + 64, :]), qm, preferred_element_type=F32) + bias2[...]
        put_scores(ha, off, sc)
        pm = jnp.max(sc.reshape(8, 8, T), axis=0)
        hi = lax.broadcasted_iota(jnp.int32, (8, T), 1) >= 64
        slot = MOFF[jq] + jq + 1
        m_blk[ha, slot * 8:(slot + 1) * 8, :] = jnp.where(hi, pltpu.roll(pm, 64, 1), -jnp.inf)
        m_blk[ha + 1, slot * 8:(slot + 1) * 8, :] = jnp.where(hi, pm, -jnp.inf)

    def row_max(h, jq, nslots):
        return jnp.max(m_blk[h, MOFF[jq] * 8:(MOFF[jq] + nslots) * 8, :], axis=0, keepdims=True)

    def pv_blk(h, jq, kb, st, role):
        w0 = (VS * h) // 16 * 16
        o = VS * h - w0
        off = SOFF[jq] + kb * T
        cols = slice(jq * T, (jq + 1) * T)
        key = role or 'a'
        sb, hz = sbuf(h)
        if kb == 0 and role != 'b':
            st['ma'] = row_max(h, jq, jq + 1 if role is None else jq + 2)
            if role == 'a':
                st['mb'] = row_max(h + 1, jq, jq + 2)
        m = st['m' + key]
        if kb < jq or role is None:
            p = jnp.exp2(sb[hz, off:off + T, :] - m).astype(BF16)
        else:
            if role == 'a':
                hi1 = lax.broadcasted_iota(jnp.int32, (1, T), 1) >= 64
                hi = lax.broadcasted_iota(jnp.int32, (64, T), 1) >= 64
                m2 = jnp.where(hi1, st['mb'], pltpu.roll(st['ma'], 64, 1))
                e2 = jnp.exp2(sb[hz, off + 64:off + T, :] - m2)
                p2 = jnp.where(hi, pltpu.roll(e2, 64, 1), 0.0)
                st['p2b'] = jnp.where(hi, e2, 0.0)
            else:
                p2 = st['p2b']
            p1 = jnp.exp2(sb[hz, off:off + 64, :] - m)
            p = jnp.concatenate([p1, p2], axis=0).astype(BF16)
        part = jnp.dot(_bf(vt[w0 // 2:w0 // 2 + 16, kb * T:(kb + 1) * T]), p, preferred_element_type=F32)
        st['pv' + key] = part if kb == 0 else st['pv' + key] + part
        if kb == jq:
            pv = st['pv' + key]
            res = pv * (gtab[1, h:h + 1, :] / pv[o + DH:o + DH + 1, :])
            mem = memt[w0:w0 + 32, cols]
            res = res + mem * (gtab[0, h:h + 1, :] / (mem[o + DH:o + DH + 1, :] + 1e-6))
            ot[VS * h // 2:VS * h // 2 + VS // 2, cols] = _u32(res.astype(BF16))[o // 2:o // 2 + VS // 2]

    def o_early(s, jt, c, ke):
        r0, r1 = T * c, min(T * (c + 1), D)
        tile = slice(jt * T, (jt + 1) * T)
        a = jnp.dot(_bf(wot[r0 // 2:r1 // 2, 0:ke]), _bf(ot[0:ke // 2, tile]), preferred_element_type=F32)
        att[r0:r1, tile] = x_v[r0:r1, seg_cols(s, jt)].astype(F32) + a

    def o_unit(s, jt, c, ke, st):
        r0, r1 = T * c, min(T * (c + 1), D)
        tile = slice(jt * T, (jt + 1) * T)
        a = jnp.dot(_bf(wot[r0 // 2:r1 // 2, ke:640]), _bf(ot[ke // 2:320, tile]), preferred_element_type=F32)
        hh = att[r0:r1, tile] + a
        att[r0:r1, tile] = hh
        if c == 0:
            st['p'] = hh[0:1, :]
        d = hh - st['p']
        s1 = jnp.sum(d, axis=0, keepdims=True)
        s2 = jnp.sum(d * d, axis=0, keepdims=True)
        st['s1'] = s1 if c == 0 else st['s1'] + s1
        st['s2'] = s2 if c == 0 else st['s2'] + s2

    def e2_unit(s, jt, c, st):
        r0, r1 = T * c, min(T * (c + 1), D)
        cols = seg_cols(s, jt)
        if c == 0:
            st['m'], st['inv'] = _ln_scale(st['p'], st['s1'], st['s2'])
        hh = att[r0:r1, jt * T:(jt + 1) * T]
        y = (hh - st['m']) * st['inv']
        cand = st.get('cand')
        out_s[r0:r1, cols] = (hh + y).astype(BF16)
        yb = y.astype(BF16)
        if cand is None:
            y_s[r0 // 2:r1 // 2, cols] = _u32(yb)
        rr = jnp.dot(wr16[:, r0:r1], yb, preferred_element_type=F32)
        st['r'] = rr if c == 0 else st['r'] + rr
        if cand is not None:
            cand.setdefault(jt, {'y': []})['y'].append(yb)
        if r1 == D:
            rrow = _rb(st['r'][0:1, :])
            if cand is None:
                r_s[s, :, jt * T:(jt + 1) * T] = jnp.broadcast_to(rrow, (8, T))
            else:
                cand[jt]['r'] = rrow

    def offer_last(best, cand):
        lane = lax.broadcasted_iota(jnp.int32, (1, T), 1)
        keys = [_rank_key(cand[jt]['r'], lane + jt * T) for jt in range(4)]
        key = jnp.max(jnp.maximum(jnp.maximum(keys[0], keys[1]), jnp.maximum(keys[2], keys[3])),
                      axis=1, keepdims=True)
        tmax = _key_score(jnp.broadcast_to(key, (1, T)))[:, 0:1]
        lane_c = 0xFFFF - (key & 0xFFFF)
        xs = None
        for jt in range(4):
            oh = (lax.broadcasted_iota(jnp.int32, (16, T), 1) == lane_c - jt * T).astype(BF16)
            part = jnp.concatenate([lax.dot_general(oh, yc, NT, preferred_element_type=F32)
                                    for yc in cand[jt]['y']], axis=1)
            xs = part if xs is None else xs + part
        take = tmax > best['r']
        best.update(r=jnp.where(take, tmax, best['r']),
                    tok=jnp.where(take, (NSEG - 1) * L + lane_c, best['tok']),
                    xs=jnp.where(take, xs, best['xs']))

    def prep_qk(i, base):
        wt = _u32(w_v[i].T)
        for g in range(NG):
            n = 9 * GH[g]
            wqkv[base + 64 * g:base + 64 * g + n, :] = wt[63 * g:63 * g + n, :]

    def prep_v():
        wt = _u32(w_v[2].T)
        for h in range(H):
            wqkv[QR + 10 * h:QR + 10 * h + 9, :] = wt[9 * h:9 * h + 9, :]

    def prep_o():
        wt = _u32(w_v[3])
        wpad = jnp.concatenate(
            [piece for h in range(H) for piece in (wt[9 * h:9 * h + 9, :], jnp.zeros((1, D), U32))], axis=0)
        wot[...] = _u32(_bf(wpad).T)

    BLKS = [(jq, kb) for jq in range(4) for kb in range(jq + 1)]

    def head_sets(heads):
        sets, i = [], 0
        while i < len(heads):
            h = heads[i]
            if h % 7 % 2 == 0 and h % 7 < 6 and i + 1 < len(heads):
                sets.append((h, h + 1))
                i += 2
            else:
                assert h % 7 == 6
                sets.append((h,))
                i += 1
        return sets

    def s_items(heads, small_tail=0):
        big, small = [], []
        for hs in head_sets(heads):
            for jq, kb in BLKS:
                halved = len(hs) == 2 and kb == jq
                for h in hs:
                    (small if halved else big).append(functools.partial(s_blk, h, jq, kb, halved))
                if halved:
                    small.append(functools.partial(s_pair, hs[0], jq))
        tail = small[len(small) - small_tail:] if small_tail else []
        small = small[:len(small) - small_tail] if small_tail else small
        order = sorted([((j + 0.5) / len(big), 0, j) for j in range(len(big))]
                       + [((j + 0.5) / len(small), 1, j) for j in range(len(small))])
        return [(big, small)[w][j] for _, w, j in order] + tail

    def phase_x():
        sb = s_items(HB)
        for it in sb[0:NS0]:
            it()
        interleave(pv_items(HA), sb[NS0:])

    def pv_items(heads):
        items = []
        for hs in head_sets(heads):
            st = {}
            roles = ('a', 'b') if len(hs) == 2 else (None,)
            for jq, kb in BLKS:
                for h, role in zip(hs, roles):
                    items.append(functools.partial(pv_blk, h, jq, kb, st, role))
        return items

    def interleave(*seqs):
        seqs = [q for q in seqs if q]
        order = []
        for i, q in enumerate(seqs):
            order += [((j + 0.5) / len(q), i, j) for j in range(len(q))]
        for _, i, j in sorted(order):
            seqs[i][j]()

    def proj_items(fn):
        return [functools.partial(fn, jt, g) for jt in range(4) for g in range(NG)]

    def out_items(s, ke, cand=None):
        sts = [{'cand': cand} for _ in range(4)]
        o_items = [functools.partial(o_unit, s, jt, c, ke, sts[jt]) for jt in range(4) for c in range(NG)]
        e_items = [functools.partial(e2_unit, s, jt, c, sts[jt]) for jt in range(4) for c in range(NG)]
        early = [functools.partial(o_early, s, jt, c, ke) for jt in range(4) for c in range(NG)]
        return early, o_items, e_items

    HA = list(range(HS))
    HB = list(range(HS, H))

    x0a.start()
    w_copy(1).start()
    x0b.start()
    zero_s[0] = 0
    beta_copy.start()
    wr_copy.start()
    kr = lax.broadcasted_iota(jnp.int32, (T, T), 0)
    qc = lax.broadcasted_iota(jnp.int32, (T, T), 1)
    bias[...] = jnp.where(kr > qc, MASKVAL, 0.0).astype(F32)
    kr2 = lax.broadcasted_iota(jnp.int32, (64, T), 0)
    qc2 = lax.broadcasted_iota(jnp.int32, (64, T), 1)
    bias2[...] = jnp.where(kr2 > (qc2 & 63), MASKVAL, 0.0).astype(F32)
    wqkv[...] = jnp.zeros(wqkv.shape, U32)
    bd[...] = jnp.zeros(bd.shape, F32)
    memt[...] = jnp.zeros(memt.shape, F32)
    row = lax.broadcasted_iota(jnp.int32, (640, T), 0)
    ones_tab[...] = jnp.where(row % VS == DH, 1.0, 0.0).astype(F32)
    for g in range(NG):
        row = lax.broadcasted_iota(jnp.int32, (160, T), 0) + (GWIN[g][0] - 140 * g)
        lane = lax.broadcasted_iota(jnp.int32, (160, T), 1)
        keep = ((row >= 0) & (row < 20 * GH[g]) & (lane >= (row // VS) * DH)
                & (lane < (row // VS) * DH + DH))
        keep_tab[g] = jnp.where(keep, 1.0, 0.0).astype(F32)
    qt[NG - 1] = jnp.zeros(qt.shape[1:], U32)
    pqt[NG - 1] = jnp.zeros(pqt.shape[1:], U32)
    pkt[NG - 1] = jnp.zeros(pkt.shape[1:], U32)

    x0a.wait()
    w_copy(0).start()
    for jt in range(2):
        ln1_stats(0, jt)
        ln1_norm(0, jt)
    w_copy(1).wait()
    w_copy(2).start()
    prep_qk(1, 0)
    for g in range(NG):
        for jt in range(2):
            q_unit(jt, g)
    w_copy(0).wait()
    x0b.wait()
    x_rest.start()
    for jt in range(2, 4):
        ln1_stats(0, jt)
        ln1_norm(0, jt)
    prep_qk(0, QR // 2)
    for jt in range(2, 4):
        for g in range(NG):
            q_unit(jt, g)
    w_copy(2).wait()
    w_copy(3).start()
    prep_v()
    for jt in range(4):
        for g in range(NG):
            k_unit(jt, g)
    beta_copy.wait()
    wr_copy.wait()
    x_rest.wait()
    beta = beta_v[...].astype(F32).reshape(1, H)
    hl = lax.broadcasted_iota(jnp.int32, (H, H), 1)
    hs = lax.broadcasted_iota(jnp.int32, (H, H), 0)
    bcol = jnp.sum(jnp.where(hl == hs, jnp.broadcast_to(beta, (H, H)), 0.0), axis=1, keepdims=True)
    gate = _rb(jax.nn.sigmoid(bcol))
    gtab[0] = jnp.broadcast_to(gate, (H, T))
    gtab[1] = jnp.broadcast_to(_rb(1.0 - gate), (H, T))
    r16 = lax.broadcasted_iota(jnp.int32, (16, D), 0)
    wr_row = wr_v[...].astype(F32).reshape(1, D)
    wr16[...] = jnp.where(r16 == 0, jnp.broadcast_to(wr_row, (16, D)), 0.0).astype(BF16)
    interleave(proj_items(v_unit) + s_items(HA, TAIL),
               [functools.partial(ln1_stats, i, jt) for i in range(1, NSEG) for jt in range(4)])
    w_copy(3).wait()

    def seg_body(s, carry):
        prep_o()
        phase_x()
        ln = [functools.partial(ln1_norm, s + 1, jt) for jt in range(4)]
        qs = proj_items(q_unit)
        early, o_items, e_items = out_items(s, KE)
        upd = [functools.partial(mem_update_unit, g) for g in range(NG)]
        ks = proj_items(k_unit)
        pre = [ln[0]] + early[0:8] + [ln[1]]
        mxu1 = early[8:14] + [ln[2]] + upd + qs[0:5] + early[14:20] + [ln[3]] + qs[5:20] + ks
        for it in pre:
            it()
        interleave(pv_items(HB), mxu1)
        vr = proj_items(v_unit) + [functools.partial(mem_read_unit, g) for g in range(NG)]
        for it in o_items:
            it()
        interleave(vr, e_items)
        for it in s_items(HA, TAIL):
            it()
        o_copy(s).start()

        @pl.when(s == 0)
        def _():
            f_copy(0).start()
            f_copy(1).start()

        @pl.when(s == 1)
        def _():
            f_copy(2).start()
        return carry

    lax.fori_loop(0, NSEG - 1, seg_body, 0)

    for i in range(3):
        f_copy(i).wait()
    best = {}

    def offer_previous():
        n = (NSEG - 1) * 8
        r_all = r_s[0:NSEG - 1].reshape(n, L)
        tok = ((lax.broadcasted_iota(jnp.int32, (n, L), 0) // 8) * L
               + lax.broadcasted_iota(jnp.int32, (n, L), 1))
        rmax = jnp.max(jnp.max(r_all, axis=1, keepdims=True), axis=0, keepdims=True)
        idx = jnp.clip(jnp.min(jnp.where(r_all == rmax, tok, S)), 0, S - 1)
        base = pl.multiple_of((idx // T) * T, T)
        onehot = (lax.broadcasted_iota(jnp.int32, (16, T), 1) == idx - base).astype(BF16)
        xs = lax.dot_general(onehot, _bf(y_s[:, pl.ds(base, T)]), NT, preferred_element_type=F32)
        best.update(r=rmax, tok=jnp.full((1, 1), idx, jnp.int32), xs=xs)

    ha1, ha2 = HA[:HA1], HA[HA1:]
    hb1, hb2 = list(range(HS, HM)), list(range(HM, H))
    sb1 = s_items(hb1)
    for it in sb1[0:NS0]:
        it()
    interleave(pv_items(ha1), sb1[NS0:])
    offer_previous()
    sb2 = s_items(hb2)
    interleave(pv_items(ha2) + pv_items(hb1), sb2)
    cand = {}
    early, o_items, e_items = out_items(NSEG - 1, KM, cand)
    for it in early[0:4]:
        it()
    interleave(pv_items(hb2), early[4:])
    for jt in range(4):
        for it in o_items[jt * NG:(jt + 1) * NG]:
            it()
        if jt > 0:
            for it in e_items[(jt - 1) * NG:jt * NG]:
                it()
    for it in e_items[3 * NG:]:
        it()
    offer_last(best, cand)
    o_copy(NSEG - 1).start()

    xs_v[...] = best['xs'].astype(BF16)
    best_v[...] = jnp.broadcast_to(best['r'], (8, T))
    idx = jnp.clip(jnp.max(best['tok']), 0, S - 1)
    base = pl.multiple_of((idx // T) * T, T)
    tile = pl.ds(base, T)

    @pl.when(zero_s[0] == 0)
    def _ffn():
        xs = xs_v[...]
        acc = None
        f0 = 0
        for fw in FCH:
            fc = slice(f0, f0 + fw)
            gt = _rb(jnp.dot(xs, wg_v[:, fc], preferred_element_type=F32))
            up = _rb(jnp.dot(xs, wu_v[:, fc], preferred_element_type=F32))
            act = _rb(_rb(gt * jax.nn.sigmoid(gt)) * up)[0:1, :]
            for t in range(fw // T):
                a = act[:, t * T:(t + 1) * T]
                term = wd_v[:, f0 + t * T:f0 + (t + 1) * T].astype(F32) * a
                acc = term if acc is None else acc + term
            f0 += fw
        ycol = _rb(jnp.sum(acc, axis=1, keepdims=True))
        ycol = _rb(ycol * _rb(jax.nn.sigmoid(best_v[0:1, 0:1])))
        sel = lax.broadcasted_iota(jnp.int32, (D, T), 1) == idx - base
        old = out_s[:, tile].astype(F32)
        fix_v[...] = jnp.where(sel, old + ycol, old).astype(BF16)

    for s in range(NSEG):
        o_copy(s).wait()
    fix = pltpu.make_async_copy(fix_v, out_hbm.at[0, :, tile], sem_o.at[0])
    fix.start()
    fix.wait()


@jax.jit
def pallas_sequential_preLN__memory_aug_infini_attn__moe_arch_mod__prompt_kernel(
    A_x: jax.Array,
    A_wq: jax.Array,
    A_wk: jax.Array,
    A_wv: jax.Array,
    A_wo: jax.Array,
    A_beta: jax.Array,
    B_x: jax.Array,
    B_w_r: jax.Array,
    B_w_gate: jax.Array,
    B_w_up: jax.Array,
    B_w_down: jax.Array,
):
    del B_x
    hbm = pl.BlockSpec(memory_space=pltpu.HBM)
    scratch = [
        pltpu.VMEM((D, S), BF16),
        pltpu.VMEM((4, D, D), BF16),
        pltpu.VMEM((QR + 320, D), U32),
        pltpu.VMEM((D // 2, 640), U32),
        pltpu.VMEM((D // 2, L), U32),
        pltpu.VMEM((NG, 64, L), U32),
        pltpu.VMEM((NG, 64, L), U32),
        pltpu.VMEM((NG, L // 2, T), U32),
        pltpu.VMEM((NG, 64, L), U32),
        pltpu.VMEM((320, L), U32),
        pltpu.VMEM((640, L), F32),
        pltpu.VMEM((NG, 160, T), F32),
        pltpu.VMEM((HS, 1280, T), F32),
        pltpu.VMEM((HM - HS, 1280, T), F32),
        pltpu.VMEM((H - HM, 1280, T), F32),
        pltpu.VMEM((H, 112, T), F32),
        pltpu.VMEM((320, L), U32),
        pltpu.VMEM((D, L), F32),
        pltpu.VMEM((NSEG, 4, 16, T), F32),
        pltpu.VMEM((D // 2, S), U32),
        pltpu.VMEM((D, S), BF16),
        pltpu.VMEM((NSEG, 8, L), F32),
        pltpu.VMEM((T, T), F32),
        pltpu.VMEM((64, T), F32),
        pltpu.VMEM((2, H, T), F32),
        pltpu.VMEM((640, T), F32),
        pltpu.VMEM((NG, 160, T), F32),
        pltpu.VMEM((D, FF), BF16),
        pltpu.VMEM((D, FF), BF16),
        pltpu.VMEM((D, FF), BF16),
        pltpu.VMEM((H,), BF16),
        pltpu.VMEM((D,), BF16),
        pltpu.VMEM((16, D), BF16),
        pltpu.VMEM((16, D), BF16),
        pltpu.VMEM((8, T), F32),
        pltpu.VMEM((D, T), BF16),
        pltpu.SMEM((1,), jnp.int32),
        pltpu.SemaphoreType.DMA((4,)),
        pltpu.SemaphoreType.DMA((4,)),
        pltpu.SemaphoreType.DMA((3,)),
        pltpu.SemaphoreType.DMA((NSEG,)),
        pltpu.SemaphoreType.DMA((2,)),
    ]
    out_t = pl.pallas_call(
        _kernel,
        out_shape=jax.ShapeDtypeStruct((1, D, S), BF16),
        in_specs=[hbm] * 10,
        out_specs=hbm,
        scratch_shapes=scratch,
        compiler_params=pltpu.CompilerParams(vmem_limit_bytes=110 * 1024 * 1024),
        name="infini_moe",
    )(jnp.transpose(A_x, (0, 2, 1)), A_wq, A_wk, A_wv, A_wo, A_beta, B_w_r,
      B_w_gate, B_w_up, jnp.transpose(B_w_down, (1, 0)))
    return jnp.transpose(out_t, (0, 2, 1))
```

```python
import functools
import math

import jax
import jax.numpy as jnp
from jax import lax
import jax.experimental.pallas as pl
import jax.experimental.pallas.tpu as pltpu

F32 = jnp.float32
BF16 = jnp.bfloat16
U32 = jnp.uint32

S = 2048
D = 576
H = 32
DH = 18
NSEG = 4
L = 512
FF = 4608
T = 128
NG = 5
GH = (7, 7, 7, 7, 4)
VS = 20
EPS = 1e-5
QSCALE = DH ** (-0.5) * math.log2(math.e)
MASKVAL = -1000000000.0 * math.log2(math.e)
SOFF = (0, 128, 384, 768)
MOFF = (0, 2, 5, 9)
GWIN = tuple(((140 * g) // 16 * 16, -(-(140 * g + 20 * GH[g]) // 16) * 16) for g in range(NG))
QR = 592
FCH = (256,) * 18

HS = 16
HM = 25
HA1 = 9
NS0 = 16
TAIL = 16
KE = (VS * HS) // T * T
KM = (VS * HM) // T * T

NT = (((1,), (1,)), ((), ()))


def _bf(x_u32):
    return pltpu.bitcast(x_u32, BF16)


def _u32(x_bf):
    return pltpu.bitcast(x_bf, U32)


def _pack(y):
    return _u32(y.astype(BF16))


def _rb(x):
    return x.astype(BF16).astype(F32)


def _phi(t):
    return jnp.where(t > 0, t + 1.0, jnp.exp(t))


def _rank_key(r, tok):
    b = pltpu.bitcast(jnp.broadcast_to(r, (8, r.shape[1])), jnp.int32)[0:1]
    b = (b ^ ((b >> 31) & 0x7FFFFFFF)) & -65536
    return b | (0xFFFF - tok)


def _key_score(key):
    u = key & -65536
    u = jnp.where(u < 0, u ^ 0x7FFF0000, u)
    return pltpu.bitcast(jnp.broadcast_to(u, (8, key.shape[1])), F32)[0:1]


def _ln_scale(pivot, s1, s2):
    md = s1 * (1.0 / D)
    v = jnp.maximum(s2 * (1.0 / D) - md * md, 0.0)
    den = _rb(jnp.sqrt(_rb(_rb(v) + EPS)))
    return pivot + md, 1.0 / den


def _kernel(x_hbm, wq_hbm, wk_hbm, wv_hbm, wo_hbm, beta_hbm, wr_hbm, wg_hbm, wu_hbm, wd_hbm,
            out_hbm,
            x_v, w_v, wqkv, wot, xn, qt, pqt, kk, pkt, vt, memt, bd, s_a, s_b1, s_b2, m_blk,
            ot, att, ln_st, y_s, out_s, r_s, bias, bias2, gtab, ones_tab, keep_tab,
            wg_v, wu_v, wd_v, beta_v, wr_v, wr16, xs_v, best_v, fix_v,
            zero_s, sem_x, sem_w, sem_f, sem_o, sem_s):
    x_rest = pltpu.make_async_copy(x_hbm.at[0, :, pl.ds(L, S - L)], x_v.at[:, pl.ds(L, S - L)], sem_x.at[2])

    x0a = pltpu.make_async_copy(x_hbm.at[0, :, pl.ds(0, L // 2)], x_v.at[:, pl.ds(0, L // 2)], sem_x.at[0])
    x0b = pltpu.make_async_copy(x_hbm.at[0, :, pl.ds(L // 2, L // 2)], x_v.at[:, pl.ds(L // 2, L // 2)], sem_x.at[1])

    w_srcs = (wk_hbm, wq_hbm, wv_hbm, wo_hbm)

    def w_copy(i):
        return pltpu.make_async_copy(w_srcs[i], w_v.at[i], sem_w.at[i])

    f_pairs = ((wg_hbm, wg_v), (wu_hbm, wu_v), (wd_hbm, wd_v))

    def f_copy(i):
        return pltpu.make_async_copy(f_pairs[i][0], f_pairs[i][1], sem_f.at[i])

    def o_copy(s):
        return pltpu.make_async_copy(out_s.at[:, pl.ds(s * L, L)], out_hbm.at[0, :, pl.ds(s * L, L)],
                                     sem_o.at[s])

    beta_copy = pltpu.make_async_copy(beta_hbm, beta_v, sem_s.at[0])
    wr_copy = pltpu.make_async_copy(wr_hbm, wr_v, sem_s.at[1])

    def seg_cols(s, jt):
        if isinstance(s, int):
            return slice(s * L + jt * T, s * L + (jt + 1) * T)
        return pl.ds(pl.multiple_of(s * L + jt * T, T), T)

    def ln1_stats(s, jt):
        cols = seg_cols(s, jt)
        pivot = a1 = a2 = None
        for c in range(D // 32):
            x = x_v[32 * c:32 * (c + 1), cols].astype(F32)
            if c == 0:
                pivot = x[0:1, :]
            d = (x - pivot).reshape(4, 8, T)
            p1 = (d[0] + d[1]) + (d[2] + d[3])
            dd = d * d
            p2 = (dd[0] + dd[1]) + (dd[2] + dd[3])
            a1 = p1 if c == 0 else a1 + p1
            a2 = p2 if c == 0 else a2 + p2
        m, inv = _ln_scale(pivot, jnp.sum(a1, axis=0, keepdims=True), jnp.sum(a2, axis=0, keepdims=True))
        ln_st[s, jt, 0:1, :] = m
        ln_st[s, jt, 8:9, :] = inv

    def ln1_norm(s, jt):
        for c in range(NG):
            r0, r1 = T * c, min(T * (c + 1), D)
            x = x_v[r0:r1, seg_cols(s, jt)].astype(F32)
            xn[r0 // 2:r1 // 2, jt * T:(jt + 1) * T] = _u32(
                ((x - ln_st[s, jt, 0:1, :]) * ln_st[s, jt, 8:9, :]).astype(BF16))

    def q_unit(jt, g):
        cols = slice(jt * T, (jt + 1) * T)
        n = min(64, QR // 2 - 64 * g)
        q = jnp.dot(_bf(wqkv[64 * g:64 * g + n, :]), _bf(xn[:, cols]), preferred_element_type=F32)
        qt[g, 0:n, cols] = _pack(q * QSCALE)
        pqt[g, 0:n, cols] = _pack(_phi(q))

    def k_unit(jt, g):
        cols = slice(jt * T, (jt + 1) * T)
        n = min(64, QR // 2 - 64 * g)
        b0 = QR // 2 + 64 * g
        k = jnp.dot(_bf(wqkv[b0:b0 + n, :]), _bf(xn[:, cols]), preferred_element_type=F32)
        pkt[g, 0:n, cols] = _pack(_phi(k))
        kb = _pack(k)
        if n < 64:
            kb = jnp.concatenate([kb, jnp.zeros((64 - n, T), U32)], axis=0)
        kk[g, jt * 64:(jt + 1) * 64, :] = _u32(_bf(kb).T)

    def v_unit(jt, c):
        cols = slice(jt * T, (jt + 1) * T)
        b0 = QR + 64 * c
        v = jnp.dot(_bf(wqkv[b0:b0 + 64, :]), _bf(xn[:, cols]), preferred_element_type=F32)
        vt[64 * c:64 * (c + 1), cols] = _pack(v + ones_tab[T * c:T * (c + 1), :])

    def mem_read_unit(g):
        w0, w1 = GWIN[g]
        b = bd[g, 0:w1 - w0, :].astype(BF16)
        res = jnp.dot(b, _bf(pqt[g]), preferred_element_type=F32)
        lo, hi = 140 * g, 140 * g + 20 * GH[g]
        memt[lo:hi, :] = res[lo - w0:hi - w0]

    def mem_update_unit(g):
        w0, w1 = GWIN[g]
        upd = lax.dot_general(_bf(vt[w0 // 2:w1 // 2, :]), _bf(pkt[g]), NT, preferred_element_type=F32)
        n = w1 - w0
        bd[g, 0:n, :] = bd[g, 0:n, :] + jnp.where(keep_tab[g, 0:n, :] > 0.5, upd, 0.0)

    def sbuf(h):
        if h < HS:
            return s_a, h
        return (s_b1, h - HS) if h < HM else (s_b2, h - HM)

    def put_scores(h, off, sc):
        sb, hi_ = sbuf(h)
        n = sc.shape[0]
        if h < HS:
            sb[hi_, off:off + n, :] = sc
        else:
            keep = lax.broadcasted_iota(jnp.int32, (n, T), 1) >= zero_s[0]
            pltpu.store(sb.at[hi_, off:off + n, :], sc, mask=keep)

    def head_rows(j):
        r = lax.broadcasted_iota(jnp.int32, (64, T), 0)
        return (r >= 9 * j) & (r < 9 * j + 9)

    def s_blk(h, jq, kb, half=False):
        g, j = divmod(h, 7)
        off = SOFF[jq] + kb * T
        n = 64 if half else T
        qm = _bf(jnp.where(head_rows(j), qt[g, :, jq * T:(jq + 1) * T], U32(0)))
        sc = jnp.dot(_bf(kk[g, kb * 64:kb * 64 + n // 2, :]), qm, preferred_element_type=F32)
        if kb == jq:
            sc = sc + bias[0:n, :]
        put_scores(h, off, sc)
        slot = MOFF[jq] + kb
        m_blk[h, slot * 8:(slot + 1) * 8, :] = jnp.max(sc.reshape(n // 8, 8, T), axis=0)

    def s_pair(ha, jq):
        g, j = divmod(ha, 7)
        off = SOFF[jq] + jq * T + 64
        lo = lax.broadcasted_iota(jnp.int32, (64, T), 1) < 64
        qu = qt[g, :, jq * T:(jq + 1) * T]
        qmix = jnp.where(lo, pltpu.roll(qu, 64, 1), qu)
        qm = _bf(jnp.where((lo & head_rows(j)) | (~lo & head_rows(j + 1)), qmix, U32(0)))
        sc = jnp.dot(_bf(kk[g, jq * 64 + 32:jq * 64 + 64, :]), qm, preferred_element_type=F32) + bias2[...]
        put_scores(ha, off, sc)
        pm = jnp.max(sc.reshape(8, 8, T), axis=0)
        hi = lax.broadcasted_iota(jnp.int32, (8, T), 1) >= 64
        slot = MOFF[jq] + jq + 1
        m_blk[ha, slot * 8:(slot + 1) * 8, :] = jnp.where(hi, pltpu.roll(pm, 64, 1), -jnp.inf)
        m_blk[ha + 1, slot * 8:(slot + 1) * 8, :] = jnp.where(hi, pm, -jnp.inf)

    def row_max(h, jq, nslots):
        return jnp.max(m_blk[h, MOFF[jq] * 8:(MOFF[jq] + nslots) * 8, :], axis=0, keepdims=True)

    def pv_blk(h, jq, kb, st, role):
        w0 = (VS * h) // 16 * 16
        o = VS * h - w0
        off = SOFF[jq] + kb * T
        cols = slice(jq * T, (jq + 1) * T)
        key = role or 'a'
        sb, hz = sbuf(h)
        if kb == 0 and role != 'b':
            st['ma'] = row_max(h, jq, jq + 1 if role is None else jq + 2)
            if role == 'a':
                st['mb'] = row_max(h + 1, jq, jq + 2)
        m = st['m' + key]
        if kb < jq or role is None:
            p = jnp.exp2(sb[hz, off:off + T, :] - m).astype(BF16)
        else:
            if role == 'a':
                hi1 = lax.broadcasted_iota(jnp.int32, (1, T), 1) >= 64
                hi = lax.broadcasted_iota(jnp.int32, (64, T), 1) >= 64
                m2 = jnp.where(hi1, st['mb'], pltpu.roll(st['ma'], 64, 1))
                e2 = jnp.exp2(sb[hz, off + 64:off + T, :] - m2)
                p2 = jnp.where(hi, pltpu.roll(e2, 64, 1), 0.0)
                st['p2b'] = jnp.where(hi, e2, 0.0)
            else:
                p2 = st['p2b']
            p1 = jnp.exp2(sb[hz, off:off + 64, :] - m)
            p = jnp.concatenate([p1, p2], axis=0).astype(BF16)
        part = jnp.dot(_bf(vt[w0 // 2:w0 // 2 + 16, kb * T:(kb + 1) * T]), p, preferred_element_type=F32)
        st['pv' + key] = part if kb == 0 else st['pv' + key] + part
        if kb == jq:
            pv = st['pv' + key]
            res = pv * (gtab[1, h:h + 1, :] / pv[o + DH:o + DH + 1, :])
            mem = memt[w0:w0 + 32, cols]
            res = res + mem * (gtab[0, h:h + 1, :] / (mem[o + DH:o + DH + 1, :] + 1e-6))
            ot[VS * h // 2:VS * h // 2 + VS // 2, cols] = _u32(res.astype(BF16))[o // 2:o // 2 + VS // 2]

    def o_early(s, jt, c, ke):
        r0, r1 = T * c, min(T * (c + 1), D)
        tile = slice(jt * T, (jt + 1) * T)
        a = jnp.dot(_bf(wot[r0 // 2:r1 // 2, 0:ke]), _bf(ot[0:ke // 2, tile]), preferred_element_type=F32)
        att[r0:r1, tile] = x_v[r0:r1, seg_cols(s, jt)].astype(F32) + a

    def o_unit(s, jt, c, ke, st):
        r0, r1 = T * c, min(T * (c + 1), D)
        tile = slice(jt * T, (jt + 1) * T)
        a = jnp.dot(_bf(wot[r0 // 2:r1 // 2, ke:640]), _bf(ot[ke // 2:320, tile]), preferred_element_type=F32)
        hh = att[r0:r1, tile] + a
        att[r0:r1, tile] = hh
        if c == 0:
            st['p'] = hh[0:1, :]
        d = hh - st['p']
        s1 = jnp.sum(d, axis=0, keepdims=True)
        s2 = jnp.sum(d * d, axis=0, keepdims=True)
        st['s1'] = s1 if c == 0 else st['s1'] + s1
        st['s2'] = s2 if c == 0 else st['s2'] + s2

    def e2_unit(s, jt, c, st):
        r0, r1 = T * c, min(T * (c + 1), D)
        cols = seg_cols(s, jt)
        if c == 0:
            st['m'], st['inv'] = _ln_scale(st['p'], st['s1'], st['s2'])
        hh = att[r0:r1, jt * T:(jt + 1) * T]
        y = (hh - st['m']) * st['inv']
        cand = st.get('cand')
        out_s[r0:r1, cols] = (hh + y).astype(BF16)
        yb = y.astype(BF16)
        if cand is None:
            y_s[r0 // 2:r1 // 2, cols] = _u32(yb)
        rr = jnp.dot(wr16[:, r0:r1], yb, preferred_element_type=F32)
        st['r'] = rr if c == 0 else st['r'] + rr
        if cand is not None:
            cand.setdefault(jt, {'y': []})['y'].append(yb)
        if r1 == D:
            rrow = _rb(st['r'][0:1, :])
            if cand is None:
                r_s[s, :, jt * T:(jt + 1) * T] = jnp.broadcast_to(rrow, (8, T))
            else:
                cand[jt]['r'] = rrow

    def offer_last(best, cand):
        lane = lax.broadcasted_iota(jnp.int32, (1, T), 1)
        keys = [_rank_key(cand[jt]['r'], lane + jt * T) for jt in range(4)]
        key = jnp.max(jnp.maximum(jnp.maximum(keys[0], keys[1]), jnp.maximum(keys[2], keys[3])),
                      axis=1, keepdims=True)
        tmax = _key_score(jnp.broadcast_to(key, (1, T)))[:, 0:1]
        lane_c = 0xFFFF - (key & 0xFFFF)
        xs = None
        for jt in range(4):
            oh = (lax.broadcasted_iota(jnp.int32, (16, T), 1) == lane_c - jt * T).astype(BF16)
            part = jnp.concatenate([lax.dot_general(oh, yc, NT, preferred_element_type=F32)
                                    for yc in cand[jt]['y']], axis=1)
            xs = part if xs is None else xs + part
        take = tmax > best['r']
        best.update(r=jnp.where(take, tmax, best['r']),
                    tok=jnp.where(take, (NSEG - 1) * L + lane_c, best['tok']),
                    xs=jnp.where(take, xs, best['xs']))

    def prep_qk(i, base):
        wt = _u32(w_v[i].T)
        for g in range(NG):
            n = 9 * GH[g]
            wqkv[base + 64 * g:base + 64 * g + n, :] = wt[63 * g:63 * g + n, :]

    def prep_v():
        wt = _u32(w_v[2].T)
        for h in range(H):
            wqkv[QR + 10 * h:QR + 10 * h + 9, :] = wt[9 * h:9 * h + 9, :]

    def prep_o():
        wt = _u32(w_v[3])
        wpad = jnp.concatenate(
            [piece for h in range(H) for piece in (wt[9 * h:9 * h + 9, :], jnp.zeros((1, D), U32))], axis=0)
        wot[...] = _u32(_bf(wpad).T)

    BLKS = [(jq, kb) for jq in range(4) for kb in range(jq + 1)]

    def head_sets(heads):
        sets, i = [], 0
        while i < len(heads):
            h = heads[i]
            if h % 7 % 2 == 0 and h % 7 < 6 and i + 1 < len(heads):
                sets.append((h, h + 1))
                i += 2
            else:
                assert h % 7 == 6
                sets.append((h,))
                i += 1
        return sets

    def s_items(heads, small_tail=0):
        big, small = [], []
        for hs in head_sets(heads):
            for jq, kb in BLKS:
                halved = len(hs) == 2 and kb == jq
                for h in hs:
                    (small if halved else big).append(functools.partial(s_blk, h, jq, kb, halved))
                if halved:
                    small.append(functools.partial(s_pair, hs[0], jq))
        tail = small[len(small) - small_tail:] if small_tail else []
        small = small[:len(small) - small_tail] if small_tail else small
        order = sorted([((j + 0.5) / len(big), 0, j) for j in range(len(big))]
                       + [((j + 0.5) / len(small), 1, j) for j in range(len(small))])
        return [(big, small)[w][j] for _, w, j in order] + tail

    def phase_x():
        sb = s_items(HB)
        for it in sb[0:NS0]:
            it()
        interleave(pv_items(HA), sb[NS0:])

    def pv_items(heads):
        items = []
        for hs in head_sets(heads):
            st = {}
            roles = ('a', 'b') if len(hs) == 2 else (None,)
            for jq, kb in BLKS:
                for h, role in zip(hs, roles):
                    items.append(functools.partial(pv_blk, h, jq, kb, st, role))
        return items

    def interleave(*seqs):
        seqs = [q for q in seqs if q]
        order = []
        for i, q in enumerate(seqs):
            order += [((j + 0.5) / len(q), i, j) for j in range(len(q))]
        for _, i, j in sorted(order):
            seqs[i][j]()

    def proj_items(fn):
        return [functools.partial(fn, jt, g) for jt in range(4) for g in range(NG)]

    def out_items(s, ke, cand=None):
        sts = [{'cand': cand} for _ in range(4)]
        o_items = [functools.partial(o_unit, s, jt, c, ke, sts[jt]) for jt in range(4) for c in range(NG)]
        e_items = [functools.partial(e2_unit, s, jt, c, sts[jt]) for jt in range(4) for c in range(NG)]
        early = [functools.partial(o_early, s, jt, c, ke) for jt in range(4) for c in range(NG)]
        return early, o_items, e_items

    HA = list(range(HS))
    HB = list(range(HS, H))

    x0a.start()
    w_copy(1).start()
    x0b.start()
    zero_s[0] = 0
    beta_copy.start()
    wr_copy.start()
    kr = lax.broadcasted_iota(jnp.int32, (T, T), 0)
    qc = lax.broadcasted_iota(jnp.int32, (T, T), 1)
    bias[...] = jnp.where(kr > qc, MASKVAL, 0.0).astype(F32)
    kr2 = lax.broadcasted_iota(jnp.int32, (64, T), 0)
    qc2 = lax.broadcasted_iota(jnp.int32, (64, T), 1)
    bias2[...] = jnp.where(kr2 > (qc2 & 63), MASKVAL, 0.0).astype(F32)
    wqkv[...] = jnp.zeros(wqkv.shape, U32)
    bd[...] = jnp.zeros(bd.shape, F32)
    memt[...] = jnp.zeros(memt.shape, F32)
    row = lax.broadcasted_iota(jnp.int32, (640, T), 0)
    ones_tab[...] = jnp.where(row % VS == DH, 1.0, 0.0).astype(F32)
    for g in range(NG):
        row = lax.broadcasted_iota(jnp.int32, (160, T), 0) + (GWIN[g][0] - 140 * g)
        lane = lax.broadcasted_iota(jnp.int32, (160, T), 1)
        keep = ((row >= 0) & (row < 20 * GH[g]) & (lane >= (row // VS) * DH)
                & (lane < (row // VS) * DH + DH))
        keep_tab[g] = jnp.where(keep, 1.0, 0.0).astype(F32)
    qt[NG - 1] = jnp.zeros(qt.shape[1:], U32)
    pqt[NG - 1] = jnp.zeros(pqt.shape[1:], U32)
    pkt[NG - 1] = jnp.zeros(pkt.shape[1:], U32)

    x0a.wait()
    w_copy(0).start()
    for jt in range(2):
        ln1_stats(0, jt)
        ln1_norm(0, jt)
    w_copy(1).wait()
    w_copy(2).start()
    prep_qk(1, 0)
    for g in range(NG):
        for jt in range(2):
            q_unit(jt, g)
    w_copy(0).wait()
    x0b.wait()
    x_rest.start()
    for jt in range(2, 4):
        ln1_stats(0, jt)
        ln1_norm(0, jt)
    prep_qk(0, QR // 2)
    for jt in range(2, 4):
        for g in range(NG):
            q_unit(jt, g)
    w_copy(2).wait()
    w_copy(3).start()
    prep_v()
    for jt in range(4):
        for g in range(NG):
            k_unit(jt, g)
    beta_copy.wait()
    wr_copy.wait()
    x_rest.wait()
    beta = beta_v[...].astype(F32).reshape(1, H)
    hl = lax.broadcasted_iota(jnp.int32, (H, H), 1)
    hs = lax.broadcasted_iota(jnp.int32, (H, H), 0)
    bcol = jnp.sum(jnp.where(hl == hs, jnp.broadcast_to(beta, (H, H)), 0.0), axis=1, keepdims=True)
    gate = _rb(jax.nn.sigmoid(bcol))
    gtab[0] = jnp.broadcast_to(gate, (H, T))
    gtab[1] = jnp.broadcast_to(_rb(1.0 - gate), (H, T))
    r16 = lax.broadcasted_iota(jnp.int32, (16, D), 0)
    wr_row = wr_v[...].astype(F32).reshape(1, D)
    wr16[...] = jnp.where(r16 == 0, jnp.broadcast_to(wr_row, (16, D)), 0.0).astype(BF16)
    interleave(proj_items(v_unit) + s_items(HA, TAIL),
               [functools.partial(ln1_stats, i, jt) for i in range(1, NSEG) for jt in range(4)])
    w_copy(3).wait()

    def seg_body(s, carry):
        prep_o()
        phase_x()
        ln = [functools.partial(ln1_norm, s + 1, jt) for jt in range(4)]
        qs = proj_items(q_unit)
        early, o_items, e_items = out_items(s, KE)
        upd = [functools.partial(mem_update_unit, g) for g in range(NG)]
        ks = proj_items(k_unit)
        pre = [ln[0]] + early[0:8] + [ln[1]]
        mxu1 = early[8:14] + [ln[2]] + upd + qs[0:5] + early[14:20] + [ln[3]] + qs[5:20] + ks
        for it in pre:
            it()
        interleave(pv_items(HB), mxu1)
        vr = proj_items(v_unit) + [functools.partial(mem_read_unit, g) for g in range(NG)]
        for it in o_items:
            it()
        interleave(vr, e_items)
        for it in s_items(HA, TAIL):
            it()
        o_copy(s).start()

        @pl.when(s == 0)
        def _():
            f_copy(0).start()
            f_copy(1).start()

        @pl.when(s == 1)
        def _():
            f_copy(2).start()
        return carry

    lax.fori_loop(0, NSEG - 1, seg_body, 0)

    for i in range(3):
        f_copy(i).wait()
    best = {}

    def offer_previous():
        n = (NSEG - 1) * 8
        r_all = r_s[0:NSEG - 1].reshape(n, L)
        tok = ((lax.broadcasted_iota(jnp.int32, (n, L), 0) // 8) * L
               + lax.broadcasted_iota(jnp.int32, (n, L), 1))
        rmax = jnp.max(jnp.max(r_all, axis=1, keepdims=True), axis=0, keepdims=True)
        idx = jnp.clip(jnp.min(jnp.where(r_all == rmax, tok, S)), 0, S - 1)
        base = pl.multiple_of((idx // T) * T, T)
        onehot = (lax.broadcasted_iota(jnp.int32, (16, T), 1) == idx - base).astype(BF16)
        xs = lax.dot_general(onehot, _bf(y_s[:, pl.ds(base, T)]), NT, preferred_element_type=F32)
        best.update(r=rmax, tok=jnp.full((1, 1), idx, jnp.int32), xs=xs)

    ha1, ha2 = HA[:HA1], HA[HA1:]
    hb1, hb2 = list(range(HS, HM)), list(range(HM, H))
    sb1 = s_items(hb1)
    for it in sb1[0:NS0]:
        it()
    interleave(pv_items(ha1), sb1[NS0:])
    offer_previous()
    sb2 = s_items(hb2)
    interleave(pv_items(ha2) + pv_items(hb1), sb2)
    cand = {}
    early, o_items, e_items = out_items(NSEG - 1, KM, cand)
    for it in early[0:4]:
        it()
    interleave(pv_items(hb2), early[4:])
    for jt in range(4):
        for it in o_items[jt * NG:(jt + 1) * NG]:
            it()
        if jt > 0:
            for it in e_items[(jt - 1) * NG:jt * NG]:
                it()
    for it in e_items[3 * NG:]:
        it()
    offer_last(best, cand)
    o_copy(NSEG - 1).start()

    xs_v[...] = best['xs'].astype(BF16)
    best_v[...] = jnp.broadcast_to(best['r'], (8, T))
    idx = jnp.clip(jnp.max(best['tok']), 0, S - 1)
    base = pl.multiple_of((idx // T) * T, T)
    tile = pl.ds(base, T)

    @pl.when(zero_s[0] == 0)
    def _ffn():
        xs = xs_v[...]
        acc = None
        f0 = 0
        for fw in FCH:
            fc = slice(f0, f0 + fw)
            gt = _rb(jnp.dot(xs, wg_v[:, fc], preferred_element_type=F32))
            up = _rb(jnp.dot(xs, wu_v[:, fc], preferred_element_type=F32))
            act = _rb(_rb(gt * jax.nn.sigmoid(gt)) * up)[0:1, :]
            for t in range(fw // T):
                a = act[:, t * T:(t + 1) * T]
                term = wd_v[:, f0 + t * T:f0 + (t + 1) * T].astype(F32) * a
                acc = term if acc is None else acc + term
            f0 += fw
        ycol = _rb(jnp.sum(acc, axis=1, keepdims=True))
        ycol = _rb(ycol * _rb(jax.nn.sigmoid(best_v[0:1, 0:1])))
        sel = lax.broadcasted_iota(jnp.int32, (D, T), 1) == idx - base
        old = out_s[:, tile].astype(F32)
        fix_v[...] = jnp.where(sel, old + ycol, old).astype(BF16)

    for s in range(NSEG):
        o_copy(s).wait()
    fix = pltpu.make_async_copy(fix_v, out_hbm.at[0, :, tile], sem_o.at[0])
    fix.start()
    fix.wait()


@jax.jit
def pallas_sequential_preLN__memory_aug_infini_attn__moe_arch_mod__prompt_kernel(
    A_x: jax.Array,
    A_wq: jax.Array,
    A_wk: jax.Array,
    A_wv: jax.Array,
    A_wo: jax.Array,
    A_beta: jax.Array,
    B_x: jax.Array,
    B_w_r: jax.Array,
    B_w_gate: jax.Array,
    B_w_up: jax.Array,
    B_w_down: jax.Array,
):
    del B_x
    hbm = pl.BlockSpec(memory_space=pltpu.HBM)
    scratch = [
        pltpu.VMEM((D, S), BF16),
        pltpu.VMEM((4, D, D), BF16),
        pltpu.VMEM((QR + 320, D), U32),
        pltpu.VMEM((D // 2, 640), U32),
        pltpu.VMEM((D // 2, L), U32),
        pltpu.VMEM((NG, 64, L), U32),
        pltpu.VMEM((NG, 64, L), U32),
        pltpu.VMEM((NG, L // 2, T), U32),
        pltpu.VMEM((NG, 64, L), U32),
        pltpu.VMEM((320, L), U32),
        pltpu.VMEM((640, L), F32),
        pltpu.VMEM((NG, 160, T), F32),
        pltpu.VMEM((HS, 1280, T), F32),
        pltpu.VMEM((HM - HS, 1280, T), F32),
        pltpu.VMEM((H - HM, 1280, T), F32),
        pltpu.VMEM((H, 112, T), F32),
        pltpu.VMEM((320, L), U32),
        pltpu.VMEM((D, L), F32),
        pltpu.VMEM((NSEG, 4, 16, T), F32),
        pltpu.VMEM((D // 2, S), U32),
        pltpu.VMEM((D, S), BF16),
        pltpu.VMEM((NSEG, 8, L), F32),
        pltpu.VMEM((T, T), F32),
        pltpu.VMEM((64, T), F32),
        pltpu.VMEM((2, H, T), F32),
        pltpu.VMEM((640, T), F32),
        pltpu.VMEM((NG, 160, T), F32),
        pltpu.VMEM((D, FF), BF16),
        pltpu.VMEM((D, FF), BF16),
        pltpu.VMEM((D, FF), BF16),
        pltpu.VMEM((H,), BF16),
        pltpu.VMEM((D,), BF16),
        pltpu.VMEM((16, D), BF16),
        pltpu.VMEM((16, D), BF16),
        pltpu.VMEM((8, T), F32),
        pltpu.VMEM((D, T), BF16),
        pltpu.SMEM((1,), jnp.int32),
        pltpu.SemaphoreType.DMA((3,)),
        pltpu.SemaphoreType.DMA((4,)),
        pltpu.SemaphoreType.DMA((3,)),
        pltpu.SemaphoreType.DMA((NSEG,)),
        pltpu.SemaphoreType.DMA((2,)),
    ]
    out_t = pl.pallas_call(
        _kernel,
        out_shape=jax.ShapeDtypeStruct((1, D, S), BF16),
        in_specs=[hbm] * 10,
        out_specs=hbm,
        scratch_shapes=scratch,
        compiler_params=pltpu.CompilerParams(vmem_limit_bytes=110 * 1024 * 1024),
        name="infini_moe",
    )(jnp.transpose(A_x, (0, 2, 1)), A_wq, A_wk, A_wv, A_wo, A_beta, B_w_r,
      B_w_gate, B_w_up, jnp.transpose(B_w_down, (1, 0)))
    return jnp.transpose(out_t, (0, 2, 1))
```
